```python
import jax
import jax.numpy as jnp

def _softmax(x, axis=-1):
    return jax.nn.softmax(x, axis=axis)
def _gelu(x):
    return jax.nn.gelu(x, approximate=True)
def _silu(x):
    return jax.nn.silu(x)
def _sigmoid(x):
    return jax.nn.sigmoid(x)
def _layernorm(x, axis=-1, eps=1e-5):
    m = jnp.mean(x, axis=axis, keepdims=True)
    v = jnp.var(x, axis=axis, keepdims=True)
    return (x - m) / jnp.sqrt(v + eps)
def _scatter_add(tgt, idx, src, axis=0):
    return tgt.at[idx].add(src)
def _segment_sum(src, seg, n):
    return jax.ops.segment_sum(src, seg, n)
class _Rng:
    def __init__(self, key):
        self._k = key
    def _next(self):
        self._k, sub = jax.random.split(self._k)
        return sub
    def normal(self, shape):
        return jax.random.normal(self._next(), shape, dtype=jnp.bfloat16)
    def randint(self, lo, hi, shape):
        return jax.random.randint(self._next(), shape, lo, hi, dtype=jnp.int32)
    def uniform(self, shape, lo=0.0, hi=1.0):
        return jax.random.uniform(self._next(), shape, jnp.bfloat16, lo, hi)
    def permutation(self, n):
        return jax.random.permutation(self._next(), n)


kernel_name = 'interleave_layers__sliding_local_dilated__softmax_full_mha__prompt'

def setup_inputs():
    _rng = _Rng(jax.random.key(int.from_bytes(__import__("os").urandom(4), "little")))
    _w = (lambda a: (lambda t: t.astype(jnp.bfloat16) if jnp.issubdtype(t.dtype, jnp.floating) else t)(jnp.asarray(a)))
    def _A_setup():
        B, S, D = 1, 2048, 1024
        return {
            "x": _w((lambda *s: _rng.normal(s) * 0.05)(B, S, D)),
            "wqkv": _w((lambda *s: _rng.normal(s) * 0.05)(D, 3 * D)),
            "wo": _w((lambda *s: _rng.normal(s) * 0.05)(D, D)),
        }
    _A_in = _A_setup()

    def _B_setup():
        B, S, D = 1, 2048, 1024
        return {
            "x": _w((lambda *s: _rng.normal(s) * 0.05)(B, S, D)),
            "wqkv": _w((lambda *s: _rng.normal(s) * 0.05)(D, 3 * D)),
            "wo": _w((lambda *s: _rng.normal(s) * 0.05)(D, D)),
        }
    _B_in = _B_setup()

    return {
        "A_x": _A_in["x"],
        "A_wqkv": _A_in["wqkv"],
        "A_wo": _A_in["wo"],
        "B_x": _B_in["x"],
        "B_wqkv": _B_in["wqkv"],
        "B_wo": _B_in["wo"],
    }

def reference(A_x, A_wqkv, A_wo, B_x, B_wqkv, B_wo):
    def _A_ref(x, wqkv, wo):
        B, S, D = x.shape
        H = 32; Dh = D // H
        W, dil = 8, 2
        qkv = (lambda x, *d: x.transpose(*d))((x @ wqkv).reshape(B, S, 3, H, Dh), 2, 0, 3, 1, 4)
        q, k, v = qkv[0], qkv[1], qkv[2]
        scale = Dh ** -0.5
        pos = jnp.arange(S)
        off = jnp.arange(W) * dil
        idx = pos[:, None] - off[None, :]
        mask = idx >= 0
        idx_c = jnp.where(mask, idx, 0).reshape(-1)
        kg = k[:, :, idx_c, :].reshape(B, H, S, W, Dh)
        vg = v[:, :, idx_c, :].reshape(B, H, S, W, Dh)
        logits = jnp.einsum("bhsd,bhswd->bhsw", q, kg) * scale
        logits = jnp.where(mask[None, None, :, :], logits, -1e9)
        attn = _softmax(logits, axis=-1)
        o = jnp.einsum("bhsw,bhswd->bhsd", attn, vg)
        return (lambda x, *d: x.transpose(*d))(o, 0, 2, 1, 3).reshape(B, S, D) @ wo

    def _B_ref(x, wqkv, wo):
        B, S, D = x.shape
        H = 32; Dh = D // H
        qkv = (lambda x, *d: x.transpose(*d))((x @ wqkv).reshape(B, S, 3, H, Dh), 2, 0, 3, 1, 4)
        q, k, v = qkv[0], qkv[1], qkv[2]
        scale = Dh ** -0.5
        scores = jnp.einsum("bhqd,bhkd->bhqk", q, k) * scale
        p = _softmax(scores, axis=-1)
        o = jnp.einsum("bhqk,bhkd->bhqd", p, v)
        return (lambda x, *d: x.transpose(*d))(o, 0, 2, 1, 3).reshape(B, S, D) @ wo

    x = A_x
    x = x + _A_ref(_layernorm(x, axis=-1), A_wqkv, A_wo)
    x = x + _B_ref(_layernorm(x, axis=-1), B_wqkv, B_wo)
    x = x + _A_ref(_layernorm(x, axis=-1), A_wqkv, A_wo)
    x = x + _B_ref(_layernorm(x, axis=-1), B_wqkv, B_wo)
    return x
```

```python
import jax
import jax.numpy as jnp
from jax import lax
import jax.experimental.pallas as pl
import jax.experimental.pallas.tpu as pltpu

S, D, H, DH = 2048, 1024, 32, 32
W_LOC, DIL = 8, 2
EPS = 1e-5
LOG2E = 1.4426950408889634
QSCALE = (DH ** -0.5) * LOG2E
NEG = -1e9 * LOG2E

BLK = 128
NB = S // BLK
NG = D // 128
NQ = 256
NQT = S // NQ
MK = 128
NC = S // MK
DL = 5
TB = 256
TF = 256

bf16 = jnp.bfloat16
f32 = jnp.float32
u32 = jnp.uint32
NT = (((1,), (1,)), ((), ()))


def _pack(x):
    return pltpu.bitcast(x.astype(bf16), u32)


def _as_bf16(x):
    return pltpu.bitcast(x, bf16)


def _dot(a, b):
    return jnp.dot(a, b, preferred_element_type=f32)


def _dot_nt(a, b):
    return lax.dot_general(a, b, NT, preferred_element_type=f32)


def _layernorm_packed(x):
    outs = []
    for r in range(x.shape[0] // 16):
        xr = x[r * 16:(r + 1) * 16]
        mu = jnp.sum(xr, axis=1, keepdims=True) * (1.0 / D)
        xc = xr - mu
        var = jnp.sum(xc * xc, axis=1, keepdims=True) * (1.0 / D)
        outs.append(_pack(xc * lax.rsqrt(var + EPS)))
    return jnp.concatenate(outs, axis=0)


def _tree(x, op):
    n = x.shape[0]
    while n > 1:
        n //= 2
        x = op(x[:n], x[n:])
    return x[0]


def _local_attention(q, kc, kp, vc, vp, pos):
    lane = lax.broadcasted_iota(jnp.int32, (16, 128), 1)
    outs = []
    for h in range(4):
        rows = slice(h * 16, (h + 1) * 16)

        def shifted(cur, prev, w):
            x = cur[rows]
            if w:
                x = jnp.where(lane >= 128 - DIL * w, prev[rows], x)
                x = pltpu.roll(x, DIL * w, axis=1)
            return _as_bf16(x).astype(f32).reshape(4, 8, 128)

        qh = q[h * 32:(h + 1) * 32].reshape(4, 8, 128)
        logits = []
        for w in range(W_LOC):
            t = jnp.sum(qh * shifted(kc, kp, w), axis=0)
            t = t + pltpu.roll(t, 4, axis=0)
            t = t + pltpu.roll(t, 2, axis=0)
            t = t + pltpu.roll(t, 1, axis=0)
            if w:
                t = jnp.where(pos >= DIL * w, t, NEG)
            logits.append(t)
        m = logits[0]
        for t in logits[1:]:
            m = jnp.maximum(m, t)
        ps = [jnp.exp2(t - m) for t in logits]
        l = ps[0]
        for p in ps[1:]:
            l = l + p
        o = None
        for w in range(W_LOC):
            t = shifted(vc, vp, w) * ps[w][None]
            o = t if o is None else o + t
        outs.append((o * (1.0 / l)[None]).reshape(32, 128))
    return jnp.concatenate(outs, axis=0)


def _kernel(x_hbm, wa_hbm, woa_hbm, wb_hbm, wob_hbm, out_hbm,
            x_ref, xio, xn1, xn2, wa_nat, wat, woa, wb_nat, wbt, wk, wob,
            khalo, vhalo, q0, k0, v0,
            qT, kN, vT, oN, otbuf,
            sem_x, sem_wa, sem_wb, sem_w, sem_o, *sbufs):

    def x_copy(i):
        rows = pl.ds(pl.multiple_of(i * BLK, BLK), BLK)
        return pltpu.make_async_copy(x_hbm.at[rows, :], xio.at[rows, :], sem_x.at[i])

    def wa_copy(g, sec):
        col = pl.multiple_of(sec * D + g * 128, 128)
        return pltpu.make_async_copy(
            wa_hbm.at[:, pl.ds(col, 128)], wa_nat.at[g * 3 + sec], sem_wa.at[g * 3 + sec])

    def wb_copy(c):
        col = pl.multiple_of(c * 128 + (c // 8) * D, 128)
        return pltpu.make_async_copy(
            wb_hbm.at[:, pl.ds(col, 128)], wb_nat.at[c], sem_wb.at[c])

    woa_copy = pltpu.make_async_copy(woa_hbm, woa, sem_w.at[0])
    wk_copy = pltpu.make_async_copy(wb_hbm.at[:, pl.ds(D, D)], wk, sem_w.at[1])
    wob_copy = pltpu.make_async_copy(wob_hbm, wob, sem_w.at[2])

    def out_copy(j):
        rows = pl.ds(pl.multiple_of(j * TF, TF), TF)
        return pltpu.make_async_copy(xio.at[rows, :], out_hbm.at[rows, :], sem_o.at[j])

    def blk_rows(i, n=BLK):
        return pl.ds(pl.multiple_of(i * n, n), n)

    def qkv_group(g, xn):
        r = _dot_nt(_as_bf16(wat[g]), xn)
        return r[0:128] * QSCALE, _pack(r[128:256]), _pack(r[256:384])

    def o_rows(i, n):
        rows = blk_rows(i, n // 2)
        return _as_bf16(jnp.concatenate([oN[t, rows, :] for t in range(NG)], axis=1))

    def proj_residual(o, w_ref, xv):
        cols = []
        for n in range(2):
            c = slice(n * 512, (n + 1) * 512)
            cols.append(xv[:, c] + _dot(o, w_ref[:, c]))
        return jnp.concatenate(cols, axis=1)

    def next_x(i, rep):
        rows = blk_rows(i)
        if rep == 0:
            xv = xio[rows, :].astype(f32)
        else:
            xv = proj_residual(o_rows(i, BLK), wob, x_ref[rows, :])
        x_ref[rows, :] = xv
        return xv

    def head_group0(xn_packed):
        q, k, v = qkv_group(0, _as_bf16(xn_packed))
        q0[...] = q
        k0[...] = k
        v0[...] = v

    def a_body(i, rep, last):
        if rep == 0:
            if not last:
                x_copy(i + 1).wait()

                @pl.when(i + 2 < NB)
                def _():
                    x_copy(jnp.minimum(i + 2, NB - 1)).start()

                wb_copy(i + 1).start()
            wb_copy(i).wait()

        xn_cur = _as_bf16(xn1[...])
        qkv0 = (q0[...], k0[...], v0[...])

        ip = jnp.maximum(i - 1, 0)
        xn2[blk_rows(ip, BLK // 2), :] = _layernorm_packed(x_ref[blk_rows(ip), :])

        if not last:
            xn_next = _layernorm_packed(next_x(i + 1, rep))
            xn1[...] = xn_next
        if rep == 0:
            wbt[i] = pltpu.bitcast(wb_nat[i].T, u32)

        pos = i * BLK + lax.broadcasted_iota(jnp.int32, (8, 128), 1)
        o_cols = []
        for g in range(NG):
            q, kc, vc = qkv0 if g == 0 else qkv_group(g, xn_cur)
            kp = khalo[g]
            vp = vhalo[g]
            khalo[g] = kc
            vhalo[g] = vc
            ot = _local_attention(q, kc, kp, vc, vp, pos)
            o_cols.append(ot.astype(bf16).T)
        if not last:
            head_group0(xn_next)
        o = jnp.concatenate(o_cols, axis=1)
        rows = blk_rows(i)
        xv = proj_residual(o, woa, x_ref[rows, :])
        x_ref[rows, :] = xv
        if last:
            xn2[blk_rows(i, BLK // 2), :] = _layernorm_packed(xv)

    def phase_a(rep):
        khalo[...] = jnp.zeros(khalo.shape, u32)
        vhalo[...] = jnp.zeros(vhalo.shape, u32)
        xn_first = _layernorm_packed(next_x(0, rep))
        xn1[...] = xn_first
        head_group0(xn_first)
        if rep == 0:
            woa_copy.wait()
            wk_copy.start()
            wob_copy.start()

        def body(i, c):
            a_body(i, rep, False)
            return c
        lax.fori_loop(0, NB - 1, body, 0)
        a_body(NB - 1, rep, True)

    def phase_b_proj():
        def body(j, c):
            rows = blk_rows(j, TB // 2)
            xn = _as_bf16(xn2[rows, :])
            for r in range(4):
                w = _as_bf16(wbt[2 * r:2 * r + 2].reshape(128, D))
                y = _pack(_dot_nt(w, xn) * QSCALE)
                for b in range(TB // NQ):
                    qT[j * (TB // NQ) + b, r * 128:(r + 1) * 128, :] = y[:, b * NQ:(b + 1) * NQ]
            for r in range(4):
                w = _as_bf16(wbt[8 + 2 * r:8 + 2 * r + 2].reshape(128, D))
                y = _pack(_dot_nt(w, xn))
                for b in range(TB // MK):
                    vT[j * (TB // MK) + b, r * 128:(r + 1) * 128, :] = y[:, b * MK:(b + 1) * MK]
            for n in range(2):
                y = _pack(_dot(xn, wk[:, n * 512:(n + 1) * 512]))
                for t in range(4):
                    kN[4 * n + t, rows, :] = y[:, t * 128:(t + 1) * 128]
            return c
        lax.fori_loop(0, S // TB, body, 0)

    def phase_b_attn():
        off = [0, 0]

        def qm_of(t, qi, j):
            q = _as_bf16(qT[qi, pl.ds(pl.multiple_of(t * 64 + j * 16, 16), 16), :])
            parts = []
            if j > 0:
                parts.append(jnp.zeros((32 * j, NQ), bf16))
            parts.append(q)
            if j < 3:
                parts.append(jnp.zeros((32 * (3 - j), NQ), bf16))
            return jnp.concatenate(parts, axis=0)

        def qk_chunk(t, qm, c, par, m):
            k = _as_bf16(kN[t, c * (MK // 2):(c + 1) * (MK // 2), :])
            s = _dot(k, qm)
            sbufs[c][pl.ds(pl.multiple_of(off[0] + par * MK, 8), MK), :] = s
            sm = _tree(s.reshape(MK // 8, 8, NQ), jnp.maximum)
            return sm if m is None else jnp.maximum(m, sm)

        def pv_chunk(h, c, par, mrow, l, o):
            s = sbufs[c][pl.ds(pl.multiple_of(off[1] + par * MK, 8), MK), :]
            p = jnp.exp2(s - mrow)
            ls = jnp.sum(p.reshape(MK // 8, 8, NQ), axis=0)
            l = ls if l is None else l + ls
            v = _as_bf16(vT[c, pl.ds(pl.multiple_of(h * 16, 16), 16), :])
            oc = _dot(v, p.astype(bf16))
            o = oc if o is None else o + oc
            return l, o

        def flush_o(g, val):
            y = pltpu.bitcast(_as_bf16(val).T, u32)
            oN[g % NG, blk_rows(g // NG, NQ // 2), :] = y

        n_groups = NQT * NG
        otbuf[...] = jnp.zeros(otbuf.shape, u32)
        qm = qm_of(0, 0, 0)
        m0 = None
        for c in range(NC):
            m0 = qk_chunk(0, qm, c, 0, m0)
        qm = qm_of(0, 0, 1)
        m1 = None
        for c in range(DL):
            m1 = qk_chunk(0, qm, c, 1, m1)

        def body(g, carry):
            qi = g // NG
            t = g % NG
            gn = jnp.minimum(g + 1, n_groups - 1)
            qin = gn // NG
            tn = gn % NG
            off[0] = lax.shift_right_logical(g, 16) * 8
            off[1] = lax.shift_right_logical(g, 17) * 8
            flush_o(jnp.maximum(g - 1, 0), otbuf[...])
            ms = {0: carry[0], 1: carry[1]}
            qms = {}
            l = o = mrow = None
            for n in range(4 * NC):
                j, c = divmod(n, NC)
                j2, c2 = divmod(n + NC + DL, NC)
                if j2 not in qms:
                    qms[j2] = qm_of(t, qi, j2) if j2 < 4 else qm_of(tn, qin, j2 - 4)
                ms[j2] = qk_chunk(t if j2 < 4 else tn, qms[j2], c2, j2 % 2, ms.get(j2))
                if c == 0:
                    mrow = jnp.max(ms[j], axis=0, keepdims=True)
                    l = o = None
                l, o = pv_chunk(t * 4 + j, c, j % 2, mrow, l, o)
                if c == NC - 1:
                    lrow = jnp.sum(l, axis=0, keepdims=True)
                    otbuf[j * 16:(j + 1) * 16, :] = _pack(o * (1.0 / lrow))
            return ms[4], ms[5]

        lax.fori_loop(0, n_groups, body, (m0, m1))
        off[0] = off[1] = 0
        flush_o(n_groups - 1, otbuf[...])

    def final():
        def body(j, c):
            rows = blk_rows(j, TF)
            xv = proj_residual(o_rows(j, TF), wob, x_ref[rows, :])
            xio[rows, :] = xv.astype(bf16)
            out_copy(j).start()
            return c
        lax.fori_loop(0, S // TF, body, 0)
        for j in range(S // TF):
            out_copy(j).wait()

    x_copy(0).start()
    for g in range(NG):
        for sec in range(3):
            wa_copy(g, sec).start()

    def wa_body(g, c):
        for sec in range(3):
            wa_copy(g, sec).wait()

        @pl.when(g == NG - 2)
        def _():
            x_copy(1).start()
            wb_copy(0).start()
            woa_copy.start()

        for sec in range(3):
            wat[g, sec * 64:(sec + 1) * 64, :] = pltpu.bitcast(wa_nat[g * 3 + sec].T, u32)
        return c
    lax.fori_loop(0, NG, wa_body, 0)
    x_copy(0).wait()

    phase_a(0)
    wk_copy.wait()
    wob_copy.wait()
    phase_b_proj()
    phase_b_attn()
    phase_a(1)
    phase_b_proj()
    phase_b_attn()
    final()


@jax.jit
def pallas_interleave_layers__sliding_local_dilated__softmax_full_mha__prompt_kernel(
    A_x: jax.Array,
    A_wqkv: jax.Array,
    A_wo: jax.Array,
    B_x: jax.Array,
    B_wqkv: jax.Array,
    B_wo: jax.Array,
):
    del B_x
    x = A_x.reshape(S, D)
    vm = pltpu.VMEM
    scratch = [
        vm((S, D), f32),
        vm((S, D), bf16),
        vm((BLK // 2, D), u32),
        vm((S // 2, D), u32),
        vm((3 * NG, D, 128), bf16),
        vm((NG, 192, D), u32),
        vm((D, D), bf16),
        vm((2 * NG, D, 128), bf16),
        vm((2 * NG, 64, D), u32),
        vm((D, D), bf16),
        vm((D, D), bf16),
        vm((NG, 64, BLK), u32),
        vm((NG, 64, BLK), u32),
        vm((128, BLK), f32),
        vm((64, BLK), u32),
        vm((64, BLK), u32),
        vm((NQT, D // 2, NQ), u32),
        vm((NG, S // 2, 128), u32),
        vm((NC, D // 2, MK), u32),
        vm((NG, S // 2, 128), u32),
        vm((64, NQ), u32),
        pltpu.SemaphoreType.DMA((NB,)),
        pltpu.SemaphoreType.DMA((3 * NG,)),
        pltpu.SemaphoreType.DMA((2 * NG,)),
        pltpu.SemaphoreType.DMA((3,)),
        pltpu.SemaphoreType.DMA((S // TF,)),
    ] + [vm((2 * MK, NQ), f32)] * NC
    out = pl.pallas_call(
        _kernel,
        out_shape=jax.ShapeDtypeStruct((S, D), bf16),
        in_specs=[pl.BlockSpec(memory_space=pl.ANY)] * 5,
        out_specs=pl.BlockSpec(memory_space=pl.ANY),
        scratch_shapes=scratch,
        compiler_params=pltpu.CompilerParams(vmem_limit_bytes=110 * 1024 * 1024),
        name="interleave_attn",
    )(x, A_wqkv, A_wo, B_wqkv, B_wo)
    return out.reshape(1, S, D)
```

```python
import jax
import jax.numpy as jnp
from jax import lax
import jax.experimental.pallas as pl
import jax.experimental.pallas.tpu as pltpu

S, D, H, DH = 2048, 1024, 32, 32
W_LOC, DIL = 8, 2
EPS = 1e-5
LOG2E = 1.4426950408889634
QSCALE = (DH ** -0.5) * LOG2E
NEG = -1e9 * LOG2E

BLK = 128
NB = S // BLK
NG = D // 128
NQ = 256
NQT = S // NQ
MK = 128
NC = S // MK
DL = 5
TB = 256
TF = 256

SEM_WA = NB
SEM_WB = SEM_WA + 3 * NG
SEM_W = SEM_WB + 2 * NG
SEM_O = SEM_W + 3

PROFILE_SCOPES = False

bf16 = jnp.bfloat16
f32 = jnp.float32
u32 = jnp.uint32
NT = (((1,), (1,)), ((), ()))


class _NoScope:
    def __enter__(self):
        return self

    def __exit__(self, *a):
        return False


def _scope(name):
    return jax.named_scope(name) if PROFILE_SCOPES else _NoScope()


def _pack(x):
    return pltpu.bitcast(x.astype(bf16), u32)


def _as_bf16(x):
    return pltpu.bitcast(x, bf16)


def _dot(a, b):
    return jnp.dot(a, b, preferred_element_type=f32)


def _dot_nt(a, b):
    return lax.dot_general(a, b, NT, preferred_element_type=f32)


def _layernorm_packed(x):
    outs = []
    for r in range(x.shape[0] // 16):
        xr = x[r * 16:(r + 1) * 16]
        mu = jnp.sum(xr, axis=1, keepdims=True) * (1.0 / D)
        xc = xr - mu
        var = jnp.sum(xc * xc, axis=1, keepdims=True) * (1.0 / D)
        outs.append(_pack(xc * lax.rsqrt(var + EPS)))
    return jnp.concatenate(outs, axis=0)


def _token(v):
    return lax.shift_right_logical(jnp.bitwise_and(v[0:8, :], jnp.uint32(0xFFFF)), jnp.uint32(16))


def _after(x, tok):
    n, m = x.shape
    z = jnp.concatenate([jnp.concatenate([tok] * (m // 128), axis=1)] * (n // 8), axis=0)
    return pltpu.bitcast(jnp.bitwise_or(pltpu.bitcast(x, u32), z), x.dtype)


def _ln16(xr):
    mu = jnp.sum(xr, axis=1, keepdims=True) * (1.0 / D)
    xc = xr - mu
    var = jnp.sum(xc * xc, axis=1, keepdims=True) * (1.0 / D)
    return _pack(xc * lax.rsqrt(var + EPS))


def _tree(x, op):
    n = x.shape[0]
    while n > 1:
        n //= 2
        x = op(x[:n], x[n:])
    return x[0]


def _local_attention(q, kc, kp, vc, vp, pos):
    lane = lax.broadcasted_iota(jnp.int32, (16, 128), 1)
    outs = []
    for h in range(4):
        rows = slice(h * 16, (h + 1) * 16)

        def shifted(cur, prev, w):
            x = cur[rows]
            if w:
                x = jnp.where(lane >= 128 - DIL * w, prev[rows], x)
                x = pltpu.roll(x, DIL * w, axis=1)
            return _as_bf16(x).astype(f32).reshape(4, 8, 128)

        qh = q[h * 32:(h + 1) * 32].reshape(4, 8, 128)
        logits = []
        for w in range(W_LOC):
            t = jnp.sum(qh * shifted(kc, kp, w), axis=0)
            t = t + pltpu.roll(t, 4, axis=0)
            t = t + pltpu.roll(t, 2, axis=0)
            t = t + pltpu.roll(t, 1, axis=0)
            if w:
                t = jnp.where(pos >= DIL * w, t, NEG)
            logits.append(t)
        m = logits[0]
        for t in logits[1:]:
            m = jnp.maximum(m, t)
        ps = [jnp.exp2(t - m) for t in logits]
        l = ps[0]
        for p in ps[1:]:
            l = l + p
        o = None
        for w in range(W_LOC):
            t = shifted(vc, vp, w) * ps[w][None]
            o = t if o is None else o + t
        outs.append((o * (1.0 / l)[None]).reshape(32, 128))
    return jnp.concatenate(outs, axis=0)


def _kernel(x_hbm, wa_hbm, woa_hbm, wb_hbm, wob_hbm, out_hbm,
            x_ref, xio, xn1, xn2, wa_nat, wat, woa, wb_nat, wbt, wk, wob,
            khalo, vhalo, q0, k0, v0,
            qT, kN, vT, oN, otbuf,
            sem, *sbufs):

    def x_copy(i):
        rows = pl.ds(pl.multiple_of(i * BLK, BLK), BLK)
        return pltpu.make_async_copy(x_hbm.at[rows, :], xio.at[rows, :], sem.at[i])

    def wa_copy(g, sec):
        col = pl.multiple_of(sec * D + g * 128, 128)
        return pltpu.make_async_copy(
            wa_hbm.at[:, pl.ds(col, 128)], wa_nat.at[g * 3 + sec], sem.at[SEM_WA + g * 3 + sec])

    def wb_copy(c):
        col = pl.multiple_of(c * 128 + (c // 8) * D, 128)
        return pltpu.make_async_copy(
            wb_hbm.at[:, pl.ds(col, 128)], wb_nat.at[c], sem.at[SEM_WB + c])

    woa_copy = pltpu.make_async_copy(woa_hbm, woa, sem.at[SEM_W])
    wk_copy = pltpu.make_async_copy(wb_hbm.at[:, pl.ds(D, D)], wk, sem.at[SEM_W + 1])
    wob_copy = pltpu.make_async_copy(wob_hbm, wob, sem.at[SEM_W + 2])

    def out_copy(j):
        rows = pl.ds(pl.multiple_of(j * TF, TF), TF)
        return pltpu.make_async_copy(xio.at[rows, :], out_hbm.at[rows, :], sem.at[SEM_O + j])

    def blk_rows(i, n=BLK):
        return pl.ds(pl.multiple_of(i * n, n), n)

    def qkv_group(g, xn):
        r = _dot_nt(_as_bf16(wat[g]), xn)
        return r[0:128] * QSCALE, _pack(r[128:256]), _pack(r[256:384])

    def o_rows(i, n):
        rows = blk_rows(i, n // 2)
        return _as_bf16(jnp.concatenate([oN[t, rows, :] for t in range(NG)], axis=1))

    def proj_residual(o, w_ref, xv):
        cols = []
        for n in range(2):
            c = slice(n * 512, (n + 1) * 512)
            cols.append(xv[:, c] + _dot(o, w_ref[:, c]))
        return jnp.concatenate(cols, axis=1)

    def next_x(i, rep):
        rows = blk_rows(i)
        if rep == 0:
            xv = xio[rows, :].astype(f32)
        else:
            xv = proj_residual(o_rows(i, BLK), wob, x_ref[rows, :])
        x_ref[rows, :] = xv
        return xv

    def head_group0(xn_packed):
        q, k, v = qkv_group(0, _as_bf16(xn_packed))
        q0[...] = q
        k0[...] = k
        v0[...] = v
        return _token(k)

    def a_body(i, rep, last):
        if rep == 0:
            if not last:
                x_copy(i + 1).wait()
            wb_copy(i).wait()

        xn_cur = _as_bf16(xn1[...])
        qkv0 = (q0[...], k0[...], v0[...])
        ip = jnp.maximum(i - 1, 0)
        if rep == 1 and not last:
            next_x(i + 1, rep)

        def rows16(blk, r):
            return pl.ds(pl.multiple_of(blk * BLK + r * 16, 16), 16)

        def ln1(r, tok):
            rows = rows16(i + 1, r)
            if rep == 0:
                xv = _after(xio[rows, :].astype(f32), tok)
                x_ref[rows, :] = xv
            else:
                xv = _after(x_ref[rows, :], tok)
            return _ln16(xv)

        def ln2(r, tok):
            y = _ln16(_after(x_ref[rows16(ip, r), :], tok))
            xn2[pl.ds(pl.multiple_of(ip * (BLK // 2) + r * 8, 8), 8), :] = y

        pos = i * BLK + lax.broadcasted_iota(jnp.int32, (8, 128), 1)
        o_cols = []
        xn_parts = []
        for g in range(NG):
            q, kc, vc = qkv0 if g == 0 else qkv_group(g, xn_cur)
            kp = khalo[g]
            vp = vhalo[g]
            khalo[g] = kc
            vhalo[g] = vc
            ot = _local_attention(q, kc, kp, vc, vp, pos)
            o_cols.append(ot.astype(bf16).T)
            if g >= 1:
                tok = _token(kc)
                if g <= 4:
                    if not last:
                        xn_parts += [ln1(2 * g - 2, tok), ln1(2 * g - 1, tok)]
                else:
                    ln2(2 * g - 10, tok)
                    ln2(2 * g - 9, tok)
                if g == 5 and rep == 0:
                    wsrc = _as_bf16(_after(pltpu.bitcast(wb_nat[i], u32), tok))
                    wbt[i] = pltpu.bitcast(wsrc.T, u32)
        if not last:
            xn_next = jnp.concatenate(xn_parts, axis=0)
            xn1[...] = xn_next
            tok = head_group0(xn_next)
        ln2(6, tok)
        ln2(7, tok)
        o = jnp.concatenate(o_cols, axis=1)
        rows = blk_rows(i)
        xv = proj_residual(o, woa, x_ref[rows, :])
        x_ref[rows, :] = xv
        if last:
            xn2[blk_rows(i, BLK // 2), :] = _layernorm_packed(xv)

    def phase_a(rep):
        khalo[...] = jnp.zeros(khalo.shape, u32)
        vhalo[...] = jnp.zeros(vhalo.shape, u32)
        xn_first = _layernorm_packed(next_x(0, rep))
        xn1[...] = xn_first
        head_group0(xn_first)
        if rep == 0:
            woa_copy.wait()

        def body(i, c):
            a_body(i, rep, False)
            return c
        with _scope("a_loop%d" % rep):
            lax.fori_loop(0, NB - 1, body, 0)
        a_body(NB - 1, rep, True)

    def phase_b_proj():
        def body(j, c):
            rows = blk_rows(j, TB // 2)
            xn = _as_bf16(xn2[rows, :])
            for r in range(4):
                w = _as_bf16(wbt[2 * r:2 * r + 2].reshape(128, D))
                y = _pack(_dot_nt(w, xn) * QSCALE)
                for b in range(TB // NQ):
                    qT[j * (TB // NQ) + b, r * 128:(r + 1) * 128, :] = y[:, b * NQ:(b + 1) * NQ]
            for r in range(4):
                w = _as_bf16(wbt[8 + 2 * r:8 + 2 * r + 2].reshape(128, D))
                y = _pack(_dot_nt(w, xn))
                for b in range(TB // MK):
                    vT[j * (TB // MK) + b, r * 128:(r + 1) * 128, :] = y[:, b * MK:(b + 1) * MK]
            for n in range(2):
                y = _pack(_dot(xn, wk[:, n * 512:(n + 1) * 512]))
                for t in range(4):
                    kN[4 * n + t, rows, :] = y[:, t * 128:(t + 1) * 128]
            return c
        lax.fori_loop(0, S // TB, body, 0)

    def phase_b_attn():
        off = [0, 0]

        def qm_of(t, qi, j):
            q = _as_bf16(qT[qi, pl.ds(pl.multiple_of(t * 64 + j * 16, 16), 16), :])
            parts = []
            if j > 0:
                parts.append(jnp.zeros((32 * j, NQ), bf16))
            parts.append(q)
            if j < 3:
                parts.append(jnp.zeros((32 * (3 - j), NQ), bf16))
            return jnp.concatenate(parts, axis=0)

        def qk_chunk(t, qm, c, par, m):
            k = _as_bf16(kN[t, c * (MK // 2):(c + 1) * (MK // 2), :])
            s = _dot(k, qm)
            sbufs[c][pl.ds(pl.multiple_of(off[0] + par * MK, 8), MK), :] = s
            sm = _tree(s.reshape(MK // 8, 8, NQ), jnp.maximum)
            return sm if m is None else jnp.maximum(m, sm)

        def pv_chunk(h, c, par, mrow, l, o):
            s = sbufs[c][pl.ds(pl.multiple_of(off[1] + par * MK, 8), MK), :]
            p = jnp.exp2(s - mrow)
            ls = jnp.sum(p.reshape(MK // 8, 8, NQ), axis=0)
            l = ls if l is None else l + ls
            v = _as_bf16(vT[c, pl.ds(pl.multiple_of(h * 16, 16), 16), :])
            oc = _dot(v, p.astype(bf16))
            o = oc if o is None else o + oc
            return l, o

        def flush_o(g, val):
            y = pltpu.bitcast(_as_bf16(val).T, u32)
            oN[g % NG, blk_rows(g // NG, NQ // 2), :] = y

        n_groups = NQT * NG
        otbuf[...] = jnp.zeros(otbuf.shape, u32)
        qm = qm_of(0, 0, 0)
        m0 = None
        for c in range(NC):
            m0 = qk_chunk(0, qm, c, 0, m0)
        qm = qm_of(0, 0, 1)
        m1 = None
        for c in range(DL):
            m1 = qk_chunk(0, qm, c, 1, m1)

        def body(g, carry):
            qi = g // NG
            t = g % NG
            gn = jnp.minimum(g + 1, n_groups - 1)
            qin = gn // NG
            tn = gn % NG
            off[0] = lax.shift_right_logical(g, 16) * 8
            off[1] = lax.shift_right_logical(g, 17) * 8
            flush_o(jnp.maximum(g - 1, 0), otbuf[...])
            ms = {0: carry[0], 1: carry[1]}
            qms = {}
            l = o = mrow = None
            for n in range(4 * NC):
                j, c = divmod(n, NC)
                j2, c2 = divmod(n + NC + DL, NC)
                if j2 not in qms:
                    qms[j2] = qm_of(t, qi, j2) if j2 < 4 else qm_of(tn, qin, j2 - 4)
                ms[j2] = qk_chunk(t if j2 < 4 else tn, qms[j2], c2, j2 % 2, ms.get(j2))
                if c == 0:
                    mrow = jnp.max(ms[j], axis=0, keepdims=True)
                    l = o = None
                l, o = pv_chunk(t * 4 + j, c, j % 2, mrow, l, o)
                if c == NC - 1:
                    lrow = jnp.sum(l, axis=0, keepdims=True)
                    otbuf[j * 16:(j + 1) * 16, :] = _pack(o * (1.0 / lrow))
            return ms[4], ms[5]

        lax.fori_loop(0, n_groups, body, (m0, m1))
        off[0] = off[1] = 0
        flush_o(n_groups - 1, otbuf[...])

    def final():
        def body(j, c):
            rows = blk_rows(j, TF)
            xv = proj_residual(o_rows(j, TF), wob, x_ref[rows, :])
            xio[rows, :] = xv.astype(bf16)
            out_copy(j).start()
            return c
        lax.fori_loop(0, S // TF, body, 0)
        for j in range(S // TF):
            out_copy(j).wait()

    x_copy(0).start()
    for g in range(NG):
        for sec in range(3):
            wa_copy(g, sec).start()
    woa_copy.start()
    for i in range(1, NB):
        x_copy(i).start()
        wb_copy(i - 1).start()
    wb_copy(NB - 1).start()
    wk_copy.start()
    wob_copy.start()

    def wa_body(g, c):
        for sec in range(3):
            wa_copy(g, sec).wait()
        for sec in range(3):
            wat[g, sec * 64:(sec + 1) * 64, :] = pltpu.bitcast(wa_nat[g * 3 + sec].T, u32)
        return c
    with _scope("wa_loop"):
        lax.fori_loop(0, NG, wa_body, 0)
        x_copy(0).wait()

    with _scope("phase_a0"):
        phase_a(0)
    wk_copy.wait()
    wob_copy.wait()
    with _scope("b_proj0"):
        phase_b_proj()
    with _scope("b_attn0"):
        phase_b_attn()
    with _scope("phase_a1"):
        phase_a(1)
    with _scope("b_proj1"):
        phase_b_proj()
    with _scope("b_attn1"):
        phase_b_attn()
    with _scope("final"):
        final()


@jax.jit
def pallas_interleave_layers__sliding_local_dilated__softmax_full_mha__prompt_kernel(
    A_x: jax.Array,
    A_wqkv: jax.Array,
    A_wo: jax.Array,
    B_x: jax.Array,
    B_wqkv: jax.Array,
    B_wo: jax.Array,
):
    del B_x
    x = A_x.reshape(S, D)
    vm = pltpu.VMEM
    scratch = [
        vm((S, D), f32),
        vm((S, D), bf16),
        vm((BLK // 2, D), u32),
        vm((S // 2, D), u32),
        vm((3 * NG, D, 128), bf16),
        vm((NG, 192, D), u32),
        vm((D, D), bf16),
        vm((2 * NG, D, 128), bf16),
        vm((2 * NG, 64, D), u32),
        vm((D, D), bf16),
        vm((D, D), bf16),
        vm((NG, 64, BLK), u32),
        vm((NG, 64, BLK), u32),
        vm((128, BLK), f32),
        vm((64, BLK), u32),
        vm((64, BLK), u32),
        vm((NQT, D // 2, NQ), u32),
        vm((NG, S // 2, 128), u32),
        vm((NC, D // 2, MK), u32),
        vm((NG, S // 2, 128), u32),
        vm((64, NQ), u32),
        pltpu.SemaphoreType.DMA((SEM_O + S // TF,)),
    ] + [vm((2 * MK, NQ), f32)] * NC
    out = pl.pallas_call(
        _kernel,
        out_shape=jax.ShapeDtypeStruct((S, D), bf16),
        in_specs=[pl.BlockSpec(memory_space=pl.ANY)] * 5,
        out_specs=pl.BlockSpec(memory_space=pl.ANY),
        scratch_shapes=scratch,
        compiler_params=pltpu.CompilerParams(vmem_limit_bytes=110 * 1024 * 1024),
        name="interleave_attn",
    )(x, A_wqkv, A_wo, B_wqkv, B_wo)
    return out.reshape(1, S, D)
```

```python
import jax
import jax.numpy as jnp
from jax import lax
import jax.experimental.pallas as pl
import jax.experimental.pallas.tpu as pltpu

S, D, H, DH = 2048, 1024, 32, 32
W_LOC, DIL = 8, 2
EPS = 1e-5
LOG2E = 1.4426950408889634
QSCALE = (DH ** -0.5) * LOG2E
NEG = -1e9 * LOG2E

BLK = 128
NB = S // BLK
NG = D // 128
NQ = 256
NQT = S // NQ
MK = 128
NC = S // MK
DL = 5
APB = 2
GPB = 4
TB = 256
TF = 256

SEM_WA = NB
SEM_WB = SEM_WA + 3 * NG
SEM_W = SEM_WB + 2 * NG
SEM_O = SEM_W + 3

PROFILE_SCOPES = False

bf16 = jnp.bfloat16
f32 = jnp.float32
u32 = jnp.uint32
NT = (((1,), (1,)), ((), ()))


class _NoScope:
    def __enter__(self):
        return self

    def __exit__(self, *a):
        return False


def _scope(name):
    return jax.named_scope(name) if PROFILE_SCOPES else _NoScope()


def _pack(x):
    return pltpu.bitcast(x.astype(bf16), u32)


def _as_bf16(x):
    return pltpu.bitcast(x, bf16)


def _dot(a, b):
    return jnp.dot(a, b, preferred_element_type=f32)


def _dot_nt(a, b):
    return lax.dot_general(a, b, NT, preferred_element_type=f32)


def _layernorm_packed(x):
    outs = []
    for r in range(x.shape[0] // 16):
        xr = x[r * 16:(r + 1) * 16]
        mu = jnp.sum(xr, axis=1, keepdims=True) * (1.0 / D)
        xc = xr - mu
        var = jnp.sum(xc * xc, axis=1, keepdims=True) * (1.0 / D)
        outs.append(_pack(xc * lax.rsqrt(var + EPS)))
    return jnp.concatenate(outs, axis=0)


def _token(v):
    return lax.shift_right_logical(jnp.bitwise_and(v[0:8, :], jnp.uint32(0xFFFF)), jnp.uint32(16))


def _after(x, tok):
    n, m = x.shape
    z = jnp.concatenate([jnp.concatenate([tok] * (m // 128), axis=1)] * (n // 8), axis=0)
    return pltpu.bitcast(jnp.bitwise_or(pltpu.bitcast(x, u32), z), x.dtype)


def _ln16(xr):
    mu = jnp.sum(xr, axis=1, keepdims=True) * (1.0 / D)
    xc = xr - mu
    var = jnp.sum(xc * xc, axis=1, keepdims=True) * (1.0 / D)
    return _pack(xc * lax.rsqrt(var + EPS))


def _tree(x, op):
    n = x.shape[0]
    while n > 1:
        n //= 2
        x = op(x[:n], x[n:])
    return x[0]


def _local_attention(q, kc, kp, vc, vp, pos):
    lane = lax.broadcasted_iota(jnp.int32, (16, 128), 1)
    outs = []
    for h in range(4):
        rows = slice(h * 16, (h + 1) * 16)

        def shifted(cur, prev, w):
            x = cur[rows]
            if w:
                x = jnp.where(lane >= 128 - DIL * w, prev[rows], x)
                x = pltpu.roll(x, DIL * w, axis=1)
            return _as_bf16(x).astype(f32).reshape(4, 8, 128)

        qh = q[h * 32:(h + 1) * 32].reshape(4, 8, 128)
        logits = []
        for w in range(W_LOC):
            t = jnp.sum(qh * shifted(kc, kp, w), axis=0)
            t = t + pltpu.roll(t, 4, axis=0)
            t = t + pltpu.roll(t, 2, axis=0)
            t = t + pltpu.roll(t, 1, axis=0)
            if w:
                t = jnp.where(pos >= DIL * w, t, NEG)
            logits.append(t)
        m = logits[0]
        for t in logits[1:]:
            m = jnp.maximum(m, t)
        ps = [jnp.exp2(t - m) for t in logits]
        l = ps[0]
        for p in ps[1:]:
            l = l + p
        o = None
        for w in range(W_LOC):
            t = shifted(vc, vp, w) * ps[w][None]
            o = t if o is None else o + t
        outs.append((o * (1.0 / l)[None]).reshape(32, 128))
    return jnp.concatenate(outs, axis=0)


def _kernel(x_hbm, wa_hbm, woa_hbm, wb_hbm, wob_hbm, out_hbm,
            x_ref, xio, xn1, xn2, wa_nat, wat, woa, wb_nat, wbt, wk, wob,
            khalo, vhalo, q0, k0, v0,
            qT, kN, vT, oN, otbuf,
            sem, *sbufs):

    def x_copy(i):
        rows = pl.ds(pl.multiple_of(i * BLK, BLK), BLK)
        return pltpu.make_async_copy(x_hbm.at[rows, :], xio.at[rows, :], sem.at[i])

    def wa_copy(g, sec):
        col = pl.multiple_of(sec * D + g * 128, 128)
        return pltpu.make_async_copy(
            wa_hbm.at[:, pl.ds(col, 128)], wa_nat.at[g * 3 + sec], sem.at[SEM_WA + g * 3 + sec])

    def wb_copy(c):
        col = pl.multiple_of(c * 128 + (c // 8) * D, 128)
        return pltpu.make_async_copy(
            wb_hbm.at[:, pl.ds(col, 128)], wb_nat.at[c], sem.at[SEM_WB + c])

    woa_copy = pltpu.make_async_copy(woa_hbm, woa, sem.at[SEM_W])
    wk_copy = pltpu.make_async_copy(wb_hbm.at[:, pl.ds(D, D)], wk, sem.at[SEM_W + 1])
    wob_copy = pltpu.make_async_copy(wob_hbm, wob, sem.at[SEM_W + 2])

    def out_copy(j):
        rows = pl.ds(pl.multiple_of(j * TF, TF), TF)
        return pltpu.make_async_copy(xio.at[rows, :], out_hbm.at[rows, :], sem.at[SEM_O + j])

    def blk_rows(i, n=BLK):
        return pl.ds(pl.multiple_of(i * n, n), n)

    def qkv_group(g, xn):
        r = _dot_nt(_as_bf16(wat[g]), xn)
        return r[0:128] * QSCALE, _pack(r[128:256]), _pack(r[256:384])

    def o_rows(i, n):
        rows = blk_rows(i, n // 2)
        return _as_bf16(jnp.concatenate([oN[t, rows, :] for t in range(NG)], axis=1))

    def proj_residual(o, w_ref, xv):
        cols = []
        for n in range(2):
            c = slice(n * 512, (n + 1) * 512)
            cols.append(xv[:, c] + _dot(o, w_ref[:, c]))
        return jnp.concatenate(cols, axis=1)

    def rows16(blk, r):
        return pl.ds(pl.multiple_of(blk * BLK + r * 16, 16), 16)

    def ln1(blk, r, tok=None):
        rows = rows16(blk, r)
        xv = xio[rows, :].astype(f32)
        if tok is not None:
            xv = _after(xv, tok)
        x_ref[rows, :] = xv
        return _ln16(xv)

    def ln2(blk, r, tok=None):
        xv = x_ref[rows16(blk, r), :]
        if tok is not None:
            xv = _after(xv, tok)
        xn2[pl.ds(pl.multiple_of(blk * (BLK // 2) + r * 8, 8), 8), :] = _ln16(xv)

    def head_group0(xn_packed):
        q, k, v = qkv_group(0, _as_bf16(xn_packed))
        q0[...] = q
        k0[...] = k
        v0[...] = v
        return _token(k)

    def a_block(i):
        xn_cur = _as_bf16(xn1[...])
        qkv0 = (q0[...], k0[...], v0[...])
        ip = jnp.maximum(i - 1, 0)
        inx = jnp.minimum(i + 1, NB - 1)
        pos = i * BLK + lax.broadcasted_iota(jnp.int32, (8, 128), 1)
        o_cols = []
        xn_parts = []
        for g in range(NG):
            q, kc, vc = qkv0 if g == 0 else qkv_group(g, xn_cur)
            kp = khalo[g]
            vp = vhalo[g]
            khalo[g] = kc
            vhalo[g] = vc
            ot = _local_attention(q, kc, kp, vc, vp, pos)
            o_cols.append(ot.astype(bf16).T)
            if g >= 1:
                tok = _token(kc)
                if g <= 4:
                    xn_parts += [ln1(inx, 2 * g - 2, tok), ln1(inx, 2 * g - 1, tok)]
                else:
                    ln2(ip, 2 * g - 10, tok)
                    ln2(ip, 2 * g - 9, tok)
                if g == 5:
                    wsrc = _as_bf16(_after(pltpu.bitcast(wb_nat[i], u32), tok))
                    wbt[i] = pltpu.bitcast(wsrc.T, u32)
        xn_next = jnp.concatenate(xn_parts, axis=0)
        xn1[...] = xn_next
        tok = head_group0(xn_next)
        ln2(ip, 6, tok)
        ln2(ip, 7, tok)
        o = jnp.concatenate(o_cols, axis=1)
        rows = blk_rows(i)
        x_ref[rows, :] = proj_residual(o, woa, x_ref[rows, :])

    def phase_a(rep):
        khalo[...] = jnp.zeros(khalo.shape, u32)
        vhalo[...] = jnp.zeros(vhalo.shape, u32)
        xn_first = jnp.concatenate([ln1(0, r) for r in range(BLK // 16)], axis=0)
        xn1[...] = xn_first
        head_group0(xn_first)

        @pl.when(rep == 0)
        def _():
            woa_copy.wait()

        def body(it, c):
            @pl.when(rep == 0)
            def _():
                for u in range(APB):
                    wb_copy(it * APB + u).wait()

            for u in range(APB):
                nxt = it * APB + u + 1

                @pl.when(jnp.logical_and(rep == 0, nxt < NB))
                def _():
                    x_copy(jnp.minimum(nxt, NB - 1)).wait()

            for u in range(APB):
                a_block(it * APB + u)
            return c
        with _scope("a_loop"):
            lax.fori_loop(0, NB // APB, body, 0)
        for r in range(BLK // 16):
            ln2(NB - 1, r)

    def phase_b_proj():
        def body(j, c):
            rows = blk_rows(j, TB // 2)
            xn = _as_bf16(xn2[rows, :])
            for r in range(4):
                w = _as_bf16(wbt[2 * r:2 * r + 2].reshape(128, D))
                y = _pack(_dot_nt(w, xn) * QSCALE)
                for b in range(TB // NQ):
                    qT[j * (TB // NQ) + b, r * 128:(r + 1) * 128, :] = y[:, b * NQ:(b + 1) * NQ]
            for r in range(4):
                w = _as_bf16(wbt[8 + 2 * r:8 + 2 * r + 2].reshape(128, D))
                y = _pack(_dot_nt(w, xn))
                for b in range(TB // MK):
                    vT[j * (TB // MK) + b, r * 128:(r + 1) * 128, :] = y[:, b * MK:(b + 1) * MK]
            for n in range(2):
                y = _pack(_dot(xn, wk[:, n * 512:(n + 1) * 512]))
                for t in range(4):
                    kN[4 * n + t, rows, :] = y[:, t * 128:(t + 1) * 128]
            return c
        lax.fori_loop(0, S // TB, body, 0)

    def phase_b_attn():
        off = [0, 0]

        def qm_of(t, qi, j):
            q = _as_bf16(qT[qi, pl.ds(pl.multiple_of(t * 64 + j * 16, 16), 16), :])
            parts = []
            if j > 0:
                parts.append(jnp.zeros((32 * j, NQ), bf16))
            parts.append(q)
            if j < 3:
                parts.append(jnp.zeros((32 * (3 - j), NQ), bf16))
            return jnp.concatenate(parts, axis=0)

        def qk_chunk(t, qm, c, par, m):
            k = _as_bf16(kN[t, c * (MK // 2):(c + 1) * (MK // 2), :])
            s = _dot(k, qm)
            sbufs[c][pl.ds(pl.multiple_of(off[0] + par * MK, 8), MK), :] = s
            sm = _tree(s.reshape(MK // 8, 8, NQ), jnp.maximum)
            return sm if m is None else jnp.maximum(m, sm)

        def pv_chunk(h, c, par, mrow, l, o):
            s = sbufs[c][pl.ds(pl.multiple_of(off[1] + par * MK, 8), MK), :]
            p = jnp.exp2(s - mrow)
            ls = jnp.sum(p.reshape(MK // 8, 8, NQ), axis=0)
            l = ls if l is None else l + ls
            v = _as_bf16(vT[c, pl.ds(pl.multiple_of(h * 16, 16), 16), :])
            oc = _dot(v, p.astype(bf16))
            o = oc if o is None else o + oc
            return l, o

        def flush_o(g, val):
            y = pltpu.bitcast(_as_bf16(val).T, u32)
            oN[g % NG, blk_rows(g // NG, NQ // 2), :] = y

        n_groups = NQT * NG
        otbuf[...] = jnp.zeros(otbuf.shape, u32)
        qm = qm_of(0, 0, 0)
        m0 = None
        for c in range(NC):
            m0 = qk_chunk(0, qm, c, 0, m0)
        qm = qm_of(0, 0, 1)
        m1 = None
        for c in range(DL):
            m1 = qk_chunk(0, qm, c, 1, m1)

        def group(g, g_next, carry, zero):
            qi = g // NG
            t = g % NG
            off[0] = lax.shift_right_logical(zero, 16) * 8
            off[1] = lax.shift_right_logical(zero, 17) * 8
            flush_o(jnp.maximum(g - 1, 0), otbuf[...])
            ms = {0: carry[0], 1: carry[1]}
            qms = {}
            l = o = mrow = None
            for n in range(4 * NC):
                j, c = divmod(n, NC)
                j2, c2 = divmod(n + NC + DL, NC)
                if j2 < 4 or g_next is not None:
                    t2 = t if j2 < 4 else g_next % NG
                    if j2 not in qms:
                        qms[j2] = qm_of(t2, qi if j2 < 4 else g_next // NG, j2 % 4)
                    ms[j2] = qk_chunk(t2, qms[j2], c2, j2 % 2, ms.get(j2))
                if c == 0:
                    mrow = jnp.max(ms[j], axis=0, keepdims=True)
                    l = o = None
                l, o = pv_chunk(t * 4 + j, c, j % 2, mrow, l, o)
                if c == NC - 1:
                    lrow = jnp.sum(l, axis=0, keepdims=True)
                    otbuf[j * 16:(j + 1) * 16, :] = _pack(o * (1.0 / lrow))
            return ms.get(4), ms.get(5)

        def body(it, ms):
            for u in range(GPB):
                g = it * GPB + u
                ms = group(g, jnp.minimum(g + 1, n_groups - 1), ms, it)
            return ms

        lax.fori_loop(0, n_groups // GPB, body, (m0, m1))
        off[0] = off[1] = 0
        flush_o(n_groups - 1, otbuf[...])

    def phase_b_out(rep):
        def body(j, c):
            rows = blk_rows(j, TF)
            xv = proj_residual(o_rows(j, TF), wob, x_ref[rows, :])
            xio[rows, :] = xv.astype(bf16)

            @pl.when(rep == 1)
            def _():
                out_copy(j).start()
            return c
        lax.fori_loop(0, S // TF, body, 0)

    x_copy(0).start()
    for g in range(NG):
        for sec in range(3):
            wa_copy(g, sec).start()
    woa_copy.start()
    for i in range(1, NB):
        x_copy(i).start()
        wb_copy(i - 1).start()
    wb_copy(NB - 1).start()
    wk_copy.start()
    wob_copy.start()

    def wa_body(g, c):
        for sec in range(3):
            wa_copy(g, sec).wait()
        for sec in range(3):
            wat[g, sec * 64:(sec + 1) * 64, :] = pltpu.bitcast(wa_nat[g * 3 + sec].T, u32)
        return c
    with _scope("wa_loop"):
        lax.fori_loop(0, NG, wa_body, 0)
        x_copy(0).wait()

    def layer_pair(rep, c):
        with _scope("phase_a"):
            phase_a(rep)

        @pl.when(rep == 0)
        def _():
            wk_copy.wait()
            wob_copy.wait()

        with _scope("b_proj"):
            phase_b_proj()
        with _scope("b_attn"):
            phase_b_attn()
        with _scope("b_out"):
            phase_b_out(rep)
        return c
    lax.fori_loop(0, 2, layer_pair, 0)
    for j in range(S // TF):
        out_copy(j).wait()


@jax.jit
def pallas_interleave_layers__sliding_local_dilated__softmax_full_mha__prompt_kernel(
    A_x: jax.Array,
    A_wqkv: jax.Array,
    A_wo: jax.Array,
    B_x: jax.Array,
    B_wqkv: jax.Array,
    B_wo: jax.Array,
):
    del B_x
    x = A_x.reshape(S, D)
    vm = pltpu.VMEM
    scratch = [
        vm((S, D), f32),
        vm((S, D), bf16),
        vm((BLK // 2, D), u32),
        vm((S // 2, D), u32),
        vm((3 * NG, D, 128), bf16),
        vm((NG, 192, D), u32),
        vm((D, D), bf16),
        vm((2 * NG, D, 128), bf16),
        vm((2 * NG, 64, D), u32),
        vm((D, D), bf16),
        vm((D, D), bf16),
        vm((NG, 64, BLK), u32),
        vm((NG, 64, BLK), u32),
        vm((128, BLK), f32),
        vm((64, BLK), u32),
        vm((64, BLK), u32),
        vm((NQT, D // 2, NQ), u32),
        vm((NG, S // 2, 128), u32),
        vm((NC, D // 2, MK), u32),
        vm((NG, S // 2, 128), u32),
        vm((64, NQ), u32),
        pltpu.SemaphoreType.DMA((SEM_O + S // TF,)),
    ] + [vm((2 * MK, NQ), f32)] * NC
    out = pl.pallas_call(
        _kernel,
        out_shape=jax.ShapeDtypeStruct((S, D), bf16),
        in_specs=[pl.BlockSpec(memory_space=pl.ANY)] * 5,
        out_specs=pl.BlockSpec(memory_space=pl.ANY),
        scratch_shapes=scratch,
        compiler_params=pltpu.CompilerParams(vmem_limit_bytes=110 * 1024 * 1024),
        name="interleave_attn",
    )(x, A_wqkv, A_wo, B_wqkv, B_wo)
    return out.reshape(1, S, D)
```

```python
import jax
import jax.numpy as jnp
from jax import lax
import jax.experimental.pallas as pl
import jax.experimental.pallas.tpu as pltpu

S, D, H, DH = 2048, 1024, 32, 32
W_LOC, DIL = 8, 2
EPS = 1e-5
LOG2E = 1.4426950408889634
QSCALE = (DH ** -0.5) * LOG2E
NEG = -1e9 * LOG2E

BLK = 128
NB = S // BLK
NG = D // 128
NQ = 256
NQT = S // NQ
MK = 128
NC = S // MK
DL = 5
APB = 2
GPB = 4
TB = 256
TF = 256

SEM_WA = NB
SEM_WB = SEM_WA + 3 * NG
SEM_W = SEM_WB + 2 * NG
SEM_O = SEM_W + 3

PACK_K = False
PACK_V = True
UCH = 2
PROFILE_SCOPES = False

bf16 = jnp.bfloat16
f32 = jnp.float32
u32 = jnp.uint32
NT = (((1,), (1,)), ((), ()))


class _NoScope:
    def __enter__(self):
        return self

    def __exit__(self, *a):
        return False


def _scope(name):
    return jax.named_scope(name) if PROFILE_SCOPES else _NoScope()


def _pack(x):
    return pltpu.bitcast(x.astype(bf16), u32)


def _as_bf16(x):
    return pltpu.bitcast(x, bf16)


def _dot(a, b):
    return jnp.dot(a, b, preferred_element_type=f32)


def _dot_nt(a, b):
    return lax.dot_general(a, b, NT, preferred_element_type=f32)


def _layernorm_packed(x):
    outs = []
    for r in range(x.shape[0] // 16):
        xr = x[r * 16:(r + 1) * 16]
        mu = jnp.sum(xr, axis=1, keepdims=True) * (1.0 / D)
        xc = xr - mu
        var = jnp.sum(xc * xc, axis=1, keepdims=True) * (1.0 / D)
        outs.append(_pack(xc * lax.rsqrt(var + EPS)))
    return jnp.concatenate(outs, axis=0)


def _token(v):
    t = pltpu.bitcast(v[0:8, :], u32)
    return lax.shift_right_logical(jnp.bitwise_and(t, jnp.uint32(0xFFFF)), jnp.uint32(16))


def _after(x, tok):
    n, m = x.shape
    z = jnp.concatenate([jnp.concatenate([tok] * (m // 128), axis=1)] * (n // 8), axis=0)
    return pltpu.bitcast(jnp.bitwise_or(pltpu.bitcast(x, u32), z), x.dtype)


def _ln16(xr):
    mu = jnp.sum(xr, axis=1, keepdims=True) * (1.0 / D)
    xc = xr - mu
    var = jnp.sum(xc * xc, axis=1, keepdims=True) * (1.0 / D)
    return _pack(xc * lax.rsqrt(var + EPS))


def _tree(x, op):
    n = x.shape[0]
    while n > 1:
        n //= 2
        x = op(x[:n], x[n:])
    return x[0]


def _local_attention(q, kc, kp, vc, vp, pos):
    def shifted(cur, prev, u, w):
        n = UCH * (4 if cur.dtype == u32 else 8)
        x = cur[u * n:(u + 1) * n]
        if w:
            lane = lax.broadcasted_iota(jnp.int32, x.shape, 1)
            x = jnp.where(lane >= 128 - DIL * w, prev[u * n:(u + 1) * n], x)
            x = pltpu.roll(x, DIL * w, axis=1)
        if x.dtype == u32:
            x = _as_bf16(x).astype(f32)
        return x.reshape(UCH, 8, 128)

    even = lax.broadcasted_iota(jnp.int32, (8, 128), 0) % 2 == 0
    acc = [None] * W_LOC
    for u in range(16 // UCH):
        qu = q[u * UCH * 8:(u + 1) * UCH * 8].reshape(UCH, 8, 128)
        for w in range(W_LOC):
            t = _tree(qu * shifted(kc, kp, u, w), jnp.add)
            acc[w] = t if acc[w] is None else acc[w] + t
    logits = []
    for w in range(W_LOC):
        t = acc[w]
        t = t + jnp.where(even, pltpu.roll(t, 7, axis=0), pltpu.roll(t, 1, axis=0))
        t = t * QSCALE
        if w:
            t = jnp.where(pos >= DIL * w, t, NEG)
        logits.append(t)
    m = logits[0]
    for t in logits[1:]:
        m = jnp.maximum(m, t)
    ps = [jnp.exp2(t - m) for t in logits]
    l = ps[0]
    for p in ps[1:]:
        l = l + p
    r = 1.0 / l
    ps = [(p * r)[None] for p in ps]
    outs = []
    for u in range(16 // UCH):
        o = None
        for w in range(W_LOC):
            t = shifted(vc, vp, u, w) * ps[w]
            o = t if o is None else o + t
        outs.append(o.reshape(UCH * 8, 128))
    return jnp.concatenate(outs, axis=0)


def _kernel(x_hbm, wa_hbm, woa_hbm, wb_hbm, wob_hbm, out_hbm,
            x_ref, xio, xn1, xn2, wa_nat, wat, woa, woap, wb_nat, wbt, wk, wob,
            khalo, vhalo, q0, k0, v0,
            qT, kN, vT, oN, otbuf,
            sem, *sbufs):

    def x_copy(i):
        rows = pl.ds(pl.multiple_of(i * BLK, BLK), BLK)
        return pltpu.make_async_copy(x_hbm.at[rows, :], xio.at[rows, :], sem.at[i])

    def wa_copy(g, sec):
        col = pl.multiple_of(sec * D + g * 128, 128)
        return pltpu.make_async_copy(
            wa_hbm.at[:, pl.ds(col, 128)], wa_nat.at[g * 3 + sec], sem.at[SEM_WA + g * 3 + sec])

    def wb_copy(c):
        col = pl.multiple_of(c * 128 + (c // 8) * D, 128)
        return pltpu.make_async_copy(
            wb_hbm.at[:, pl.ds(col, 128)], wb_nat.at[c], sem.at[SEM_WB + c])

    woa_copy = pltpu.make_async_copy(woa_hbm, woa, sem.at[SEM_W])
    wk_copy = pltpu.make_async_copy(wb_hbm.at[:, pl.ds(D, D)], wk, sem.at[SEM_W + 1])
    wob_copy = pltpu.make_async_copy(wob_hbm, wob, sem.at[SEM_W + 2])

    def out_copy(j):
        rows = pl.ds(pl.multiple_of(j * TF, TF), TF)
        return pltpu.make_async_copy(xio.at[rows, :], out_hbm.at[rows, :], sem.at[SEM_O + j])

    def blk_rows(i, n=BLK):
        return pl.ds(pl.multiple_of(i * n, n), n)

    def qkv_group(g, xn):
        w = jnp.concatenate([wat[g, kt] for kt in range(NG)], axis=1)
        r = _dot_nt(_as_bf16(w), xn)
        k = r[128:256]
        v = r[256:384]
        return r[0:128], _pack(k) if PACK_K else k, _pack(v) if PACK_V else v

    def o_rows(i, n):
        rows = blk_rows(i, n // 2)
        return _as_bf16(jnp.concatenate([oN[t, rows, :] for t in range(NG)], axis=1))

    def proj_residual(o, w_cols, xv):
        cols = []
        for n in range(2):
            cols.append(xv[:, n * 512:(n + 1) * 512] + _dot(o, w_cols(n)))
        return jnp.concatenate(cols, axis=1)

    def woa_cols(n):
        return _as_bf16(jnp.concatenate([woap[4 * n + t] for t in range(4)], axis=1))

    def wob_cols(n):
        return wob[:, n * 512:(n + 1) * 512]

    def store_permuted(dst_ref, row0, val):
        for h in range(4):
            dst_ref[pl.ds(row0 + h, 16, stride=4), :] = val[h * 16:(h + 1) * 16]

    def rows16(blk, r):
        return pl.ds(pl.multiple_of(blk * BLK + r * 16, 16), 16)

    def ln1(blk, r, tok=None):
        rows = rows16(blk, r)
        xv = xio[rows, :].astype(f32)
        if tok is not None:
            xv = _after(xv, tok)
        x_ref[rows, :] = xv
        return _ln16(xv)

    def ln2(blk, r, tok=None):
        xv = x_ref[rows16(blk, r), :]
        if tok is not None:
            xv = _after(xv, tok)
        xn2[pl.ds(pl.multiple_of(blk * (BLK // 2) + r * 8, 8), 8), :] = _ln16(xv)

    def head_group0(xn_packed):
        q, k, v = qkv_group(0, _as_bf16(xn_packed))
        q0[...] = q
        k0[...] = k
        v0[...] = v
        return _token(k)

    def a_block(i):
        xn_cur = _as_bf16(xn1[...])
        qkv0 = (q0[...], k0[...], v0[...])
        ip = jnp.maximum(i - 1, 0)
        inx = jnp.minimum(i + 1, NB - 1)
        pos = i * BLK + lax.broadcasted_iota(jnp.int32, (8, 128), 1)
        o_cols = []
        xn_parts = []
        for g in range(NG):
            q, kc, vc = qkv0 if g == 0 else qkv_group(g, xn_cur)
            kp = khalo[g]
            vp = vhalo[g]
            khalo[g] = kc
            vhalo[g] = vc
            ot = _local_attention(q, kc, kp, vc, vp, pos)
            o_cols.append(ot.astype(bf16).T)
            if g >= 1:
                tok = _token(kc)
                if g <= 4:
                    xn_parts += [ln1(inx, 2 * g - 2, tok), ln1(inx, 2 * g - 1, tok)]
                else:
                    ln2(ip, 2 * g - 10, tok)
                    ln2(ip, 2 * g - 9, tok)
                if g == 5:
                    wsrc = _as_bf16(_after(pltpu.bitcast(wb_nat[i], u32), tok))
                    wbt[i] = pltpu.bitcast(wsrc.T, u32)
        xn_next = jnp.concatenate(xn_parts, axis=0)
        xn1[...] = xn_next
        tok = head_group0(xn_next)
        ln2(ip, 6, tok)
        ln2(ip, 7, tok)
        o = jnp.concatenate(o_cols, axis=1)
        rows = blk_rows(i)
        x_ref[rows, :] = proj_residual(o, woa_cols, x_ref[rows, :])

    def phase_a(rep):
        khalo[...] = jnp.zeros(khalo.shape, khalo.dtype)
        vhalo[...] = jnp.zeros(vhalo.shape, vhalo.dtype)
        xn_first = jnp.concatenate([ln1(0, r) for r in range(BLK // 16)], axis=0)
        xn1[...] = xn_first
        head_group0(xn_first)

        @pl.when(rep == 0)
        def _():
            woa_copy.wait()
            for g in range(NG):
                wv = pltpu.bitcast(woa[g * 128:(g + 1) * 128, :], u32)
                for t in range(NG):
                    store_permuted(woap.at[t], g * 64, wv[:, t * 128:(t + 1) * 128])

        def body(it, c):
            @pl.when(rep == 0)
            def _():
                for u in range(APB):
                    wb_copy(it * APB + u).wait()

            for u in range(APB):
                nxt = it * APB + u + 1

                @pl.when(jnp.logical_and(rep == 0, nxt < NB))
                def _():
                    x_copy(jnp.minimum(nxt, NB - 1)).wait()

            for u in range(APB):
                a_block(it * APB + u)
            return c
        with _scope("a_loop"):
            lax.fori_loop(0, NB // APB, body, 0)
        for r in range(BLK // 16):
            ln2(NB - 1, r)

    def phase_b_proj():
        def body(j, c):
            rows = blk_rows(j, TB // 2)
            xn = _as_bf16(xn2[rows, :])
            for r in range(4):
                w = _as_bf16(wbt[2 * r:2 * r + 2].reshape(128, D))
                y = _pack(_dot_nt(w, xn) * QSCALE)
                for b in range(TB // NQ):
                    qT[j * (TB // NQ) + b, r * 128:(r + 1) * 128, :] = y[:, b * NQ:(b + 1) * NQ]
            for r in range(4):
                w = _as_bf16(wbt[8 + 2 * r:8 + 2 * r + 2].reshape(128, D))
                y = _pack(_dot_nt(w, xn))
                for b in range(TB // MK):
                    vT[j * (TB // MK) + b, r * 128:(r + 1) * 128, :] = y[:, b * MK:(b + 1) * MK]
            for n in range(2):
                y = _pack(_dot(xn, wk[:, n * 512:(n + 1) * 512]))
                for t in range(4):
                    kN[4 * n + t, rows, :] = y[:, t * 128:(t + 1) * 128]
            return c
        lax.fori_loop(0, S // TB, body, 0)

    def phase_b_attn():
        off = [0, 0]

        def qm_of(t, qi, j):
            q = _as_bf16(qT[qi, pl.ds(pl.multiple_of(t * 64 + j * 16, 16), 16), :])
            parts = []
            if j > 0:
                parts.append(jnp.zeros((32 * j, NQ), bf16))
            parts.append(q)
            if j < 3:
                parts.append(jnp.zeros((32 * (3 - j), NQ), bf16))
            return jnp.concatenate(parts, axis=0)

        def qk_chunk(t, qm, c, par, m):
            k = _as_bf16(kN[t, c * (MK // 2):(c + 1) * (MK // 2), :])
            s = _dot(k, qm)
            sbufs[c][pl.ds(pl.multiple_of(off[0] + par * MK, 8), MK), :] = s
            sm = _tree(s.reshape(MK // 8, 8, NQ), jnp.maximum)
            return sm if m is None else jnp.maximum(m, sm)

        def pv_chunk(h, c, par, mrow, l, o):
            s = sbufs[c][pl.ds(pl.multiple_of(off[1] + par * MK, 8), MK), :]
            p = jnp.exp2(s - mrow)
            ls = jnp.sum(p.reshape(MK // 8, 8, NQ), axis=0)
            l = ls if l is None else l + ls
            v = _as_bf16(vT[c, pl.ds(pl.multiple_of(h * 16, 16), 16), :])
            oc = _dot(v, p.astype(bf16))
            o = oc if o is None else o + oc
            return l, o

        def flush_o(g, val):
            y = pltpu.bitcast(_as_bf16(val).T, u32)
            oN[g % NG, blk_rows(g // NG, NQ // 2), :] = y

        n_groups = NQT * NG
        otbuf[...] = jnp.zeros(otbuf.shape, u32)
        qm = qm_of(0, 0, 0)
        m0 = None
        for c in range(NC):
            m0 = qk_chunk(0, qm, c, 0, m0)
        qm = qm_of(0, 0, 1)
        m1 = None
        for c in range(DL):
            m1 = qk_chunk(0, qm, c, 1, m1)

        def group(g, g_next, carry, zero):
            qi = g // NG
            t = g % NG
            off[0] = lax.shift_right_logical(zero, 16) * 8
            off[1] = lax.shift_right_logical(zero, 17) * 8
            flush_o(jnp.maximum(g - 1, 0), otbuf[...])
            ms = {0: carry[0], 1: carry[1]}
            qms = {}
            l = o = mrow = None
            for n in range(4 * NC):
                j, c = divmod(n, NC)
                j2, c2 = divmod(n + NC + DL, NC)
                if j2 < 4 or g_next is not None:
                    t2 = t if j2 < 4 else g_next % NG
                    if j2 not in qms:
                        qms[j2] = qm_of(t2, qi if j2 < 4 else g_next // NG, j2 % 4)
                    ms[j2] = qk_chunk(t2, qms[j2], c2, j2 % 2, ms.get(j2))
                if c == 0:
                    mrow = jnp.max(ms[j], axis=0, keepdims=True)
                    l = o = None
                l, o = pv_chunk(t * 4 + j, c, j % 2, mrow, l, o)
                if c == NC - 1:
                    lrow = jnp.sum(l, axis=0, keepdims=True)
                    otbuf[j * 16:(j + 1) * 16, :] = _pack(o * (1.0 / lrow))
            return ms.get(4), ms.get(5)

        def body(it, ms):
            for u in range(GPB):
                g = it * GPB + u
                ms = group(g, jnp.minimum(g + 1, n_groups - 1), ms, it)
            return ms

        lax.fori_loop(0, n_groups // GPB, body, (m0, m1))
        off[0] = off[1] = 0
        flush_o(n_groups - 1, otbuf[...])

    def phase_b_out(rep):
        def body(j, c):
            rows = blk_rows(j, TF)
            xv = proj_residual(o_rows(j, TF), wob_cols, x_ref[rows, :])
            xio[rows, :] = xv.astype(bf16)

            @pl.when(rep == 1)
            def _():
                out_copy(j).start()
            return c
        lax.fori_loop(0, S // TF, body, 0)

    x_copy(0).start()
    for g in range(NG):
        for sec in range(3):
            wa_copy(g, sec).start()
    woa_copy.start()
    for i in range(1, NB):
        x_copy(i).start()
        wb_copy(i - 1).start()
    wb_copy(NB - 1).start()
    wk_copy.start()
    wob_copy.start()

    def wa_body(g, c):
        for sec in range(3):
            wa_copy(g, sec).wait()
        for sec in range(3):
            wv = pltpu.bitcast(wa_nat[g * 3 + sec].T, u32)
            for kt in range(NG):
                store_permuted(wat.at[g, kt], sec * 64, wv[:, kt * 128:(kt + 1) * 128])
        return c
    with _scope("wa_loop"):
        lax.fori_loop(0, NG, wa_body, 0)
        x_copy(0).wait()

    def layer_pair(rep, c):
        with _scope("phase_a"):
            phase_a(rep)

        @pl.when(rep == 0)
        def _():
            wk_copy.wait()
            wob_copy.wait()

        with _scope("b_proj"):
            phase_b_proj()
        with _scope("b_attn"):
            phase_b_attn()
        with _scope("b_out"):
            phase_b_out(rep)
        return c
    lax.fori_loop(0, 2, layer_pair, 0)
    for j in range(S // TF):
        out_copy(j).wait()


@jax.jit
def pallas_interleave_layers__sliding_local_dilated__softmax_full_mha__prompt_kernel(
    A_x: jax.Array,
    A_wqkv: jax.Array,
    A_wo: jax.Array,
    B_x: jax.Array,
    B_wqkv: jax.Array,
    B_wo: jax.Array,
):
    del B_x
    x = A_x.reshape(S, D)
    vm = pltpu.VMEM
    kshape, kdt = ((64, BLK), u32) if PACK_K else ((128, BLK), f32)
    vshape, vdt = ((64, BLK), u32) if PACK_V else ((128, BLK), f32)
    scratch = [
        vm((S, D), f32),
        vm((S, D), bf16),
        vm((BLK // 2, D), u32),
        vm((S // 2, D), u32),
        vm((3 * NG, D, 128), bf16),
        vm((NG, NG, 192, 128), u32),
        vm((D, D), bf16),
        vm((NG, D // 2, 128), u32),
        vm((2 * NG, D, 128), bf16),
        vm((2 * NG, 64, D), u32),
        vm((D, D), bf16),
        vm((D, D), bf16),
        vm((NG,) + kshape, kdt),
        vm((NG,) + vshape, vdt),
        vm((128, BLK), f32),
        vm(kshape, kdt),
        vm(vshape, vdt),
        vm((NQT, D // 2, NQ), u32),
        vm((NG, S // 2, 128), u32),
        vm((NC, D // 2, MK), u32),
        vm((NG, S // 2, 128), u32),
        vm((64, NQ), u32),
        pltpu.SemaphoreType.DMA((SEM_O + S // TF,)),
    ] + [vm((2 * MK, NQ), f32)] * NC
    out = pl.pallas_call(
        _kernel,
        out_shape=jax.ShapeDtypeStruct((S, D), bf16),
        in_specs=[pl.BlockSpec(memory_space=pl.ANY)] * 5,
        out_specs=pl.BlockSpec(memory_space=pl.ANY),
        scratch_shapes=scratch,
        compiler_params=pltpu.CompilerParams(vmem_limit_bytes=110 * 1024 * 1024),
        name="interleave_attn",
    )(x, A_wqkv, A_wo, B_wqkv, B_wo)
    return out.reshape(1, S, D)
```

```python
import jax
import jax.numpy as jnp
from jax import lax
import jax.experimental.pallas as pl
import jax.experimental.pallas.tpu as pltpu

S, D, H, DH = 2048, 1024, 32, 32
W_LOC, DIL = 8, 2
EPS = 1e-5
LOG2E = 1.4426950408889634
QSCALE = (DH ** -0.5) * LOG2E
NEG = -1e9 * LOG2E

BLK = 128
NB = S // BLK
NG = D // 128
NQ = 256
NQT = S // NQ
MK = 128
NC = S // MK
DL = 5
APB = 2
GPB = 4
TB = 256
TF = 256

SEM_WA = NB
SEM_WB = SEM_WA + 3 * NG
SEM_W = SEM_WB + 2 * NG
SEM_O = SEM_W + 3

PACK_K = False
PACK_V = True
UCH = 2
PROFILE_SCOPES = False

bf16 = jnp.bfloat16
f32 = jnp.float32
u32 = jnp.uint32
NT = (((1,), (1,)), ((), ()))


class _NoScope:
    def __enter__(self):
        return self

    def __exit__(self, *a):
        return False


def _scope(name):
    return jax.named_scope(name) if PROFILE_SCOPES else _NoScope()


def _pack(x):
    return pltpu.bitcast(x.astype(bf16), u32)


def _as_bf16(x):
    return pltpu.bitcast(x, bf16)


def _dot(a, b):
    return jnp.dot(a, b, preferred_element_type=f32)


def _dot_nt(a, b):
    return lax.dot_general(a, b, NT, preferred_element_type=f32)


def _layernorm_packed(x):
    outs = []
    for r in range(x.shape[0] // 16):
        xr = x[r * 16:(r + 1) * 16]
        mu = jnp.sum(xr, axis=1, keepdims=True) * (1.0 / D)
        xc = xr - mu
        var = jnp.sum(xc * xc, axis=1, keepdims=True) * (1.0 / D)
        outs.append(_pack(xc * lax.rsqrt(var + EPS)))
    return jnp.concatenate(outs, axis=0)


def _token(v):
    t = pltpu.bitcast(v[0:8, :], u32)
    return lax.shift_right_logical(jnp.bitwise_and(t, jnp.uint32(0xFFFF)), jnp.uint32(16))


def _after(x, tok):
    n, m = x.shape
    z = jnp.concatenate([jnp.concatenate([tok] * (m // 128), axis=1)] * (n // 8), axis=0)
    return pltpu.bitcast(jnp.bitwise_or(pltpu.bitcast(x, u32), z), x.dtype)


def _ln16(xr):
    mu = jnp.sum(xr, axis=1, keepdims=True) * (1.0 / D)
    xc = xr - mu
    var = jnp.sum(xc * xc, axis=1, keepdims=True) * (1.0 / D)
    return _pack(xc * lax.rsqrt(var + EPS))


def _tree(x, op):
    n = x.shape[0]
    while n > 1:
        n //= 2
        x = op(x[:n], x[n:])
    return x[0]


def _local_attention(q, kc, kp, vc, vp, pos):
    def shifted(cur, prev, u, w):
        n = UCH * (4 if cur.dtype == u32 else 8)
        x = cur[u * n:(u + 1) * n]
        if w:
            lane = lax.broadcasted_iota(jnp.int32, x.shape, 1)
            x = jnp.where(lane >= 128 - DIL * w, prev[u * n:(u + 1) * n], x)
            x = pltpu.roll(x, DIL * w, axis=1)
        if x.dtype == u32:
            x = _as_bf16(x).astype(f32)
        return x.reshape(UCH, 8, 128)

    even = lax.broadcasted_iota(jnp.int32, (8, 128), 0) % 2 == 0
    acc = [None] * W_LOC
    for u in range(16 // UCH):
        qu = q[u * UCH * 8:(u + 1) * UCH * 8].reshape(UCH, 8, 128)
        for w in range(W_LOC):
            t = _tree(qu * shifted(kc, kp, u, w), jnp.add)
            acc[w] = t if acc[w] is None else acc[w] + t
    logits = []
    for w in range(W_LOC):
        t = acc[w]
        t = t + jnp.where(even, pltpu.roll(t, 7, axis=0), pltpu.roll(t, 1, axis=0))
        t = t * QSCALE
        if w:
            t = jnp.where(pos >= DIL * w, t, NEG)
        logits.append(t)
    m = logits[0]
    for t in logits[1:]:
        m = jnp.maximum(m, t)
    ps = [jnp.exp2(t - m) for t in logits]
    l = ps[0]
    for p in ps[1:]:
        l = l + p
    r = 1.0 / l
    ps = [(p * r)[None] for p in ps]
    outs = []
    for u in range(16 // UCH):
        o = None
        for w in range(W_LOC):
            t = shifted(vc, vp, u, w) * ps[w]
            o = t if o is None else o + t
        outs.append(o.reshape(UCH * 8, 128))
    return jnp.concatenate(outs, axis=0)


def _kernel(x_hbm, wa_hbm, woa_hbm, wb_hbm, wob_hbm, out_hbm,
            x_ref, xio, xn1, xn2, wa_nat, wat, woa, woap, wb_nat, wbt, wk, wob,
            khalo, vhalo, q0, k0, v0, wstage, pxn, pbuf, po,
            qT, kN, vT, oN, otbuf,
            sem, *sbufs):

    def x_copy(i):
        rows = pl.ds(pl.multiple_of(i * BLK, BLK), BLK)
        return pltpu.make_async_copy(x_hbm.at[rows, :], xio.at[rows, :], sem.at[i])

    def wa_copy(g, sec):
        col = pl.multiple_of(sec * D + g * 128, 128)
        return pltpu.make_async_copy(
            wa_hbm.at[:, pl.ds(col, 128)], wa_nat.at[g * 3 + sec], sem.at[SEM_WA + g * 3 + sec])

    def wb_copy(c):
        col = pl.multiple_of(c * 128 + (c // 8) * D, 128)
        return pltpu.make_async_copy(
            wb_hbm.at[:, pl.ds(col, 128)], wb_nat.at[c], sem.at[SEM_WB + c])

    woa_copy = pltpu.make_async_copy(woa_hbm, woa, sem.at[SEM_W])
    wk_copy = pltpu.make_async_copy(wb_hbm.at[:, pl.ds(D, D)], wk, sem.at[SEM_W + 1])
    wob_copy = pltpu.make_async_copy(wob_hbm, wob, sem.at[SEM_W + 2])

    def out_copy(j):
        rows = pl.ds(pl.multiple_of(j * TF, TF), TF)
        return pltpu.make_async_copy(xio.at[rows, :], out_hbm.at[rows, :], sem.at[SEM_O + j])

    def blk_rows(i, n=BLK):
        return pl.ds(pl.multiple_of(i * n, n), n)

    def qkv_group(g, xn):
        w = jnp.concatenate([wat[g, kt] for kt in range(NG)], axis=1)
        r = _dot_nt(_as_bf16(w), xn)
        k = r[128:256]
        v = r[256:384]
        return r[0:128], _pack(k) if PACK_K else k, _pack(v) if PACK_V else v

    def o_rows(i, n):
        rows = blk_rows(i, n // 2)
        return _as_bf16(jnp.concatenate([oN[t, rows, :] for t in range(NG)], axis=1))

    def proj_residual(o, w_cols, xv):
        cols = []
        for n in range(2):
            cols.append(xv[:, n * 512:(n + 1) * 512] + _dot(o, w_cols(n)))
        return jnp.concatenate(cols, axis=1)

    def woa_cols(n):
        return _as_bf16(jnp.concatenate([woap[4 * n + t] for t in range(4)], axis=1))

    def wob_cols(n):
        return wob[:, n * 512:(n + 1) * 512]

    def store_permuted(dst_ref, row0, val):
        for h in range(4):
            dst_ref[pl.ds(row0 + h, 16, stride=4), :] = val[h * 16:(h + 1) * 16]

    def rows16(blk, r):
        return pl.ds(pl.multiple_of(blk * BLK + r * 16, 16), 16)

    def ln1(blk, r, tok=None):
        rows = rows16(blk, r)
        xv = xio[rows, :].astype(f32)
        if tok is not None:
            xv = _after(xv, tok)
        x_ref[rows, :] = xv
        return _ln16(xv)

    def ln2(blk, r, tok=None):
        xv = x_ref[rows16(blk, r), :]
        if tok is not None:
            xv = _after(xv, tok)
        xn2[pl.ds(pl.multiple_of(blk * (BLK // 2) + r * 8, 8), 8), :] = _ln16(xv)

    def head_group0(xn_packed):
        q, k, v = qkv_group(0, _as_bf16(xn_packed))
        q0[...] = q
        k0[...] = k
        v0[...] = v
        return _token(k)

    def a_block(i):
        xn_cur = _as_bf16(xn1[...])
        qkv0 = (q0[...], k0[...], v0[...])
        ip = jnp.maximum(i - 1, 0)
        inx = jnp.minimum(i + 1, NB - 1)
        pos = i * BLK + lax.broadcasted_iota(jnp.int32, (8, 128), 1)
        o_cols = []
        xn_parts = []
        for g in range(NG):
            q, kc, vc = qkv0 if g == 0 else qkv_group(g, xn_cur)
            kp = khalo[g]
            vp = vhalo[g]
            khalo[g] = kc
            vhalo[g] = vc
            ot = _local_attention(q, kc, kp, vc, vp, pos)
            o_cols.append(ot.astype(bf16).T)
            if g >= 1:
                tok = _token(kc)
                if g <= 4:
                    xn_parts += [ln1(inx, 2 * g - 2, tok), ln1(inx, 2 * g - 1, tok)]
                else:
                    ln2(ip, 2 * g - 10, tok)
                    ln2(ip, 2 * g - 9, tok)
                if g == 5:
                    wsrc = _as_bf16(_after(pltpu.bitcast(wb_nat[i], u32), tok))
                    wbt[i] = pltpu.bitcast(wsrc.T, u32)
        xn_next = jnp.concatenate(xn_parts, axis=0)
        xn1[...] = xn_next
        tok = head_group0(xn_next)
        ln2(ip, 6, tok)
        ln2(ip, 7, tok)
        o = jnp.concatenate(o_cols, axis=1)
        rows = blk_rows(i)
        x_ref[rows, :] = proj_residual(o, woa_cols, x_ref[rows, :])

    def startup():
        def transpose_wa(g):
            for sec in range(3):
                wv = pltpu.bitcast(wa_nat[g * 3 + sec].T, u32)
                for kt in range(NG):
                    store_permuted(wstage.at[kt], sec * 64, wv[:, kt * 128:(kt + 1) * 128])

        def project(g):
            w = wstage[...]
            wat[g] = w
            w = jnp.concatenate([w[kt] for kt in range(NG)], axis=1)
            return _dot_nt(_as_bf16(w), _as_bf16(pxn[...]))

        def attend(g, r):
            pos = lax.broadcasted_iota(jnp.int32, (8, 128), 1)
            kp = jnp.zeros(khalo.shape[1:], khalo.dtype)
            vp = jnp.zeros(vhalo.shape[1:], vhalo.dtype)
            for b in range(2):
                rb = r[:, b * BLK:(b + 1) * BLK]
                kc = _pack(rb[128:256]) if PACK_K else rb[128:256]
                vc = _pack(rb[256:384]) if PACK_V else rb[256:384]
                ot = _local_attention(rb[0:128], kc, kp, vc, vp, pos + b * BLK)
                po[g, b * 64:(b + 1) * 64, :] = pltpu.bitcast(ot.astype(bf16).T, u32)
                kp, vp = kc, vc
            khalo[g] = kp
            vhalo[g] = vp

        pbuf[...] = jnp.zeros(pbuf.shape, f32)
        x_copy(0).wait()
        x_copy(1).wait()
        for b in range(2):
            for r in range(BLK // 16):
                pxn[b * 64 + r * 8:b * 64 + (r + 1) * 8, :] = ln1(b, r)
        for sec in range(3):
            wa_copy(0, sec).wait()
        transpose_wa(0)

        def body(g, c):
            for sec in range(3):
                wa_copy(g + 1, sec).wait()
            prev = pbuf[...]
            pbuf[...] = project(g)
            transpose_wa(g + 1)
            attend(jnp.maximum(g - 1, 0), prev)
            return c
        lax.fori_loop(0, NG - 1, body, 0)

        x_copy(2).wait()
        prev = pbuf[...]
        r = project(NG - 1)
        attend(NG - 2, prev)
        xn_next = jnp.concatenate([ln1(2, r16) for r16 in range(BLK // 16)], axis=0)
        xn1[...] = xn_next
        head_group0(xn_next)
        attend(NG - 1, r)

        woa_copy.wait()
        wb_copy(0).wait()
        wb_copy(1).wait()
        for t in range(NG):
            wv = pltpu.bitcast(woa[:, t * 128:(t + 1) * 128], u32)
            for g in range(NG):
                store_permuted(woap.at[t], g * 64, wv[g * 64:(g + 1) * 64])
        for b in range(2):
            o = jnp.concatenate([po[g, b * 64:(b + 1) * 64, :] for g in range(NG)], axis=1)
            rows = blk_rows(b)
            x_ref[rows, :] = proj_residual(_as_bf16(o), woa_cols, x_ref[rows, :])
            wbt[b] = pltpu.bitcast(wb_nat[b].T, u32)
        for r16 in range(BLK // 16):
            ln2(0, r16)

    def phase_a(rep):
        @pl.when(rep == 1)
        def _():
            khalo[...] = jnp.zeros(khalo.shape, khalo.dtype)
            vhalo[...] = jnp.zeros(vhalo.shape, vhalo.dtype)
            xn_first = jnp.concatenate([ln1(0, r) for r in range(BLK // 16)], axis=0)
            xn1[...] = xn_first
            head_group0(xn_first)

        def body(it, c):
            @pl.when(rep == 0)
            def _():
                for u in range(APB):
                    wb_copy(it * APB + u).wait()

            for u in range(APB):
                nxt = it * APB + u + 1

                @pl.when(jnp.logical_and(rep == 0, nxt < NB))
                def _():
                    x_copy(jnp.minimum(nxt, NB - 1)).wait()

            for u in range(APB):
                a_block(it * APB + u)
            return c
        with _scope("a_loop"):
            lax.fori_loop(1 - rep, NB // APB, body, 0)
        for r in range(BLK // 16):
            ln2(NB - 1, r)

    def phase_b_proj():
        def body(j, c):
            rows = blk_rows(j, TB // 2)
            xn = _as_bf16(xn2[rows, :])
            for r in range(4):
                w = _as_bf16(wbt[2 * r:2 * r + 2].reshape(128, D))
                y = _pack(_dot_nt(w, xn) * QSCALE)
                for b in range(TB // NQ):
                    qT[j * (TB // NQ) + b, r * 128:(r + 1) * 128, :] = y[:, b * NQ:(b + 1) * NQ]
            for r in range(4):
                w = _as_bf16(wbt[8 + 2 * r:8 + 2 * r + 2].reshape(128, D))
                y = _pack(_dot_nt(w, xn))
                for b in range(TB // MK):
                    vT[j * (TB // MK) + b, r * 128:(r + 1) * 128, :] = y[:, b * MK:(b + 1) * MK]
            for n in range(2):
                y = _pack(_dot(xn, wk[:, n * 512:(n + 1) * 512]))
                for t in range(4):
                    kN[4 * n + t, rows, :] = y[:, t * 128:(t + 1) * 128]
            return c
        lax.fori_loop(0, S // TB, body, 0)

    def phase_b_attn():
        off = [0, 0]

        def qm_of(t, qi, j):
            q = _as_bf16(qT[qi, pl.ds(pl.multiple_of(t * 64 + j * 16, 16), 16), :])
            parts = []
            if j > 0:
                parts.append(jnp.zeros((32 * j, NQ), bf16))
            parts.append(q)
            if j < 3:
                parts.append(jnp.zeros((32 * (3 - j), NQ), bf16))
            return jnp.concatenate(parts, axis=0)

        def qk_chunk(t, qm, c, par, m):
            k = _as_bf16(kN[t, c * (MK // 2):(c + 1) * (MK // 2), :])
            s = _dot(k, qm)
            sbufs[c][pl.ds(pl.multiple_of(off[0] + par * MK, 8), MK), :] = s
            sm = _tree(s.reshape(MK // 8, 8, NQ), jnp.maximum)
            return sm if m is None else jnp.maximum(m, sm)

        def pv_chunk(h, c, par, mrow, l, o):
            s = sbufs[c][pl.ds(pl.multiple_of(off[1] + par * MK, 8), MK), :]
            p = jnp.exp2(s - mrow)
            ls = jnp.sum(p.reshape(MK // 8, 8, NQ), axis=0)
            l = ls if l is None else l + ls
            v = _as_bf16(vT[c, pl.ds(pl.multiple_of(h * 16, 16), 16), :])
            oc = _dot(v, p.astype(bf16))
            o = oc if o is None else o + oc
            return l, o

        def flush_o(g, val):
            y = pltpu.bitcast(_as_bf16(val).T, u32)
            oN[g % NG, blk_rows(g // NG, NQ // 2), :] = y

        n_groups = NQT * NG
        otbuf[...] = jnp.zeros(otbuf.shape, u32)
        qm = qm_of(0, 0, 0)
        m0 = None
        for c in range(NC):
            m0 = qk_chunk(0, qm, c, 0, m0)
        qm = qm_of(0, 0, 1)
        m1 = None
        for c in range(DL):
            m1 = qk_chunk(0, qm, c, 1, m1)

        def group(g, g_next, carry, zero):
            qi = g // NG
            t = g % NG
            off[0] = lax.shift_right_logical(zero, 16) * 8
            off[1] = lax.shift_right_logical(zero, 17) * 8
            flush_o(jnp.maximum(g - 1, 0), otbuf[...])
            ms = {0: carry[0], 1: carry[1]}
            qms = {}
            l = o = mrow = None
            for n in range(4 * NC):
                j, c = divmod(n, NC)
                j2, c2 = divmod(n + NC + DL, NC)
                if j2 < 4 or g_next is not None:
                    t2 = t if j2 < 4 else g_next % NG
                    if j2 not in qms:
                        qms[j2] = qm_of(t2, qi if j2 < 4 else g_next // NG, j2 % 4)
                    ms[j2] = qk_chunk(t2, qms[j2], c2, j2 % 2, ms.get(j2))
                if c == 0:
                    mrow = jnp.max(ms[j], axis=0, keepdims=True)
                    l = o = None
                l, o = pv_chunk(t * 4 + j, c, j % 2, mrow, l, o)
                if c == NC - 1:
                    lrow = jnp.sum(l, axis=0, keepdims=True)
                    otbuf[j * 16:(j + 1) * 16, :] = _pack(o * (1.0 / lrow))
            return ms.get(4), ms.get(5)

        def body(it, ms):
            for u in range(GPB):
                g = it * GPB + u
                ms = group(g, jnp.minimum(g + 1, n_groups - 1), ms, it)
            return ms

        lax.fori_loop(0, n_groups // GPB, body, (m0, m1))
        off[0] = off[1] = 0
        flush_o(n_groups - 1, otbuf[...])

    def phase_b_out(rep):
        def body(j, c):
            rows = blk_rows(j, TF)
            xv = proj_residual(o_rows(j, TF), wob_cols, x_ref[rows, :])
            xio[rows, :] = xv.astype(bf16)

            @pl.when(rep == 1)
            def _():
                out_copy(j).start()
            return c
        lax.fori_loop(0, S // TF, body, 0)

    x_copy(0).start()
    x_copy(1).start()
    for g in range(NG):
        for sec in range(3):
            wa_copy(g, sec).start()
    x_copy(2).start()
    woa_copy.start()
    wb_copy(0).start()
    wb_copy(1).start()
    for i in range(2, NB, 2):
        x_copy(i + 1).start()
        if i + 2 < NB:
            x_copy(i + 2).start()
        wb_copy(i).start()
        wb_copy(i + 1).start()
    wk_copy.start()
    wob_copy.start()

    with _scope("startup"):
        startup()

    def layer_pair(rep, c):
        with _scope("phase_a"):
            phase_a(rep)

        @pl.when(rep == 0)
        def _():
            wk_copy.wait()
            wob_copy.wait()

        with _scope("b_proj"):
            phase_b_proj()
        with _scope("b_attn"):
            phase_b_attn()
        with _scope("b_out"):
            phase_b_out(rep)
        return c
    lax.fori_loop(0, 2, layer_pair, 0)
    for j in range(S // TF):
        out_copy(j).wait()


@jax.jit
def pallas_interleave_layers__sliding_local_dilated__softmax_full_mha__prompt_kernel(
    A_x: jax.Array,
    A_wqkv: jax.Array,
    A_wo: jax.Array,
    B_x: jax.Array,
    B_wqkv: jax.Array,
    B_wo: jax.Array,
):
    del B_x
    x = A_x.reshape(S, D)
    vm = pltpu.VMEM
    kshape, kdt = ((64, BLK), u32) if PACK_K else ((128, BLK), f32)
    vshape, vdt = ((64, BLK), u32) if PACK_V else ((128, BLK), f32)
    scratch = [
        vm((S, D), f32),
        vm((S, D), bf16),
        vm((BLK // 2, D), u32),
        vm((S // 2, D), u32),
        vm((3 * NG, D, 128), bf16),
        vm((NG, NG, 192, 128), u32),
        vm((D, D), bf16),
        vm((NG, D // 2, 128), u32),
        vm((2 * NG, D, 128), bf16),
        vm((2 * NG, 64, D), u32),
        vm((D, D), bf16),
        vm((D, D), bf16),
        vm((NG,) + kshape, kdt),
        vm((NG,) + vshape, vdt),
        vm((128, BLK), f32),
        vm(kshape, kdt),
        vm(vshape, vdt),
        vm((NG, 192, 128), u32),
        vm((BLK, D), u32),
        vm((384, 2 * BLK), f32),
        vm((NG, BLK, 128), u32),
        vm((NQT, D // 2, NQ), u32),
        vm((NG, S // 2, 128), u32),
        vm((NC, D // 2, MK), u32),
        vm((NG, S // 2, 128), u32),
        vm((64, NQ), u32),
        pltpu.SemaphoreType.DMA((SEM_O + S // TF,)),
    ] + [vm((2 * MK, NQ), f32)] * NC
    out = pl.pallas_call(
        _kernel,
        out_shape=jax.ShapeDtypeStruct((S, D), bf16),
        in_specs=[pl.BlockSpec(memory_space=pl.ANY)] * 5,
        out_specs=pl.BlockSpec(memory_space=pl.ANY),
        scratch_shapes=scratch,
        compiler_params=pltpu.CompilerParams(vmem_limit_bytes=110 * 1024 * 1024),
        name="interleave_attn",
    )(x, A_wqkv, A_wo, B_wqkv, B_wo)
    return out.reshape(1, S, D)
```

```python
import jax
import jax.numpy as jnp
from jax import lax
import jax.experimental.pallas as pl
import jax.experimental.pallas.tpu as pltpu

S, D, H, DH = 2048, 1024, 32, 32
W_LOC, DIL = 8, 2
EPS = 1e-5
LOG2E = 1.4426950408889634
QSCALE = (DH ** -0.5) * LOG2E
NEG = -1e9 * LOG2E

BLK = 128
NB = S // BLK
NG = D // 128
NQ = 256
NQT = S // NQ
MK = 128
NC = S // MK
DL = 5
APB = 2
GPB = 4
TB = 256
TF = 256

SEM_WA = NB
SEM_WB = SEM_WA + 3 * NG
SEM_W = SEM_WB + 2 * NG
SEM_O = SEM_W + 3

PACK_K = False
PACK_V = True
UCH = 2
PROFILE_SCOPES = False

bf16 = jnp.bfloat16
f32 = jnp.float32
u32 = jnp.uint32
NT = (((1,), (1,)), ((), ()))


class _NoScope:
    def __enter__(self):
        return self

    def __exit__(self, *a):
        return False


def _scope(name):
    return jax.named_scope(name) if PROFILE_SCOPES else _NoScope()


def _pack(x):
    return pltpu.bitcast(x.astype(bf16), u32)


def _as_bf16(x):
    return pltpu.bitcast(x, bf16)


def _dot(a, b):
    return jnp.dot(a, b, preferred_element_type=f32)


def _dot_nt(a, b):
    return lax.dot_general(a, b, NT, preferred_element_type=f32)


def _layernorm_packed(x):
    outs = []
    for r in range(x.shape[0] // 16):
        xr = x[r * 16:(r + 1) * 16]
        mu = jnp.sum(xr, axis=1, keepdims=True) * (1.0 / D)
        xc = xr - mu
        var = jnp.sum(xc * xc, axis=1, keepdims=True) * (1.0 / D)
        outs.append(_pack(xc * lax.rsqrt(var + EPS)))
    return jnp.concatenate(outs, axis=0)


def _token(v):
    t = pltpu.bitcast(v[0:8, :], u32)
    return lax.shift_right_logical(jnp.bitwise_and(t, jnp.uint32(0xFFFF)), jnp.uint32(16))


def _after(x, tok):
    n, m = x.shape
    z = jnp.concatenate([jnp.concatenate([tok] * (m // 128), axis=1)] * (n // 8), axis=0)
    return pltpu.bitcast(jnp.bitwise_or(pltpu.bitcast(x, u32), z), x.dtype)


def _ln16(xr):
    mu = jnp.sum(xr, axis=1, keepdims=True) * (1.0 / D)
    xc = xr - mu
    var = jnp.sum(xc * xc, axis=1, keepdims=True) * (1.0 / D)
    return _pack(xc * lax.rsqrt(var + EPS))


def _tree(x, op):
    n = x.shape[0]
    while n > 1:
        n //= 2
        x = op(x[:n], x[n:])
    return x[0]


def _local_attention(q, kc, kp, vc, vp, pos):
    def shifted(cur, prev, u, w):
        n = UCH * (4 if cur.dtype == u32 else 8)
        x = cur[u * n:(u + 1) * n]
        if w:
            lane = lax.broadcasted_iota(jnp.int32, x.shape, 1)
            x = jnp.where(lane >= 128 - DIL * w, prev[u * n:(u + 1) * n], x)
            x = pltpu.roll(x, DIL * w, axis=1)
        if x.dtype == u32:
            x = _as_bf16(x).astype(f32)
        return x.reshape(UCH, 8, 128)

    even = lax.broadcasted_iota(jnp.int32, (8, 128), 0) % 2 == 0
    acc = [None] * W_LOC
    for u in range(16 // UCH):
        qu = q[u * UCH * 8:(u + 1) * UCH * 8].reshape(UCH, 8, 128)
        for w in range(W_LOC):
            t = _tree(qu * shifted(kc, kp, u, w), jnp.add)
            acc[w] = t if acc[w] is None else acc[w] + t
    logits = []
    for w in range(W_LOC):
        t = acc[w]
        t = t + jnp.where(even, pltpu.roll(t, 7, axis=0), pltpu.roll(t, 1, axis=0))
        t = t * QSCALE
        if w:
            t = jnp.where(pos >= DIL * w, t, NEG)
        logits.append(t)
    m = logits[0]
    for t in logits[1:]:
        m = jnp.maximum(m, t)
    ps = [jnp.exp2(t - m) for t in logits]
    l = ps[0]
    for p in ps[1:]:
        l = l + p
    r = 1.0 / l
    ps = [(p * r)[None] for p in ps]
    outs = []
    for u in range(16 // UCH):
        o = None
        for w in range(W_LOC):
            t = shifted(vc, vp, u, w) * ps[w]
            o = t if o is None else o + t
        outs.append(o.reshape(UCH * 8, 128))
    return jnp.concatenate(outs, axis=0)


def _kernel(x_hbm, wa_hbm, woa_hbm, wb_hbm, wob_hbm, out_hbm,
            x_ref, xio, xn1, xn2, wa_nat, wat, woa, woap, wb_nat, wbt, wk, wob,
            khalo, vhalo, q0, k0, v0, wstage, pxn, pbuf, po,
            qT, kN, vT, oN, otbuf,
            sem, *sbufs):

    def x_copy(i):
        rows = pl.ds(pl.multiple_of(i * BLK, BLK), BLK)
        return pltpu.make_async_copy(x_hbm.at[rows, :], xio.at[rows, :], sem.at[i])

    def wa_copy(g, sec):
        col = pl.multiple_of(sec * D + g * 128, 128)
        return pltpu.make_async_copy(
            wa_hbm.at[:, pl.ds(col, 128)], wa_nat.at[g * 3 + sec], sem.at[SEM_WA + g * 3 + sec])

    def wb_copy(c):
        col = pl.multiple_of(c * 128 + (c // 8) * D, 128)
        return pltpu.make_async_copy(
            wb_hbm.at[:, pl.ds(col, 128)], wb_nat.at[c], sem.at[SEM_WB + c])

    woa_copy = pltpu.make_async_copy(woa_hbm, woa, sem.at[SEM_W])
    wk_copy = pltpu.make_async_copy(wb_hbm.at[:, pl.ds(D, D)], wk, sem.at[SEM_W + 1])
    wob_copy = pltpu.make_async_copy(wob_hbm, wob, sem.at[SEM_W + 2])

    def out_copy(j):
        rows = pl.ds(pl.multiple_of(j * TF, TF), TF)
        return pltpu.make_async_copy(xio.at[rows, :], out_hbm.at[rows, :], sem.at[SEM_O + j])

    def blk_rows(i, n=BLK):
        return pl.ds(pl.multiple_of(i * n, n), n)

    def qkv_group(g, xn):
        w = jnp.concatenate([wat[g, kt] for kt in range(NG)], axis=1)
        r = _dot_nt(_as_bf16(w), xn)
        k = r[128:256]
        v = r[256:384]
        return r[0:128], _pack(k) if PACK_K else k, _pack(v) if PACK_V else v

    def o_rows(i, n):
        rows = blk_rows(i, n // 2)
        return _as_bf16(jnp.concatenate([oN[t, rows, :] for t in range(NG)], axis=1))

    def proj_residual(o, w_cols, xv):
        cols = []
        for n in range(2):
            cols.append(xv[:, n * 512:(n + 1) * 512] + _dot(o, w_cols(n)))
        return jnp.concatenate(cols, axis=1)

    def woa_cols(n):
        return _as_bf16(jnp.concatenate([woap[4 * n + t] for t in range(4)], axis=1))

    def wob_cols(n):
        return wob[:, n * 512:(n + 1) * 512]

    def store_permuted(dst_ref, row0, val):
        for h in range(4):
            dst_ref[pl.ds(row0 + h, 16, stride=4), :] = val[h * 16:(h + 1) * 16]

    def rows16(blk, r):
        return pl.ds(pl.multiple_of(blk * BLK + r * 16, 16), 16)

    def ln1(blk, r, tok=None):
        rows = rows16(blk, r)
        xv = xio[rows, :].astype(f32)
        if tok is not None:
            xv = _after(xv, tok)
        x_ref[rows, :] = xv
        return _ln16(xv)

    def ln2(blk, r, tok=None):
        xv = x_ref[rows16(blk, r), :]
        if tok is not None:
            xv = _after(xv, tok)
        xn2[pl.ds(pl.multiple_of(blk * (BLK // 2) + r * 8, 8), 8), :] = _ln16(xv)

    def head_group0(xn_packed):
        q, k, v = qkv_group(0, _as_bf16(xn_packed))
        q0[...] = q
        k0[...] = k
        v0[...] = v
        return _token(k)

    def a_block(i):
        xn_cur = _as_bf16(xn1[...])
        qkv0 = (q0[...], k0[...], v0[...])
        ip = jnp.maximum(i - 1, 0)
        inx = jnp.minimum(i + 1, NB - 1)
        pos = i * BLK + lax.broadcasted_iota(jnp.int32, (8, 128), 1)
        o_cols = []
        xn_parts = []
        for g in range(NG):
            q, kc, vc = qkv0 if g == 0 else qkv_group(g, xn_cur)
            kp = khalo[g]
            vp = vhalo[g]
            khalo[g] = kc
            vhalo[g] = vc
            ot = _local_attention(q, kc, kp, vc, vp, pos)
            o_cols.append(ot.astype(bf16).T)
            if g >= 1:
                tok = _token(kc)
                if g <= 4:
                    xn_parts += [ln1(inx, 2 * g - 2, tok), ln1(inx, 2 * g - 1, tok)]
                else:
                    ln2(ip, 2 * g - 10, tok)
                    ln2(ip, 2 * g - 9, tok)
                if g == 5:
                    wsrc = _as_bf16(_after(pltpu.bitcast(wb_nat[i], u32), tok))
                    wbt[i] = pltpu.bitcast(wsrc.T, u32)
        xn_next = jnp.concatenate(xn_parts, axis=0)
        xn1[...] = xn_next
        tok = head_group0(xn_next)
        ln2(ip, 6, tok)
        ln2(ip, 7, tok)
        o = jnp.concatenate(o_cols, axis=1)
        rows = blk_rows(i)
        x_ref[rows, :] = proj_residual(o, woa_cols, x_ref[rows, :])

    def startup():
        def transpose_wa(g, secs=(0, 1, 2)):
            for sec in secs:
                wv = pltpu.bitcast(wa_nat[g * 3 + sec].T, u32)
                for kt in range(NG):
                    store_permuted(wstage.at[kt], sec * 64, wv[:, kt * 128:(kt + 1) * 128])

        def project(g):
            w = wstage[...]
            wat[g] = w
            w = jnp.concatenate([w[kt] for kt in range(NG)], axis=1)
            return _dot_nt(_as_bf16(w), _as_bf16(pxn[...]))

        def attend(g, r):
            pos = lax.broadcasted_iota(jnp.int32, (8, 128), 1)
            kp = jnp.zeros(khalo.shape[1:], khalo.dtype)
            vp = jnp.zeros(vhalo.shape[1:], vhalo.dtype)
            for b in range(2):
                rb = r[:, b * BLK:(b + 1) * BLK]
                kc = _pack(rb[128:256]) if PACK_K else rb[128:256]
                vc = _pack(rb[256:384]) if PACK_V else rb[256:384]
                ot = _local_attention(rb[0:128], kc, kp, vc, vp, pos + b * BLK)
                po[g, b * 64:(b + 1) * 64, :] = pltpu.bitcast(ot.astype(bf16).T, u32)
                kp, vp = kc, vc
            khalo[g] = kp
            vhalo[g] = vp

        pbuf[...] = jnp.zeros(pbuf.shape, f32)
        x_copy(0).wait()
        x_copy(1).wait()
        for b in range(2):
            for r in range(BLK // 16):
                pxn[b * 64 + r * 8:b * 64 + (r + 1) * 8, :] = ln1(b, r)
        for sec in range(3):
            wa_copy(0, sec).wait()
            transpose_wa(0, (sec,))

        def body(g, c):
            for sec in range(3):
                wa_copy(g + 1, sec).wait()
            prev = pbuf[...]
            pbuf[...] = project(g)
            transpose_wa(g + 1)
            attend(jnp.maximum(g - 1, 0), prev)
            return c
        lax.fori_loop(0, NG - 1, body, 0)

        x_copy(2).wait()
        prev = pbuf[...]
        r = project(NG - 1)
        xn_next = jnp.concatenate([ln1(2, r16) for r16 in range(BLK // 16)], axis=0)
        xn1[...] = xn_next
        attend(NG - 2, _after(prev, _token(xn_next[56:64, 0:128])))
        head_group0(xn_next)
        attend(NG - 1, r)

        woa_copy.wait()
        wb_copy(0).wait()
        wb_copy(1).wait()
        for t in range(NG):
            wv = pltpu.bitcast(woa[:, t * 128:(t + 1) * 128], u32)
            for g in range(NG):
                store_permuted(woap.at[t], g * 64, wv[g * 64:(g + 1) * 64])
        for b in range(2):
            o = jnp.concatenate([po[g, b * 64:(b + 1) * 64, :] for g in range(NG)], axis=1)
            rows = blk_rows(b)
            x_ref[rows, :] = proj_residual(_as_bf16(o), woa_cols, x_ref[rows, :])
            wbt[b] = pltpu.bitcast(wb_nat[b].T, u32)
        for r16 in range(BLK // 16):
            ln2(0, r16)

    def phase_a(rep):
        @pl.when(rep == 1)
        def _():
            khalo[...] = jnp.zeros(khalo.shape, khalo.dtype)
            vhalo[...] = jnp.zeros(vhalo.shape, vhalo.dtype)
            xn_first = jnp.concatenate([ln1(0, r) for r in range(BLK // 16)], axis=0)
            xn1[...] = xn_first
            head_group0(xn_first)

        def body(it, c):
            @pl.when(rep == 0)
            def _():
                for u in range(APB):
                    wb_copy(it * APB + u).wait()

            for u in range(APB):
                nxt = it * APB + u + 1

                @pl.when(jnp.logical_and(rep == 0, nxt < NB))
                def _():
                    x_copy(jnp.minimum(nxt, NB - 1)).wait()

            for u in range(APB):
                a_block(it * APB + u)
            return c
        with _scope("a_loop"):
            lax.fori_loop(1 - rep, NB // APB, body, 0)
        for r in range(BLK // 16):
            ln2(NB - 1, r)

    def phase_b_proj():
        def body(j, c):
            rows = blk_rows(j, TB // 2)
            xn = _as_bf16(xn2[rows, :])
            for r in range(4):
                w = _as_bf16(wbt[2 * r:2 * r + 2].reshape(128, D))
                y = _pack(_dot_nt(w, xn) * QSCALE)
                for b in range(TB // NQ):
                    qT[j * (TB // NQ) + b, r * 128:(r + 1) * 128, :] = y[:, b * NQ:(b + 1) * NQ]
            for r in range(4):
                w = _as_bf16(wbt[8 + 2 * r:8 + 2 * r + 2].reshape(128, D))
                y = _pack(_dot_nt(w, xn))
                for b in range(TB // MK):
                    vT[j * (TB // MK) + b, r * 128:(r + 1) * 128, :] = y[:, b * MK:(b + 1) * MK]
            for n in range(2):
                y = _pack(_dot(xn, wk[:, n * 512:(n + 1) * 512]))
                for t in range(4):
                    kN[4 * n + t, rows, :] = y[:, t * 128:(t + 1) * 128]
            return c
        lax.fori_loop(0, S // TB, body, 0)

    def phase_b_attn():
        off = [0, 0]

        def qm_of(t, qi, j):
            q = _as_bf16(qT[qi, pl.ds(pl.multiple_of(t * 64 + j * 16, 16), 16), :])
            parts = []
            if j > 0:
                parts.append(jnp.zeros((32 * j, NQ), bf16))
            parts.append(q)
            if j < 3:
                parts.append(jnp.zeros((32 * (3 - j), NQ), bf16))
            return jnp.concatenate(parts, axis=0)

        def qk_chunk(t, qm, c, par, m):
            k = _as_bf16(kN[t, c * (MK // 2):(c + 1) * (MK // 2), :])
            s = _dot(k, qm)
            sbufs[c][pl.ds(pl.multiple_of(off[0] + par * MK, 8), MK), :] = s
            sm = _tree(s.reshape(MK // 8, 8, NQ), jnp.maximum)
            return sm if m is None else jnp.maximum(m, sm)

        def pv_chunk(h, c, par, mrow, l, o):
            s = sbufs[c][pl.ds(pl.multiple_of(off[1] + par * MK, 8), MK), :]
            p = jnp.exp2(s - mrow)
            ls = jnp.sum(p.reshape(MK // 8, 8, NQ), axis=0)
            l = ls if l is None else l + ls
            v = _as_bf16(vT[c, pl.ds(pl.multiple_of(h * 16, 16), 16), :])
            oc = _dot(v, p.astype(bf16))
            o = oc if o is None else o + oc
            return l, o

        def flush_o(g, val):
            y = pltpu.bitcast(_as_bf16(val).T, u32)
            oN[g % NG, blk_rows(g // NG, NQ // 2), :] = y

        n_groups = NQT * NG
        otbuf[...] = jnp.zeros(otbuf.shape, u32)
        qm = qm_of(0, 0, 0)
        m0 = None
        for c in range(NC):
            m0 = qk_chunk(0, qm, c, 0, m0)
        qm = qm_of(0, 0, 1)
        m1 = None
        for c in range(DL):
            m1 = qk_chunk(0, qm, c, 1, m1)

        def group(g, g_next, carry, zero):
            qi = g // NG
            t = g % NG
            off[0] = lax.shift_right_logical(zero, 16) * 8
            off[1] = lax.shift_right_logical(zero, 17) * 8
            flush_o(jnp.maximum(g - 1, 0), otbuf[...])
            ms = {0: carry[0], 1: carry[1]}
            qms = {}
            l = o = mrow = None
            for n in range(4 * NC):
                j, c = divmod(n, NC)
                j2, c2 = divmod(n + NC + DL, NC)
                if j2 < 4 or g_next is not None:
                    t2 = t if j2 < 4 else g_next % NG
                    if j2 not in qms:
                        qms[j2] = qm_of(t2, qi if j2 < 4 else g_next // NG, j2 % 4)
                    ms[j2] = qk_chunk(t2, qms[j2], c2, j2 % 2, ms.get(j2))
                if c == 0:
                    mrow = jnp.max(ms[j], axis=0, keepdims=True)
                    l = o = None
                l, o = pv_chunk(t * 4 + j, c, j % 2, mrow, l, o)
                if c == NC - 1:
                    lrow = jnp.sum(l, axis=0, keepdims=True)
                    otbuf[j * 16:(j + 1) * 16, :] = _pack(o * (1.0 / lrow))
            return ms.get(4), ms.get(5)

        def body(it, ms):
            for u in range(GPB):
                g = it * GPB + u
                ms = group(g, jnp.minimum(g + 1, n_groups - 1), ms, it)
            return ms

        lax.fori_loop(0, n_groups // GPB, body, (m0, m1))
        off[0] = off[1] = 0
        flush_o(n_groups - 1, otbuf[...])

    def phase_b_out(rep):
        def body(j, c):
            rows = blk_rows(j, TF)
            xv = proj_residual(o_rows(j, TF), wob_cols, x_ref[rows, :])
            xio[rows, :] = xv.astype(bf16)

            @pl.when(rep == 1)
            def _():
                out_copy(j).start()
            return c
        lax.fori_loop(0, S // TF, body, 0)

    x_copy(0).start()
    x_copy(1).start()
    for g in range(NG):
        if g == NG - 2:
            x_copy(2).start()
        for sec in range(3):
            wa_copy(g, sec).start()
    woa_copy.start()
    wb_copy(0).start()
    wb_copy(1).start()
    for i in range(2, NB, 2):
        x_copy(i + 1).start()
        if i + 2 < NB:
            x_copy(i + 2).start()
        wb_copy(i).start()
        wb_copy(i + 1).start()
    wk_copy.start()
    wob_copy.start()

    with _scope("startup"):
        startup()

    def layer_pair(rep, c):
        with _scope("phase_a"):
            phase_a(rep)

        @pl.when(rep == 0)
        def _():
            wk_copy.wait()
            wob_copy.wait()

        with _scope("b_proj"):
            phase_b_proj()
        with _scope("b_attn"):
            phase_b_attn()
        with _scope("b_out"):
            phase_b_out(rep)
        return c
    lax.fori_loop(0, 2, layer_pair, 0)
    for j in range(S // TF):
        out_copy(j).wait()


@jax.jit
def pallas_interleave_layers__sliding_local_dilated__softmax_full_mha__prompt_kernel(
    A_x: jax.Array,
    A_wqkv: jax.Array,
    A_wo: jax.Array,
    B_x: jax.Array,
    B_wqkv: jax.Array,
    B_wo: jax.Array,
):
    del B_x
    x = A_x.reshape(S, D)
    vm = pltpu.VMEM
    kshape, kdt = ((64, BLK), u32) if PACK_K else ((128, BLK), f32)
    vshape, vdt = ((64, BLK), u32) if PACK_V else ((128, BLK), f32)
    scratch = [
        vm((S, D), f32),
        vm((S, D), bf16),
        vm((BLK // 2, D), u32),
        vm((S // 2, D), u32),
        vm((3 * NG, D, 128), bf16),
        vm((NG, NG, 192, 128), u32),
        vm((D, D), bf16),
        vm((NG, D // 2, 128), u32),
        vm((2 * NG, D, 128), bf16),
        vm((2 * NG, 64, D), u32),
        vm((D, D), bf16),
        vm((D, D), bf16),
        vm((NG,) + kshape, kdt),
        vm((NG,) + vshape, vdt),
        vm((128, BLK), f32),
        vm(kshape, kdt),
        vm(vshape, vdt),
        vm((NG, 192, 128), u32),
        vm((BLK, D), u32),
        vm((384, 2 * BLK), f32),
        vm((NG, BLK, 128), u32),
        vm((NQT, D // 2, NQ), u32),
        vm((NG, S // 2, 128), u32),
        vm((NC, D // 2, MK), u32),
        vm((NG, S // 2, 128), u32),
        vm((64, NQ), u32),
        pltpu.SemaphoreType.DMA((SEM_O + S // TF,)),
    ] + [vm((2 * MK, NQ), f32)] * NC
    out = pl.pallas_call(
        _kernel,
        out_shape=jax.ShapeDtypeStruct((S, D), bf16),
        in_specs=[pl.BlockSpec(memory_space=pl.ANY)] * 5,
        out_specs=pl.BlockSpec(memory_space=pl.ANY),
        scratch_shapes=scratch,
        compiler_params=pltpu.CompilerParams(vmem_limit_bytes=110 * 1024 * 1024),
        name="interleave_attn",
    )(x, A_wqkv, A_wo, B_wqkv, B_wo)
    return out.reshape(1, S, D)
```

```python
import jax
import jax.numpy as jnp
from jax import lax
import jax.experimental.pallas as pl
import jax.experimental.pallas.tpu as pltpu

S, D, H, DH = 2048, 1024, 32, 32
W_LOC, DIL = 8, 2
EPS = 1e-5
LOG2E = 1.4426950408889634
QSCALE = (DH ** -0.5) * LOG2E
NEG = -1e9 * LOG2E

BLK = 128
NB = S // BLK
NG = D // 128
NQ = 256
NQT = S // NQ
MK = 128
NC = S // MK
DL = 5
APB = 2
GPB = 4
TB = 256
TF = 256

SEM_WA = NB
SEM_WB = SEM_WA + 3 * NG
SEM_W = SEM_WB + 2 * NG
SEM_O = SEM_W + 3

PACK_K = True
GM = 128
PACK_V = True
UCH = 2
LOCAL_OFF = False
LNMODE = 0
KLAG = 0
VLAG = 0
PROFILE_SCOPES = False

bf16 = jnp.bfloat16
f32 = jnp.float32
u32 = jnp.uint32
NT = (((1,), (1,)), ((), ()))


class _NoScope:
    def __enter__(self):
        return self

    def __exit__(self, *a):
        return False


def _scope(name):
    return jax.named_scope(name) if PROFILE_SCOPES else _NoScope()


def _pack(x):
    return pltpu.bitcast(x.astype(bf16), u32)


def _as_bf16(x):
    return pltpu.bitcast(x, bf16)


def _dot(a, b):
    return jnp.dot(a, b, preferred_element_type=f32)


def _dot_nt(a, b):
    return lax.dot_general(a, b, NT, preferred_element_type=f32)


def _layernorm_packed(x):
    outs = []
    for r in range(x.shape[0] // 16):
        xr = x[r * 16:(r + 1) * 16]
        mu = jnp.sum(xr, axis=1, keepdims=True) * (1.0 / D)
        xc = xr - mu
        var = jnp.sum(xc * xc, axis=1, keepdims=True) * (1.0 / D)
        outs.append(_pack(xc * lax.rsqrt(var + EPS)))
    return jnp.concatenate(outs, axis=0)


def _token(v):
    t = pltpu.bitcast(v[0:8, :], u32)
    return lax.shift_right_logical(jnp.bitwise_and(t, jnp.uint32(0xFFFF)), jnp.uint32(16))


def _after(x, tok):
    n, m = x.shape
    z = jnp.concatenate([jnp.concatenate([tok] * (m // 128), axis=1)] * (n // 8), axis=0)
    return pltpu.bitcast(jnp.bitwise_or(pltpu.bitcast(x, u32), z), x.dtype)


def _ln16(xr):
    if LNMODE == 1:
        return _pack(xr)
    if LNMODE == 2:
        mu = jnp.sum(xr, axis=1, keepdims=True) * (1.0 / D)
        ms = jnp.sum(xr * xr, axis=1, keepdims=True) * (1.0 / D)
        rs = lax.rsqrt(ms - mu * mu + EPS)
        return _pack(xr * rs - mu * rs)
    mu = jnp.sum(xr, axis=1, keepdims=True) * (1.0 / D)
    xc = xr - mu
    var = jnp.sum(xc * xc, axis=1, keepdims=True) * (1.0 / D)
    return _pack(xc * lax.rsqrt(var + EPS))


def _tree(x, op):
    n = x.shape[0]
    while n > 1:
        n //= 2
        x = op(x[:n], x[n:])
    return x[0]


def _local_attention(q, kc, kp, vc, vp, pos):
    def chunk(x, u, tok):
        if callable(x):
            return x(u)
        n = UCH * (4 if x.dtype == u32 else 8)
        x = x[u * n:(u + 1) * n]
        return x if tok is None else _after(x, tok)

    def shifted(cur, prev, w):
        x = cur
        if w:
            lane = lax.broadcasted_iota(jnp.int32, x.shape, 1)
            x = jnp.where(lane >= 128 - DIL * w, prev, x)
            x = pltpu.roll(x, DIL * w, axis=1)
        if x.dtype == u32:
            x = _as_bf16(x).astype(f32)
        return x.reshape(UCH, 8, 128)

    nu = 16 // UCH
    if LOCAL_OFF:
        return jnp.concatenate([chunk(q, u, None) for u in range(nu)], axis=0)
    even = lax.broadcasted_iota(jnp.int32, (8, 128), 0) % 2 == 0
    acc = [None] * W_LOC
    done = []
    for u in range(nu):
        tok = _token(done[u - KLAG]) if KLAG and u >= KLAG else None
        cur, prev = chunk(kc, u, tok), chunk(kp, u, None)
        qu = chunk(q, u, None).reshape(UCH, 8, 128)
        for w in range(W_LOC):
            t = _tree(qu * shifted(cur, prev, w), jnp.add)
            acc[w] = t if acc[w] is None else acc[w] + t
        done.append(acc[W_LOC - 1])
    logits = []
    for w in range(W_LOC):
        t = acc[w]
        t = t + jnp.where(even, pltpu.roll(t, 7, axis=0), pltpu.roll(t, 1, axis=0))
        t = t * QSCALE
        if w:
            t = jnp.where(pos >= DIL * w, t, NEG)
        logits.append(t)
    m = logits[0]
    for t in logits[1:]:
        m = jnp.maximum(m, t)
    ps = [jnp.exp2(t - m) for t in logits]
    l = ps[0]
    for p in ps[1:]:
        l = l + p
    r = 1.0 / l
    ps = [(p * r)[None] for p in ps]
    outs = []
    for u in range(nu):
        tok = None
        if VLAG:
            tok = _token(outs[u - VLAG] if u >= VLAG else done[nu - VLAG + u])
        cur, prev = chunk(vc, u, tok), chunk(vp, u, None)
        o = None
        for w in range(W_LOC):
            t = shifted(cur, prev, w) * ps[w]
            o = t if o is None else o + t
        outs.append(o.reshape(UCH * 8, 128))
    return jnp.concatenate(outs, axis=0)


def _kernel(x_hbm, wa_hbm, woa_hbm, wb_hbm, wob_hbm, out_hbm,
            x_ref, xio, xn1, xn2, wa_nat, wat, woa, woap, wb_nat, wbt, wk, wob,
            khalo, vhalo, wstage, pxn, pbuf, po,
            qT, kN, vT, oN, otbuf,
            sem, *bufs):
    sbufs = bufs[:NC]
    stg = [bufs[NC + 3 * g:NC + 3 * g + 3] for g in range(NG)]

    def x_copy(i):
        rows = pl.ds(pl.multiple_of(i * BLK, BLK), BLK)
        return pltpu.make_async_copy(x_hbm.at[rows, :], xio.at[rows, :], sem.at[i])

    def wa_copy(g, sec):
        col = pl.multiple_of(sec * D + g * 128, 128)
        return pltpu.make_async_copy(
            wa_hbm.at[:, pl.ds(col, 128)], wa_nat.at[g * 3 + sec], sem.at[SEM_WA + g * 3 + sec])

    def wb_copy(c):
        col = pl.multiple_of(c * 128 + (c // 8) * D, 128)
        return pltpu.make_async_copy(
            wb_hbm.at[:, pl.ds(col, 128)], wb_nat.at[c], sem.at[SEM_WB + c])

    woa_copy = pltpu.make_async_copy(woa_hbm, woa, sem.at[SEM_W])
    wk_copy = pltpu.make_async_copy(wb_hbm.at[:, pl.ds(D, D)], wk, sem.at[SEM_W + 1])
    wob_copy = pltpu.make_async_copy(wob_hbm, wob, sem.at[SEM_W + 2])

    def out_copy(j):
        rows = pl.ds(pl.multiple_of(j * TF, TF), TF)
        return pltpu.make_async_copy(xio.at[rows, :], out_hbm.at[rows, :], sem.at[SEM_O + j])

    def blk_rows(i, n=BLK):
        return pl.ds(pl.multiple_of(i * n, n), n)

    def qkv_group(g, xn):
        w = jnp.concatenate([wat[g, kt] for kt in range(NG)], axis=1)
        r = jnp.concatenate(
            [_dot_nt(_as_bf16(w[a:a + GM // 2]), xn) for a in range(0, 192, GM // 2)], axis=0)
        k = r[128:256]
        v = r[256:384]
        return r[0:128], _pack(k) if PACK_K else k, _pack(v) if PACK_V else v

    def o_rows(i, n):
        rows = blk_rows(i, n // 2)
        return _as_bf16(jnp.concatenate([oN[t, rows, :] for t in range(NG)], axis=1))

    def proj_residual(o, w_cols, xv):
        cols = []
        for n in range(2):
            cols.append(xv[:, n * 512:(n + 1) * 512] + _dot(o, w_cols(n)))
        return jnp.concatenate(cols, axis=1)

    def woa_cols(n):
        return _as_bf16(jnp.concatenate([woap[4 * n + t] for t in range(4)], axis=1))

    def wob_cols(n):
        return wob[:, n * 512:(n + 1) * 512]

    def store_permuted(dst_ref, row0, val):
        for h in range(4):
            dst_ref[pl.ds(row0 + h, 16, stride=4), :] = val[h * 16:(h + 1) * 16]

    def rows16(blk, r):
        return pl.ds(pl.multiple_of(blk * BLK + r * 16, 16), 16)

    def ln1(blk, r, tok=None):
        rows = rows16(blk, r)
        xv = xio[rows, :].astype(f32)
        if tok is not None:
            xv = _after(xv, tok)
        x_ref[rows, :] = xv
        return _ln16(xv)

    def ln2(blk, r, tok=None):
        xv = x_ref[rows16(blk, r), :]
        if tok is not None:
            xv = _after(xv, tok)
        xn2[pl.ds(pl.multiple_of(blk * (BLK // 2) + r * 8, 8), 8), :] = _ln16(xv)

    def head_group0(xn_packed):
        for ref, val in zip(stg[0], qkv_group(0, _as_bf16(xn_packed))):
            ref[0:val.shape[0], :] = val

    def a_block(i, par, z0, z1):
        xn_cur = _as_bf16(xn1[...])
        ip = jnp.maximum(i - 1, 0)
        inx = jnp.minimum(i + 1, NB - 1)
        pos = i * BLK + lax.broadcasted_iota(jnp.int32, (8, 128), 1)

        def stage(g, slot, qkv):
            for ref, val in zip(stg[g], qkv):
                n = val.shape[0]
                ref[pl.ds(pl.multiple_of(z0 + slot * n, 8), n), :] = val

        def getter(ref, slot):
            n = ref.shape[0] // 2
            m = n // (16 // UCH)
            return lambda u: ref[pl.ds(pl.multiple_of(z1 + slot * n + u * m, 8), m), :]

        o_cols = []
        xn_parts = []
        for g in range(NG):
            if g:
                qkv = qkv_group(g, xn_cur)
                stage(g, par, qkv)
            qs, ks, vs = stg[g]
            ot = _local_attention(getter(qs, par), getter(ks, par), getter(ks, 1 - par),
                                  getter(vs, par), getter(vs, 1 - par), pos)
            o_cols.append(ot.astype(bf16).T)
            if g >= 1:
                tok = _token(qkv[1])
                if g <= 4:
                    xn_parts += [ln1(inx, 2 * g - 2, tok), ln1(inx, 2 * g - 1, tok)]
                else:
                    ln2(ip, 2 * g - 10, tok)
                    ln2(ip, 2 * g - 9, tok)
                if g == 5:
                    wsrc = _as_bf16(_after(pltpu.bitcast(wb_nat[i], u32), tok))
                    wbt[i] = pltpu.bitcast(wsrc.T, u32)
        xn_next = jnp.concatenate(xn_parts, axis=0)
        xn1[...] = xn_next
        qkv = qkv_group(0, _as_bf16(xn_next))
        stage(0, 1 - par, qkv)
        tok = _token(qkv[1])
        ln2(ip, 6, tok)
        ln2(ip, 7, tok)
        o = jnp.concatenate(o_cols, axis=1)
        rows = blk_rows(i)
        x_ref[rows, :] = proj_residual(o, woa_cols, x_ref[rows, :])

    def startup():
        def transpose_wa(g, secs=(0, 1, 2)):
            for sec in secs:
                wv = pltpu.bitcast(wa_nat[g * 3 + sec].T, u32)
                for kt in range(NG):
                    store_permuted(wstage.at[kt], sec * 64, wv[:, kt * 128:(kt + 1) * 128])

        def project(g):
            w = wstage[...]
            wat[g] = w
            w = jnp.concatenate([w[kt] for kt in range(NG)], axis=1)
            return _dot_nt(_as_bf16(w), _as_bf16(pxn[...]))

        def attend(g, r):
            pos = lax.broadcasted_iota(jnp.int32, (8, 128), 1)
            kp = jnp.zeros(khalo.shape[1:], khalo.dtype)
            vp = jnp.zeros(vhalo.shape[1:], vhalo.dtype)
            for b in range(2):
                rb = r[:, b * BLK:(b + 1) * BLK]
                kc = _pack(rb[128:256]) if PACK_K else rb[128:256]
                vc = _pack(rb[256:384]) if PACK_V else rb[256:384]
                ot = _local_attention(rb[0:128], kc, kp, vc, vp, pos + b * BLK)
                po[g, b * 64:(b + 1) * 64, :] = pltpu.bitcast(ot.astype(bf16).T, u32)
                kp, vp = kc, vc
            khalo[g] = kp
            vhalo[g] = vp

        pbuf[...] = jnp.zeros(pbuf.shape, f32)
        x_copy(0).wait()
        x_copy(1).wait()
        for b in range(2):
            for r in range(BLK // 16):
                pxn[b * 64 + r * 8:b * 64 + (r + 1) * 8, :] = ln1(b, r)
        for sec in range(3):
            wa_copy(0, sec).wait()
            transpose_wa(0, (sec,))

        def body(g, c):
            for sec in range(3):
                wa_copy(g + 1, sec).wait()
            prev = pbuf[...]
            pbuf[...] = project(g)
            transpose_wa(g + 1)
            attend(jnp.maximum(g - 1, 0), prev)
            return c
        lax.fori_loop(0, NG - 1, body, 0)

        x_copy(2).wait()
        prev = pbuf[...]
        r = project(NG - 1)
        xn_next = jnp.concatenate([ln1(2, r16) for r16 in range(BLK // 16)], axis=0)
        xn1[...] = xn_next
        attend(NG - 2, _after(prev, _token(xn_next[56:64, 0:128])))
        head_group0(xn_next)
        attend(NG - 1, r)

        woa_copy.wait()
        wb_copy(0).wait()
        wb_copy(1).wait()
        for t in range(NG):
            wv = pltpu.bitcast(woa[:, t * 128:(t + 1) * 128], u32)
            for g in range(NG):
                store_permuted(woap.at[t], g * 64, wv[g * 64:(g + 1) * 64])
        for b in range(2):
            o = jnp.concatenate([po[g, b * 64:(b + 1) * 64, :] for g in range(NG)], axis=1)
            rows = blk_rows(b)
            x_ref[rows, :] = proj_residual(_as_bf16(o), woa_cols, x_ref[rows, :])
            wbt[b] = pltpu.bitcast(wb_nat[b].T, u32)
        for r16 in range(BLK // 16):
            ln2(0, r16)
        for g in range(NG):
            for ref, src in ((stg[g][1], khalo), (stg[g][2], vhalo)):
                n = src.shape[1]
                ref[n:2 * n, :] = src[g]

    def phase_a(rep):
        @pl.when(rep == 1)
        def _():
            for g in range(NG):
                for ref in stg[g][1:]:
                    n = ref.shape[0] // 2
                    ref[n:2 * n, :] = jnp.zeros((n, BLK), ref.dtype)
            xn_first = jnp.concatenate([ln1(0, r) for r in range(BLK // 16)], axis=0)
            xn1[...] = xn_first
            head_group0(xn_first)

        def body(it, c):
            @pl.when(rep == 0)
            def _():
                for u in range(APB):
                    wb_copy(it * APB + u).wait()

            for u in range(APB):
                nxt = it * APB + u + 1

                @pl.when(jnp.logical_and(rep == 0, nxt < NB))
                def _():
                    x_copy(jnp.minimum(nxt, NB - 1)).wait()

            z0 = lax.shift_right_logical(it, 16) * 8
            z1 = lax.shift_right_logical(it, 17) * 8
            for u in range(APB):
                a_block(it * APB + u, u % 2, z0, z1)
            return c
        with _scope("a_loop"):
            lax.fori_loop(1 - rep, NB // APB, body, 0)
        for r in range(BLK // 16):
            ln2(NB - 1, r)

    def phase_b_proj():
        def body(j, c):
            rows = blk_rows(j, TB // 2)
            xn = _as_bf16(xn2[rows, :])
            for n in range(2):
                y = _pack(_dot(xn, wk[:, n * 512:(n + 1) * 512]))
                for t in range(4):
                    kN[4 * n + t, rows, :] = y[:, t * 128:(t + 1) * 128]
            for r in range(4):
                w = _as_bf16(wbt[2 * r:2 * r + 2].reshape(128, D))
                y = _pack(_dot_nt(w, xn) * QSCALE)
                for b in range(TB // NQ):
                    qT[j * (TB // NQ) + b, r * 128:(r + 1) * 128, :] = y[:, b * NQ:(b + 1) * NQ]
            for r in range(4):
                w = _as_bf16(wbt[8 + 2 * r:8 + 2 * r + 2].reshape(128, D))
                y = _pack(_dot_nt(w, xn))
                for b in range(TB // MK):
                    vT[j * (TB // MK) + b, r * 128:(r + 1) * 128, :] = y[:, b * MK:(b + 1) * MK]
            return c
        lax.fori_loop(0, S // TB, body, 0)

    def phase_b_attn():
        off = [0, 0]

        def qm_of(t, qi, j):
            q = _as_bf16(qT[qi, pl.ds(pl.multiple_of(t * 64 + j * 16, 16), 16), :])
            parts = []
            if j > 0:
                parts.append(jnp.zeros((32 * j, NQ), bf16))
            parts.append(q)
            if j < 3:
                parts.append(jnp.zeros((32 * (3 - j), NQ), bf16))
            return jnp.concatenate(parts, axis=0)

        def qk_chunk(t, qm, c, par, m):
            k = _as_bf16(kN[t, c * (MK // 2):(c + 1) * (MK // 2), :])
            s = _dot(k, qm)
            sbufs[c][pl.ds(pl.multiple_of(off[0] + par * MK, 8), MK), :] = s
            sm = _tree(s.reshape(MK // 8, 8, NQ), jnp.maximum)
            return sm if m is None else jnp.maximum(m, sm)

        def pv_chunk(h, c, par, mrow, l, o):
            s = sbufs[c][pl.ds(pl.multiple_of(off[1] + par * MK, 8), MK), :]
            p = jnp.exp2(s - mrow)
            ls = jnp.sum(p.reshape(MK // 8, 8, NQ), axis=0)
            l = ls if l is None else l + ls
            v = _as_bf16(vT[c, pl.ds(pl.multiple_of(h * 16, 16), 16), :])
            oc = _dot(v, p.astype(bf16))
            o = oc if o is None else o + oc
            return l, o

        def flush_o(g, val):
            y = pltpu.bitcast(_as_bf16(val).T, u32)
            oN[g % NG, blk_rows(g // NG, NQ // 2), :] = y

        n_groups = NQT * NG
        otbuf[...] = jnp.zeros(otbuf.shape, u32)
        qm = qm_of(0, 0, 0)
        m0 = None
        for c in range(NC):
            m0 = qk_chunk(0, qm, c, 0, m0)
        qm = qm_of(0, 0, 1)
        m1 = None
        for c in range(DL):
            m1 = qk_chunk(0, qm, c, 1, m1)

        def group(g, g_next, carry, zero):
            qi = g // NG
            t = g % NG
            off[0] = lax.shift_right_logical(zero, 16) * 8
            off[1] = lax.shift_right_logical(zero, 17) * 8
            flush_o(jnp.maximum(g - 1, 0), otbuf[...])
            ms = {0: carry[0], 1: carry[1]}
            qms = {}
            l = o = mrow = None
            for n in range(4 * NC):
                j, c = divmod(n, NC)
                j2, c2 = divmod(n + NC + DL, NC)
                if j2 < 4 or g_next is not None:
                    t2 = t if j2 < 4 else g_next % NG
                    if j2 not in qms:
                        qms[j2] = qm_of(t2, qi if j2 < 4 else g_next // NG, j2 % 4)
                    ms[j2] = qk_chunk(t2, qms[j2], c2, j2 % 2, ms.get(j2))
                if c == 0:
                    mrow = jnp.max(ms[j], axis=0, keepdims=True)
                    l = o = None
                l, o = pv_chunk(t * 4 + j, c, j % 2, mrow, l, o)
                if c == NC - 1:
                    lrow = jnp.sum(l, axis=0, keepdims=True)
                    otbuf[j * 16:(j + 1) * 16, :] = _pack(o * (1.0 / lrow))
            return ms.get(4), ms.get(5)

        def body(it, ms):
            for u in range(GPB):
                g = it * GPB + u
                ms = group(g, jnp.minimum(g + 1, n_groups - 1), ms, it)
            return ms

        lax.fori_loop(0, n_groups // GPB, body, (m0, m1))
        off[0] = off[1] = 0
        flush_o(n_groups - 1, otbuf[...])

    def phase_b_out(rep):
        def body(j, c):
            rows = blk_rows(j, TF)
            xv = proj_residual(o_rows(j, TF), wob_cols, x_ref[rows, :])
            xio[rows, :] = xv.astype(bf16)

            @pl.when(rep == 1)
            def _():
                out_copy(j).start()
            return c
        lax.fori_loop(0, S // TF, body, 0)

    x_copy(0).start()
    x_copy(1).start()
    for g in range(NG):
        if g == NG - 2:
            x_copy(2).start()
        for sec in range(3):
            wa_copy(g, sec).start()
    woa_copy.start()
    wb_copy(0).start()
    wb_copy(1).start()
    for i in range(2, NB, 2):
        x_copy(i + 1).start()
        if i + 2 < NB:
            x_copy(i + 2).start()
        wb_copy(i).start()
        wb_copy(i + 1).start()
    wk_copy.start()
    wob_copy.start()

    with _scope("startup"):
        startup()

    def layer_pair(rep, c):
        with _scope("phase_a"):
            phase_a(rep)

        @pl.when(rep == 0)
        def _():
            wk_copy.wait()
            wob_copy.wait()

        with _scope("b_proj"):
            phase_b_proj()
        with _scope("b_attn"):
            phase_b_attn()
        with _scope("b_out"):
            phase_b_out(rep)
        return c
    lax.fori_loop(0, 2, layer_pair, 0)
    for j in range(S // TF):
        out_copy(j).wait()


@jax.jit
def pallas_interleave_layers__sliding_local_dilated__softmax_full_mha__prompt_kernel(
    A_x: jax.Array,
    A_wqkv: jax.Array,
    A_wo: jax.Array,
    B_x: jax.Array,
    B_wqkv: jax.Array,
    B_wo: jax.Array,
):
    del B_x
    x = A_x.reshape(S, D)
    vm = pltpu.VMEM
    kshape, kdt = ((64, BLK), u32) if PACK_K else ((128, BLK), f32)
    vshape, vdt = ((64, BLK), u32) if PACK_V else ((128, BLK), f32)
    scratch = [
        vm((S, D), f32),
        vm((S, D), bf16),
        vm((BLK // 2, D), u32),
        vm((S // 2, D), u32),
        vm((3 * NG, D, 128), bf16),
        vm((NG, NG, 192, 128), u32),
        vm((D, D), bf16),
        vm((NG, D // 2, 128), u32),
        vm((2 * NG, D, 128), bf16),
        vm((2 * NG, 64, D), u32),
        vm((D, D), bf16),
        vm((D, D), bf16),
        vm((NG,) + kshape, kdt),
        vm((NG,) + vshape, vdt),
        vm((NG, 192, 128), u32),
        vm((BLK, D), u32),
        vm((384, 2 * BLK), f32),
        vm((NG, BLK, 128), u32),
        vm((NQT, D // 2, NQ), u32),
        vm((NG, S // 2, 128), u32),
        vm((NC, D // 2, MK), u32),
        vm((NG, S // 2, 128), u32),
        vm((64, NQ), u32),
        pltpu.SemaphoreType.DMA((SEM_O + S // TF,)),
    ] + [vm((2 * MK, NQ), f32)] * NC + [
        vm((256, BLK), f32), vm((2 * kshape[0], BLK), kdt), vm((2 * vshape[0], BLK), vdt)] * NG
    out = pl.pallas_call(
        _kernel,
        out_shape=jax.ShapeDtypeStruct((S, D), bf16),
        in_specs=[pl.BlockSpec(memory_space=pl.ANY)] * 5,
        out_specs=pl.BlockSpec(memory_space=pl.ANY),
        scratch_shapes=scratch,
        compiler_params=pltpu.CompilerParams(vmem_limit_bytes=110 * 1024 * 1024),
        name="interleave_attn",
    )(x, A_wqkv, A_wo, B_wqkv, B_wo)
    return out.reshape(1, S, D)
```

```python
import jax
import jax.numpy as jnp
from jax import lax
import jax.experimental.pallas as pl
import jax.experimental.pallas.tpu as pltpu

S, D, H, DH = 2048, 1024, 32, 32
W_LOC, DIL = 8, 2
EPS = 1e-5
LOG2E = 1.4426950408889634
QSCALE = (DH ** -0.5) * LOG2E
NEG = -1e9 * LOG2E

BLK = 128
NB = S // BLK
NG = D // 128
NQ = 256
NQT = S // NQ
MK = 128
NC = S // MK
DL = 5
APB = 2
GPB = 4
TB = 256
TF = 256

SEM_X01, SEM_X2, SEM_WOB, SEM_OUT = 0, 1, 2, 3
SEM_WA = 4
SEM_IT = SEM_WA + NG
N_SEM = SEM_IT + NB // APB

PACK_K = True
GM = 128
PACK_V = True
UCH = 2
LOCAL_OFF = False
LNMODE = 0
KLAG = 0
VLAG = 0
PROFILE_SCOPES = False

bf16 = jnp.bfloat16
f32 = jnp.float32
u32 = jnp.uint32
NT = (((1,), (1,)), ((), ()))


class _NoScope:
    def __enter__(self):
        return self

    def __exit__(self, *a):
        return False


def _scope(name):
    return jax.named_scope(name) if PROFILE_SCOPES else _NoScope()


def _pack(x):
    return pltpu.bitcast(x.astype(bf16), u32)


def _as_bf16(x):
    return pltpu.bitcast(x, bf16)


def _dot(a, b):
    return jnp.dot(a, b, preferred_element_type=f32)


def _dot_nt(a, b):
    return lax.dot_general(a, b, NT, preferred_element_type=f32)


def _layernorm_packed(x):
    outs = []
    for r in range(x.shape[0] // 16):
        xr = x[r * 16:(r + 1) * 16]
        mu = jnp.sum(xr, axis=1, keepdims=True) * (1.0 / D)
        xc = xr - mu
        var = jnp.sum(xc * xc, axis=1, keepdims=True) * (1.0 / D)
        outs.append(_pack(xc * lax.rsqrt(var + EPS)))
    return jnp.concatenate(outs, axis=0)


def _token(v):
    t = pltpu.bitcast(v[0:8, :], u32)
    return lax.shift_right_logical(jnp.bitwise_and(t, jnp.uint32(0xFFFF)), jnp.uint32(16))


def _after(x, tok):
    n, m = x.shape
    z = jnp.concatenate([jnp.concatenate([tok] * (m // 128), axis=1)] * (n // 8), axis=0)
    return pltpu.bitcast(jnp.bitwise_or(pltpu.bitcast(x, u32), z), x.dtype)


def _ln16(xr):
    if LNMODE == 1:
        return _pack(xr)
    if LNMODE == 2:
        mu = jnp.sum(xr, axis=1, keepdims=True) * (1.0 / D)
        ms = jnp.sum(xr * xr, axis=1, keepdims=True) * (1.0 / D)
        rs = lax.rsqrt(ms - mu * mu + EPS)
        return _pack(xr * rs - mu * rs)
    mu = jnp.sum(xr, axis=1, keepdims=True) * (1.0 / D)
    xc = xr - mu
    var = jnp.sum(xc * xc, axis=1, keepdims=True) * (1.0 / D)
    return _pack(xc * lax.rsqrt(var + EPS))


def _tree(x, op):
    n = x.shape[0]
    while n > 1:
        n //= 2
        x = op(x[:n], x[n:])
    return x[0]


def _local_attention(q, kc, kp, vc, vp, pos):
    def chunk(x, u, tok):
        if callable(x):
            return x(u)
        n = UCH * (4 if x.dtype == u32 else 8)
        x = x[u * n:(u + 1) * n]
        return x if tok is None else _after(x, tok)

    def shifted(cur, prev, w):
        x = cur
        if w:
            lane = lax.broadcasted_iota(jnp.int32, x.shape, 1)
            x = jnp.where(lane >= 128 - DIL * w, prev, x)
            x = pltpu.roll(x, DIL * w, axis=1)
        if x.dtype == u32:
            x = _as_bf16(x).astype(f32)
        return x.reshape(UCH, 8, 128)

    nu = 16 // UCH
    if LOCAL_OFF:
        return jnp.concatenate([chunk(q, u, None) for u in range(nu)], axis=0)
    even = lax.broadcasted_iota(jnp.int32, (8, 128), 0) % 2 == 0
    acc = [None] * W_LOC
    done = []
    for u in range(nu):
        tok = _token(done[u - KLAG]) if KLAG and u >= KLAG else None
        cur, prev = chunk(kc, u, tok), chunk(kp, u, None)
        qu = chunk(q, u, None).reshape(UCH, 8, 128)
        for w in range(W_LOC):
            t = _tree(qu * shifted(cur, prev, w), jnp.add)
            acc[w] = t if acc[w] is None else acc[w] + t
        done.append(acc[W_LOC - 1])
    logits = []
    for w in range(W_LOC):
        t = acc[w]
        t = t + jnp.where(even, pltpu.roll(t, 7, axis=0), pltpu.roll(t, 1, axis=0))
        t = t * QSCALE
        if w:
            t = jnp.where(pos >= DIL * w, t, NEG)
        logits.append(t)
    m = logits[0]
    for t in logits[1:]:
        m = jnp.maximum(m, t)
    ps = [jnp.exp2(t - m) for t in logits]
    l = ps[0]
    for p in ps[1:]:
        l = l + p
    r = 1.0 / l
    ps = [(p * r)[None] for p in ps]
    outs = []
    for u in range(nu):
        tok = None
        if VLAG:
            tok = _token(outs[u - VLAG] if u >= VLAG else done[nu - VLAG + u])
        cur, prev = chunk(vc, u, tok), chunk(vp, u, None)
        o = None
        for w in range(W_LOC):
            t = shifted(cur, prev, w) * ps[w]
            o = t if o is None else o + t
        outs.append(o.reshape(UCH * 8, 128))
    return jnp.concatenate(outs, axis=0)


def _kernel(x_hbm, wa_hbm, woa_hbm, wb_hbm, wob_hbm, out_hbm,
            x_ref, xio, xn1, xn2, wa_nat, wat, woa, woap, wb_nat, wbt, wk, wkp, wob, wobp,
            khalo, vhalo, wstage, pxn, pbuf, po,
            qT, kN, vT, oN, otbuf,
            sem, *bufs):
    sbufs = bufs[:NC]
    stg = [bufs[NC + 3 * g:NC + 3 * g + 3] for g in range(NG)]

    def x_copy(i, sid):
        rows = pl.ds(i * BLK, BLK)
        return pltpu.make_async_copy(x_hbm.at[rows, :], xio.at[rows, :], sem.at[sid])

    def wa_copies(g):
        return [pltpu.make_async_copy(
            wa_hbm.at[:, pl.ds(pl.multiple_of(sec * D + g * 128, 128), 128)],
            wa_nat.at[g * 3 + sec], sem.at[SEM_WA + g]) for sec in range(3)]

    def wb_copy(c, sid):
        col = c * 128 + (c // 8) * D
        return pltpu.make_async_copy(
            wb_hbm.at[:, pl.ds(col, 128)], wb_nat.at[c], sem.at[sid])

    def wk_copy(c, sid):
        rows = pl.ds(c * 128, 128)
        return pltpu.make_async_copy(
            wb_hbm.at[rows, pl.ds(D, D)], wk.at[rows, :], sem.at[sid])

    def iter_copies(it):
        sid = SEM_IT + it
        if it == 0:
            cps = [pltpu.make_async_copy(woa_hbm, woa, sem.at[sid])]
        else:
            cps = [x_copy(i, sid) for i in (2 * it + 1, 2 * it + 2) if i < NB]
        return cps + [wb_copy(2 * it, sid), wb_copy(2 * it + 1, sid), wk_copy(it, sid)]

    x01_copies = [x_copy(0, SEM_X01), x_copy(1, SEM_X01)]
    x2_copy = x_copy(2, SEM_X2)
    wob_copy = pltpu.make_async_copy(wob_hbm, wob, sem.at[SEM_WOB])

    def out_copy(j):
        rows = pl.ds(pl.multiple_of(j * TF, TF), TF)
        return pltpu.make_async_copy(xio.at[rows, :], out_hbm.at[rows, :], sem.at[SEM_OUT])

    def blk_rows(i, n=BLK):
        return pl.ds(pl.multiple_of(i * n, n), n)

    def qkv_group(g, xn):
        w = jnp.concatenate([wat[g, kt] for kt in range(NG)], axis=1)
        r = jnp.concatenate(
            [_dot_nt(_as_bf16(w[a:a + GM // 2]), xn) for a in range(0, 192, GM // 2)], axis=0)
        k = r[128:256]
        v = r[256:384]
        return r[0:128], _pack(k) if PACK_K else k, _pack(v) if PACK_V else v

    def o_rows(i, n):
        rows = blk_rows(i, n // 2)
        return _as_bf16(jnp.concatenate([oN[t, rows, :] for t in range(NG)], axis=1))

    def proj_residual(o, w_cols, xv):
        cols = []
        for n in range(2):
            cols.append(xv[:, n * 512:(n + 1) * 512] + _dot(o, w_cols(n)))
        return jnp.concatenate(cols, axis=1)

    def packed_cols(w_ref):
        return lambda n: _as_bf16(
            jnp.concatenate([w_ref[4 * n + t] for t in range(4)], axis=1))

    woa_cols, wob_cols, wk_cols = packed_cols(woap), packed_cols(wobp), packed_cols(wkp)

    def repack(dst_ref, src_ref, c, n, tok=None):
        wv = pltpu.bitcast(src_ref[blk_rows(c, n), :], u32)
        if tok is not None:
            wv = _after(wv, tok)
        for t in range(NG):
            dst_ref[t, blk_rows(c, n // 2), :] = wv[:, t * 128:(t + 1) * 128]

    def store_permuted(dst_ref, row0, val):
        for h in range(4):
            dst_ref[pl.ds(row0 + h, 16, stride=4), :] = val[h * 16:(h + 1) * 16]

    def rows16(blk, r):
        return pl.ds(pl.multiple_of(blk * BLK + r * 16, 16), 16)

    def ln1(blk, r, tok=None):
        rows = rows16(blk, r)
        xv = xio[rows, :].astype(f32)
        if tok is not None:
            xv = _after(xv, tok)
        x_ref[rows, :] = xv
        return _ln16(xv)

    def ln2(blk, r, tok=None):
        xv = x_ref[rows16(blk, r), :]
        if tok is not None:
            xv = _after(xv, tok)
        xn2[pl.ds(pl.multiple_of(blk * (BLK // 2) + r * 8, 8), 8), :] = _ln16(xv)

    def head_group0(xn_packed):
        for ref, val in zip(stg[0], qkv_group(0, _as_bf16(xn_packed))):
            ref[0:val.shape[0], :] = val

    def a_block(i, par, z0, z1):
        xn_cur = _as_bf16(xn1[...])
        ip = jnp.maximum(i - 1, 0)
        inx = jnp.minimum(i + 1, NB - 1)
        pos = i * BLK + lax.broadcasted_iota(jnp.int32, (8, 128), 1)

        def stage(g, slot, qkv):
            for ref, val in zip(stg[g], qkv):
                n = val.shape[0]
                ref[pl.ds(pl.multiple_of(z0 + slot * n, 8), n), :] = val

        def getter(ref, slot):
            n = ref.shape[0] // 2
            m = n // (16 // UCH)
            return lambda u: ref[pl.ds(pl.multiple_of(z1 + slot * n + u * m, 8), m), :]

        o_cols = []
        xn_parts = []
        for g in range(NG):
            if g:
                qkv = qkv_group(g, xn_cur)
                stage(g, par, qkv)
            qs, ks, vs = stg[g]
            ot = _local_attention(getter(qs, par), getter(ks, par), getter(ks, 1 - par),
                                  getter(vs, par), getter(vs, 1 - par), pos)
            o_cols.append(ot.astype(bf16).T)
            if g >= 1:
                tok = _token(qkv[1])
                if g <= 4:
                    xn_parts += [ln1(inx, 2 * g - 2, tok), ln1(inx, 2 * g - 1, tok)]
                else:
                    ln2(ip, 2 * g - 10, tok)
                    ln2(ip, 2 * g - 9, tok)
                if g == 5:
                    wsrc = _as_bf16(_after(pltpu.bitcast(wb_nat[i], u32), tok))
                    wbt[i] = pltpu.bitcast(wsrc.T, u32)
                if g == 6:
                    repack(wkp, wk, i, 64, tok)
        xn_next = jnp.concatenate(xn_parts, axis=0)
        xn1[...] = xn_next
        qkv = qkv_group(0, _as_bf16(xn_next))
        stage(0, 1 - par, qkv)
        tok = _token(qkv[1])
        ln2(ip, 6, tok)
        ln2(ip, 7, tok)
        o = jnp.concatenate(o_cols, axis=1)
        rows = blk_rows(i)
        x_ref[rows, :] = proj_residual(o, woa_cols, x_ref[rows, :])

    def startup():
        def transpose_wa(g):
            for sec in range(3):
                wv = pltpu.bitcast(wa_nat[g * 3 + sec].T, u32)
                for kt in range(NG):
                    store_permuted(wstage.at[kt], sec * 64, wv[:, kt * 128:(kt + 1) * 128])

        def project(g):
            w = wstage[...]
            wat[g] = w
            w = jnp.concatenate([w[kt] for kt in range(NG)], axis=1)
            return _dot_nt(_as_bf16(w), _as_bf16(pxn[...]))

        def attend(g, r):
            pos = lax.broadcasted_iota(jnp.int32, (8, 128), 1)
            kp = jnp.zeros(khalo.shape[1:], khalo.dtype)
            vp = jnp.zeros(vhalo.shape[1:], vhalo.dtype)
            for b in range(2):
                rb = r[:, b * BLK:(b + 1) * BLK]
                kc = _pack(rb[128:256]) if PACK_K else rb[128:256]
                vc = _pack(rb[256:384]) if PACK_V else rb[256:384]
                ot = _local_attention(rb[0:128], kc, kp, vc, vp, pos + b * BLK)
                po[g, b * 64:(b + 1) * 64, :] = pltpu.bitcast(ot.astype(bf16).T, u32)
                kp, vp = kc, vc
            khalo[g] = kp
            vhalo[g] = vp

        pbuf[...] = jnp.zeros(pbuf.shape, f32)
        for cp in x01_copies:
            cp.wait()
        for b in range(2):
            for r in range(BLK // 16):
                pxn[b * 64 + r * 8:b * 64 + (r + 1) * 8, :] = ln1(b, r)
        for cp in wa_copies(0):
            cp.wait()
        transpose_wa(0)

        def body(g, c):
            for cp in wa_copies(g + 1):
                cp.wait()
            prev = pbuf[...]
            pbuf[...] = project(g)
            transpose_wa(g + 1)
            attend(jnp.maximum(g - 1, 0), prev)
            return c
        lax.fori_loop(0, NG - 1, body, 0)

        x2_copy.wait()
        prev = pbuf[...]
        r = project(NG - 1)
        xn_next = jnp.concatenate([ln1(2, r16) for r16 in range(BLK // 16)], axis=0)
        xn1[...] = xn_next
        attend(NG - 2, _after(prev, _token(xn_next[56:64, 0:128])))
        head_group0(xn_next)
        attend(NG - 1, r)

        for cp in iter_copies(0):
            cp.wait()
        for t in range(NG):
            wv = pltpu.bitcast(woa[:, t * 128:(t + 1) * 128], u32)
            for g in range(NG):
                store_permuted(woap.at[t], g * 64, wv[g * 64:(g + 1) * 64])
        for b in range(2):
            o = jnp.concatenate([po[g, b * 64:(b + 1) * 64, :] for g in range(NG)], axis=1)
            rows = blk_rows(b)
            x_ref[rows, :] = proj_residual(_as_bf16(o), woa_cols, x_ref[rows, :])
            wbt[b] = pltpu.bitcast(wb_nat[b].T, u32)
        repack(wkp, wk, 0, 128)
        for r16 in range(BLK // 16):
            ln2(0, r16)
        for g in range(NG):
            for ref, src in ((stg[g][1], khalo), (stg[g][2], vhalo)):
                n = src.shape[1]
                ref[n:2 * n, :] = src[g]

    def phase_a(rep):
        @pl.when(rep == 1)
        def _():
            for g in range(NG):
                for ref in stg[g][1:]:
                    n = ref.shape[0] // 2
                    ref[n:2 * n, :] = jnp.zeros((n, BLK), ref.dtype)
            xn_first = jnp.concatenate([ln1(0, r) for r in range(BLK // 16)], axis=0)
            xn1[...] = xn_first
            head_group0(xn_first)

        def body(it, c):
            for k in range(1, NB // APB):
                @pl.when(jnp.logical_and(rep == 0, it == k))
                def _():
                    for cp in iter_copies(k):
                        cp.wait()

            z0 = lax.shift_right_logical(it, 16) * 8
            z1 = lax.shift_right_logical(it, 17) * 8
            for u in range(APB):
                a_block(it * APB + u, u % 2, z0, z1)
            return c
        with _scope("a_loop"):
            lax.fori_loop(1 - rep, NB // APB, body, 0)
        for r in range(BLK // 16):
            ln2(NB - 1, r)

    def phase_b_proj():
        def body(j, c):
            rows = blk_rows(j, TB // 2)
            xn = _as_bf16(xn2[rows, :])
            for n in range(2):
                y = _pack(_dot(xn, wk_cols(n)))
                for t in range(4):
                    kN[4 * n + t, rows, :] = y[:, t * 128:(t + 1) * 128]
            for r in range(4):
                w = _as_bf16(wbt[2 * r:2 * r + 2].reshape(128, D))
                y = _pack(_dot_nt(w, xn) * QSCALE)
                for b in range(TB // NQ):
                    qT[j * (TB // NQ) + b, r * 128:(r + 1) * 128, :] = y[:, b * NQ:(b + 1) * NQ]
            for r in range(4):
                w = _as_bf16(wbt[8 + 2 * r:8 + 2 * r + 2].reshape(128, D))
                y = _pack(_dot_nt(w, xn))
                for b in range(TB // MK):
                    vT[j * (TB // MK) + b, r * 128:(r + 1) * 128, :] = y[:, b * MK:(b + 1) * MK]
            return c
        lax.fori_loop(0, S // TB, body, 0)

    def phase_b_attn():
        off = [0, 0]

        def qm_of(t, qi, j):
            q = _as_bf16(qT[qi, pl.ds(pl.multiple_of(t * 64 + j * 16, 16), 16), :])
            parts = []
            if j > 0:
                parts.append(jnp.zeros((32 * j, NQ), bf16))
            parts.append(q)
            if j < 3:
                parts.append(jnp.zeros((32 * (3 - j), NQ), bf16))
            return jnp.concatenate(parts, axis=0)

        def qk_chunk(t, qm, c, par, m):
            k = _as_bf16(kN[t, c * (MK // 2):(c + 1) * (MK // 2), :])
            s = _dot(k, qm)
            sbufs[c][pl.ds(pl.multiple_of(off[0] + par * MK, 8), MK), :] = s
            sm = _tree(s.reshape(MK // 8, 8, NQ), jnp.maximum)
            return sm if m is None else jnp.maximum(m, sm)

        def pv_chunk(h, c, par, mrow, l, o):
            s = sbufs[c][pl.ds(pl.multiple_of(off[1] + par * MK, 8), MK), :]
            p = jnp.exp2(s - mrow)
            ls = jnp.sum(p.reshape(MK // 8, 8, NQ), axis=0)
            l = ls if l is None else l + ls
            v = _as_bf16(vT[c, pl.ds(pl.multiple_of(h * 16, 16), 16), :])
            oc = _dot(v, p.astype(bf16))
            o = oc if o is None else o + oc
            return l, o

        def flush_o(g, val):
            y = pltpu.bitcast(_as_bf16(val).T, u32)
            oN[g % NG, blk_rows(g // NG, NQ // 2), :] = y

        n_groups = NQT * NG
        otbuf[...] = jnp.zeros(otbuf.shape, u32)
        qm = qm_of(0, 0, 0)
        m0 = None
        for c in range(NC):
            m0 = qk_chunk(0, qm, c, 0, m0)
        qm = qm_of(0, 0, 1)
        m1 = None
        for c in range(DL):
            m1 = qk_chunk(0, qm, c, 1, m1)

        def group(g, g_next, carry, zero):
            qi = g // NG
            t = g % NG
            off[0] = lax.shift_right_logical(zero, 16) * 8
            off[1] = lax.shift_right_logical(zero, 17) * 8
            flush_o(jnp.maximum(g - 1, 0), otbuf[...])
            ms = {0: carry[0], 1: carry[1]}
            qms = {}
            l = o = mrow = None
            for n in range(4 * NC):
                j, c = divmod(n, NC)
                j2, c2 = divmod(n + NC + DL, NC)
                if j2 < 4 or g_next is not None:
                    t2 = t if j2 < 4 else g_next % NG
                    if j2 not in qms:
                        qms[j2] = qm_of(t2, qi if j2 < 4 else g_next // NG, j2 % 4)
                    ms[j2] = qk_chunk(t2, qms[j2], c2, j2 % 2, ms.get(j2))
                if c == 0:
                    mrow = jnp.max(ms[j], axis=0, keepdims=True)
                    l = o = None
                l, o = pv_chunk(t * 4 + j, c, j % 2, mrow, l, o)
                if c == NC - 1:
                    lrow = jnp.sum(l, axis=0, keepdims=True)
                    otbuf[j * 16:(j + 1) * 16, :] = _pack(o * (1.0 / lrow))
            return ms.get(4), ms.get(5)

        def body(it, ms):
            repack(wobp, wob, it, D * GPB // n_groups)
            for u in range(GPB):
                g = it * GPB + u
                ms = group(g, jnp.minimum(g + 1, n_groups - 1), ms, it)
            return ms

        lax.fori_loop(0, n_groups // GPB, body, (m0, m1))
        off[0] = off[1] = 0
        flush_o(n_groups - 1, otbuf[...])

    def phase_b_out(rep):
        def body(j, c):
            rows = blk_rows(j, TF)
            xv = proj_residual(o_rows(j, TF), wob_cols, x_ref[rows, :])
            xio[rows, :] = xv.astype(bf16)

            @pl.when(rep == 1)
            def _():
                out_copy(j).start()
            return c
        lax.fori_loop(0, S // TF, body, 0)

    for cp in x01_copies:
        cp.start()
    for g in range(NG):
        if g == NG - 2:
            x2_copy.start()
        for cp in wa_copies(g):
            cp.start()
    for it in range(NB // APB):
        for cp in iter_copies(it):
            cp.start()
    wob_copy.start()

    with _scope("startup"):
        startup()

    def layer_pair(rep, c):
        with _scope("phase_a"):
            phase_a(rep)

        @pl.when(rep == 0)
        def _():
            wob_copy.wait()

        with _scope("b_proj"):
            phase_b_proj()
        with _scope("b_attn"):
            phase_b_attn()
        with _scope("b_out"):
            phase_b_out(rep)
        return c
    lax.fori_loop(0, 2, layer_pair, 0)
    for j in range(S // TF):
        out_copy(j).wait()


@jax.jit
def pallas_interleave_layers__sliding_local_dilated__softmax_full_mha__prompt_kernel(
    A_x: jax.Array,
    A_wqkv: jax.Array,
    A_wo: jax.Array,
    B_x: jax.Array,
    B_wqkv: jax.Array,
    B_wo: jax.Array,
):
    del B_x
    x = A_x.reshape(S, D)
    vm = pltpu.VMEM
    kshape, kdt = ((64, BLK), u32) if PACK_K else ((128, BLK), f32)
    vshape, vdt = ((64, BLK), u32) if PACK_V else ((128, BLK), f32)
    scratch = [
        vm((S, D), f32),
        vm((S, D), bf16),
        vm((BLK // 2, D), u32),
        vm((S // 2, D), u32),
        vm((3 * NG, D, 128), bf16),
        vm((NG, NG, 192, 128), u32),
        vm((D, D), bf16),
        vm((NG, D // 2, 128), u32),
        vm((2 * NG, D, 128), bf16),
        vm((2 * NG, 64, D), u32),
        vm((D, D), bf16),
        vm((NG, D // 2, 128), u32),
        vm((D, D), bf16),
        vm((NG, D // 2, 128), u32),
        vm((NG,) + kshape, kdt),
        vm((NG,) + vshape, vdt),
        vm((NG, 192, 128), u32),
        vm((BLK, D), u32),
        vm((384, 2 * BLK), f32),
        vm((NG, BLK, 128), u32),
        vm((NQT, D // 2, NQ), u32),
        vm((NG, S // 2, 128), u32),
        vm((NC, D // 2, MK), u32),
        vm((NG, S // 2, 128), u32),
        vm((64, NQ), u32),
        pltpu.SemaphoreType.DMA((N_SEM,)),
    ] + [vm((2 * MK, NQ), f32)] * NC + [
        vm((256, BLK), f32), vm((2 * kshape[0], BLK), kdt), vm((2 * vshape[0], BLK), vdt)] * NG
    out = pl.pallas_call(
        _kernel,
        out_shape=jax.ShapeDtypeStruct((S, D), bf16),
        in_specs=[pl.BlockSpec(memory_space=pl.ANY)] * 5,
        out_specs=pl.BlockSpec(memory_space=pl.ANY),
        scratch_shapes=scratch,
        compiler_params=pltpu.CompilerParams(vmem_limit_bytes=110 * 1024 * 1024),
        name="interleave_attn",
    )(x, A_wqkv, A_wo, B_wqkv, B_wo)
    return out.reshape(1, S, D)
```

```python
import jax
import jax.numpy as jnp
from jax import lax
import jax.experimental.pallas as pl
import jax.experimental.pallas.tpu as pltpu

S, D, H, DH = 2048, 1024, 32, 32
W_LOC, DIL = 8, 2
EPS = 1e-5
LOG2E = 1.4426950408889634
QSCALE = (DH ** -0.5) * LOG2E
NEG = -1e9 * LOG2E

BLK = 128
NB = S // BLK
NG = D // 128
NQ = 256
NQT = S // NQ
MK = 128
NC = S // MK
DL = 5
APB = 2
GPB = 4
TB = 256
TF = 256

SEM_X01, SEM_X2, SEM_WOB, SEM_OUT = 0, 1, 2, 3
SEM_WA = 4
SEM_IT = SEM_WA + NG
N_SEM = SEM_IT + 4

PACK_K = True
GM = 128
PACK_V = True
UCH = 4
ONLY_A = False
S4N = 2
LNORD = 0
XBASE = True
WKSLOT = 5
LSKEW = 1
L1S = (0, 0, 1, 1, 2, 2, 3, 3)
L2S = (4, 5, 6, 7, 8, 8, 8, 8)
RSMODE = 0
NOTOK = False
SKIP1 = False
SKIP2 = False
TOKMODE = 1
WBSLOT = 4
LOCAL_OFF = False
LNMODE = 0
KLAG = 0
VLAG = 0
PROFILE_SCOPES = False

bf16 = jnp.bfloat16
f32 = jnp.float32
u32 = jnp.uint32
NT = (((1,), (1,)), ((), ()))


class _NoScope:
    def __enter__(self):
        return self

    def __exit__(self, *a):
        return False


def _scope(name):
    return jax.named_scope(name) if PROFILE_SCOPES else _NoScope()


def _pack(x):
    return pltpu.bitcast(x.astype(bf16), u32)


def _as_bf16(x):
    return pltpu.bitcast(x, bf16)


def _dot(a, b):
    return jnp.dot(a, b, preferred_element_type=f32)


def _dot_nt(a, b):
    return lax.dot_general(a, b, NT, preferred_element_type=f32)


def _layernorm_packed(x):
    outs = []
    for r in range(x.shape[0] // 16):
        xr = x[r * 16:(r + 1) * 16]
        mu = jnp.sum(xr, axis=1, keepdims=True) * (1.0 / D)
        xc = xr - mu
        var = jnp.sum(xc * xc, axis=1, keepdims=True) * (1.0 / D)
        outs.append(_pack(xc * lax.rsqrt(var + EPS)))
    return jnp.concatenate(outs, axis=0)


def _token(v):
    t = pltpu.bitcast(v[0:8, :], u32)
    return lax.shift_right_logical(jnp.bitwise_and(t, jnp.uint32(0xFFFF)), jnp.uint32(16))


def _after(x, tok):
    n, m = x.shape
    z = jnp.concatenate([jnp.concatenate([tok] * (m // 128), axis=1)] * (n // 8), axis=0)
    return pltpu.bitcast(jnp.bitwise_or(pltpu.bitcast(x, u32), z), x.dtype)


def _rowsum(x):
    if RSMODE == 1:
        t = x[:, 0:128]
        parts = [x[:, k * 128:(k + 1) * 128] for k in range(x.shape[1] // 128)]
        while len(parts) > 1:
            parts = [a + b for a, b in zip(parts[0::2], parts[1::2])]
        return jnp.sum(parts[0], axis=1, keepdims=True)
    return jnp.sum(x, axis=1, keepdims=True)


def _ln16(xr):
    if LNMODE == 1:
        return _pack(xr)
    if LNMODE == 2:
        mu = _rowsum(xr) * (1.0 / D)
        ms = _rowsum(xr * xr) * (1.0 / D)
        rs = lax.rsqrt(ms - mu * mu + EPS)
        return _pack(xr * rs - mu * rs)
    if LNMODE == 3:
        mu = _rowsum(xr) * (1.0 / D)
        xc = xr - mu
        var = _rowsum(xc * xc) * (1.0 / D)
        return _pack(xc * (var + EPS))
    if LNMODE == 4:
        mu = _rowsum(xr) * (1.0 / D)
        return _pack(xr - mu)
    mu = _rowsum(xr) * (1.0 / D)
    xc = xr - mu
    var = _rowsum(xc * xc) * (1.0 / D)
    return _pack(xc * lax.rsqrt(var + EPS))


def _tree(x, op):
    n = x.shape[0]
    while n > 1:
        n //= 2
        x = op(x[:n], x[n:])
    return x[0]


def _local_attention(q, kc, kp, vc, vp, pos):
    def chunk(x, u, tok):
        if callable(x):
            return x(u)
        n = UCH * (4 if x.dtype == u32 else 8)
        x = x[u * n:(u + 1) * n]
        return x if tok is None else _after(x, tok)

    def shifted(cur, prev, w):
        x = cur
        if w:
            lane = lax.broadcasted_iota(jnp.int32, x.shape, 1)
            x = jnp.where(lane >= 128 - DIL * w, prev, x)
            x = pltpu.roll(x, DIL * w, axis=1)
        if x.dtype == u32:
            x = _as_bf16(x).astype(f32)
        return x.reshape(UCH, 8, 128)

    nu = 16 // UCH
    if LOCAL_OFF:
        return jnp.concatenate([chunk(q, u, None) for u in range(nu)], axis=0)
    even = lax.broadcasted_iota(jnp.int32, (8, 128), 0) % 2 == 0
    acc = [None] * W_LOC
    done = []
    for u in range(nu):
        tok = _token(done[u - KLAG]) if KLAG and u >= KLAG else None
        cur, prev = chunk(kc, u, tok), chunk(kp, u, None)
        qu = chunk(q, u, None).reshape(UCH, 8, 128)
        for w in range(W_LOC):
            t = _tree(qu * shifted(cur, prev, w), jnp.add)
            acc[w] = t if acc[w] is None else acc[w] + t
        done.append(acc[W_LOC - 1])
    logits = []
    for w in range(W_LOC):
        t = acc[w]
        t = t + jnp.where(even, pltpu.roll(t, 7, axis=0), pltpu.roll(t, 1, axis=0))
        t = t * QSCALE
        if w:
            t = jnp.where(pos >= DIL * w, t, NEG)
        logits.append(t)
    m = logits[0]
    for t in logits[1:]:
        m = jnp.maximum(m, t)
    ps = [jnp.exp2(t - m) for t in logits]
    l = ps[0]
    for p in ps[1:]:
        l = l + p
    r = 1.0 / l
    ps = [(p * r)[None] for p in ps]
    outs = []
    for u in range(nu):
        tok = None
        if VLAG:
            tok = _token(outs[u - VLAG] if u >= VLAG else done[nu - VLAG + u])
        cur, prev = chunk(vc, u, tok), chunk(vp, u, None)
        o = None
        for w in range(W_LOC):
            t = shifted(cur, prev, w) * ps[w]
            o = t if o is None else o + t
        outs.append(o.reshape(UCH * 8, 128))
    return jnp.concatenate(outs, axis=0)


def _kernel(x_hbm, wa_hbm, woa_hbm, wb_hbm, wob_hbm, out_hbm,
            x_ref, xio, xn1a, xn1b, xn2, wa_nat, wat, woa, woap, wb_nat, wbt, wk, wkp, wob, wobp,
            khalo, vhalo, wstage, pxn, pbuf, po,
            qT, kN, vT, oN, otbuf,
            sem, *bufs):
    xn1 = (xn1a, xn1b)
    sbufs = bufs[:NC]
    stg = [bufs[NC + 3 * g:NC + 3 * g + 3] for g in range(NG)]

    def x_copy(i, sid):
        rows = pl.ds(i * BLK, BLK)
        return pltpu.make_async_copy(x_hbm.at[rows, :], xio.at[rows, :], sem.at[sid])

    def wa_copies(g):
        return [pltpu.make_async_copy(
            wa_hbm.at[:, pl.ds(pl.multiple_of(sec * D + g * 128, 128), 128)],
            wa_nat.at[g * 3 + sec], sem.at[SEM_WA + g]) for sec in range(3)]

    def wb_copy(c, sid):
        col = c * 128 + (c // 8) * D
        return pltpu.make_async_copy(
            wb_hbm.at[:, pl.ds(col, 128)], wb_nat.at[c], sem.at[sid])

    def wk_copy(c, sid):
        rows = pl.ds(c * 128, 128)
        return pltpu.make_async_copy(
            wb_hbm.at[rows, pl.ds(D, D)], wk.at[rows, :], sem.at[sid])

    def iter_copies(it):
        sid = SEM_IT + min(it, 3)
        if it == 0:
            cps = [pltpu.make_async_copy(woa_hbm, woa, sem.at[sid])]
        else:
            cps = [x_copy(i, sid) for i in (2 * it + 1, 2 * it + 2) if i < NB]
        return cps + [wb_copy(2 * it, sid), wb_copy(2 * it + 1, sid), wk_copy(it, sid)]

    x01_copies = [x_copy(0, SEM_X01), x_copy(1, SEM_X01)]
    x2_copy = x_copy(2, SEM_X2)
    wob_copy = pltpu.make_async_copy(wob_hbm, wob, sem.at[SEM_WOB])

    def out_copy(j):
        rows = pl.ds(pl.multiple_of(j * TF, TF), TF)
        return pltpu.make_async_copy(xio.at[rows, :], out_hbm.at[rows, :], sem.at[SEM_OUT])

    def blk_rows(i, n=BLK):
        return pl.ds(pl.multiple_of(i * n, n), n)

    def qkv_group(g, xn):
        w = jnp.concatenate([wat[g, kt] for kt in range(NG)], axis=1)
        r = jnp.concatenate(
            [_dot_nt(_as_bf16(w[a:a + GM // 2]), xn) for a in range(0, 192, GM // 2)], axis=0)
        k = r[128:256]
        v = r[256:384]
        return r[0:128], _pack(k) if PACK_K else k, _pack(v) if PACK_V else v

    def o_rows(i, n):
        rows = blk_rows(i, n // 2)
        return _as_bf16(jnp.concatenate([oN[t, rows, :] for t in range(NG)], axis=1))

    def proj_residual(o, w_cols, xv, ns=2):
        cols = []
        w = D // ns
        for n in range(ns):
            cols.append(xv[:, n * w:(n + 1) * w] + _dot(o, w_cols(n, ns)))
        return jnp.concatenate(cols, axis=1)

    def packed_cols(w_ref):
        return lambda n, ns=2: _as_bf16(jnp.concatenate(
            [w_ref[NG // ns * n + t] for t in range(NG // ns)], axis=1))

    woa_cols, wob_cols, wk_cols = packed_cols(woap), packed_cols(wobp), packed_cols(wkp)

    def repack(dst_ref, src_ref, c, n, tok=None):
        wv = pltpu.bitcast(src_ref[blk_rows(c, n), :], u32)
        if tok is not None:
            wv = _after(wv, tok)
        for t in range(NG):
            dst_ref[t, blk_rows(c, n // 2), :] = wv[:, t * 128:(t + 1) * 128]

    def store_permuted(dst_ref, row0, val):
        for h in range(4):
            dst_ref[pl.ds(row0 + h, 16, stride=4), :] = val[h * 16:(h + 1) * 16]

    def rows16(blk, r):
        return pl.ds(pl.multiple_of(blk * BLK + r * 16, 16), 16)

    def ln1(blk, r, tok=None):
        rows = rows16(blk, r)
        xv = xio[rows, :].astype(f32)
        if SKIP1:
            return _pack(xv)
        if tok is not None and not NOTOK:
            xv = _after(xv, tok)
        if not XBASE:
            x_ref[rows, :] = xv
        return _ln16(xv)

    def ln2(blk, r, tok=None):
        if SKIP2:
            return
        xv = x_ref[rows16(blk, r), :]
        if tok is not None and not NOTOK:
            xv = _after(xv, tok)
        xn2[pl.ds(pl.multiple_of(blk * (BLK // 2) + r * 8, 8), 8), :] = _ln16(xv)

    def head_group0(xn_packed):
        for ref, val in zip(stg[0], qkv_group(0, _as_bf16(xn_packed))):
            ref[0:val.shape[0], :] = val

    def a_block(i, par, z0, z1):
        def xn_cur():
            if LSKEW == 1:
                return _as_bf16(xn1[par][...])
            return _as_bf16(xn1[par][pl.ds(pl.multiple_of(z1, 8), BLK // 2), :])

        ip = jnp.maximum(i - 1, 0)
        inx = jnp.minimum(i + LSKEW, NB - 1)
        dst = xn1[(par + LSKEW) % 2]
        pos = i * BLK + lax.broadcasted_iota(jnp.int32, (8, 128), 1)

        def stage(g, slot, qkv):
            for ref, val in zip(stg[g], qkv):
                n = val.shape[0]
                ref[pl.ds(pl.multiple_of(z0 + slot * n, 8), n), :] = val

        def getter(ref, slot):
            n = ref.shape[0] // 2
            m = n // (16 // UCH)
            return lambda u: ref[pl.ds(pl.multiple_of(z1 + slot * n + u * m, 8), m), :]

        def ln_jobs(slot, tok):
            for r in range(8):
                if L1S[r] == slot:
                    dst[pl.ds(pl.multiple_of(z0 + r * 8, 8), 8), :] = ln1(inx, r, tok)
            for r in range(8):
                if L2S[r] == slot:
                    ln2(ip, r, tok)

        o_cols = []
        for g in range(NG):
            if g:
                qkv = qkv_group(g, xn_cur())
                stage(g, par, qkv)
            qs, ks, vs = stg[g]
            ot = _local_attention(getter(qs, par), getter(ks, par), getter(ks, 1 - par),
                                  getter(vs, par), getter(vs, 1 - par), pos)
            o_cols.append(ot.astype(bf16).T)
            if TOKMODE == 0:
                tok = _token(qkv[1]) if g else None
                slot = g - 1
            else:
                tok = _token(ot[120:128])
                slot = g
            ln_jobs(slot, tok)
            if slot == WBSLOT:
                wsrc = _as_bf16(_after(pltpu.bitcast(wb_nat[i], u32), tok))
                wbt[i] = pltpu.bitcast(wsrc.T, u32)
            if slot == WKSLOT:
                repack(wkp, wk, i, 64, tok)
        xn_next = xn1[1 - par][pl.ds(pl.multiple_of(z1, 8), BLK // 2), :]
        qkv = qkv_group(0, _as_bf16(xn_next))
        stage(0, 1 - par, qkv)
        ln_jobs(7 + TOKMODE, _token(qkv[1]))
        o = jnp.concatenate(o_cols, axis=1)
        rows = blk_rows(i)
        base = xio[rows, :].astype(f32) if XBASE else x_ref[rows, :]
        xv = proj_residual(o, woa_cols, base, S4N)
        x_ref[rows, :] = xv
        for k in range(4):
            ln_jobs(9 + k, _token(xv[0:8, k * 256:k * 256 + 128]))

    def startup():
        def transpose_wa(g):
            for sec in range(3):
                wv = pltpu.bitcast(wa_nat[g * 3 + sec].T, u32)
                for kt in range(NG):
                    store_permuted(wstage.at[kt], sec * 64, wv[:, kt * 128:(kt + 1) * 128])

        def project(g):
            w = wstage[...]
            wat[g] = w
            w = jnp.concatenate([w[kt] for kt in range(NG)], axis=1)
            return _dot_nt(_as_bf16(w), _as_bf16(pxn[...]))

        def attend(g, r):
            pos = lax.broadcasted_iota(jnp.int32, (8, 128), 1)
            kp = jnp.zeros(khalo.shape[1:], khalo.dtype)
            vp = jnp.zeros(vhalo.shape[1:], vhalo.dtype)
            for b in range(2):
                rb = r[:, b * BLK:(b + 1) * BLK]
                kc = _pack(rb[128:256]) if PACK_K else rb[128:256]
                vc = _pack(rb[256:384]) if PACK_V else rb[256:384]
                ot = _local_attention(rb[0:128], kc, kp, vc, vp, pos + b * BLK)
                po[g, b * 64:(b + 1) * 64, :] = pltpu.bitcast(ot.astype(bf16).T, u32)
                kp, vp = kc, vc
            khalo[g] = kp
            vhalo[g] = vp

        pbuf[...] = jnp.zeros(pbuf.shape, f32)
        for cp in x01_copies:
            cp.wait()
        for b in range(2):
            for r in range(BLK // 16):
                pxn[b * 64 + r * 8:b * 64 + (r + 1) * 8, :] = ln1(b, r)
        for cp in wa_copies(0):
            cp.wait()
        transpose_wa(0)

        def body(g, c):
            for cp in wa_copies(g + 1):
                cp.wait()
            prev = pbuf[...]
            pbuf[...] = project(g)
            transpose_wa(g + 1)
            attend(jnp.maximum(g - 1, 0), prev)
            return c
        lax.fori_loop(0, NG - 1, body, 0)

        x2_copy.wait()
        prev = pbuf[...]
        r = project(NG - 1)
        xn_next = jnp.concatenate([ln1(2, r16) for r16 in range(BLK // 16)], axis=0)
        xn1[0][...] = xn_next
        attend(NG - 2, _after(prev, _token(xn_next[56:64, 0:128])))
        head_group0(xn_next)
        attend(NG - 1, r)

        for cp in iter_copies(0):
            cp.wait()
        for t in range(NG):
            wv = pltpu.bitcast(woa[:, t * 128:(t + 1) * 128], u32)
            for g in range(NG):
                store_permuted(woap.at[t], g * 64, wv[g * 64:(g + 1) * 64])
        for b in range(2):
            o = jnp.concatenate([po[g, b * 64:(b + 1) * 64, :] for g in range(NG)], axis=1)
            rows = blk_rows(b)
            base = xio[rows, :].astype(f32) if XBASE else x_ref[rows, :]
            x_ref[rows, :] = proj_residual(_as_bf16(o), woa_cols, base)
            wbt[b] = pltpu.bitcast(wb_nat[b].T, u32)
        repack(wkp, wk, 0, 128)
        for r16 in range(BLK // 16):
            ln2(0, r16)
        for g in range(NG):
            for ref, src in ((stg[g][1], khalo), (stg[g][2], vhalo)):
                n = src.shape[1]
                ref[n:2 * n, :] = src[g]
        for cp in iter_copies(1):
            cp.wait()

    def phase_a(rep):
        @pl.when(rep == 1)
        def _():
            for g in range(NG):
                for ref in stg[g][1:]:
                    n = ref.shape[0] // 2
                    ref[n:2 * n, :] = jnp.zeros((n, BLK), ref.dtype)
            xn_first = jnp.concatenate([ln1(0, r) for r in range(BLK // 16)], axis=0)
            xn1[0][...] = xn_first
            head_group0(xn_first)

        def body(it, c):
            @pl.when(it == 2 - rep * NB)
            def _():
                for cp in iter_copies(2):
                    cp.wait()

            @pl.when(it == 3 - rep * NB)
            def _():
                for k in range(3, NB // APB):
                    for cp in iter_copies(k):
                        cp.wait()

            z0 = lax.shift_right_logical(it, 16) * 8
            z1 = lax.shift_right_logical(it, 17) * 8
            with _scope("a_iter"):
                for u in range(APB):
                    a_block(it * APB + u, u % 2, z0, z1)
            return c
        with _scope("a_loop"):
            lax.fori_loop(1 - rep, NB // APB, body, 0)
        for r in range(BLK // 16):
            ln2(NB - 1, r)

    def phase_b_proj():
        def body(j, c):
            rows = blk_rows(j, TB // 2)
            xn = _as_bf16(xn2[rows, :])
            for n in range(2):
                y = _pack(_dot(xn, wk_cols(n)))
                for t in range(4):
                    kN[4 * n + t, rows, :] = y[:, t * 128:(t + 1) * 128]
            for r in range(4):
                w = _as_bf16(wbt[2 * r:2 * r + 2].reshape(128, D))
                y = _pack(_dot_nt(w, xn) * QSCALE)
                for b in range(TB // NQ):
                    qT[j * (TB // NQ) + b, r * 128:(r + 1) * 128, :] = y[:, b * NQ:(b + 1) * NQ]
            for r in range(4):
                w = _as_bf16(wbt[8 + 2 * r:8 + 2 * r + 2].reshape(128, D))
                y = _pack(_dot_nt(w, xn))
                for b in range(TB // MK):
                    vT[j * (TB // MK) + b, r * 128:(r + 1) * 128, :] = y[:, b * MK:(b + 1) * MK]
            return c
        lax.fori_loop(0, S // TB, body, 0)

    def phase_b_attn():
        off = [0, 0]

        def qm_of(t, qi, j):
            q = _as_bf16(qT[qi, pl.ds(pl.multiple_of(t * 64 + j * 16, 16), 16), :])
            parts = []
            if j > 0:
                parts.append(jnp.zeros((32 * j, NQ), bf16))
            parts.append(q)
            if j < 3:
                parts.append(jnp.zeros((32 * (3 - j), NQ), bf16))
            return jnp.concatenate(parts, axis=0)

        def qk_chunk(t, qm, c, par, m):
            k = _as_bf16(kN[t, c * (MK // 2):(c + 1) * (MK // 2), :])
            s = _dot(k, qm)
            sbufs[c][pl.ds(pl.multiple_of(off[0] + par * MK, 8), MK), :] = s
            sm = _tree(s.reshape(MK // 8, 8, NQ), jnp.maximum)
            return sm if m is None else jnp.maximum(m, sm)

        def pv_chunk(h, c, par, mrow, l, o):
            s = sbufs[c][pl.ds(pl.multiple_of(off[1] + par * MK, 8), MK), :]
            p = jnp.exp2(s - mrow)
            ls = jnp.sum(p.reshape(MK // 8, 8, NQ), axis=0)
            l = ls if l is None else l + ls
            v = _as_bf16(vT[c, pl.ds(pl.multiple_of(h * 16, 16), 16), :])
            oc = _dot(v, p.astype(bf16))
            o = oc if o is None else o + oc
            return l, o

        def flush_o(g, val):
            y = pltpu.bitcast(_as_bf16(val).T, u32)
            oN[g % NG, blk_rows(g // NG, NQ // 2), :] = y

        n_groups = NQT * NG
        otbuf[...] = jnp.zeros(otbuf.shape, u32)
        qm = qm_of(0, 0, 0)
        m0 = None
        for c in range(NC):
            m0 = qk_chunk(0, qm, c, 0, m0)
        qm = qm_of(0, 0, 1)
        m1 = None
        for c in range(DL):
            m1 = qk_chunk(0, qm, c, 1, m1)

        def group(g, g_next, carry, zero, side_job=None):
            qi = g // NG
            t = g % NG
            off[0] = lax.shift_right_logical(zero, 16) * 8
            off[1] = lax.shift_right_logical(zero, 17) * 8
            flush_o(jnp.maximum(g - 1, 0), otbuf[...])
            ms = {0: carry[0], 1: carry[1]}
            qms = {}
            l = o = mrow = None
            for n in range(4 * NC):
                j, c = divmod(n, NC)
                j2, c2 = divmod(n + NC + DL, NC)
                if j2 < 4 or g_next is not None:
                    t2 = t if j2 < 4 else g_next % NG
                    if j2 not in qms:
                        qms[j2] = qm_of(t2, qi if j2 < 4 else g_next // NG, j2 % 4)
                    ms[j2] = qk_chunk(t2, qms[j2], c2, j2 % 2, ms.get(j2))
                if c == 0:
                    mrow = jnp.max(ms[j], axis=0, keepdims=True)
                    l = o = None
                l, o = pv_chunk(t * 4 + j, c, j % 2, mrow, l, o)
                if side_job is not None and n == NC // 2:
                    side_job(_token(l[:, 0:128]))
                if c == NC - 1:
                    lrow = jnp.sum(l, axis=0, keepdims=True)
                    otbuf[j * 16:(j + 1) * 16, :] = _pack(o * (1.0 / lrow))
            return ms.get(4), ms.get(5)

        def body(it, ms):
            def side_job(tok):
                repack(wobp, wob, it, D * GPB // n_groups, tok)

            for u in range(GPB):
                g = it * GPB + u
                ms = group(g, jnp.minimum(g + 1, n_groups - 1), ms, it,
                           side_job if u == 0 else None)
            return ms

        lax.fori_loop(0, n_groups // GPB, body, (m0, m1))
        off[0] = off[1] = 0
        flush_o(n_groups - 1, otbuf[...])

    def phase_b_out(rep):
        def body(j, c):
            rows = blk_rows(j, TF)
            xv = proj_residual(o_rows(j, TF), wob_cols, x_ref[rows, :])
            xio[rows, :] = xv.astype(bf16)

            @pl.when(rep == 1)
            def _():
                out_copy(j).start()
            return c
        lax.fori_loop(0, S // TF, body, 0)

    def sem_dummy():
        return lax.fori_loop(0, 3, lambda i, c: c + i, 0)

    if ONLY_A:
        phase_a(lax.shift_right_logical(sem_dummy(), 1))
        xio[0:8, :] = (_as_bf16(wbt[0, 0:4, :]) + _as_bf16(xn2[0:4, :])
                       + jnp.concatenate([_as_bf16(wkp[0, 0:4, :])] * 8, axis=1))
        return

    for cp in x01_copies:
        cp.start()
    for g in range(NG):
        if g == NG - 2:
            x2_copy.start()
        for cp in wa_copies(g):
            cp.start()
    for it in range(NB // APB):
        for cp in iter_copies(it):
            cp.start()
    wob_copy.start()

    with _scope("startup"):
        startup()

    def layer_pair(rep, c):
        with _scope("phase_a"):
            phase_a(rep)

        @pl.when(rep == 0)
        def _():
            wob_copy.wait()

        with _scope("b_proj"):
            phase_b_proj()
        with _scope("b_attn"):
            phase_b_attn()
        with _scope("b_out"):
            phase_b_out(rep)
        return c
    lax.fori_loop(0, 2, layer_pair, 0)
    for j in range(S // TF):
        out_copy(j).wait()


@jax.jit
def pallas_interleave_layers__sliding_local_dilated__softmax_full_mha__prompt_kernel(
    A_x: jax.Array,
    A_wqkv: jax.Array,
    A_wo: jax.Array,
    B_x: jax.Array,
    B_wqkv: jax.Array,
    B_wo: jax.Array,
):
    del B_x
    x = A_x.reshape(S, D)
    vm = pltpu.VMEM
    kshape, kdt = ((64, BLK), u32) if PACK_K else ((128, BLK), f32)
    vshape, vdt = ((64, BLK), u32) if PACK_V else ((128, BLK), f32)
    scratch = [
        vm((S, D), f32),
        vm((S, D), bf16),
        vm((BLK // 2, D), u32),
        vm((BLK // 2, D), u32),
        vm((S // 2, D), u32),
        vm((3 * NG, D, 128), bf16),
        vm((NG, NG, 192, 128), u32),
        vm((D, D), bf16),
        vm((NG, D // 2, 128), u32),
        vm((2 * NG, D, 128), bf16),
        vm((2 * NG, 64, D), u32),
        vm((D, D), bf16),
        vm((NG, D // 2, 128), u32),
        vm((D, D), bf16),
        vm((NG, D // 2, 128), u32),
        vm((NG,) + kshape, kdt),
        vm((NG,) + vshape, vdt),
        vm((NG, 192, 128), u32),
        vm((BLK, D), u32),
        vm((384, 2 * BLK), f32),
        vm((NG, BLK, 128), u32),
        vm((NQT, D // 2, NQ), u32),
        vm((NG, S // 2, 128), u32),
        vm((NC, D // 2, MK), u32),
        vm((NG, S // 2, 128), u32),
        vm((64, NQ), u32),
        pltpu.SemaphoreType.DMA((N_SEM,)),
    ] + [vm((2 * MK, NQ), f32)] * NC + [
        vm((256, BLK), f32), vm((2 * kshape[0], BLK), kdt), vm((2 * vshape[0], BLK), vdt)] * NG
    out = pl.pallas_call(
        _kernel,
        out_shape=jax.ShapeDtypeStruct((S, D), bf16),
        in_specs=[pl.BlockSpec(memory_space=pl.ANY)] * 5,
        out_specs=pl.BlockSpec(memory_space=pl.ANY),
        scratch_shapes=scratch,
        compiler_params=pltpu.CompilerParams(vmem_limit_bytes=110 * 1024 * 1024),
        name="interleave_attn",
    )(x, A_wqkv, A_wo, B_wqkv, B_wo)
    return out.reshape(1, S, D)
```

```python
import jax
import jax.numpy as jnp
from jax import lax
import jax.experimental.pallas as pl
import jax.experimental.pallas.tpu as pltpu

S, D, H, DH = 2048, 1024, 32, 32
W_LOC, DIL = 8, 2
EPS = 1e-5
LOG2E = 1.4426950408889634
QSCALE = (DH ** -0.5) * LOG2E
NEG = -1e9 * LOG2E

BLK = 128
NB = S // BLK
NG = D // 128
NQ = 256
NQT = S // NQ
MK = 128
NC = S // MK
DL = 5
APB = 2
GPB = 4
TB = 256
TF = 256

SEM_X01, SEM_X2, SEM_WOB, SEM_OUT = 0, 1, 2, 3
SEM_WA = 4
SEM_IT = SEM_WA + NG
N_SEM = SEM_IT + 4

PACK_K = True
GM = 128
PACK_V = True
UCH = 4
ONLY_A = False
MIDWAIT = False
NOBC = False
OPB = 2
S4N = 2
LNORD = 0
XBASE = True
WKSLOT = 5
LSKEW = 1
L1S = (0, 0, 1, 1, 2, 2, 3, 3)
L2S = (4, 5, 6, 7, 8, 8, 8, 8)
RSMODE = 0
NOTOK = False
SKIP1 = False
SKIP2 = False
TOKMODE = 1
WBSLOT = 4
LOCAL_OFF = False
LNMODE = 0
KLAG = 0
VLAG = 0
PROFILE_SCOPES = False

bf16 = jnp.bfloat16
f32 = jnp.float32
u32 = jnp.uint32
NT = (((1,), (1,)), ((), ()))


class _NoScope:
    def __enter__(self):
        return self

    def __exit__(self, *a):
        return False


def _scope(name):
    return jax.named_scope(name) if PROFILE_SCOPES else _NoScope()


def _pack(x):
    return pltpu.bitcast(x.astype(bf16), u32)


def _as_bf16(x):
    return pltpu.bitcast(x, bf16)


def _dot(a, b):
    return jnp.dot(a, b, preferred_element_type=f32)


def _dot_nt(a, b):
    return lax.dot_general(a, b, NT, preferred_element_type=f32)


def _layernorm_packed(x):
    outs = []
    for r in range(x.shape[0] // 16):
        xr = x[r * 16:(r + 1) * 16]
        mu = jnp.sum(xr, axis=1, keepdims=True) * (1.0 / D)
        xc = xr - mu
        var = jnp.sum(xc * xc, axis=1, keepdims=True) * (1.0 / D)
        outs.append(_pack(xc * lax.rsqrt(var + EPS)))
    return jnp.concatenate(outs, axis=0)


def _token(v):
    t = pltpu.bitcast(v[0:8, :], u32)
    return lax.shift_right_logical(jnp.bitwise_and(t, jnp.uint32(0xFFFF)), jnp.uint32(16))


def _after(x, tok):
    n, m = x.shape
    z = jnp.concatenate([jnp.concatenate([tok] * (m // 128), axis=1)] * (n // 8), axis=0)
    return pltpu.bitcast(jnp.bitwise_or(pltpu.bitcast(x, u32), z), x.dtype)


def _rowsum(x):
    if RSMODE == 1:
        t = x[:, 0:128]
        parts = [x[:, k * 128:(k + 1) * 128] for k in range(x.shape[1] // 128)]
        while len(parts) > 1:
            parts = [a + b for a, b in zip(parts[0::2], parts[1::2])]
        return jnp.sum(parts[0], axis=1, keepdims=True)
    return jnp.sum(x, axis=1, keepdims=True)


def _ln16(xr):
    if LNMODE == 1:
        return _pack(xr)
    if LNMODE == 2:
        mu = _rowsum(xr) * (1.0 / D)
        ms = _rowsum(xr * xr) * (1.0 / D)
        rs = lax.rsqrt(ms - mu * mu + EPS)
        return _pack(xr * rs - mu * rs)
    if LNMODE == 3:
        mu = _rowsum(xr) * (1.0 / D)
        xc = xr - mu
        var = _rowsum(xc * xc) * (1.0 / D)
        return _pack(xc * (var + EPS))
    if LNMODE == 4:
        mu = _rowsum(xr) * (1.0 / D)
        return _pack(xr - mu)
    mu = _rowsum(xr) * (1.0 / D)
    xc = xr - mu
    var = _rowsum(xc * xc) * (1.0 / D)
    return _pack(xc * lax.rsqrt(var + EPS))


def _tree(x, op):
    n = x.shape[0]
    while n > 1:
        n //= 2
        x = op(x[:n], x[n:])
    return x[0]


def _local_attention(q, kc, kp, vc, vp, pos):
    def chunk(x, u, tok):
        if callable(x):
            return x(u)
        n = UCH * (4 if x.dtype == u32 else 8)
        x = x[u * n:(u + 1) * n]
        return x if tok is None else _after(x, tok)

    def shifted(cur, prev, w):
        x = cur
        if w:
            lane = lax.broadcasted_iota(jnp.int32, x.shape, 1)
            x = jnp.where(lane >= 128 - DIL * w, prev, x)
            x = pltpu.roll(x, DIL * w, axis=1)
        if x.dtype == u32:
            x = _as_bf16(x).astype(f32)
        return x.reshape(UCH, 8, 128)

    nu = 16 // UCH
    if LOCAL_OFF:
        return jnp.concatenate([chunk(q, u, None) for u in range(nu)], axis=0)
    even = lax.broadcasted_iota(jnp.int32, (8, 128), 0) % 2 == 0
    acc = [None] * W_LOC
    done = []
    for u in range(nu):
        tok = _token(done[u - KLAG]) if KLAG and u >= KLAG else None
        cur, prev = chunk(kc, u, tok), chunk(kp, u, None)
        qu = chunk(q, u, None).reshape(UCH, 8, 128)
        for w in range(W_LOC):
            t = _tree(qu * shifted(cur, prev, w), jnp.add)
            acc[w] = t if acc[w] is None else acc[w] + t
        done.append(acc[W_LOC - 1])
    logits = []
    for w in range(W_LOC):
        t = acc[w]
        t = t + jnp.where(even, pltpu.roll(t, 7, axis=0), pltpu.roll(t, 1, axis=0))
        t = t * QSCALE
        if w:
            t = jnp.where(pos >= DIL * w, t, NEG)
        logits.append(t)
    m = logits[0]
    for t in logits[1:]:
        m = jnp.maximum(m, t)
    ps = [jnp.exp2(t - m) for t in logits]
    l = ps[0]
    for p in ps[1:]:
        l = l + p
    r = 1.0 / l
    ps = [(p * r)[None] for p in ps]
    outs = []
    for u in range(nu):
        tok = None
        if VLAG:
            tok = _token(outs[u - VLAG] if u >= VLAG else done[nu - VLAG + u])
        cur, prev = chunk(vc, u, tok), chunk(vp, u, None)
        o = None
        for w in range(W_LOC):
            t = shifted(cur, prev, w) * ps[w]
            o = t if o is None else o + t
        outs.append(o.reshape(UCH * 8, 128))
    return jnp.concatenate(outs, axis=0)


def _kernel(x_hbm, wa_hbm, woa_hbm, wb_hbm, wob_hbm, out_hbm,
            x_ref, xio, xn1a, xn1b, xn2, wa_nat, wat, woa, woap, wb_nat, wbt, wk, wkp, wob, wobp,
            khalo, vhalo, wstage, pxn, pbuf, po,
            qT, kN, vT, oN, otbuf,
            sem, *bufs):
    xn1 = (xn1a, xn1b)
    sbufs = bufs[:NC]
    stg = [bufs[NC + 3 * g:NC + 3 * g + 3] for g in range(NG)]

    def x_copy(i, sid):
        rows = pl.ds(i * BLK, BLK)
        return pltpu.make_async_copy(x_hbm.at[rows, :], xio.at[rows, :], sem.at[sid])

    def wa_copies(g):
        return [pltpu.make_async_copy(
            wa_hbm.at[:, pl.ds(pl.multiple_of(sec * D + g * 128, 128), 128)],
            wa_nat.at[g * 3 + sec], sem.at[SEM_WA + g]) for sec in range(3)]

    def wb_copy(c, sid):
        col = c * 128 + (c // 8) * D
        return pltpu.make_async_copy(
            wb_hbm.at[:, pl.ds(col, 128)], wb_nat.at[c], sem.at[sid])

    def wk_copy(c, sid):
        rows = pl.ds(c * 128, 128)
        return pltpu.make_async_copy(
            wb_hbm.at[rows, pl.ds(D, D)], wk.at[rows, :], sem.at[sid])

    def iter_copies(it):
        sid = SEM_IT + min(it, 3)
        if it == 0:
            cps = [pltpu.make_async_copy(woa_hbm, woa, sem.at[sid])]
        else:
            cps = [x_copy(i, sid) for i in (2 * it + 1, 2 * it + 2) if i < NB]
        return cps + [wb_copy(2 * it, sid), wb_copy(2 * it + 1, sid), wk_copy(it, sid)]

    x01_copies = [x_copy(0, SEM_X01), x_copy(1, SEM_X01)]
    x2_copy = x_copy(2, SEM_X2)
    wob_copy = pltpu.make_async_copy(wob_hbm, wob, sem.at[SEM_WOB])

    def out_copy(j):
        rows = pl.ds(pl.multiple_of(j * TF, TF), TF)
        return pltpu.make_async_copy(xio.at[rows, :], out_hbm.at[rows, :], sem.at[SEM_OUT])

    def blk_rows(i, n=BLK):
        return pl.ds(pl.multiple_of(i * n, n), n)

    def qkv_group(g, xn):
        w = jnp.concatenate([wat[g, kt] for kt in range(NG)], axis=1)
        r = jnp.concatenate(
            [_dot_nt(_as_bf16(w[a:a + GM // 2]), xn) for a in range(0, 192, GM // 2)], axis=0)
        k = r[128:256]
        v = r[256:384]
        return r[0:128], _pack(k) if PACK_K else k, _pack(v) if PACK_V else v

    def o_rows(i, n):
        rows = blk_rows(i, n // 2)
        return _as_bf16(jnp.concatenate([oN[t, rows, :] for t in range(NG)], axis=1))

    def proj_residual(o, w_cols, xv, ns=2):
        cols = []
        w = D // ns
        for n in range(ns):
            cols.append(xv[:, n * w:(n + 1) * w] + _dot(o, w_cols(n, ns)))
        return jnp.concatenate(cols, axis=1)

    def packed_cols(w_ref):
        return lambda n, ns=2: _as_bf16(jnp.concatenate(
            [w_ref[NG // ns * n + t] for t in range(NG // ns)], axis=1))

    woa_cols, wob_cols, wk_cols = packed_cols(woap), packed_cols(wobp), packed_cols(wkp)

    def repack(dst_ref, src_ref, c, n, tok=None):
        wv = pltpu.bitcast(src_ref[blk_rows(c, n), :], u32)
        if tok is not None:
            wv = _after(wv, tok)
        for t in range(NG):
            dst_ref[t, blk_rows(c, n // 2), :] = wv[:, t * 128:(t + 1) * 128]

    def store_permuted(dst_ref, row0, val):
        for h in range(4):
            dst_ref[pl.ds(row0 + h, 16, stride=4), :] = val[h * 16:(h + 1) * 16]

    def rows16(blk, r):
        return pl.ds(pl.multiple_of(blk * BLK + r * 16, 16), 16)

    def ln1(blk, r, tok=None):
        rows = rows16(blk, r)
        xv = xio[rows, :].astype(f32)
        if SKIP1:
            return _pack(xv)
        if tok is not None and not NOTOK:
            xv = _after(xv, tok)
        if not XBASE:
            x_ref[rows, :] = xv
        return _ln16(xv)

    def ln2(blk, r, tok=None):
        if SKIP2:
            return
        xv = x_ref[rows16(blk, r), :]
        if tok is not None and not NOTOK:
            xv = _after(xv, tok)
        xn2[pl.ds(pl.multiple_of(blk * (BLK // 2) + r * 8, 8), 8), :] = _ln16(xv)

    def head_group0(xn_packed):
        for ref, val in zip(stg[0], qkv_group(0, _as_bf16(xn_packed))):
            ref[0:val.shape[0], :] = val

    def a_block(i, par, z0, z1):
        def xn_cur():
            if LSKEW == 1:
                return _as_bf16(xn1[par][...])
            return _as_bf16(xn1[par][pl.ds(pl.multiple_of(z1, 8), BLK // 2), :])

        ip = jnp.maximum(i - 1, 0)
        inx = jnp.minimum(i + LSKEW, NB - 1)
        dst = xn1[(par + LSKEW) % 2]
        pos = i * BLK + lax.broadcasted_iota(jnp.int32, (8, 128), 1)

        def stage(g, slot, qkv):
            for ref, val in zip(stg[g], qkv):
                n = val.shape[0]
                ref[pl.ds(pl.multiple_of(z0 + slot * n, 8), n), :] = val

        def getter(ref, slot):
            n = ref.shape[0] // 2
            m = n // (16 // UCH)
            return lambda u: ref[pl.ds(pl.multiple_of(z1 + slot * n + u * m, 8), m), :]

        def ln_jobs(slot, tok):
            for r in range(8):
                if L1S[r] == slot:
                    dst[pl.ds(pl.multiple_of(z0 + r * 8, 8), 8), :] = ln1(inx, r, tok)
            for r in range(8):
                if L2S[r] == slot:
                    ln2(ip, r, tok)

        o_cols = []
        for g in range(NG):
            if g:
                qkv = qkv_group(g, xn_cur())
                stage(g, par, qkv)
            qs, ks, vs = stg[g]
            ot = _local_attention(getter(qs, par), getter(ks, par), getter(ks, 1 - par),
                                  getter(vs, par), getter(vs, 1 - par), pos)
            o_cols.append(ot.astype(bf16).T)
            if TOKMODE == 0:
                tok = _token(qkv[1]) if g else None
                slot = g - 1
            else:
                tok = _token(ot[120:128])
                slot = g
            ln_jobs(slot, tok)
            if slot == WBSLOT:
                wsrc = _as_bf16(_after(pltpu.bitcast(wb_nat[i], u32), tok))
                wbt[i] = pltpu.bitcast(wsrc.T, u32)
            if slot == WKSLOT:
                repack(wkp, wk, i, 64, tok)
        xn_next = xn1[1 - par][pl.ds(pl.multiple_of(z1, 8), BLK // 2), :]
        qkv = qkv_group(0, _as_bf16(xn_next))
        stage(0, 1 - par, qkv)
        ln_jobs(7 + TOKMODE, _token(qkv[1]))
        o = jnp.concatenate(o_cols, axis=1)
        rows = blk_rows(i)
        base = xio[rows, :].astype(f32) if XBASE else x_ref[rows, :]
        xv = proj_residual(o, woa_cols, base, S4N)
        x_ref[rows, :] = xv
        for k in range(4):
            ln_jobs(9 + k, _token(xv[0:8, k * 256:k * 256 + 128]))

    def startup():
        def transpose_wa(g):
            for sec in range(3):
                wv = pltpu.bitcast(wa_nat[g * 3 + sec].T, u32)
                for kt in range(NG):
                    store_permuted(wstage.at[kt], sec * 64, wv[:, kt * 128:(kt + 1) * 128])

        def project(g):
            w = wstage[...]
            wat[g] = w
            w = jnp.concatenate([w[kt] for kt in range(NG)], axis=1)
            return _dot_nt(_as_bf16(w), _as_bf16(pxn[...]))

        def attend(g, r):
            pos = lax.broadcasted_iota(jnp.int32, (8, 128), 1)
            kp = jnp.zeros(khalo.shape[1:], khalo.dtype)
            vp = jnp.zeros(vhalo.shape[1:], vhalo.dtype)
            for b in range(2):
                rb = r[:, b * BLK:(b + 1) * BLK]
                kc = _pack(rb[128:256]) if PACK_K else rb[128:256]
                vc = _pack(rb[256:384]) if PACK_V else rb[256:384]
                ot = _local_attention(rb[0:128], kc, kp, vc, vp, pos + b * BLK)
                po[g, b * 64:(b + 1) * 64, :] = pltpu.bitcast(ot.astype(bf16).T, u32)
                kp, vp = kc, vc
            khalo[g] = kp
            vhalo[g] = vp

        pbuf[...] = jnp.zeros(pbuf.shape, f32)
        for cp in x01_copies:
            cp.wait()
        for b in range(2):
            for r in range(BLK // 16):
                pxn[b * 64 + r * 8:b * 64 + (r + 1) * 8, :] = ln1(b, r)
        for cp in wa_copies(0):
            cp.wait()
        transpose_wa(0)

        def body(g, c):
            if not MIDWAIT:
                for cp in wa_copies(g + 1):
                    cp.wait()
            prev = pbuf[...]
            r = project(g)
            if MIDWAIT:
                attend(jnp.maximum(g - 1, 0), prev)
                for cp in wa_copies(g + 1):
                    cp.wait()
            transpose_wa(g + 1)
            pbuf[...] = r
            if not MIDWAIT:
                attend(jnp.maximum(g - 1, 0), prev)
            return c
        lax.fori_loop(0, NG - 1, body, 0)

        x2_copy.wait()
        prev = pbuf[...]
        r = project(NG - 1)
        xn_next = jnp.concatenate([ln1(2, r16) for r16 in range(BLK // 16)], axis=0)
        xn1[0][...] = xn_next
        attend(NG - 2, _after(prev, _token(xn_next[56:64, 0:128])))
        head_group0(xn_next)
        attend(NG - 1, r)

        for cp in iter_copies(0):
            cp.wait()
        for t in range(NG):
            wv = pltpu.bitcast(woa[:, t * 128:(t + 1) * 128], u32)
            for g in range(NG):
                store_permuted(woap.at[t], g * 64, wv[g * 64:(g + 1) * 64])
        for b in range(2):
            o = jnp.concatenate([po[g, b * 64:(b + 1) * 64, :] for g in range(NG)], axis=1)
            rows = blk_rows(b)
            base = xio[rows, :].astype(f32) if XBASE else x_ref[rows, :]
            x_ref[rows, :] = proj_residual(_as_bf16(o), woa_cols, base)
            wbt[b] = pltpu.bitcast(wb_nat[b].T, u32)
        repack(wkp, wk, 0, 128)
        for r16 in range(BLK // 16):
            ln2(0, r16)
        for g in range(NG):
            for ref, src in ((stg[g][1], khalo), (stg[g][2], vhalo)):
                n = src.shape[1]
                ref[n:2 * n, :] = src[g]
        for cp in iter_copies(1):
            cp.wait()

    def phase_a(rep):
        @pl.when(rep == 1)
        def _():
            for g in range(NG):
                for ref in stg[g][1:]:
                    n = ref.shape[0] // 2
                    ref[n:2 * n, :] = jnp.zeros((n, BLK), ref.dtype)
            xn_first = jnp.concatenate([ln1(0, r) for r in range(BLK // 16)], axis=0)
            xn1[0][...] = xn_first
            head_group0(xn_first)

        def body(it, c):
            @pl.when(it == 2 - rep * NB)
            def _():
                for cp in iter_copies(2):
                    cp.wait()

            @pl.when(it == 3 - rep * NB)
            def _():
                for k in range(3, NB // APB):
                    for cp in iter_copies(k):
                        cp.wait()

            z0 = lax.shift_right_logical(it, 16) * 8
            z1 = lax.shift_right_logical(it, 17) * 8
            with _scope("a_iter"):
                for u in range(APB):
                    a_block(it * APB + u, u % 2, z0, z1)
            return c
        with _scope("a_loop"):
            lax.fori_loop(1 - rep, NB // APB, body, 0)
        for r in range(BLK // 16):
            ln2(NB - 1, r)

    def phase_b_proj():
        def body(j, c):
            rows = blk_rows(j, TB // 2)
            xn = _as_bf16(xn2[rows, :])
            for n in range(2):
                y = _pack(_dot(xn, wk_cols(n)))
                for t in range(4):
                    kN[4 * n + t, rows, :] = y[:, t * 128:(t + 1) * 128]
            for r in range(4):
                w = _as_bf16(wbt[2 * r:2 * r + 2].reshape(128, D))
                y = _pack(_dot_nt(w, xn) * QSCALE)
                for b in range(TB // NQ):
                    qT[j * (TB // NQ) + b, r * 128:(r + 1) * 128, :] = y[:, b * NQ:(b + 1) * NQ]
            for r in range(4):
                w = _as_bf16(wbt[8 + 2 * r:8 + 2 * r + 2].reshape(128, D))
                y = _pack(_dot_nt(w, xn))
                for b in range(TB // MK):
                    vT[j * (TB // MK) + b, r * 128:(r + 1) * 128, :] = y[:, b * MK:(b + 1) * MK]
            return c
        lax.fori_loop(0, S // TB, body, 0)

    def phase_b_attn():
        off = [0, 0]

        def qm_of(t, qi, j):
            q = _as_bf16(qT[qi, pl.ds(pl.multiple_of(t * 64 + j * 16, 16), 16), :])
            parts = []
            if j > 0:
                parts.append(jnp.zeros((32 * j, NQ), bf16))
            parts.append(q)
            if j < 3:
                parts.append(jnp.zeros((32 * (3 - j), NQ), bf16))
            return jnp.concatenate(parts, axis=0)

        def qk_chunk(t, qm, c, par, m):
            k = _as_bf16(kN[t, c * (MK // 2):(c + 1) * (MK // 2), :])
            s = _dot(k, qm)
            sbufs[c][pl.ds(pl.multiple_of(off[0] + par * MK, 8), MK), :] = s
            sm = _tree(s.reshape(MK // 8, 8, NQ), jnp.maximum)
            return sm if m is None else jnp.maximum(m, sm)

        def pv_chunk(h, c, par, mrow, l, o):
            s = sbufs[c][pl.ds(pl.multiple_of(off[1] + par * MK, 8), MK), :]
            p = jnp.exp2(s - mrow)
            ls = jnp.sum(p.reshape(MK // 8, 8, NQ), axis=0)
            l = ls if l is None else l + ls
            v = _as_bf16(vT[c, pl.ds(pl.multiple_of(h * 16, 16), 16), :])
            oc = _dot(v, p.astype(bf16))
            o = oc if o is None else o + oc
            return l, o

        def flush_o(g, val):
            y = pltpu.bitcast(_as_bf16(val).T, u32)
            oN[g % NG, blk_rows(g // NG, NQ // 2), :] = y

        n_groups = NQT * NG
        otbuf[...] = jnp.zeros(otbuf.shape, u32)
        qm = qm_of(0, 0, 0)
        m0 = None
        for c in range(NC):
            m0 = qk_chunk(0, qm, c, 0, m0)
        qm = qm_of(0, 0, 1)
        m1 = None
        for c in range(DL):
            m1 = qk_chunk(0, qm, c, 1, m1)

        def group(g, g_next, carry, zero, side_job=None):
            qi = g // NG
            t = g % NG
            off[0] = lax.shift_right_logical(zero, 16) * 8
            off[1] = lax.shift_right_logical(zero, 17) * 8
            flush_o(jnp.maximum(g - 1, 0), otbuf[...])
            ms = {0: carry[0], 1: carry[1]}
            qms = {}
            l = o = mrow = None
            for n in range(4 * NC):
                j, c = divmod(n, NC)
                j2, c2 = divmod(n + NC + DL, NC)
                if j2 < 4 or g_next is not None:
                    t2 = t if j2 < 4 else g_next % NG
                    if j2 not in qms:
                        qms[j2] = qm_of(t2, qi if j2 < 4 else g_next // NG, j2 % 4)
                    ms[j2] = qk_chunk(t2, qms[j2], c2, j2 % 2, ms.get(j2))
                if c == 0:
                    mrow = jnp.max(ms[j], axis=0, keepdims=True)
                    l = o = None
                l, o = pv_chunk(t * 4 + j, c, j % 2, mrow, l, o)
                if side_job is not None and n == NC // 2:
                    side_job(_token(l[:, 0:128]))
                if c == NC - 1:
                    lrow = jnp.sum(l, axis=0, keepdims=True)
                    otbuf[j * 16:(j + 1) * 16, :] = _pack(o * (1.0 / lrow))
            return ms.get(4), ms.get(5)

        def body(it, ms):
            def side_job(tok):
                repack(wobp, wob, it, D * GPB // n_groups, tok)

            for u in range(GPB):
                g = it * GPB + u
                ms = group(g, jnp.minimum(g + 1, n_groups - 1), ms, it,
                           side_job if u == 0 else None)
            return ms

        lax.fori_loop(0, n_groups // GPB, body, (m0, m1))
        off[0] = off[1] = 0
        flush_o(n_groups - 1, otbuf[...])

    def phase_b_out(rep):
        def body(jj, c):
            for u in range(OPB):
                j = jj * OPB + u
                rows = blk_rows(j, TF)
                xv = proj_residual(o_rows(j, TF), wob_cols, x_ref[rows, :])
                xio[rows, :] = xv.astype(bf16)

                @pl.when(rep == 1)
                def _():
                    out_copy(j).start()
            return c
        lax.fori_loop(0, S // (TF * OPB), body, 0)

    def sem_dummy():
        return lax.fori_loop(0, 3, lambda i, c: c + i, 0)

    if ONLY_A:
        phase_a(lax.shift_right_logical(sem_dummy(), 1))
        xio[0:8, :] = (_as_bf16(wbt[0, 0:4, :]) + _as_bf16(xn2[0:4, :])
                       + jnp.concatenate([_as_bf16(wkp[0, 0:4, :])] * 8, axis=1))
        return

    for cp in x01_copies:
        cp.start()
    for g in range(NG):
        if g == NG - 2:
            x2_copy.start()
        for cp in wa_copies(g):
            cp.start()
    for it in range(NB // APB):
        for cp in iter_copies(it):
            cp.start()
    wob_copy.start()

    with _scope("startup"):
        startup()

    def layer_pair(rep, c):
        with _scope("phase_a"):
            phase_a(rep)

        @pl.when(rep == 0)
        def _():
            wob_copy.wait()

        with _scope("b_proj"):
            phase_b_proj()
        with _scope("b_attn"):
            phase_b_attn()
        with _scope("b_out"):
            phase_b_out(rep)
        return c
    lax.fori_loop(0, 2, layer_pair, 0)
    for j in range(S // TF):
        out_copy(j).wait()


@jax.jit
def pallas_interleave_layers__sliding_local_dilated__softmax_full_mha__prompt_kernel(
    A_x: jax.Array,
    A_wqkv: jax.Array,
    A_wo: jax.Array,
    B_x: jax.Array,
    B_wqkv: jax.Array,
    B_wo: jax.Array,
):
    del B_x
    x = A_x.reshape(S, D)
    vm = pltpu.VMEM
    kshape, kdt = ((64, BLK), u32) if PACK_K else ((128, BLK), f32)
    vshape, vdt = ((64, BLK), u32) if PACK_V else ((128, BLK), f32)
    scratch = [
        vm((S, D), f32),
        vm((S, D), bf16),
        vm((BLK // 2, D), u32),
        vm((BLK // 2, D), u32),
        vm((S // 2, D), u32),
        vm((3 * NG, D, 128), bf16),
        vm((NG, NG, 192, 128), u32),
        vm((D, D), bf16),
        vm((NG, D // 2, 128), u32),
        vm((2 * NG, D, 128), bf16),
        vm((2 * NG, 64, D), u32),
        vm((D, D), bf16),
        vm((NG, D // 2, 128), u32),
        vm((D, D), bf16),
        vm((NG, D // 2, 128), u32),
        vm((NG,) + kshape, kdt),
        vm((NG,) + vshape, vdt),
        vm((NG, 192, 128), u32),
        vm((BLK, D), u32),
        vm((384, 2 * BLK), f32),
        vm((NG, BLK, 128), u32),
        vm((NQT, D // 2, NQ), u32),
        vm((NG, S // 2, 128), u32),
        vm((NC, D // 2, MK), u32),
        vm((NG, S // 2, 128), u32),
        vm((64, NQ), u32),
        pltpu.SemaphoreType.DMA((N_SEM,)),
    ] + [vm((2 * MK, NQ), f32)] * NC + [
        vm((256, BLK), f32), vm((2 * kshape[0], BLK), kdt), vm((2 * vshape[0], BLK), vdt)] * NG
    out = pl.pallas_call(
        _kernel,
        out_shape=jax.ShapeDtypeStruct((S, D), bf16),
        in_specs=[pl.BlockSpec(memory_space=pl.ANY)] * 5,
        out_specs=pl.BlockSpec(memory_space=pl.ANY),
        scratch_shapes=scratch,
        compiler_params=pltpu.CompilerParams(
            vmem_limit_bytes=110 * 1024 * 1024, disable_bounds_checks=NOBC),
        name="interleave_attn",
    )(x, A_wqkv, A_wo, B_wqkv, B_wo)
    return out.reshape(1, S, D)
```

```python
import jax
import jax.numpy as jnp
from jax import lax
import jax.experimental.pallas as pl
import jax.experimental.pallas.tpu as pltpu

S, D, H, DH = 2048, 1024, 32, 32
W_LOC, DIL = 8, 2
EPS = 1e-5
LOG2E = 1.4426950408889634
QSCALE = (DH ** -0.5) * LOG2E
NEG = -1e9 * LOG2E

BLK = 128
NB = S // BLK
NG = D // 128
NQ = 256
NQT = S // NQ
MK = 128
NC = S // MK
DL = 6
APB = 2
GPB = 4
TB = 256
TF = 256

SEM_X01, SEM_X2, SEM_WOB, SEM_OUT = 0, 1, 2, 3
SEM_WA = 4
SEM_IT = SEM_WA + NG
N_SEM = SEM_IT + 4

PACK_K = True
GM = 128
PACK_V = True
UCH = 4
ONLY_A = False
ONLY_B = False
ZINIT = True
PVFIRST = False
MIDWAIT = False
NOBC = False
OPB = 2
S4N = 2
LNORD = 0
XBASE = True
WKSLOT = 5
LSKEW = 1
L1S = (0, 0, 1, 1, 2, 2, 3, 3)
L2S = (4, 5, 6, 7, 8, 8, 8, 8)
RSMODE = 0
NOTOK = False
SKIP1 = False
SKIP2 = False
TOKMODE = 1
WBSLOT = 4
LOCAL_OFF = False
LNMODE = 0
KLAG = 0
VLAG = 0
PROFILE_SCOPES = False

bf16 = jnp.bfloat16
f32 = jnp.float32
u32 = jnp.uint32
NT = (((1,), (1,)), ((), ()))


class _NoScope:
    def __enter__(self):
        return self

    def __exit__(self, *a):
        return False


def _scope(name):
    return jax.named_scope(name) if PROFILE_SCOPES else _NoScope()


def _pack(x):
    return pltpu.bitcast(x.astype(bf16), u32)


def _as_bf16(x):
    return pltpu.bitcast(x, bf16)


def _dot(a, b):
    return jnp.dot(a, b, preferred_element_type=f32)


def _dot_nt(a, b):
    return lax.dot_general(a, b, NT, preferred_element_type=f32)


def _layernorm_packed(x):
    outs = []
    for r in range(x.shape[0] // 16):
        xr = x[r * 16:(r + 1) * 16]
        mu = jnp.sum(xr, axis=1, keepdims=True) * (1.0 / D)
        xc = xr - mu
        var = jnp.sum(xc * xc, axis=1, keepdims=True) * (1.0 / D)
        outs.append(_pack(xc * lax.rsqrt(var + EPS)))
    return jnp.concatenate(outs, axis=0)


def _token(v):
    t = pltpu.bitcast(v[0:8, :], u32)
    return lax.shift_right_logical(jnp.bitwise_and(t, jnp.uint32(0xFFFF)), jnp.uint32(16))


def _after(x, tok):
    n, m = x.shape
    z = jnp.concatenate([jnp.concatenate([tok] * (m // 128), axis=1)] * (n // 8), axis=0)
    return pltpu.bitcast(jnp.bitwise_or(pltpu.bitcast(x, u32), z), x.dtype)


def _rowsum(x):
    if RSMODE == 1:
        t = x[:, 0:128]
        parts = [x[:, k * 128:(k + 1) * 128] for k in range(x.shape[1] // 128)]
        while len(parts) > 1:
            parts = [a + b for a, b in zip(parts[0::2], parts[1::2])]
        return jnp.sum(parts[0], axis=1, keepdims=True)
    return jnp.sum(x, axis=1, keepdims=True)


def _ln16(xr):
    if LNMODE == 1:
        return _pack(xr)
    if LNMODE == 2:
        mu = _rowsum(xr) * (1.0 / D)
        ms = _rowsum(xr * xr) * (1.0 / D)
        rs = lax.rsqrt(ms - mu * mu + EPS)
        return _pack(xr * rs - mu * rs)
    if LNMODE == 3:
        mu = _rowsum(xr) * (1.0 / D)
        xc = xr - mu
        var = _rowsum(xc * xc) * (1.0 / D)
        return _pack(xc * (var + EPS))
    if LNMODE == 4:
        mu = _rowsum(xr) * (1.0 / D)
        return _pack(xr - mu)
    mu = _rowsum(xr) * (1.0 / D)
    xc = xr - mu
    var = _rowsum(xc * xc) * (1.0 / D)
    return _pack(xc * lax.rsqrt(var + EPS))


def _tree(x, op):
    n = x.shape[0]
    while n > 1:
        n //= 2
        x = op(x[:n], x[n:])
    return x[0]


def _local_attention(q, kc, kp, vc, vp, pos):
    def chunk(x, u, tok):
        if callable(x):
            return x(u)
        n = UCH * (4 if x.dtype == u32 else 8)
        x = x[u * n:(u + 1) * n]
        return x if tok is None else _after(x, tok)

    def shifted(cur, prev, w):
        x = cur
        if w:
            lane = lax.broadcasted_iota(jnp.int32, x.shape, 1)
            x = jnp.where(lane >= 128 - DIL * w, prev, x)
            x = pltpu.roll(x, DIL * w, axis=1)
        if x.dtype == u32:
            x = _as_bf16(x).astype(f32)
        return x.reshape(UCH, 8, 128)

    nu = 16 // UCH
    if LOCAL_OFF:
        return jnp.concatenate([chunk(q, u, None) for u in range(nu)], axis=0)
    even = lax.broadcasted_iota(jnp.int32, (8, 128), 0) % 2 == 0
    acc = [None] * W_LOC
    done = []
    for u in range(nu):
        tok = _token(done[u - KLAG]) if KLAG and u >= KLAG else None
        cur, prev = chunk(kc, u, tok), chunk(kp, u, None)
        qu = chunk(q, u, None).reshape(UCH, 8, 128)
        for w in range(W_LOC):
            t = _tree(qu * shifted(cur, prev, w), jnp.add)
            acc[w] = t if acc[w] is None else acc[w] + t
        done.append(acc[W_LOC - 1])
    logits = []
    for w in range(W_LOC):
        t = acc[w]
        t = t + jnp.where(even, pltpu.roll(t, 7, axis=0), pltpu.roll(t, 1, axis=0))
        t = t * QSCALE
        if w:
            t = jnp.where(pos >= DIL * w, t, NEG)
        logits.append(t)
    m = logits[0]
    for t in logits[1:]:
        m = jnp.maximum(m, t)
    ps = [jnp.exp2(t - m) for t in logits]
    l = ps[0]
    for p in ps[1:]:
        l = l + p
    r = 1.0 / l
    ps = [(p * r)[None] for p in ps]
    outs = []
    for u in range(nu):
        tok = None
        if VLAG:
            tok = _token(outs[u - VLAG] if u >= VLAG else done[nu - VLAG + u])
        cur, prev = chunk(vc, u, tok), chunk(vp, u, None)
        o = None
        for w in range(W_LOC):
            t = shifted(cur, prev, w) * ps[w]
            o = t if o is None else o + t
        outs.append(o.reshape(UCH * 8, 128))
    return jnp.concatenate(outs, axis=0)


def _kernel(x_hbm, wa_hbm, woa_hbm, wb_hbm, wob_hbm, out_hbm,
            x_ref, xio, xn1a, xn1b, xn2, wa_nat, wat, woa, woap, wb_nat, wbt, wk, wkp, wob, wobp,
            khalo, vhalo, wstage, pxn, pbuf, po,
            qT, kN, vT, oN, otbuf,
            sem, *bufs):
    xn1 = (xn1a, xn1b)
    sbufs = bufs[:NC]
    stg = [bufs[NC + 3 * g:NC + 3 * g + 3] for g in range(NG)]

    def x_copy(i, sid):
        rows = pl.ds(i * BLK, BLK)
        return pltpu.make_async_copy(x_hbm.at[rows, :], xio.at[rows, :], sem.at[sid])

    def wa_copies(g):
        return [pltpu.make_async_copy(
            wa_hbm.at[:, pl.ds(pl.multiple_of(sec * D + g * 128, 128), 128)],
            wa_nat.at[g * 3 + sec], sem.at[SEM_WA + g]) for sec in range(3)]

    def wb_copy(c, sid):
        col = c * 128 + (c // 8) * D
        return pltpu.make_async_copy(
            wb_hbm.at[:, pl.ds(col, 128)], wb_nat.at[c], sem.at[sid])

    def wk_copy(c, sid):
        rows = pl.ds(c * 128, 128)
        return pltpu.make_async_copy(
            wb_hbm.at[rows, pl.ds(D, D)], wk.at[rows, :], sem.at[sid])

    def iter_copies(it):
        sid = SEM_IT + min(it, 3)
        if it == 0:
            cps = [pltpu.make_async_copy(woa_hbm, woa, sem.at[sid])]
        else:
            cps = [x_copy(i, sid) for i in (2 * it + 1, 2 * it + 2) if i < NB]
        return cps + [wb_copy(2 * it, sid), wb_copy(2 * it + 1, sid), wk_copy(it, sid)]

    x01_copies = [x_copy(0, SEM_X01), x_copy(1, SEM_X01)]
    x2_copy = x_copy(2, SEM_X2)
    wob_copy = pltpu.make_async_copy(wob_hbm, wob, sem.at[SEM_WOB])

    def out_copy(j):
        rows = pl.ds(pl.multiple_of(j * TF, TF), TF)
        return pltpu.make_async_copy(xio.at[rows, :], out_hbm.at[rows, :], sem.at[SEM_OUT])

    def blk_rows(i, n=BLK):
        return pl.ds(pl.multiple_of(i * n, n), n)

    def qkv_group(g, xn):
        w = jnp.concatenate([wat[g, kt] for kt in range(NG)], axis=1)
        r = jnp.concatenate(
            [_dot_nt(_as_bf16(w[a:a + GM // 2]), xn) for a in range(0, 192, GM // 2)], axis=0)
        k = r[128:256]
        v = r[256:384]
        return r[0:128], _pack(k) if PACK_K else k, _pack(v) if PACK_V else v

    def o_rows(i, n):
        rows = blk_rows(i, n // 2)
        return _as_bf16(jnp.concatenate([oN[t, rows, :] for t in range(NG)], axis=1))

    def proj_residual(o, w_cols, xv, ns=2):
        cols = []
        w = D // ns
        for n in range(ns):
            cols.append(xv[:, n * w:(n + 1) * w] + _dot(o, w_cols(n, ns)))
        return jnp.concatenate(cols, axis=1)

    def packed_cols(w_ref):
        return lambda n, ns=2: _as_bf16(jnp.concatenate(
            [w_ref[NG // ns * n + t] for t in range(NG // ns)], axis=1))

    woa_cols, wob_cols, wk_cols = packed_cols(woap), packed_cols(wobp), packed_cols(wkp)

    def repack(dst_ref, src_ref, c, n, tok=None):
        wv = pltpu.bitcast(src_ref[blk_rows(c, n), :], u32)
        if tok is not None:
            wv = _after(wv, tok)
        for t in range(NG):
            dst_ref[t, blk_rows(c, n // 2), :] = wv[:, t * 128:(t + 1) * 128]

    def store_permuted(dst_ref, row0, val):
        for h in range(4):
            dst_ref[pl.ds(row0 + h, 16, stride=4), :] = val[h * 16:(h + 1) * 16]

    def rows16(blk, r):
        return pl.ds(pl.multiple_of(blk * BLK + r * 16, 16), 16)

    def ln1(blk, r, tok=None):
        rows = rows16(blk, r)
        xv = xio[rows, :].astype(f32)
        if SKIP1:
            return _pack(xv)
        if tok is not None and not NOTOK:
            xv = _after(xv, tok)
        if not XBASE:
            x_ref[rows, :] = xv
        return _ln16(xv)

    def ln2(blk, r, tok=None):
        if SKIP2:
            return
        xv = x_ref[rows16(blk, r), :]
        if tok is not None and not NOTOK:
            xv = _after(xv, tok)
        xn2[pl.ds(pl.multiple_of(blk * (BLK // 2) + r * 8, 8), 8), :] = _ln16(xv)

    def head_group0(xn_packed):
        for ref, val in zip(stg[0], qkv_group(0, _as_bf16(xn_packed))):
            ref[0:val.shape[0], :] = val

    def a_block(i, par, z0, z1):
        def xn_cur():
            if LSKEW == 1:
                return _as_bf16(xn1[par][...])
            return _as_bf16(xn1[par][pl.ds(pl.multiple_of(z1, 8), BLK // 2), :])

        ip = jnp.maximum(i - 1, 0)
        inx = jnp.minimum(i + LSKEW, NB - 1)
        dst = xn1[(par + LSKEW) % 2]
        pos = i * BLK + lax.broadcasted_iota(jnp.int32, (8, 128), 1)

        def stage(g, slot, qkv):
            for ref, val in zip(stg[g], qkv):
                n = val.shape[0]
                ref[pl.ds(pl.multiple_of(z0 + slot * n, 8), n), :] = val

        def getter(ref, slot):
            n = ref.shape[0] // 2
            m = n // (16 // UCH)
            return lambda u: ref[pl.ds(pl.multiple_of(z1 + slot * n + u * m, 8), m), :]

        def ln_jobs(slot, tok):
            for r in range(8):
                if L1S[r] == slot:
                    dst[pl.ds(pl.multiple_of(z0 + r * 8, 8), 8), :] = ln1(inx, r, tok)
            for r in range(8):
                if L2S[r] == slot:
                    ln2(ip, r, tok)

        o_cols = []
        for g in range(NG):
            if g:
                qkv = qkv_group(g, xn_cur())
                stage(g, par, qkv)
            qs, ks, vs = stg[g]
            ot = _local_attention(getter(qs, par), getter(ks, par), getter(ks, 1 - par),
                                  getter(vs, par), getter(vs, 1 - par), pos)
            o_cols.append(ot.astype(bf16).T)
            if TOKMODE == 0:
                tok = _token(qkv[1]) if g else None
                slot = g - 1
            else:
                tok = _token(ot[120:128])
                slot = g
            ln_jobs(slot, tok)
            if slot == WBSLOT:
                wsrc = _as_bf16(_after(pltpu.bitcast(wb_nat[i], u32), tok))
                wbt[i] = pltpu.bitcast(wsrc.T, u32)
            if slot == WKSLOT:
                repack(wkp, wk, i, 64, tok)
        xn_next = xn1[1 - par][pl.ds(pl.multiple_of(z1, 8), BLK // 2), :]
        qkv = qkv_group(0, _as_bf16(xn_next))
        stage(0, 1 - par, qkv)
        ln_jobs(7 + TOKMODE, _token(qkv[1]))
        o = jnp.concatenate(o_cols, axis=1)
        rows = blk_rows(i)
        base = xio[rows, :].astype(f32) if XBASE else x_ref[rows, :]
        xv = proj_residual(o, woa_cols, base, S4N)
        x_ref[rows, :] = xv
        for k in range(4):
            ln_jobs(9 + k, _token(xv[0:8, k * 256:k * 256 + 128]))

    def startup():
        def transpose_wa(g):
            for sec in range(3):
                wv = pltpu.bitcast(wa_nat[g * 3 + sec].T, u32)
                for kt in range(NG):
                    store_permuted(wstage.at[kt], sec * 64, wv[:, kt * 128:(kt + 1) * 128])

        def project(g):
            w = wstage[...]
            wat[g] = w
            w = jnp.concatenate([w[kt] for kt in range(NG)], axis=1)
            return _dot_nt(_as_bf16(w), _as_bf16(pxn[...]))

        def attend(g, r):
            pos = lax.broadcasted_iota(jnp.int32, (8, 128), 1)
            kp = jnp.zeros(khalo.shape[1:], khalo.dtype)
            vp = jnp.zeros(vhalo.shape[1:], vhalo.dtype)
            for b in range(2):
                rb = r[:, b * BLK:(b + 1) * BLK]
                kc = _pack(rb[128:256]) if PACK_K else rb[128:256]
                vc = _pack(rb[256:384]) if PACK_V else rb[256:384]
                ot = _local_attention(rb[0:128], kc, kp, vc, vp, pos + b * BLK)
                po[g, b * 64:(b + 1) * 64, :] = pltpu.bitcast(ot.astype(bf16).T, u32)
                kp, vp = kc, vc
            khalo[g] = kp
            vhalo[g] = vp

        pbuf[...] = jnp.zeros(pbuf.shape, f32)

        def zero_scores(k, c):
            for sb in sbufs:
                sb[blk_rows(k, 32), :] = jnp.zeros((32, NQ), f32)
            return c
        lax.fori_loop(0, 2 * MK // 32, zero_scores, 0)
        for cp in x01_copies:
            cp.wait()
        for b in range(2):
            for r in range(BLK // 16):
                pxn[b * 64 + r * 8:b * 64 + (r + 1) * 8, :] = ln1(b, r)
        for cp in wa_copies(0):
            cp.wait()
        transpose_wa(0)

        def body(g, c):
            if not MIDWAIT:
                for cp in wa_copies(g + 1):
                    cp.wait()
            prev = pbuf[...]
            r = project(g)
            if MIDWAIT:
                attend(jnp.maximum(g - 1, 0), prev)
                for cp in wa_copies(g + 1):
                    cp.wait()
            transpose_wa(g + 1)
            pbuf[...] = r
            if not MIDWAIT:
                attend(jnp.maximum(g - 1, 0), prev)
            return c
        lax.fori_loop(0, NG - 1, body, 0)

        x2_copy.wait()
        prev = pbuf[...]
        r = project(NG - 1)
        xn_next = jnp.concatenate([ln1(2, r16) for r16 in range(BLK // 16)], axis=0)
        xn1[0][...] = xn_next
        attend(NG - 2, _after(prev, _token(xn_next[56:64, 0:128])))
        head_group0(xn_next)
        attend(NG - 1, r)

        for cp in iter_copies(0):
            cp.wait()
        for t in range(NG):
            wv = pltpu.bitcast(woa[:, t * 128:(t + 1) * 128], u32)
            for g in range(NG):
                store_permuted(woap.at[t], g * 64, wv[g * 64:(g + 1) * 64])
        for b in range(2):
            o = jnp.concatenate([po[g, b * 64:(b + 1) * 64, :] for g in range(NG)], axis=1)
            rows = blk_rows(b)
            base = xio[rows, :].astype(f32) if XBASE else x_ref[rows, :]
            x_ref[rows, :] = proj_residual(_as_bf16(o), woa_cols, base)
            wbt[b] = pltpu.bitcast(wb_nat[b].T, u32)
        repack(wkp, wk, 0, 128)
        for r16 in range(BLK // 16):
            ln2(0, r16)
        for g in range(NG):
            for ref, src in ((stg[g][1], khalo), (stg[g][2], vhalo)):
                n = src.shape[1]
                ref[n:2 * n, :] = src[g]
        for cp in iter_copies(1):
            cp.wait()

    def phase_a(rep):
        @pl.when(rep == 1)
        def _():
            for g in range(NG):
                for ref in stg[g][1:]:
                    n = ref.shape[0] // 2
                    ref[n:2 * n, :] = jnp.zeros((n, BLK), ref.dtype)
            xn_first = jnp.concatenate([ln1(0, r) for r in range(BLK // 16)], axis=0)
            xn1[0][...] = xn_first
            head_group0(xn_first)

        def body(it, c):
            @pl.when(it == 2 - rep * NB)
            def _():
                for cp in iter_copies(2):
                    cp.wait()

            @pl.when(it == 3 - rep * NB)
            def _():
                for k in range(3, NB // APB):
                    for cp in iter_copies(k):
                        cp.wait()

            z0 = lax.shift_right_logical(it, 16) * 8
            z1 = lax.shift_right_logical(it, 17) * 8
            with _scope("a_iter"):
                for u in range(APB):
                    a_block(it * APB + u, u % 2, z0, z1)
            return c
        with _scope("a_loop"):
            lax.fori_loop(1 - rep, NB // APB, body, 0)
        for r in range(BLK // 16):
            ln2(NB - 1, r)

    def phase_b_proj():
        def body(j, c):
            rows = blk_rows(j, TB // 2)
            xn = _as_bf16(xn2[rows, :])
            for n in range(2):
                y = _pack(_dot(xn, wk_cols(n)))
                for t in range(4):
                    kN[4 * n + t, rows, :] = y[:, t * 128:(t + 1) * 128]
            for r in range(4):
                w = _as_bf16(wbt[2 * r:2 * r + 2].reshape(128, D))
                y = _pack(_dot_nt(w, xn) * QSCALE)
                for b in range(TB // NQ):
                    qT[j * (TB // NQ) + b, r * 128:(r + 1) * 128, :] = y[:, b * NQ:(b + 1) * NQ]
            for r in range(4):
                w = _as_bf16(wbt[8 + 2 * r:8 + 2 * r + 2].reshape(128, D))
                y = _pack(_dot_nt(w, xn))
                for b in range(TB // MK):
                    vT[j * (TB // MK) + b, r * 128:(r + 1) * 128, :] = y[:, b * MK:(b + 1) * MK]
            return c
        lax.fori_loop(0, S // TB, body, 0)

    def phase_b_attn():
        off = [0, 0]

        def qm_of(t, qi, j):
            q = _as_bf16(qT[qi, pl.ds(pl.multiple_of(t * 64 + j * 16, 16), 16), :])
            parts = []
            if j > 0:
                parts.append(jnp.zeros((32 * j, NQ), bf16))
            parts.append(q)
            if j < 3:
                parts.append(jnp.zeros((32 * (3 - j), NQ), bf16))
            return jnp.concatenate(parts, axis=0)

        def qk_chunk(t, qm, c, par, m):
            k = _as_bf16(kN[t, c * (MK // 2):(c + 1) * (MK // 2), :])
            s = _dot(k, qm)
            sbufs[c][pl.ds(pl.multiple_of(off[0] + par * MK, 8), MK), :] = s
            sm = _tree(s.reshape(MK // 8, 8, NQ), jnp.maximum)
            return sm if m is None else jnp.maximum(m, sm)

        def pv_chunk(h, c, par, mrow, l, o):
            s = sbufs[c][pl.ds(pl.multiple_of(off[1] + par * MK, 8), MK), :]
            p = jnp.exp2(s - mrow)
            ls = jnp.sum(p.reshape(MK // 8, 8, NQ), axis=0)
            l = ls if l is None else l + ls
            v = _as_bf16(vT[c, pl.ds(pl.multiple_of(h * 16, 16), 16), :])
            oc = _dot(v, p.astype(bf16))
            o = oc if o is None else o + oc
            return l, o

        def flush_o(g, val):
            y = pltpu.bitcast(_as_bf16(val).T, u32)
            oN[g % NG, blk_rows(g // NG, NQ // 2), :] = y

        n_groups = NQT * NG
        lag = NC + DL
        n_steps = 4 * NC

        def set_offsets(zero):
            off[0] = lax.shift_right_logical(zero, 16) * 8
            off[1] = lax.shift_right_logical(zero, 17) * 8

        def pv_step(g, n, ms, st):
            j, c = divmod(n, NC)
            l, o, mrow = st
            if c == 0:
                mrow = jnp.max(ms[j], axis=0, keepdims=True)
                l = o = None
            l, o = pv_chunk((g % NG) * 4 + j, c, j % 2, mrow, l, o)
            if c == NC - 1:
                lrow = jnp.sum(l, axis=0, keepdims=True)
                otbuf[j * 16:(j + 1) * 16, :] = _pack(o * (1.0 / lrow))
                if j == 3:
                    flush_o(g, otbuf[...])
            return l, o, mrow

        def group(g, g_prev, carry, side_job=None):
            st, ms_prev = carry[:3], {3: carry[3]}
            ms = {}
            for n in range(n_steps):
                j, c = divmod(n, NC)
                if c == 0:
                    qm = qm_of(g % NG, g // NG, j)
                if not PVFIRST:
                    ms[j] = qk_chunk(g % NG, qm, c, j % 2, ms.get(j))
                if n < lag:
                    st = pv_step(g_prev, n + n_steps - lag, ms_prev, st)
                else:
                    st = pv_step(g, n - lag, ms, st)
                if PVFIRST:
                    ms[j] = qk_chunk(g % NG, qm, c, j % 2, ms.get(j))
                if side_job is not None and n == n_steps // 2:
                    side_job(_token(st[0][:, 0:128]))
            return st + (ms[3],)

        def body(it, carry):
            def side_job(tok):
                repack(wobp, wob, it, D * GPB // n_groups, tok)

            set_offsets(it)
            carry = carry[:4]
            for u in range(GPB):
                g = it * GPB + u
                carry = group(g, jnp.maximum(g - 1, 0), carry, side_job if u == 0 else None)
            return carry + (it,)

        otbuf[...] = jnp.zeros(otbuf.shape, u32)
        init = (jnp.zeros((8, NQ), f32), jnp.zeros((DH, NQ), f32),
                jnp.zeros((1, NQ), f32), jnp.zeros((8, NQ), f32), jnp.int32(0))
        carry = lax.fori_loop(0, n_groups // GPB, body, init)
        set_offsets(carry[4])
        st, ms = carry[:3], {3: carry[3]}
        for n in range(n_steps - lag, n_steps):
            st = pv_step(n_groups - 1, n, ms, st)
        off[0] = off[1] = 0

    def phase_b_out(rep):
        def body(jj, c):
            for u in range(OPB):
                j = jj * OPB + u
                rows = blk_rows(j, TF)
                xv = proj_residual(o_rows(j, TF), wob_cols, x_ref[rows, :])
                xio[rows, :] = xv.astype(bf16)

                @pl.when(rep == 1)
                def _():
                    out_copy(j).start()
            return c
        lax.fori_loop(0, S // (TF * OPB), body, 0)

    def sem_dummy():
        return lax.fori_loop(0, 3, lambda i, c: c + i, 0)

    if ONLY_B:
        phase_b_attn()
        xio[0:8, :] = jnp.concatenate([_as_bf16(oN[0, 0:4, :]) + _as_bf16(wobp[0, 0:4, :])] * 8, axis=1)
        return
    if ONLY_A:
        phase_a(lax.shift_right_logical(sem_dummy(), 1))
        xio[0:8, :] = (_as_bf16(wbt[0, 0:4, :]) + _as_bf16(xn2[0:4, :])
                       + jnp.concatenate([_as_bf16(wkp[0, 0:4, :])] * 8, axis=1))
        return

    for cp in x01_copies:
        cp.start()
    for g in range(NG):
        if g == NG - 2:
            x2_copy.start()
        for cp in wa_copies(g):
            cp.start()
    for it in range(NB // APB):
        for cp in iter_copies(it):
            cp.start()
    wob_copy.start()

    with _scope("startup"):
        startup()

    def layer_pair(rep, c):
        with _scope("phase_a"):
            phase_a(rep)

        @pl.when(rep == 0)
        def _():
            wob_copy.wait()

        with _scope("b_proj"):
            phase_b_proj()
        with _scope("b_attn"):
            phase_b_attn()
        with _scope("b_out"):
            phase_b_out(rep)
        return c
    lax.fori_loop(0, 2, layer_pair, 0)
    for j in range(S // TF):
        out_copy(j).wait()


@jax.jit
def pallas_interleave_layers__sliding_local_dilated__softmax_full_mha__prompt_kernel(
    A_x: jax.Array,
    A_wqkv: jax.Array,
    A_wo: jax.Array,
    B_x: jax.Array,
    B_wqkv: jax.Array,
    B_wo: jax.Array,
):
    del B_x
    x = A_x.reshape(S, D)
    vm = pltpu.VMEM
    kshape, kdt = ((64, BLK), u32) if PACK_K else ((128, BLK), f32)
    vshape, vdt = ((64, BLK), u32) if PACK_V else ((128, BLK), f32)
    scratch = [
        vm((S, D), f32),
        vm((S, D), bf16),
        vm((BLK // 2, D), u32),
        vm((BLK // 2, D), u32),
        vm((S // 2, D), u32),
        vm((3 * NG, D, 128), bf16),
        vm((NG, NG, 192, 128), u32),
        vm((D, D), bf16),
        vm((NG, D // 2, 128), u32),
        vm((2 * NG, D, 128), bf16),
        vm((2 * NG, 64, D), u32),
        vm((D, D), bf16),
        vm((NG, D // 2, 128), u32),
        vm((D, D), bf16),
        vm((NG, D // 2, 128), u32),
        vm((NG,) + kshape, kdt),
        vm((NG,) + vshape, vdt),
        vm((NG, 192, 128), u32),
        vm((BLK, D), u32),
        vm((384, 2 * BLK), f32),
        vm((NG, BLK, 128), u32),
        vm((NQT, D // 2, NQ), u32),
        vm((NG, S // 2, 128), u32),
        vm((NC, D // 2, MK), u32),
        vm((NG, S // 2, 128), u32),
        vm((64, NQ), u32),
        pltpu.SemaphoreType.DMA((N_SEM,)),
    ] + [vm((2 * MK, NQ), f32)] * NC + [
        vm((256, BLK), f32), vm((2 * kshape[0], BLK), kdt), vm((2 * vshape[0], BLK), vdt)] * NG
    out = pl.pallas_call(
        _kernel,
        out_shape=jax.ShapeDtypeStruct((S, D), bf16),
        in_specs=[pl.BlockSpec(memory_space=pl.ANY)] * 5,
        out_specs=pl.BlockSpec(memory_space=pl.ANY),
        scratch_shapes=scratch,
        compiler_params=pltpu.CompilerParams(
            vmem_limit_bytes=110 * 1024 * 1024, disable_bounds_checks=NOBC),
        name="interleave_attn",
    )(x, A_wqkv, A_wo, B_wqkv, B_wo)
    return out.reshape(1, S, D)
```

```python
import jax
import jax.numpy as jnp
from jax import lax
import jax.experimental.pallas as pl
import jax.experimental.pallas.tpu as pltpu

S, D, H, DH = 2048, 1024, 32, 32
W_LOC, DIL = 8, 2
EPS = 1e-5
LOG2E = 1.4426950408889634
QSCALE = (DH ** -0.5) * LOG2E
NEG = -1e9 * LOG2E

BLK = 128
NB = S // BLK
NG = D // 128
NQ = 256
NQT = S // NQ
MK = 128
NC = S // MK
DL = 6
APB = 2
GPB = 4
TB = 256
TF = 256

SEM_X01, SEM_X2, SEM_WOB, SEM_OUT = 0, 1, 2, 3
SEM_WA = 4
SEM_IT = SEM_WA + NG
N_SEM = SEM_IT + 4

PACK_K = True
GM = 128
PACK_V = True
UCH = 4
ONLY_A = False
ONLY_B = False
LATEFLUSH = True
PVFIRST = False
MIDWAIT = False
NOBC = False
OPB = 2
S4N = 2
LNORD = 0
XBASE = True
WKSLOT = 5
LSKEW = 1
L1S = (0, 0, 1, 1, 2, 2, 3, 3)
L2S = (4, 5, 6, 7, 8, 8, 8, 8)
RSMODE = 0
NOTOK = False
SKIP1 = False
SKIP2 = False
TOKMODE = 1
WBSLOT = 4
LOCAL_OFF = False
LNMODE = 0
KLAG = 0
VLAG = 0
PROFILE_SCOPES = False

bf16 = jnp.bfloat16
f32 = jnp.float32
u32 = jnp.uint32
NT = (((1,), (1,)), ((), ()))


class _NoScope:
    def __enter__(self):
        return self

    def __exit__(self, *a):
        return False


def _scope(name):
    return jax.named_scope(name) if PROFILE_SCOPES else _NoScope()


def _pack(x):
    return pltpu.bitcast(x.astype(bf16), u32)


def _as_bf16(x):
    return pltpu.bitcast(x, bf16)


def _dot(a, b):
    return jnp.dot(a, b, preferred_element_type=f32)


def _dot_nt(a, b):
    return lax.dot_general(a, b, NT, preferred_element_type=f32)


def _layernorm_packed(x):
    outs = []
    for r in range(x.shape[0] // 16):
        xr = x[r * 16:(r + 1) * 16]
        mu = jnp.sum(xr, axis=1, keepdims=True) * (1.0 / D)
        xc = xr - mu
        var = jnp.sum(xc * xc, axis=1, keepdims=True) * (1.0 / D)
        outs.append(_pack(xc * lax.rsqrt(var + EPS)))
    return jnp.concatenate(outs, axis=0)


def _token(v):
    t = pltpu.bitcast(v[0:8, :], u32)
    return lax.shift_right_logical(jnp.bitwise_and(t, jnp.uint32(0xFFFF)), jnp.uint32(16))


def _after(x, tok):
    n, m = x.shape
    z = jnp.concatenate([jnp.concatenate([tok] * (m // 128), axis=1)] * (n // 8), axis=0)
    return pltpu.bitcast(jnp.bitwise_or(pltpu.bitcast(x, u32), z), x.dtype)


def _rowsum(x):
    if RSMODE == 1:
        t = x[:, 0:128]
        parts = [x[:, k * 128:(k + 1) * 128] for k in range(x.shape[1] // 128)]
        while len(parts) > 1:
            parts = [a + b for a, b in zip(parts[0::2], parts[1::2])]
        return jnp.sum(parts[0], axis=1, keepdims=True)
    return jnp.sum(x, axis=1, keepdims=True)


def _ln16(xr):
    if LNMODE == 1:
        return _pack(xr)
    if LNMODE == 2:
        mu = _rowsum(xr) * (1.0 / D)
        ms = _rowsum(xr * xr) * (1.0 / D)
        rs = lax.rsqrt(ms - mu * mu + EPS)
        return _pack(xr * rs - mu * rs)
    if LNMODE == 3:
        mu = _rowsum(xr) * (1.0 / D)
        xc = xr - mu
        var = _rowsum(xc * xc) * (1.0 / D)
        return _pack(xc * (var + EPS))
    if LNMODE == 4:
        mu = _rowsum(xr) * (1.0 / D)
        return _pack(xr - mu)
    mu = _rowsum(xr) * (1.0 / D)
    xc = xr - mu
    var = _rowsum(xc * xc) * (1.0 / D)
    return _pack(xc * lax.rsqrt(var + EPS))


def _tree(x, op):
    n = x.shape[0]
    while n > 1:
        n //= 2
        x = op(x[:n], x[n:])
    return x[0]


def _local_attention(q, kc, kp, vc, vp, pos):
    def chunk(x, u, tok):
        if callable(x):
            return x(u)
        n = UCH * (4 if x.dtype == u32 else 8)
        x = x[u * n:(u + 1) * n]
        return x if tok is None else _after(x, tok)

    def shifted(cur, prev, w):
        x = cur
        if w:
            lane = lax.broadcasted_iota(jnp.int32, x.shape, 1)
            x = jnp.where(lane >= 128 - DIL * w, prev, x)
            x = pltpu.roll(x, DIL * w, axis=1)
        if x.dtype == u32:
            x = _as_bf16(x).astype(f32)
        return x.reshape(UCH, 8, 128)

    nu = 16 // UCH
    if LOCAL_OFF:
        return jnp.concatenate([chunk(q, u, None) for u in range(nu)], axis=0)
    even = lax.broadcasted_iota(jnp.int32, (8, 128), 0) % 2 == 0
    acc = [None] * W_LOC
    done = []
    for u in range(nu):
        tok = _token(done[u - KLAG]) if KLAG and u >= KLAG else None
        cur, prev = chunk(kc, u, tok), chunk(kp, u, None)
        qu = chunk(q, u, None).reshape(UCH, 8, 128)
        for w in range(W_LOC):
            t = _tree(qu * shifted(cur, prev, w), jnp.add)
            acc[w] = t if acc[w] is None else acc[w] + t
        done.append(acc[W_LOC - 1])
    logits = []
    for w in range(W_LOC):
        t = acc[w]
        t = t + jnp.where(even, pltpu.roll(t, 7, axis=0), pltpu.roll(t, 1, axis=0))
        t = t * QSCALE
        if w:
            t = jnp.where(pos >= DIL * w, t, NEG)
        logits.append(t)
    m = logits[0]
    for t in logits[1:]:
        m = jnp.maximum(m, t)
    ps = [jnp.exp2(t - m) for t in logits]
    l = ps[0]
    for p in ps[1:]:
        l = l + p
    r = 1.0 / l
    ps = [(p * r)[None] for p in ps]
    outs = []
    for u in range(nu):
        tok = None
        if VLAG:
            tok = _token(outs[u - VLAG] if u >= VLAG else done[nu - VLAG + u])
        cur, prev = chunk(vc, u, tok), chunk(vp, u, None)
        o = None
        for w in range(W_LOC):
            t = shifted(cur, prev, w) * ps[w]
            o = t if o is None else o + t
        outs.append(o.reshape(UCH * 8, 128))
    return jnp.concatenate(outs, axis=0)


def _kernel(x_hbm, wa_hbm, woa_hbm, wb_hbm, wob_hbm, out_hbm,
            x_ref, xio, xn1a, xn1b, xn2, wa_nat, wat, woa, woap, wb_nat, wbt, wk, wkp, wob, wobp,
            khalo, vhalo, wstage, pxn, pbuf, po,
            qT, kN, vT, oN, otbuf,
            sem, *bufs):
    xn1 = (xn1a, xn1b)
    sbufs = bufs[:NC]
    stg = [bufs[NC + 3 * g:NC + 3 * g + 3] for g in range(NG)]

    def x_copy(i, sid):
        rows = pl.ds(i * BLK, BLK)
        return pltpu.make_async_copy(x_hbm.at[rows, :], xio.at[rows, :], sem.at[sid])

    def wa_copies(g):
        return [pltpu.make_async_copy(
            wa_hbm.at[:, pl.ds(pl.multiple_of(sec * D + g * 128, 128), 128)],
            wa_nat.at[g * 3 + sec], sem.at[SEM_WA + g]) for sec in range(3)]

    def wb_copy(c, sid):
        col = c * 128 + (c // 8) * D
        return pltpu.make_async_copy(
            wb_hbm.at[:, pl.ds(col, 128)], wb_nat.at[c], sem.at[sid])

    def wk_copy(c, sid):
        rows = pl.ds(c * 128, 128)
        return pltpu.make_async_copy(
            wb_hbm.at[rows, pl.ds(D, D)], wk.at[rows, :], sem.at[sid])

    def iter_copies(it):
        sid = SEM_IT + min(it, 3)
        if it == 0:
            cps = [pltpu.make_async_copy(woa_hbm, woa, sem.at[sid])]
        else:
            cps = [x_copy(i, sid) for i in (2 * it + 1, 2 * it + 2) if i < NB]
        return cps + [wb_copy(2 * it, sid), wb_copy(2 * it + 1, sid), wk_copy(it, sid)]

    x01_copies = [x_copy(0, SEM_X01), x_copy(1, SEM_X01)]
    x2_copy = x_copy(2, SEM_X2)
    wob_copy = pltpu.make_async_copy(wob_hbm, wob, sem.at[SEM_WOB])

    def out_copy(j):
        rows = pl.ds(pl.multiple_of(j * TF, TF), TF)
        return pltpu.make_async_copy(xio.at[rows, :], out_hbm.at[rows, :], sem.at[SEM_OUT])

    def blk_rows(i, n=BLK):
        return pl.ds(pl.multiple_of(i * n, n), n)

    def qkv_group(g, xn):
        w = jnp.concatenate([wat[g, kt] for kt in range(NG)], axis=1)
        r = jnp.concatenate(
            [_dot_nt(_as_bf16(w[a:a + GM // 2]), xn) for a in range(0, 192, GM // 2)], axis=0)
        k = r[128:256]
        v = r[256:384]
        return r[0:128], _pack(k) if PACK_K else k, _pack(v) if PACK_V else v

    def o_rows(i, n):
        rows = blk_rows(i, n // 2)
        return _as_bf16(jnp.concatenate([oN[t, rows, :] for t in range(NG)], axis=1))

    def proj_residual(o, w_cols, xv, ns=2):
        cols = []
        w = D // ns
        for n in range(ns):
            cols.append(xv[:, n * w:(n + 1) * w] + _dot(o, w_cols(n, ns)))
        return jnp.concatenate(cols, axis=1)

    def packed_cols(w_ref):
        return lambda n, ns=2: _as_bf16(jnp.concatenate(
            [w_ref[NG // ns * n + t] for t in range(NG // ns)], axis=1))

    woa_cols, wob_cols, wk_cols = packed_cols(woap), packed_cols(wobp), packed_cols(wkp)

    def repack(dst_ref, src_ref, c, n, tok=None):
        wv = pltpu.bitcast(src_ref[blk_rows(c, n), :], u32)
        if tok is not None:
            wv = _after(wv, tok)
        for t in range(NG):
            dst_ref[t, blk_rows(c, n // 2), :] = wv[:, t * 128:(t + 1) * 128]

    def store_permuted(dst_ref, row0, val):
        for h in range(4):
            dst_ref[pl.ds(row0 + h, 16, stride=4), :] = val[h * 16:(h + 1) * 16]

    def rows16(blk, r):
        return pl.ds(pl.multiple_of(blk * BLK + r * 16, 16), 16)

    def ln1(blk, r, tok=None):
        rows = rows16(blk, r)
        xv = xio[rows, :].astype(f32)
        if SKIP1:
            return _pack(xv)
        if tok is not None and not NOTOK:
            xv = _after(xv, tok)
        if not XBASE:
            x_ref[rows, :] = xv
        return _ln16(xv)

    def ln2(blk, r, tok=None):
        if SKIP2:
            return
        xv = x_ref[rows16(blk, r), :]
        if tok is not None and not NOTOK:
            xv = _after(xv, tok)
        xn2[pl.ds(pl.multiple_of(blk * (BLK // 2) + r * 8, 8), 8), :] = _ln16(xv)

    def head_group0(xn_packed):
        for ref, val in zip(stg[0], qkv_group(0, _as_bf16(xn_packed))):
            ref[0:val.shape[0], :] = val

    def a_block(i, par, z0, z1):
        def xn_cur():
            if LSKEW == 1:
                return _as_bf16(xn1[par][...])
            return _as_bf16(xn1[par][pl.ds(pl.multiple_of(z1, 8), BLK // 2), :])

        ip = jnp.maximum(i - 1, 0)
        inx = jnp.minimum(i + LSKEW, NB - 1)
        dst = xn1[(par + LSKEW) % 2]
        pos = i * BLK + lax.broadcasted_iota(jnp.int32, (8, 128), 1)

        def stage(g, slot, qkv):
            for ref, val in zip(stg[g], qkv):
                n = val.shape[0]
                ref[pl.ds(pl.multiple_of(z0 + slot * n, 8), n), :] = val

        def getter(ref, slot):
            n = ref.shape[0] // 2
            m = n // (16 // UCH)
            return lambda u: ref[pl.ds(pl.multiple_of(z1 + slot * n + u * m, 8), m), :]

        def ln_jobs(slot, tok):
            for r in range(8):
                if L1S[r] == slot:
                    dst[pl.ds(pl.multiple_of(z0 + r * 8, 8), 8), :] = ln1(inx, r, tok)
            for r in range(8):
                if L2S[r] == slot:
                    ln2(ip, r, tok)

        o_cols = []
        for g in range(NG):
            if g:
                qkv = qkv_group(g, xn_cur())
                stage(g, par, qkv)
            qs, ks, vs = stg[g]
            ot = _local_attention(getter(qs, par), getter(ks, par), getter(ks, 1 - par),
                                  getter(vs, par), getter(vs, 1 - par), pos)
            o_cols.append(ot.astype(bf16).T)
            if TOKMODE == 0:
                tok = _token(qkv[1]) if g else None
                slot = g - 1
            else:
                tok = _token(ot[120:128])
                slot = g
            ln_jobs(slot, tok)
            if slot == WBSLOT:
                wsrc = _as_bf16(_after(pltpu.bitcast(wb_nat[i], u32), tok))
                wbt[i] = pltpu.bitcast(wsrc.T, u32)
            if slot == WKSLOT:
                repack(wkp, wk, i, 64, tok)
        xn_next = xn1[1 - par][pl.ds(pl.multiple_of(z1, 8), BLK // 2), :]
        qkv = qkv_group(0, _as_bf16(xn_next))
        stage(0, 1 - par, qkv)
        ln_jobs(7 + TOKMODE, _token(qkv[1]))
        o = jnp.concatenate(o_cols, axis=1)
        rows = blk_rows(i)
        base = xio[rows, :].astype(f32) if XBASE else x_ref[rows, :]
        xv = proj_residual(o, woa_cols, base, S4N)
        x_ref[rows, :] = xv
        for k in range(4):
            ln_jobs(9 + k, _token(xv[0:8, k * 256:k * 256 + 128]))

    def startup():
        def transpose_wa(g):
            for sec in range(3):
                wv = pltpu.bitcast(wa_nat[g * 3 + sec].T, u32)
                for kt in range(NG):
                    store_permuted(wstage.at[kt], sec * 64, wv[:, kt * 128:(kt + 1) * 128])

        def project(g):
            w = wstage[...]
            wat[g] = w
            w = jnp.concatenate([w[kt] for kt in range(NG)], axis=1)
            return _dot_nt(_as_bf16(w), _as_bf16(pxn[...]))

        def attend(g, r):
            pos = lax.broadcasted_iota(jnp.int32, (8, 128), 1)
            kp = jnp.zeros(khalo.shape[1:], khalo.dtype)
            vp = jnp.zeros(vhalo.shape[1:], vhalo.dtype)
            for b in range(2):
                rb = r[:, b * BLK:(b + 1) * BLK]
                kc = _pack(rb[128:256]) if PACK_K else rb[128:256]
                vc = _pack(rb[256:384]) if PACK_V else rb[256:384]
                ot = _local_attention(rb[0:128], kc, kp, vc, vp, pos + b * BLK)
                po[g, b * 64:(b + 1) * 64, :] = pltpu.bitcast(ot.astype(bf16).T, u32)
                kp, vp = kc, vc
            khalo[g] = kp
            vhalo[g] = vp

        pbuf[...] = jnp.zeros(pbuf.shape, f32)

        def zero_scores(k, c):
            for sb in sbufs:
                sb[blk_rows(k, 32), :] = jnp.zeros((32, NQ), f32)
            return c
        lax.fori_loop(0, 2 * MK // 32, zero_scores, 0)
        for cp in x01_copies:
            cp.wait()
        for b in range(2):
            for r in range(BLK // 16):
                pxn[b * 64 + r * 8:b * 64 + (r + 1) * 8, :] = ln1(b, r)
        for cp in wa_copies(0):
            cp.wait()
        transpose_wa(0)

        def body(g, c):
            if not MIDWAIT:
                for cp in wa_copies(g + 1):
                    cp.wait()
            prev = pbuf[...]
            r = project(g)
            if MIDWAIT:
                attend(jnp.maximum(g - 1, 0), prev)
                for cp in wa_copies(g + 1):
                    cp.wait()
            transpose_wa(g + 1)
            pbuf[...] = r
            if not MIDWAIT:
                attend(jnp.maximum(g - 1, 0), prev)
            return c
        lax.fori_loop(0, NG - 1, body, 0)

        x2_copy.wait()
        prev = pbuf[...]
        r = project(NG - 1)
        xn_next = jnp.concatenate([ln1(2, r16) for r16 in range(BLK // 16)], axis=0)
        xn1[0][...] = xn_next
        attend(NG - 2, _after(prev, _token(xn_next[56:64, 0:128])))
        head_group0(xn_next)
        attend(NG - 1, r)

        for cp in iter_copies(0):
            cp.wait()
        for t in range(NG):
            wv = pltpu.bitcast(woa[:, t * 128:(t + 1) * 128], u32)
            for g in range(NG):
                store_permuted(woap.at[t], g * 64, wv[g * 64:(g + 1) * 64])
        for b in range(2):
            o = jnp.concatenate([po[g, b * 64:(b + 1) * 64, :] for g in range(NG)], axis=1)
            rows = blk_rows(b)
            base = xio[rows, :].astype(f32) if XBASE else x_ref[rows, :]
            x_ref[rows, :] = proj_residual(_as_bf16(o), woa_cols, base)
            wbt[b] = pltpu.bitcast(wb_nat[b].T, u32)
        repack(wkp, wk, 0, 128)
        for r16 in range(BLK // 16):
            ln2(0, r16)
        for g in range(NG):
            for ref, src in ((stg[g][1], khalo), (stg[g][2], vhalo)):
                n = src.shape[1]
                ref[n:2 * n, :] = src[g]
        for cp in iter_copies(1):
            cp.wait()

    def phase_a(rep):
        @pl.when(rep == 1)
        def _():
            for g in range(NG):
                for ref in stg[g][1:]:
                    n = ref.shape[0] // 2
                    ref[n:2 * n, :] = jnp.zeros((n, BLK), ref.dtype)
            xn_first = jnp.concatenate([ln1(0, r) for r in range(BLK // 16)], axis=0)
            xn1[0][...] = xn_first
            head_group0(xn_first)

        def body(it, c):
            @pl.when(it == 2 - rep * NB)
            def _():
                for cp in iter_copies(2):
                    cp.wait()

            @pl.when(it == 3 - rep * NB)
            def _():
                for k in range(3, NB // APB):
                    for cp in iter_copies(k):
                        cp.wait()

            z0 = lax.shift_right_logical(it, 16) * 8
            z1 = lax.shift_right_logical(it, 17) * 8
            with _scope("a_iter"):
                for u in range(APB):
                    a_block(it * APB + u, u % 2, z0, z1)
            return c
        with _scope("a_loop"):
            lax.fori_loop(1 - rep, NB // APB, body, 0)
        for r in range(BLK // 16):
            ln2(NB - 1, r)

    def phase_b_proj():
        def body(j, c):
            rows = blk_rows(j, TB // 2)
            xn = _as_bf16(xn2[rows, :])
            for n in range(2):
                y = _pack(_dot(xn, wk_cols(n)))
                for t in range(4):
                    kN[4 * n + t, rows, :] = y[:, t * 128:(t + 1) * 128]
            for r in range(4):
                w = _as_bf16(wbt[2 * r:2 * r + 2].reshape(128, D))
                y = _pack(_dot_nt(w, xn) * QSCALE)
                for b in range(TB // NQ):
                    qT[j * (TB // NQ) + b, r * 128:(r + 1) * 128, :] = y[:, b * NQ:(b + 1) * NQ]
            for r in range(4):
                w = _as_bf16(wbt[8 + 2 * r:8 + 2 * r + 2].reshape(128, D))
                y = _pack(_dot_nt(w, xn))
                for b in range(TB // MK):
                    vT[j * (TB // MK) + b, r * 128:(r + 1) * 128, :] = y[:, b * MK:(b + 1) * MK]
            return c
        lax.fori_loop(0, S // TB, body, 0)

    def flush_o(g, val):
        y = pltpu.bitcast(_as_bf16(val).T, u32)
        oN[g % NG, blk_rows(g // NG, NQ // 2), :] = y

    def phase_b_attn():
        off = [0, 0]

        def qm_of(t, qi, j):
            q = _as_bf16(qT[qi, pl.ds(pl.multiple_of(t * 64 + j * 16, 16), 16), :])
            parts = []
            if j > 0:
                parts.append(jnp.zeros((32 * j, NQ), bf16))
            parts.append(q)
            if j < 3:
                parts.append(jnp.zeros((32 * (3 - j), NQ), bf16))
            return jnp.concatenate(parts, axis=0)

        def qk_chunk(t, qm, c, par, m):
            k = _as_bf16(kN[t, c * (MK // 2):(c + 1) * (MK // 2), :])
            s = _dot(k, qm)
            sbufs[c][pl.ds(pl.multiple_of(off[0] + par * MK, 8), MK), :] = s
            sm = _tree(s.reshape(MK // 8, 8, NQ), jnp.maximum)
            return sm if m is None else jnp.maximum(m, sm)

        def pv_chunk(h, c, par, mrow, l, o):
            s = sbufs[c][pl.ds(pl.multiple_of(off[1] + par * MK, 8), MK), :]
            p = jnp.exp2(s - mrow)
            ls = jnp.sum(p.reshape(MK // 8, 8, NQ), axis=0)
            l = ls if l is None else l + ls
            v = _as_bf16(vT[c, pl.ds(pl.multiple_of(h * 16, 16), 16), :])
            oc = _dot(v, p.astype(bf16))
            o = oc if o is None else o + oc
            return l, o

        n_groups = NQT * NG
        lag = NC + DL
        n_steps = 4 * NC

        def set_offsets(zero):
            off[0] = lax.shift_right_logical(zero, 16) * 8
            off[1] = lax.shift_right_logical(zero, 17) * 8

        def pv_step(g, n, ms, st, flush=True):
            j, c = divmod(n, NC)
            l, o, mrow = st
            if c == 0:
                mrow = jnp.max(ms[j], axis=0, keepdims=True)
                l = o = None
            l, o = pv_chunk((g % NG) * 4 + j, c, j % 2, mrow, l, o)
            if c == NC - 1:
                lrow = jnp.sum(l, axis=0, keepdims=True)
                otbuf[j * 16:(j + 1) * 16, :] = _pack(o * (1.0 / lrow))
                if j == 3 and flush:
                    flush_o(g, otbuf[...])
            return l, o, mrow

        def group(g, g_prev, carry, side_job=None):
            st, ms_prev = carry[:3], {3: carry[3]}
            ms = {}
            for n in range(n_steps):
                j, c = divmod(n, NC)
                if c == 0:
                    qm = qm_of(g % NG, g // NG, j)
                if not PVFIRST:
                    ms[j] = qk_chunk(g % NG, qm, c, j % 2, ms.get(j))
                if n < lag:
                    st = pv_step(g_prev, n + n_steps - lag, ms_prev, st)
                else:
                    st = pv_step(g, n - lag, ms, st)
                if PVFIRST:
                    ms[j] = qk_chunk(g % NG, qm, c, j % 2, ms.get(j))
                if side_job is not None and n == n_steps // 2:
                    side_job(_token(st[0][:, 0:128]))
            return st + (ms[3],)

        def body(it, carry):
            def side_job(tok):
                repack(wobp, wob, it, D * GPB // n_groups, tok)

            set_offsets(it)
            carry = carry[:4]
            for u in range(GPB):
                g = it * GPB + u
                carry = group(g, jnp.maximum(g - 1, 0), carry, side_job if u == 0 else None)
            return carry + (it,)

        otbuf[...] = jnp.zeros(otbuf.shape, u32)
        init = (jnp.zeros((8, NQ), f32), jnp.zeros((DH, NQ), f32),
                jnp.zeros((1, NQ), f32), jnp.zeros((8, NQ), f32), jnp.int32(0))
        carry = lax.fori_loop(0, n_groups // GPB, body, init)
        set_offsets(carry[4])
        st, ms = carry[:3], {3: carry[3]}
        for n in range(n_steps - lag, n_steps):
            st = pv_step(n_groups - 1, n, ms, st, not LATEFLUSH)
        off[0] = off[1] = 0

    def phase_b_out(rep):
        def body(jj, c):
            for u in range(OPB):
                j = jj * OPB + u
                rows = blk_rows(j, TF)
                xv = proj_residual(o_rows(j, TF), wob_cols, x_ref[rows, :])
                xio[rows, :] = xv.astype(bf16)

                @pl.when(rep == 1)
                def _():
                    out_copy(j).start()
            if LATEFLUSH:
                flush_o(NQT * NG - 1, otbuf[...])
            return c
        lax.fori_loop(0, S // (TF * OPB), body, 0)

    def sem_dummy():
        return lax.fori_loop(0, 3, lambda i, c: c + i, 0)

    if ONLY_B:
        phase_b_attn()
        xio[0:8, :] = jnp.concatenate([_as_bf16(oN[0, 0:4, :]) + _as_bf16(wobp[0, 0:4, :])] * 8, axis=1)
        return
    if ONLY_A:
        phase_a(lax.shift_right_logical(sem_dummy(), 1))
        xio[0:8, :] = (_as_bf16(wbt[0, 0:4, :]) + _as_bf16(xn2[0:4, :])
                       + jnp.concatenate([_as_bf16(wkp[0, 0:4, :])] * 8, axis=1))
        return

    for cp in x01_copies:
        cp.start()
    for g in range(NG):
        if g == NG - 2:
            x2_copy.start()
        for cp in wa_copies(g):
            cp.start()
    for it in range(NB // APB):
        for cp in iter_copies(it):
            cp.start()
    wob_copy.start()

    with _scope("startup"):
        startup()

    def layer_pair(rep, c):
        with _scope("phase_a"):
            phase_a(rep)

        @pl.when(rep == 0)
        def _():
            wob_copy.wait()

        with _scope("b_proj"):
            phase_b_proj()
        with _scope("b_attn"):
            phase_b_attn()
        with _scope("b_out"):
            phase_b_out(rep)
        return c
    lax.fori_loop(0, 2, layer_pair, 0)
    for j in range(S // TF):
        out_copy(j).wait()


@jax.jit
def pallas_interleave_layers__sliding_local_dilated__softmax_full_mha__prompt_kernel(
    A_x: jax.Array,
    A_wqkv: jax.Array,
    A_wo: jax.Array,
    B_x: jax.Array,
    B_wqkv: jax.Array,
    B_wo: jax.Array,
):
    del B_x
    x = A_x.reshape(S, D)
    vm = pltpu.VMEM
    kshape, kdt = ((64, BLK), u32) if PACK_K else ((128, BLK), f32)
    vshape, vdt = ((64, BLK), u32) if PACK_V else ((128, BLK), f32)
    scratch = [
        vm((S, D), f32),
        vm((S, D), bf16),
        vm((BLK // 2, D), u32),
        vm((BLK // 2, D), u32),
        vm((S // 2, D), u32),
        vm((3 * NG, D, 128), bf16),
        vm((NG, NG, 192, 128), u32),
        vm((D, D), bf16),
        vm((NG, D // 2, 128), u32),
        vm((2 * NG, D, 128), bf16),
        vm((2 * NG, 64, D), u32),
        vm((D, D), bf16),
        vm((NG, D // 2, 128), u32),
        vm((D, D), bf16),
        vm((NG, D // 2, 128), u32),
        vm((NG,) + kshape, kdt),
        vm((NG,) + vshape, vdt),
        vm((NG, 192, 128), u32),
        vm((BLK, D), u32),
        vm((384, 2 * BLK), f32),
        vm((NG, BLK, 128), u32),
        vm((NQT, D // 2, NQ), u32),
        vm((NG, S // 2, 128), u32),
        vm((NC, D // 2, MK), u32),
        vm((NG, S // 2, 128), u32),
        vm((64, NQ), u32),
        pltpu.SemaphoreType.DMA((N_SEM,)),
    ] + [vm((2 * MK, NQ), f32)] * NC + [
        vm((256, BLK), f32), vm((2 * kshape[0], BLK), kdt), vm((2 * vshape[0], BLK), vdt)] * NG
    out = pl.pallas_call(
        _kernel,
        out_shape=jax.ShapeDtypeStruct((S, D), bf16),
        in_specs=[pl.BlockSpec(memory_space=pl.ANY)] * 5,
        out_specs=pl.BlockSpec(memory_space=pl.ANY),
        scratch_shapes=scratch,
        compiler_params=pltpu.CompilerParams(
            vmem_limit_bytes=110 * 1024 * 1024, disable_bounds_checks=NOBC),
        name="interleave_attn",
    )(x, A_wqkv, A_wo, B_wqkv, B_wo)
    return out.reshape(1, S, D)
```

```python
import jax
import jax.numpy as jnp
from jax import lax
import jax.experimental.pallas as pl
import jax.experimental.pallas.tpu as pltpu

S, D, H, DH = 2048, 1024, 32, 32
W_LOC, DIL = 8, 2
EPS = 1e-5
LOG2E = 1.4426950408889634
QSCALE = (DH ** -0.5) * LOG2E
NEG = -1e9 * LOG2E

BLK = 128
NB = S // BLK
NG = D // 128
NQ = 256
NQT = S // NQ
MK = 128
NC = S // MK
DL = 6
APB = 2
GPB = 4
TB = 256
TF = 256
OPB = 2

SEM_X01, SEM_X2, SEM_WOB, SEM_OUT = 0, 1, 2, 3
SEM_WA = 4
SEM_IT = SEM_WA + NG
N_SEM = SEM_IT + 4

UCH = 2
L1S = (0, 0, 1, 1, 2, 2, 3, 4)
L2S = (5, 5, 5, 5, 6, 7, 7, 8)
WBSLOT = 1
WKSLOT = 6

ONLY = None
PROFILE_SCOPES = False

bf16 = jnp.bfloat16
f32 = jnp.float32
u32 = jnp.uint32
NT = (((1,), (1,)), ((), ()))


class _NoScope:
    def __enter__(self):
        return self

    def __exit__(self, *a):
        return False


def _scope(name):
    return jax.named_scope(name) if PROFILE_SCOPES else _NoScope()


def _pack(x):
    return pltpu.bitcast(x.astype(bf16), u32)


def _as_bf16(x):
    return pltpu.bitcast(x, bf16)


def _dot(a, b):
    return jnp.dot(a, b, preferred_element_type=f32)


def _dot_nt(a, b):
    return lax.dot_general(a, b, NT, preferred_element_type=f32)


def _token(v):
    t = pltpu.bitcast(v[0:8, :], u32)
    return lax.shift_right_logical(jnp.bitwise_and(t, jnp.uint32(0xFFFF)), jnp.uint32(16))


def _after(x, tok):
    n, m = x.shape
    z = jnp.concatenate([jnp.concatenate([tok] * (m // 128), axis=1)] * (n // 8), axis=0)
    return pltpu.bitcast(jnp.bitwise_or(pltpu.bitcast(x, u32), z), x.dtype)


def _ln16(x):
    mu = jnp.sum(x, axis=1, keepdims=True) * (1.0 / D)
    xc = x - mu
    var = jnp.sum(xc * xc, axis=1, keepdims=True) * (1.0 / D)
    return _pack(xc * lax.rsqrt(var + EPS))


def _tree(x, op):
    n = x.shape[0]
    while n > 1:
        n //= 2
        x = op(x[:n], x[n:])
    return x[0]


def _local_attention(q, kc, kp, vc, vp, pos):
    lane = lax.broadcasted_iota(jnp.int32, (UCH * 4, 128), 1)

    def shifted(cur, prev, u, w):
        rows = slice(u * UCH * 4, (u + 1) * UCH * 4)
        x = cur[rows]
        if w:
            x = jnp.where(lane >= 128 - DIL * w, prev[rows], x)
            x = pltpu.roll(x, DIL * w, axis=1)
        return _as_bf16(x).astype(f32).reshape(UCH, 8, 128)

    nu = 16 // UCH
    even = lax.broadcasted_iota(jnp.int32, (8, 128), 0) % 2 == 0
    acc = [None] * W_LOC
    for u in range(nu):
        qu = q[u * UCH * 8:(u + 1) * UCH * 8].reshape(UCH, 8, 128)
        for w in range(W_LOC):
            t = _tree(qu * shifted(kc, kp, u, w), jnp.add)
            acc[w] = t if acc[w] is None else acc[w] + t
    logits = []
    for w in range(W_LOC):
        t = acc[w]
        t = t + jnp.where(even, pltpu.roll(t, 7, axis=0), pltpu.roll(t, 1, axis=0))
        t = t * QSCALE
        if w:
            t = jnp.where(pos >= DIL * w, t, NEG)
        logits.append(t)
    m = logits[0]
    for t in logits[1:]:
        m = jnp.maximum(m, t)
    ps = [jnp.exp2(t - m) for t in logits]
    l = ps[0]
    for p in ps[1:]:
        l = l + p
    r = 1.0 / l
    ps = [(p * r)[None] for p in ps]
    outs = []
    for u in range(nu):
        o = None
        for w in range(W_LOC):
            t = shifted(vc, vp, u, w) * ps[w]
            o = t if o is None else o + t
        outs.append(o.reshape(UCH * 8, 128))
    return jnp.concatenate(outs, axis=0)


def _kernel(x_hbm, wa_hbm, woa_hbm, wb_hbm, wob_hbm, out_hbm,
            x_ref, xio, xn1a, xn1b, xn2, wa_nat, wat, woa, woap, wb_nat, wbt, wk, wkp, wob, wobp,
            khalo, vhalo, wstage, pxn, pbuf, po,
            qT, kN, vT, oN, otbuf,
            sem, *bufs):
    xn1 = (xn1a, xn1b)
    sbufs = bufs[:NC]
    stg = [bufs[NC + 3 * g:NC + 3 * g + 3] for g in range(NG)]

    def x_copy(i, sid):
        rows = pl.ds(i * BLK, BLK)
        return pltpu.make_async_copy(x_hbm.at[rows, :], xio.at[rows, :], sem.at[sid])

    def wa_copies(g):
        return [pltpu.make_async_copy(
            wa_hbm.at[:, pl.ds(pl.multiple_of(sec * D + g * 128, 128), 128)],
            wa_nat.at[g * 3 + sec], sem.at[SEM_WA + g]) for sec in range(3)]

    def wb_copy(c, sid):
        col = c * 128 + (c // 8) * D
        return pltpu.make_async_copy(
            wb_hbm.at[:, pl.ds(col, 128)], wb_nat.at[c], sem.at[sid])

    def wk_copy(c, sid):
        rows = pl.ds(c * 128, 128)
        return pltpu.make_async_copy(
            wb_hbm.at[rows, pl.ds(D, D)], wk.at[rows, :], sem.at[sid])

    def iter_copies(it):
        sid = SEM_IT + min(it, 3)
        if it == 0:
            cps = [pltpu.make_async_copy(woa_hbm, woa, sem.at[sid])]
        else:
            cps = [x_copy(i, sid) for i in (2 * it + 1, 2 * it + 2) if i < NB]
        return cps + [wb_copy(2 * it, sid), wb_copy(2 * it + 1, sid), wk_copy(it, sid)]

    x01_copies = [x_copy(0, SEM_X01), x_copy(1, SEM_X01)]
    x2_copy = x_copy(2, SEM_X2)
    wob_copy = pltpu.make_async_copy(wob_hbm, wob, sem.at[SEM_WOB])

    def out_copy(j):
        rows = pl.ds(pl.multiple_of(j * TF, TF), TF)
        return pltpu.make_async_copy(xio.at[rows, :], out_hbm.at[rows, :], sem.at[SEM_OUT])

    def blk_rows(i, n=BLK):
        return pl.ds(pl.multiple_of(i * n, n), n)

    def qkv_group(g, xn):
        w = jnp.concatenate([wat[g, kt] for kt in range(NG)], axis=1)
        q, k, v = [_dot_nt(_as_bf16(w[a:a + 64]), xn) for a in (0, 64, 128)]
        return q, _pack(k), _pack(v)

    def o_rows(i, n):
        rows = blk_rows(i, n // 2)
        return _as_bf16(jnp.concatenate([oN[t, rows, :] for t in range(NG)], axis=1))

    def proj_residual(o, w_cols, xv):
        cols = []
        for n in range(2):
            cols.append(xv[:, n * 512:(n + 1) * 512] + _dot(o, w_cols(n)))
        return jnp.concatenate(cols, axis=1)

    def packed_cols(w_ref):
        return lambda n: _as_bf16(
            jnp.concatenate([w_ref[4 * n + t] for t in range(4)], axis=1))

    woa_cols, wob_cols, wk_cols = packed_cols(woap), packed_cols(wobp), packed_cols(wkp)

    def repack(dst_ref, src_ref, c, n, tok=None):
        wv = pltpu.bitcast(src_ref[blk_rows(c, n), :], u32)
        if tok is not None:
            wv = _after(wv, tok)
        for t in range(NG):
            dst_ref[t, blk_rows(c, n // 2), :] = wv[:, t * 128:(t + 1) * 128]

    def store_permuted(dst_ref, row0, val):
        for h in range(4):
            dst_ref[pl.ds(row0 + h, 16, stride=4), :] = val[h * 16:(h + 1) * 16]

    def rows16(blk, r):
        return pl.ds(pl.multiple_of(blk * BLK + r * 16, 16), 16)

    def ln1(blk, r, tok=None):
        xv = xio[rows16(blk, r), :].astype(f32)
        return _ln16(xv if tok is None else _after(xv, tok))

    def ln2(blk, r, tok=None):
        xv = x_ref[rows16(blk, r), :]
        xn2[pl.ds(pl.multiple_of(blk * (BLK // 2) + r * 8, 8), 8), :] = _ln16(
            xv if tok is None else _after(xv, tok))

    def stage(g, slot, qkv):
        for ref, val in zip(stg[g], qkv):
            ref[slot] = val

    def a_block(i, par):
        ip = jnp.maximum(i - 1, 0)
        inx = jnp.minimum(i + 1, NB - 1)
        pos = i * BLK + lax.broadcasted_iota(jnp.int32, (8, 128), 1)

        def side_jobs(slot, src):
            if slot not in L1S + L2S + (WBSLOT, WKSLOT):
                return
            tok = _token(src)
            if slot == WBSLOT:
                wsrc = _as_bf16(_after(pltpu.bitcast(wb_nat[i], u32), tok))
                wbt[i] = pltpu.bitcast(wsrc.T, u32)
            if slot == WKSLOT:
                repack(wkp, wk, i, 64, tok)
            for r in range(8):
                if L1S[r] == slot:
                    xn1[1 - par][r * 8:(r + 1) * 8, :] = ln1(inx, r, tok)
            for r in range(8):
                if L2S[r] == slot:
                    ln2(ip, r, tok)

        o_cols = []
        for g in range(NG):
            if g:
                stage(g, par, qkv_group(g, _as_bf16(xn1[par][...])))
            qs, ks, vs = stg[g]
            ot = _local_attention(qs[par], ks[par], ks[1 - par], vs[par], vs[1 - par], pos)
            o_cols.append(ot.astype(bf16).T)
            side_jobs(g, ot[120:128])
        qkv = qkv_group(0, _as_bf16(xn1[1 - par][...]))
        stage(0, 1 - par, qkv)
        side_jobs(NG, qkv[1])
        rows = blk_rows(i)
        x_ref[rows, :] = proj_residual(
            jnp.concatenate(o_cols, axis=1), woa_cols, xio[rows, :].astype(f32))

    def startup():
        def transpose_wa(g):
            for sec in range(3):
                wv = pltpu.bitcast(wa_nat[g * 3 + sec].T, u32)
                for kt in range(NG):
                    store_permuted(wstage.at[kt], sec * 64, wv[:, kt * 128:(kt + 1) * 128])

        def project(g):
            w = wstage[...]
            wat[g] = w
            w = jnp.concatenate([w[kt] for kt in range(NG)], axis=1)
            return _dot_nt(_as_bf16(w), _as_bf16(pxn[...]))

        def attend(g, r):
            pos = lax.broadcasted_iota(jnp.int32, (8, 128), 1)
            kp = vp = jnp.zeros((64, BLK), u32)
            for b in range(2):
                rb = r[:, b * BLK:(b + 1) * BLK]
                kc = _pack(rb[128:256])
                vc = _pack(rb[256:384])
                ot = _local_attention(rb[0:128], kc, kp, vc, vp, pos + b * BLK)
                po[g, b * 64:(b + 1) * 64, :] = pltpu.bitcast(ot.astype(bf16).T, u32)
                kp, vp = kc, vc
            khalo[g] = kp
            vhalo[g] = vp

        pbuf[...] = jnp.zeros(pbuf.shape, f32)

        def zero_scores(k, c):
            for sb in sbufs:
                sb[blk_rows(k, 32), :] = jnp.zeros((32, NQ), f32)
            return c
        lax.fori_loop(0, 2 * MK // 32, zero_scores, 0)
        for cp in x01_copies:
            cp.wait()
        for b in range(2):
            for r in range(BLK // 16):
                pxn[b * 64 + r * 8:b * 64 + (r + 1) * 8, :] = ln1(b, r)
        for cp in wa_copies(0):
            cp.wait()
        transpose_wa(0)

        def body(g, c):
            for cp in wa_copies(g + 1):
                cp.wait()
            prev = pbuf[...]
            pbuf[...] = project(g)
            transpose_wa(g + 1)
            attend(jnp.maximum(g - 1, 0), prev)
            return c
        lax.fori_loop(0, NG - 1, body, 0)

        x2_copy.wait()
        prev = pbuf[...]
        r = project(NG - 1)
        xn_next = jnp.concatenate([ln1(2, r16) for r16 in range(BLK // 16)], axis=0)
        xn1[0][...] = xn_next
        attend(NG - 2, _after(prev, _token(xn_next[56:64, 0:128])))
        stage(0, 0, qkv_group(0, _as_bf16(xn_next)))
        attend(NG - 1, r)

        for cp in iter_copies(0):
            cp.wait()
        for t in range(NG):
            wv = pltpu.bitcast(woa[:, t * 128:(t + 1) * 128], u32)
            for g in range(NG):
                store_permuted(woap.at[t], g * 64, wv[g * 64:(g + 1) * 64])
        for b in range(2):
            o = jnp.concatenate([po[g, b * 64:(b + 1) * 64, :] for g in range(NG)], axis=1)
            rows = blk_rows(b)
            x_ref[rows, :] = proj_residual(_as_bf16(o), woa_cols, xio[rows, :].astype(f32))
            wbt[b] = pltpu.bitcast(wb_nat[b].T, u32)
        repack(wkp, wk, 0, 128)
        for r16 in range(BLK // 16):
            ln2(0, r16)
        for g in range(NG):
            stg[g][1][1] = khalo[g]
            stg[g][2][1] = vhalo[g]
        for cp in iter_copies(1):
            cp.wait()

    def phase_a(rep):
        @pl.when(rep == 1)
        def _():
            for g in range(NG):
                for ref in stg[g][1:]:
                    ref[1] = jnp.zeros((64, BLK), u32)
            xn_first = jnp.concatenate([ln1(0, r) for r in range(BLK // 16)], axis=0)
            xn1[0][...] = xn_first
            stage(0, 0, qkv_group(0, _as_bf16(xn_first)))

        def body(it, c):
            @pl.when(it == 2 - rep * NB)
            def _():
                for cp in iter_copies(2):
                    cp.wait()

            @pl.when(it == 3 - rep * NB)
            def _():
                for k in range(3, NB // APB):
                    for cp in iter_copies(k):
                        cp.wait()

            for u in range(APB):
                a_block(it * APB + u, u % 2)
            return c
        with _scope("a_loop"):
            lax.fori_loop(1 - rep, NB // APB, body, 0)
        for r in range(BLK // 16):
            ln2(NB - 1, r)

    def phase_b_proj():
        def body(j, c):
            rows = blk_rows(j, TB // 2)
            xn = _as_bf16(xn2[rows, :])
            for n in range(2):
                y = _pack(_dot(xn, wk_cols(n)))
                for t in range(4):
                    kN[4 * n + t, rows, :] = y[:, t * 128:(t + 1) * 128]
            for r in range(4):
                w = _as_bf16(wbt[2 * r:2 * r + 2].reshape(128, D))
                y = _pack(_dot_nt(w, xn) * QSCALE)
                for b in range(TB // NQ):
                    qT[j * (TB // NQ) + b, r * 128:(r + 1) * 128, :] = y[:, b * NQ:(b + 1) * NQ]
            for r in range(4):
                w = _as_bf16(wbt[8 + 2 * r:8 + 2 * r + 2].reshape(128, D))
                y = _pack(_dot_nt(w, xn))
                for b in range(TB // MK):
                    vT[j * (TB // MK) + b, r * 128:(r + 1) * 128, :] = y[:, b * MK:(b + 1) * MK]
            return c
        lax.fori_loop(0, S // TB, body, 0)

    def flush_o(g, val):
        y = pltpu.bitcast(_as_bf16(val).T, u32)
        oN[g % NG, blk_rows(g // NG, NQ // 2), :] = y

    def phase_b_attn():
        off = [0, 0]

        def qm_of(t, qi, j):
            q = _as_bf16(qT[qi, pl.ds(pl.multiple_of(t * 64 + j * 16, 16), 16), :])
            parts = []
            if j > 0:
                parts.append(jnp.zeros((32 * j, NQ), bf16))
            parts.append(q)
            if j < 3:
                parts.append(jnp.zeros((32 * (3 - j), NQ), bf16))
            return jnp.concatenate(parts, axis=0)

        def qk_chunk(t, qm, c, par, m):
            k = _as_bf16(kN[t, c * (MK // 2):(c + 1) * (MK // 2), :])
            s = _dot(k, qm)
            sbufs[c][pl.ds(pl.multiple_of(off[0] + par * MK, 8), MK), :] = s
            sm = _tree(s.reshape(MK // 8, 8, NQ), jnp.maximum)
            return sm if m is None else jnp.maximum(m, sm)

        def pv_chunk(h, c, par, mrow, l, o):
            s = sbufs[c][pl.ds(pl.multiple_of(off[1] + par * MK, 8), MK), :]
            p = jnp.exp2(s - mrow)
            ls = jnp.sum(p.reshape(MK // 8, 8, NQ), axis=0)
            l = ls if l is None else l + ls
            v = _as_bf16(vT[c, pl.ds(pl.multiple_of(h * 16, 16), 16), :])
            oc = _dot(v, p.astype(bf16))
            o = oc if o is None else o + oc
            return l, o

        n_groups = NQT * NG
        lag = NC + DL
        n_steps = 4 * NC

        def set_offsets(zero):
            off[0] = lax.shift_right_logical(zero, 16) * 8
            off[1] = lax.shift_right_logical(zero, 17) * 8

        def pv_step(g, n, ms, st, flush=True):
            j, c = divmod(n, NC)
            l, o, mrow = st
            if c == 0:
                mrow = jnp.max(ms[j], axis=0, keepdims=True)
                l = o = None
            l, o = pv_chunk((g % NG) * 4 + j, c, j % 2, mrow, l, o)
            if c == NC - 1:
                lrow = jnp.sum(l, axis=0, keepdims=True)
                otbuf[j * 16:(j + 1) * 16, :] = _pack(o * (1.0 / lrow))
                if j == 3 and flush:
                    flush_o(g, otbuf[...])
            return l, o, mrow

        def group(g, g_prev, carry, side_job=None):
            st, ms_prev = carry[:3], {3: carry[3]}
            ms = {}
            for n in range(n_steps):
                j, c = divmod(n, NC)
                if c == 0:
                    qm = qm_of(g % NG, g // NG, j)
                ms[j] = qk_chunk(g % NG, qm, c, j % 2, ms.get(j))
                if n < lag:
                    st = pv_step(g_prev, n + n_steps - lag, ms_prev, st)
                else:
                    st = pv_step(g, n - lag, ms, st)
                if side_job is not None and n == n_steps // 2:
                    side_job(_token(st[0][:, 0:128]))
            return st + (ms[3],)

        def body(it, carry):
            def side_job(tok):
                repack(wobp, wob, it, D * GPB // n_groups, tok)

            set_offsets(it)
            carry = carry[:4]
            for u in range(GPB):
                g = it * GPB + u
                carry = group(g, jnp.maximum(g - 1, 0), carry, side_job if u == 0 else None)
            return carry + (it,)

        otbuf[...] = jnp.zeros(otbuf.shape, u32)
        init = (jnp.zeros((8, NQ), f32), jnp.zeros((DH, NQ), f32),
                jnp.zeros((1, NQ), f32), jnp.zeros((8, NQ), f32), jnp.int32(0))
        carry = lax.fori_loop(0, n_groups // GPB, body, init)
        set_offsets(carry[4])
        st, ms = carry[:3], {3: carry[3]}
        for n in range(n_steps - lag, n_steps):
            st = pv_step(n_groups - 1, n, ms, st, False)
        off[0] = off[1] = 0

    def phase_b_out(rep):
        def body(jj, c):
            for u in range(OPB):
                j = jj * OPB + u
                rows = blk_rows(j, TF)
                xv = proj_residual(o_rows(j, TF), wob_cols, x_ref[rows, :])
                xio[rows, :] = xv.astype(bf16)

                @pl.when(rep == 1)
                def _():
                    out_copy(j).start()
            flush_o(NQT * NG - 1, otbuf[...])
            return c
        lax.fori_loop(0, S // (TF * OPB), body, 0)

    if ONLY == "A":
        phase_a(lax.fori_loop(0, 2, lambda i, c: c + i, 0))
        xio[0:8, :] = (_as_bf16(wbt[0, 0:4, :]) + _as_bf16(xn2[0:4, :])
                       + jnp.concatenate([_as_bf16(wkp[0, 0:4, :])] * 8, axis=1))
        return
    if ONLY == "B":
        phase_b_attn()
        xio[0:8, :] = jnp.concatenate(
            [_as_bf16(oN[0, 0:4, :]) + _as_bf16(wobp[0, 0:4, :])] * 8, axis=1)
        return

    for cp in x01_copies:
        cp.start()
    for g in range(NG):
        if g == NG - 2:
            x2_copy.start()
        for cp in wa_copies(g):
            cp.start()
    for it in range(NB // APB):
        for cp in iter_copies(it):
            cp.start()
    wob_copy.start()

    with _scope("startup"):
        startup()

    def layer_pair(rep, c):
        with _scope("phase_a"):
            phase_a(rep)

        @pl.when(rep == 0)
        def _():
            wob_copy.wait()

        with _scope("b_proj"):
            phase_b_proj()
        with _scope("b_attn"):
            phase_b_attn()
        with _scope("b_out"):
            phase_b_out(rep)
        return c
    lax.fori_loop(0, 2, layer_pair, 0)
    for j in range(S // TF):
        out_copy(j).wait()


@jax.jit
def pallas_interleave_layers__sliding_local_dilated__softmax_full_mha__prompt_kernel(
    A_x: jax.Array,
    A_wqkv: jax.Array,
    A_wo: jax.Array,
    B_x: jax.Array,
    B_wqkv: jax.Array,
    B_wo: jax.Array,
):
    del B_x
    x = A_x.reshape(S, D)
    vm = pltpu.VMEM
    scratch = [
        vm((S, D), f32),
        vm((S, D), bf16),
        vm((BLK // 2, D), u32),
        vm((BLK // 2, D), u32),
        vm((S // 2, D), u32),
        vm((3 * NG, D, 128), bf16),
        vm((NG, NG, 192, 128), u32),
        vm((D, D), bf16),
        vm((NG, D // 2, 128), u32),
        vm((2 * NG, D, 128), bf16),
        vm((2 * NG, 64, D), u32),
        vm((D, D), bf16),
        vm((NG, D // 2, 128), u32),
        vm((D, D), bf16),
        vm((NG, D // 2, 128), u32),
        vm((NG, 64, BLK), u32),
        vm((NG, 64, BLK), u32),
        vm((NG, 192, 128), u32),
        vm((BLK, D), u32),
        vm((384, 2 * BLK), f32),
        vm((NG, BLK, 128), u32),
        vm((NQT, D // 2, NQ), u32),
        vm((NG, S // 2, 128), u32),
        vm((NC, D // 2, MK), u32),
        vm((NG, S // 2, 128), u32),
        vm((64, NQ), u32),
        pltpu.SemaphoreType.DMA((N_SEM,)),
    ] + [vm((2 * MK, NQ), f32)] * NC + [
        vm((2, 128, BLK), f32), vm((2, 64, BLK), u32), vm((2, 64, BLK), u32)] * NG
    out = pl.pallas_call(
        _kernel,
        out_shape=jax.ShapeDtypeStruct((S, D), bf16),
        in_specs=[pl.BlockSpec(memory_space=pl.ANY)] * 5,
        out_specs=pl.BlockSpec(memory_space=pl.ANY),
        scratch_shapes=scratch,
        compiler_params=pltpu.CompilerParams(vmem_limit_bytes=110 * 1024 * 1024),
        name="interleave_attn",
    )(x, A_wqkv, A_wo, B_wqkv, B_wo)
    return out.reshape(1, S, D)
```

```python
import jax
import jax.numpy as jnp
from jax import lax
import jax.experimental.pallas as pl
import jax.experimental.pallas.tpu as pltpu

S, D, H, DH = 2048, 1024, 32, 32
W_LOC, DIL = 8, 2
EPS = 1e-5
LOG2E = 1.4426950408889634
QSCALE = (DH ** -0.5) * LOG2E
NEG = -1e9 * LOG2E

BLK = 128
NB = S // BLK
NG = D // 128
NQ = 256
NQT = S // NQ
MK = 128
NC = S // MK
DL = 6
APB = 2
GPB = 4
TB = 256
TF = 256
OPB = 2

SEM_X01, SEM_X2, SEM_WOB, SEM_OUT = 0, 1, 2, 3
SEM_WA = 4
SEM_IT = SEM_WA + NG
N_SEM = SEM_IT + 4

UCH = 2
L1S = (0, 0, 1, 1, 1, 2, 3, 4)
L2S = (4, 5, 6, 6, 7, 7, 8, 8)
WBSLOT = 6
WKSLOT = 2
PM = 192

ONLY = None
PROFILE_SCOPES = False

bf16 = jnp.bfloat16
f32 = jnp.float32
u32 = jnp.uint32
NT = (((1,), (1,)), ((), ()))


class _NoScope:
    def __enter__(self):
        return self

    def __exit__(self, *a):
        return False


def _scope(name):
    return jax.named_scope(name) if PROFILE_SCOPES else _NoScope()


def _pack(x):
    return pltpu.bitcast(x.astype(bf16), u32)


def _as_bf16(x):
    return pltpu.bitcast(x, bf16)


def _dot(a, b):
    return jnp.dot(a, b, preferred_element_type=f32)


def _dot_nt(a, b):
    return lax.dot_general(a, b, NT, preferred_element_type=f32)


def _token(v):
    t = pltpu.bitcast(v[0:8, :], u32)
    return lax.shift_right_logical(jnp.bitwise_and(t, jnp.uint32(0xFFFF)), jnp.uint32(16))


def _after(x, tok):
    n, m = x.shape
    z = jnp.concatenate([jnp.concatenate([tok] * (m // 128), axis=1)] * (n // 8), axis=0)
    return pltpu.bitcast(jnp.bitwise_or(pltpu.bitcast(x, u32), z), x.dtype)


def _ln16(x):
    mu = jnp.sum(x, axis=1, keepdims=True) * (1.0 / D)
    xc = x - mu
    var = jnp.sum(xc * xc, axis=1, keepdims=True) * (1.0 / D)
    return _pack(xc * lax.rsqrt(var + EPS))


def _tree(x, op):
    n = x.shape[0]
    while n > 1:
        n //= 2
        x = op(x[:n], x[n:])
    return x[0]


def _local_attention(q, kc, kp, vc, vp, pos):
    lane = lax.broadcasted_iota(jnp.int32, (UCH * 4, 128), 1)

    def shifted(cur, prev, u, w):
        rows = slice(u * UCH * 4, (u + 1) * UCH * 4)
        x = cur[rows]
        if w:
            x = jnp.where(lane >= 128 - DIL * w, prev[rows], x)
            x = pltpu.roll(x, DIL * w, axis=1)
        return _as_bf16(x).astype(f32).reshape(UCH, 8, 128)

    nu = 16 // UCH
    even = lax.broadcasted_iota(jnp.int32, (8, 128), 0) % 2 == 0
    acc = [None] * W_LOC
    for u in range(nu):
        qu = q[u * UCH * 8:(u + 1) * UCH * 8].reshape(UCH, 8, 128)
        for w in range(W_LOC):
            t = _tree(qu * shifted(kc, kp, u, w), jnp.add)
            acc[w] = t if acc[w] is None else acc[w] + t
    logits = []
    for w in range(W_LOC):
        t = acc[w]
        t = t + jnp.where(even, pltpu.roll(t, 7, axis=0), pltpu.roll(t, 1, axis=0))
        t = t * QSCALE
        if w:
            t = jnp.where(pos >= DIL * w, t, NEG)
        logits.append(t)
    m = logits[0]
    for t in logits[1:]:
        m = jnp.maximum(m, t)
    ps = [jnp.exp2(t - m) for t in logits]
    l = ps[0]
    for p in ps[1:]:
        l = l + p
    r = 1.0 / l
    ps = [(p * r)[None] for p in ps]
    outs = []
    for u in range(nu):
        o = None
        for w in range(W_LOC):
            t = shifted(vc, vp, u, w) * ps[w]
            o = t if o is None else o + t
        outs.append(o.reshape(UCH * 8, 128))
    return jnp.concatenate(outs, axis=0)


def _kernel(x_hbm, wa_hbm, woa_hbm, wb_hbm, wob_hbm, out_hbm,
            x_ref, xio, xn1a, xn1b, xn2, wa_nat, wat, woa, woap, wb_nat, wbt, wk, wkp, wob, wobp,
            khalo, vhalo, wstage, pxn, pbuf, po,
            qT, kN, vT, oN, otbuf,
            sem, *bufs):
    xn1 = (xn1a, xn1b)
    sbufs = bufs[:NC]
    stg = [bufs[NC + 3 * g:NC + 3 * g + 3] for g in range(NG)]

    def x_copy(i, sid):
        rows = pl.ds(i * BLK, BLK)
        return pltpu.make_async_copy(x_hbm.at[rows, :], xio.at[rows, :], sem.at[sid])

    def wa_copies(g):
        return [pltpu.make_async_copy(
            wa_hbm.at[:, pl.ds(pl.multiple_of(sec * D + g * 128, 128), 128)],
            wa_nat.at[g * 3 + sec], sem.at[SEM_WA + g]) for sec in range(3)]

    def wb_copy(c, sid):
        col = c * 128 + (c // 8) * D
        return pltpu.make_async_copy(
            wb_hbm.at[:, pl.ds(col, 128)], wb_nat.at[c], sem.at[sid])

    def wk_copy(c, sid):
        rows = pl.ds(c * 128, 128)
        return pltpu.make_async_copy(
            wb_hbm.at[rows, pl.ds(D, D)], wk.at[rows, :], sem.at[sid])

    def iter_copies(it):
        sid = SEM_IT + min(it, 3)
        if it == 0:
            cps = [pltpu.make_async_copy(woa_hbm, woa, sem.at[sid])]
        else:
            cps = [x_copy(i, sid) for i in (2 * it + 1, 2 * it + 2) if i < NB]
        return cps + [wb_copy(2 * it, sid), wb_copy(2 * it + 1, sid), wk_copy(it, sid)]

    x01_copies = [x_copy(0, SEM_X01), x_copy(1, SEM_X01)]
    x2_copy = x_copy(2, SEM_X2)
    wob_copy = pltpu.make_async_copy(wob_hbm, wob, sem.at[SEM_WOB])

    def out_copy(j):
        rows = pl.ds(pl.multiple_of(j * TF, TF), TF)
        return pltpu.make_async_copy(xio.at[rows, :], out_hbm.at[rows, :], sem.at[SEM_OUT])

    def blk_rows(i, n=BLK):
        return pl.ds(pl.multiple_of(i * n, n), n)

    def qkv_group(g, xn):
        w = jnp.concatenate([wat[g, kt] for kt in range(NG)], axis=1)
        q, k, v = [_dot_nt(_as_bf16(w[a:a + 64]), xn) for a in (0, 64, 128)]
        return q, _pack(k), _pack(v)

    def o_rows(i, n):
        rows = blk_rows(i, n // 2)
        return _as_bf16(jnp.concatenate([oN[t, rows, :] for t in range(NG)], axis=1))

    def proj_residual(o, w_cols, xv):
        cols = []
        for n in range(2):
            cols.append(xv[:, n * 512:(n + 1) * 512] + _dot(o, w_cols(n)))
        return jnp.concatenate(cols, axis=1)

    def packed_cols(w_ref):
        return lambda n: _as_bf16(
            jnp.concatenate([w_ref[4 * n + t] for t in range(4)], axis=1))

    woa_cols, wob_cols, wk_cols = packed_cols(woap), packed_cols(wobp), packed_cols(wkp)

    def repack(dst_ref, src_ref, c, n, tok=None):
        wv = pltpu.bitcast(src_ref[blk_rows(c, n), :], u32)
        if tok is not None:
            wv = _after(wv, tok)
        for t in range(NG):
            dst_ref[t, blk_rows(c, n // 2), :] = wv[:, t * 128:(t + 1) * 128]

    def store_permuted(dst_ref, row0, val):
        for h in range(4):
            dst_ref[pl.ds(row0 + h, 16, stride=4), :] = val[h * 16:(h + 1) * 16]

    def rows16(blk, r):
        return pl.ds(pl.multiple_of(blk * BLK + r * 16, 16), 16)

    def ln1(blk, r, tok=None):
        xv = xio[rows16(blk, r), :].astype(f32)
        return _ln16(xv if tok is None else _after(xv, tok))

    def ln2(blk, r, tok=None):
        xv = x_ref[rows16(blk, r), :]
        xn2[pl.ds(pl.multiple_of(blk * (BLK // 2) + r * 8, 8), 8), :] = _ln16(
            xv if tok is None else _after(xv, tok))

    def stage(g, slot, qkv):
        for ref, val in zip(stg[g], qkv):
            ref[slot] = val

    def a_block(i, par):
        ip = jnp.maximum(i - 1, 0)
        inx = jnp.minimum(i + 1, NB - 1)
        pos = i * BLK + lax.broadcasted_iota(jnp.int32, (8, 128), 1)

        def side_jobs(slot, src):
            if slot not in L1S + L2S + (WBSLOT, WKSLOT):
                return
            tok = _token(src)
            if slot == WBSLOT:
                wsrc = _as_bf16(_after(pltpu.bitcast(wb_nat[i], u32), tok))
                wbt[i] = pltpu.bitcast(wsrc.T, u32)
            if slot == WKSLOT:
                repack(wkp, wk, i, 64, tok)
            for r in range(8):
                if L1S[r] == slot:
                    xn1[1 - par][r * 8:(r + 1) * 8, :] = ln1(inx, r, tok)
            for r in range(8):
                if L2S[r] == slot:
                    ln2(ip, r, tok)

        o_cols = []
        for g in range(NG):
            if g:
                stage(g, par, qkv_group(g, _as_bf16(xn1[par][...])))
            qs, ks, vs = stg[g]
            ot = _local_attention(qs[par], ks[par], ks[1 - par], vs[par], vs[1 - par], pos)
            o_cols.append(ot.astype(bf16).T)
            side_jobs(g, ot[120:128])
        qkv = qkv_group(0, _as_bf16(xn1[1 - par][...]))
        stage(0, 1 - par, qkv)
        side_jobs(NG, qkv[1])
        rows = blk_rows(i)
        x_ref[rows, :] = proj_residual(
            jnp.concatenate(o_cols, axis=1), woa_cols, xio[rows, :].astype(f32))

    def startup():
        def transpose_wa(g):
            for sec in range(3):
                wv = pltpu.bitcast(wa_nat[g * 3 + sec].T, u32)
                for kt in range(NG):
                    store_permuted(wstage.at[kt], sec * 64, wv[:, kt * 128:(kt + 1) * 128])

        def project(g):
            w = wstage[...]
            wat[g] = w
            w = jnp.concatenate([w[kt] for kt in range(NG)], axis=1)
            return jnp.concatenate(
                [_dot_nt(_as_bf16(w[a:a + PM]), _as_bf16(pxn[...])) for a in range(0, 192, PM)],
                axis=0)

        def attend(g, r):
            pos = lax.broadcasted_iota(jnp.int32, (8, 128), 1)
            kp = vp = jnp.zeros((64, BLK), u32)
            for b in range(2):
                rb = r[:, b * BLK:(b + 1) * BLK]
                kc = _pack(rb[128:256])
                vc = _pack(rb[256:384])
                ot = _local_attention(rb[0:128], kc, kp, vc, vp, pos + b * BLK)
                po[g, b * 64:(b + 1) * 64, :] = pltpu.bitcast(ot.astype(bf16).T, u32)
                kp, vp = kc, vc
            khalo[g] = kp
            vhalo[g] = vp

        pbuf[...] = jnp.zeros(pbuf.shape, f32)

        def zero_scores(k, c):
            for sb in sbufs:
                sb[blk_rows(k, 32), :] = jnp.zeros((32, NQ), f32)
            return c
        lax.fori_loop(0, 2 * MK // 32, zero_scores, 0)
        for cp in x01_copies:
            cp.wait()
        for b in range(2):
            for r in range(BLK // 16):
                pxn[b * 64 + r * 8:b * 64 + (r + 1) * 8, :] = ln1(b, r)
        for cp in wa_copies(0):
            cp.wait()
        transpose_wa(0)

        def body(g, c):
            for cp in wa_copies(g + 1):
                cp.wait()
            prev = pbuf[...]
            pbuf[...] = project(g)
            transpose_wa(g + 1)
            attend(jnp.maximum(g - 1, 0), prev)
            return c
        lax.fori_loop(0, NG - 1, body, 0)

        x2_copy.wait()
        prev = pbuf[...]
        r = project(NG - 1)
        xn_next = jnp.concatenate([ln1(2, r16) for r16 in range(BLK // 16)], axis=0)
        xn1[0][...] = xn_next
        attend(NG - 2, _after(prev, _token(xn_next[56:64, 0:128])))
        stage(0, 0, qkv_group(0, _as_bf16(xn_next)))
        attend(NG - 1, r)

        for cp in iter_copies(0):
            cp.wait()
        for t in range(NG):
            wv = pltpu.bitcast(woa[:, t * 128:(t + 1) * 128], u32)
            for g in range(NG):
                store_permuted(woap.at[t], g * 64, wv[g * 64:(g + 1) * 64])
        for b in range(2):
            o = jnp.concatenate([po[g, b * 64:(b + 1) * 64, :] for g in range(NG)], axis=1)
            rows = blk_rows(b)
            x_ref[rows, :] = proj_residual(_as_bf16(o), woa_cols, xio[rows, :].astype(f32))
            wbt[b] = pltpu.bitcast(wb_nat[b].T, u32)
        repack(wkp, wk, 0, 128)
        for r16 in range(BLK // 16):
            ln2(0, r16)
        for g in range(NG):
            stg[g][1][1] = khalo[g]
            stg[g][2][1] = vhalo[g]
        for cp in iter_copies(1):
            cp.wait()

    def phase_a(rep):
        @pl.when(rep == 1)
        def _():
            for g in range(NG):
                for ref in stg[g][1:]:
                    ref[1] = jnp.zeros((64, BLK), u32)
            xn_first = jnp.concatenate([ln1(0, r) for r in range(BLK // 16)], axis=0)
            xn1[0][...] = xn_first
            stage(0, 0, qkv_group(0, _as_bf16(xn_first)))

        def body(it, c):
            @pl.when(it == 2 - rep * NB)
            def _():
                for cp in iter_copies(2):
                    cp.wait()

            @pl.when(it == 3 - rep * NB)
            def _():
                for k in range(3, NB // APB):
                    for cp in iter_copies(k):
                        cp.wait()

            for u in range(APB):
                a_block(it * APB + u, u % 2)
            return c
        with _scope("a_loop"):
            lax.fori_loop(1 - rep, NB // APB, body, 0)
        for r in range(BLK // 16):
            ln2(NB - 1, r)

    def phase_b_proj():
        def body(j, c):
            rows = blk_rows(j, TB // 2)
            xn = _as_bf16(xn2[rows, :])
            for n in range(2):
                y = _pack(_dot(xn, wk_cols(n)))
                for t in range(4):
                    kN[4 * n + t, rows, :] = y[:, t * 128:(t + 1) * 128]
            for r in range(4):
                w = _as_bf16(wbt[2 * r:2 * r + 2].reshape(128, D))
                y = _pack(_dot_nt(w, xn) * QSCALE)
                for b in range(TB // NQ):
                    qT[j * (TB // NQ) + b, r * 128:(r + 1) * 128, :] = y[:, b * NQ:(b + 1) * NQ]
            for r in range(4):
                w = _as_bf16(wbt[8 + 2 * r:8 + 2 * r + 2].reshape(128, D))
                y = _pack(_dot_nt(w, xn))
                for b in range(TB // MK):
                    vT[j * (TB // MK) + b, r * 128:(r + 1) * 128, :] = y[:, b * MK:(b + 1) * MK]
            return c
        lax.fori_loop(0, S // TB, body, 0)

    def flush_o(g, val):
        y = pltpu.bitcast(_as_bf16(val).T, u32)
        oN[g % NG, blk_rows(g // NG, NQ // 2), :] = y

    def phase_b_attn():
        off = [0, 0]

        def qm_of(t, qi, j):
            q = _as_bf16(qT[qi, pl.ds(pl.multiple_of(t * 64 + j * 16, 16), 16), :])
            parts = []
            if j > 0:
                parts.append(jnp.zeros((32 * j, NQ), bf16))
            parts.append(q)
            if j < 3:
                parts.append(jnp.zeros((32 * (3 - j), NQ), bf16))
            return jnp.concatenate(parts, axis=0)

        def qk_chunk(t, qm, c, par, m):
            k = _as_bf16(kN[t, c * (MK // 2):(c + 1) * (MK // 2), :])
            s = _dot(k, qm)
            sbufs[c][pl.ds(pl.multiple_of(off[0] + par * MK, 8), MK), :] = s
            sm = _tree(s.reshape(MK // 8, 8, NQ), jnp.maximum)
            return sm if m is None else jnp.maximum(m, sm)

        def pv_chunk(h, c, par, mrow, l, o):
            s = sbufs[c][pl.ds(pl.multiple_of(off[1] + par * MK, 8), MK), :]
            p = jnp.exp2(s - mrow)
            ls = jnp.sum(p.reshape(MK // 8, 8, NQ), axis=0)
            l = ls if l is None else l + ls
            v = _as_bf16(vT[c, pl.ds(pl.multiple_of(h * 16, 16), 16), :])
            oc = _dot(v, p.astype(bf16))
            o = oc if o is None else o + oc
            return l, o

        n_groups = NQT * NG
        lag = NC + DL
        n_steps = 4 * NC

        def set_offsets(zero):
            off[0] = lax.shift_right_logical(zero, 16) * 8
            off[1] = lax.shift_right_logical(zero, 17) * 8

        def pv_step(g, n, ms, st, flush=True):
            j, c = divmod(n, NC)
            l, o, mrow = st
            if c == 0:
                mrow = jnp.max(ms[j], axis=0, keepdims=True)
                l = o = None
            l, o = pv_chunk((g % NG) * 4 + j, c, j % 2, mrow, l, o)
            if c == NC - 1:
                lrow = jnp.sum(l, axis=0, keepdims=True)
                otbuf[j * 16:(j + 1) * 16, :] = _pack(o * (1.0 / lrow))
                if j == 3 and flush:
                    flush_o(g, otbuf[...])
            return l, o, mrow

        def group(g, g_prev, carry, side_job=None):
            st, ms_prev = carry[:3], {3: carry[3]}
            ms = {}
            for n in range(n_steps):
                j, c = divmod(n, NC)
                if c == 0:
                    qm = qm_of(g % NG, g // NG, j)
                ms[j] = qk_chunk(g % NG, qm, c, j % 2, ms.get(j))
                if n < lag:
                    st = pv_step(g_prev, n + n_steps - lag, ms_prev, st)
                else:
                    st = pv_step(g, n - lag, ms, st)
                if side_job is not None and n == n_steps // 2:
                    side_job(_token(st[0][:, 0:128]))
            return st + (ms[3],)

        def body(it, carry):
            def side_job(tok):
                repack(wobp, wob, it, D * GPB // n_groups, tok)

            set_offsets(it)
            carry = carry[:4]
            for u in range(GPB):
                g = it * GPB + u
                carry = group(g, jnp.maximum(g - 1, 0), carry, side_job if u == 0 else None)
            return carry + (it,)

        otbuf[...] = jnp.zeros(otbuf.shape, u32)
        init = (jnp.zeros((8, NQ), f32), jnp.zeros((DH, NQ), f32),
                jnp.zeros((1, NQ), f32), jnp.zeros((8, NQ), f32), jnp.int32(0))
        carry = lax.fori_loop(0, n_groups // GPB, body, init)
        set_offsets(carry[4])
        st, ms = carry[:3], {3: carry[3]}
        for n in range(n_steps - lag, n_steps):
            st = pv_step(n_groups - 1, n, ms, st, False)
        off[0] = off[1] = 0

    def phase_b_out(rep):
        def body(jj, c):
            for u in range(OPB):
                j = jj * OPB + u
                rows = blk_rows(j, TF)
                xv = proj_residual(o_rows(j, TF), wob_cols, x_ref[rows, :])
                xio[rows, :] = xv.astype(bf16)

                @pl.when(rep == 1)
                def _():
                    out_copy(j).start()
            flush_o(NQT * NG - 1, otbuf[...])
            return c
        lax.fori_loop(0, S // (TF * OPB), body, 0)

    if ONLY == "A":
        phase_a(lax.fori_loop(0, 2, lambda i, c: c + i, 0))
        xio[0:8, :] = (_as_bf16(wbt[0, 0:4, :]) + _as_bf16(xn2[0:4, :])
                       + jnp.concatenate([_as_bf16(wkp[0, 0:4, :])] * 8, axis=1))
        return
    if ONLY == "S":
        for cp in x01_copies + [x2_copy] + iter_copies(0) + iter_copies(1):
            cp.start()
        for g in range(NG):
            for cp in wa_copies(g):
                cp.start()
        startup()
        xio[0:8, :] = (_as_bf16(wbt[0, 0:4, :]) + _as_bf16(xn2[0:4, :]) + _as_bf16(xn1[0][0:4, :])
                       + x_ref[0:8, :].astype(bf16)
                       + jnp.concatenate([_as_bf16(wkp[0, 0:4, :]) + _as_bf16(wat[1, 0, 0:4, :])
                                          + _as_bf16(stg[0][1][0, 0:4, :]) + _as_bf16(stg[3][2][1, 0:4, :])] * 8, axis=1))
        return
    if ONLY == "B":
        phase_b_attn()
        xio[0:8, :] = jnp.concatenate(
            [_as_bf16(oN[0, 0:4, :]) + _as_bf16(wobp[0, 0:4, :])] * 8, axis=1)
        return

    for cp in x01_copies:
        cp.start()
    for g in range(NG):
        if g == NG - 2:
            x2_copy.start()
        for cp in wa_copies(g):
            cp.start()
    for it in range(NB // APB):
        for cp in iter_copies(it):
            cp.start()
    wob_copy.start()

    with _scope("startup"):
        startup()

    def layer_pair(rep, c):
        with _scope("phase_a"):
            phase_a(rep)

        @pl.when(rep == 0)
        def _():
            wob_copy.wait()

        with _scope("b_proj"):
            phase_b_proj()
        with _scope("b_attn"):
            phase_b_attn()
        with _scope("b_out"):
            phase_b_out(rep)
        return c
    lax.fori_loop(0, 2, layer_pair, 0)
    for j in range(S // TF):
        out_copy(j).wait()


@jax.jit
def pallas_interleave_layers__sliding_local_dilated__softmax_full_mha__prompt_kernel(
    A_x: jax.Array,
    A_wqkv: jax.Array,
    A_wo: jax.Array,
    B_x: jax.Array,
    B_wqkv: jax.Array,
    B_wo: jax.Array,
):
    del B_x
    x = A_x.reshape(S, D)
    vm = pltpu.VMEM
    scratch = [
        vm((S, D), f32),
        vm((S, D), bf16),
        vm((BLK // 2, D), u32),
        vm((BLK // 2, D), u32),
        vm((S // 2, D), u32),
        vm((3 * NG, D, 128), bf16),
        vm((NG, NG, 192, 128), u32),
        vm((D, D), bf16),
        vm((NG, D // 2, 128), u32),
        vm((2 * NG, D, 128), bf16),
        vm((2 * NG, 64, D), u32),
        vm((D, D), bf16),
        vm((NG, D // 2, 128), u32),
        vm((D, D), bf16),
        vm((NG, D // 2, 128), u32),
        vm((NG, 64, BLK), u32),
        vm((NG, 64, BLK), u32),
        vm((NG, 192, 128), u32),
        vm((BLK, D), u32),
        vm((384, 2 * BLK), f32),
        vm((NG, BLK, 128), u32),
        vm((NQT, D // 2, NQ), u32),
        vm((NG, S // 2, 128), u32),
        vm((NC, D // 2, MK), u32),
        vm((NG, S // 2, 128), u32),
        vm((64, NQ), u32),
        pltpu.SemaphoreType.DMA((N_SEM,)),
    ] + [vm((2 * MK, NQ), f32)] * NC + [
        vm((2, 128, BLK), f32), vm((2, 64, BLK), u32), vm((2, 64, BLK), u32)] * NG
    out = pl.pallas_call(
        _kernel,
        out_shape=jax.ShapeDtypeStruct((S, D), bf16),
        in_specs=[pl.BlockSpec(memory_space=pl.ANY)] * 5,
        out_specs=pl.BlockSpec(memory_space=pl.ANY),
        scratch_shapes=scratch,
        compiler_params=pltpu.CompilerParams(vmem_limit_bytes=110 * 1024 * 1024),
        name="interleave_attn",
    )(x, A_wqkv, A_wo, B_wqkv, B_wo)
    return out.reshape(1, S, D)
```

```python
import jax
import jax.numpy as jnp
from jax import lax
import jax.experimental.pallas as pl
import jax.experimental.pallas.tpu as pltpu

S, D, H, DH = 2048, 1024, 32, 32
W_LOC, DIL = 8, 2
EPS = 1e-5
LOG2E = 1.4426950408889634
QSCALE = (DH ** -0.5) * LOG2E
NEG = -1e9 * LOG2E

BLK = 128
NB = S // BLK
NG = D // 128
NQ = 256
NQT = S // NQ
MK = 128
NC = S // MK
DL = 6
APB = 2
GPB = 4
TB = 256
TF = 128
OPRE = 1
OPB = 3

SEM_X01, SEM_X2, SEM_WOB, SEM_OUT = 0, 1, 2, 3
SEM_WA = 4
SEM_IT = SEM_WA + NG
N_SEM = SEM_IT + 4

UCH = 2
L1S = (0, 0, 1, 1, 1, 2, 3, 4)
L2S = (4, 5, 6, 6, 7, 7, 8, 8)
WBSLOT = 6
WKSLOT = 2
PM = 192

ONLY = None
PROFILE_SCOPES = False

bf16 = jnp.bfloat16
f32 = jnp.float32
u32 = jnp.uint32
NT = (((1,), (1,)), ((), ()))


class _NoScope:
    def __enter__(self):
        return self

    def __exit__(self, *a):
        return False


def _scope(name):
    return jax.named_scope(name) if PROFILE_SCOPES else _NoScope()


def _pack(x):
    return pltpu.bitcast(x.astype(bf16), u32)


def _as_bf16(x):
    return pltpu.bitcast(x, bf16)


def _dot(a, b):
    return jnp.dot(a, b, preferred_element_type=f32)


def _dot_nt(a, b):
    return lax.dot_general(a, b, NT, preferred_element_type=f32)


def _token(v):
    t = pltpu.bitcast(v[0:8, :], u32)
    return lax.shift_right_logical(jnp.bitwise_and(t, jnp.uint32(0xFFFF)), jnp.uint32(16))


def _after(x, tok):
    n, m = x.shape
    z = jnp.concatenate([jnp.concatenate([tok] * (m // 128), axis=1)] * (n // 8), axis=0)
    return pltpu.bitcast(jnp.bitwise_or(pltpu.bitcast(x, u32), z), x.dtype)


def _ln16(x):
    mu = jnp.sum(x, axis=1, keepdims=True) * (1.0 / D)
    xc = x - mu
    var = jnp.sum(xc * xc, axis=1, keepdims=True) * (1.0 / D)
    return _pack(xc * lax.rsqrt(var + EPS))


def _tree(x, op):
    n = x.shape[0]
    while n > 1:
        n //= 2
        x = op(x[:n], x[n:])
    return x[0]


def _local_attention(q, kc, kp, vc, vp, pos):
    lane = lax.broadcasted_iota(jnp.int32, (UCH * 4, 128), 1)

    def shifted(cur, prev, u, w):
        rows = slice(u * UCH * 4, (u + 1) * UCH * 4)
        x = cur[rows]
        if w:
            x = jnp.where(lane >= 128 - DIL * w, prev[rows], x)
            x = pltpu.roll(x, DIL * w, axis=1)
        return _as_bf16(x).astype(f32).reshape(UCH, 8, 128)

    nu = 16 // UCH
    even = lax.broadcasted_iota(jnp.int32, (8, 128), 0) % 2 == 0
    acc = [None] * W_LOC
    for u in range(nu):
        qu = q[u * UCH * 8:(u + 1) * UCH * 8].reshape(UCH, 8, 128)
        for w in range(W_LOC):
            t = _tree(qu * shifted(kc, kp, u, w), jnp.add)
            acc[w] = t if acc[w] is None else acc[w] + t
    logits = []
    for w in range(W_LOC):
        t = acc[w]
        t = t + jnp.where(even, pltpu.roll(t, 7, axis=0), pltpu.roll(t, 1, axis=0))
        t = t * QSCALE
        if w:
            t = jnp.where(pos >= DIL * w, t, NEG)
        logits.append(t)
    m = logits[0]
    for t in logits[1:]:
        m = jnp.maximum(m, t)
    ps = [jnp.exp2(t - m) for t in logits]
    l = ps[0]
    for p in ps[1:]:
        l = l + p
    r = 1.0 / l
    ps = [(p * r)[None] for p in ps]
    outs = []
    for u in range(nu):
        o = None
        for w in range(W_LOC):
            t = shifted(vc, vp, u, w) * ps[w]
            o = t if o is None else o + t
        outs.append(o.reshape(UCH * 8, 128))
    return jnp.concatenate(outs, axis=0)


def _kernel(x_hbm, wa_hbm, woa_hbm, wb_hbm, wob_hbm, out_hbm,
            x_ref, xio, xn1a, xn1b, xn2, wa_nat, wat, woa, woap, wb_nat, wbt, wk, wkp, wob, wobp,
            khalo, vhalo, wstage, pxn, pbuf, po,
            qT, kN, vT, oN, otbuf,
            sem, *bufs):
    xn1 = (xn1a, xn1b)
    sbufs = bufs[:NC]
    stg = [bufs[NC + 3 * g:NC + 3 * g + 3] for g in range(NG)]

    def x_copy(i, sid):
        rows = pl.ds(i * BLK, BLK)
        return pltpu.make_async_copy(x_hbm.at[rows, :], xio.at[rows, :], sem.at[sid])

    def wa_copies(g):
        return [pltpu.make_async_copy(
            wa_hbm.at[:, pl.ds(pl.multiple_of(sec * D + g * 128, 128), 128)],
            wa_nat.at[g * 3 + sec], sem.at[SEM_WA + g]) for sec in range(3)]

    def wb_copy(c, sid):
        col = c * 128 + (c // 8) * D
        return pltpu.make_async_copy(
            wb_hbm.at[:, pl.ds(col, 128)], wb_nat.at[c], sem.at[sid])

    def wk_copy(c, sid):
        rows = pl.ds(c * 128, 128)
        return pltpu.make_async_copy(
            wb_hbm.at[rows, pl.ds(D, D)], wk.at[rows, :], sem.at[sid])

    def iter_copies(it):
        sid = SEM_IT + min(it, 3)
        if it == 0:
            cps = [pltpu.make_async_copy(woa_hbm, woa, sem.at[sid])]
        else:
            cps = [x_copy(i, sid) for i in (2 * it + 1, 2 * it + 2) if i < NB]
        return cps + [wb_copy(2 * it, sid), wb_copy(2 * it + 1, sid), wk_copy(it, sid)]

    x01_copies = [x_copy(0, SEM_X01), x_copy(1, SEM_X01)]
    x2_copy = x_copy(2, SEM_X2)
    wob_copy = pltpu.make_async_copy(wob_hbm, wob, sem.at[SEM_WOB])

    def out_copy(j):
        rows = pl.ds(pl.multiple_of(j * TF, TF), TF)
        return pltpu.make_async_copy(xio.at[rows, :], out_hbm.at[rows, :], sem.at[SEM_OUT])

    def blk_rows(i, n=BLK):
        return pl.ds(pl.multiple_of(i * n, n), n)

    def qkv_group(g, xn):
        w = jnp.concatenate([wat[g, kt] for kt in range(NG)], axis=1)
        q, k, v = [_dot_nt(_as_bf16(w[a:a + 64]), xn) for a in (0, 64, 128)]
        return q, _pack(k), _pack(v)

    def o_rows(i, n):
        rows = blk_rows(i, n // 2)
        return _as_bf16(jnp.concatenate([oN[t, rows, :] for t in range(NG)], axis=1))

    def proj_residual(o, w_cols, xv):
        cols = []
        for n in range(2):
            cols.append(xv[:, n * 512:(n + 1) * 512] + _dot(o, w_cols(n)))
        return jnp.concatenate(cols, axis=1)

    def packed_cols(w_ref):
        return lambda n: _as_bf16(
            jnp.concatenate([w_ref[4 * n + t] for t in range(4)], axis=1))

    woa_cols, wob_cols, wk_cols = packed_cols(woap), packed_cols(wobp), packed_cols(wkp)

    def repack(dst_ref, src_ref, c, n, tok=None):
        wv = pltpu.bitcast(src_ref[blk_rows(c, n), :], u32)
        if tok is not None:
            wv = _after(wv, tok)
        for t in range(NG):
            dst_ref[t, blk_rows(c, n // 2), :] = wv[:, t * 128:(t + 1) * 128]

    def store_permuted(dst_ref, row0, val):
        for h in range(4):
            dst_ref[pl.ds(row0 + h, 16, stride=4), :] = val[h * 16:(h + 1) * 16]

    def rows16(blk, r):
        return pl.ds(pl.multiple_of(blk * BLK + r * 16, 16), 16)

    def ln1(blk, r, tok=None):
        xv = xio[rows16(blk, r), :].astype(f32)
        return _ln16(xv if tok is None else _after(xv, tok))

    def ln2(blk, r, tok=None):
        xv = x_ref[rows16(blk, r), :]
        xn2[pl.ds(pl.multiple_of(blk * (BLK // 2) + r * 8, 8), 8), :] = _ln16(
            xv if tok is None else _after(xv, tok))

    def stage(g, slot, qkv):
        for ref, val in zip(stg[g], qkv):
            ref[slot] = val

    def a_block(i, par):
        ip = jnp.maximum(i - 1, 0)
        inx = jnp.minimum(i + 1, NB - 1)
        pos = i * BLK + lax.broadcasted_iota(jnp.int32, (8, 128), 1)

        def side_jobs(slot, src):
            if slot not in L1S + L2S + (WBSLOT, WKSLOT):
                return
            tok = _token(src)
            if slot == WBSLOT:
                wsrc = _as_bf16(_after(pltpu.bitcast(wb_nat[i], u32), tok))
                wbt[i] = pltpu.bitcast(wsrc.T, u32)
            if slot == WKSLOT:
                repack(wkp, wk, i, 64, tok)
            for r in range(8):
                if L1S[r] == slot:
                    xn1[1 - par][r * 8:(r + 1) * 8, :] = ln1(inx, r, tok)
            for r in range(8):
                if L2S[r] == slot:
                    ln2(ip, r, tok)

        o_cols = []
        for g in range(NG):
            if g:
                stage(g, par, qkv_group(g, _as_bf16(xn1[par][...])))
            qs, ks, vs = stg[g]
            ot = _local_attention(qs[par], ks[par], ks[1 - par], vs[par], vs[1 - par], pos)
            o_cols.append(ot.astype(bf16).T)
            side_jobs(g, ot[120:128])
        qkv = qkv_group(0, _as_bf16(xn1[1 - par][...]))
        stage(0, 1 - par, qkv)
        side_jobs(NG, qkv[1])
        rows = blk_rows(i)
        x_ref[rows, :] = proj_residual(
            jnp.concatenate(o_cols, axis=1), woa_cols, xio[rows, :].astype(f32))

    def startup():
        def transpose_wa(g):
            for sec in range(3):
                wv = pltpu.bitcast(wa_nat[g * 3 + sec].T, u32)
                for kt in range(NG):
                    store_permuted(wstage.at[kt], sec * 64, wv[:, kt * 128:(kt + 1) * 128])

        def project(g):
            w = wstage[...]
            wat[g] = w
            w = jnp.concatenate([w[kt] for kt in range(NG)], axis=1)
            return jnp.concatenate(
                [_dot_nt(_as_bf16(w[a:a + PM]), _as_bf16(pxn[...])) for a in range(0, 192, PM)],
                axis=0)

        def attend(g, r):
            pos = lax.broadcasted_iota(jnp.int32, (8, 128), 1)
            kp = vp = jnp.zeros((64, BLK), u32)
            for b in range(2):
                rb = r[:, b * BLK:(b + 1) * BLK]
                kc = _pack(rb[128:256])
                vc = _pack(rb[256:384])
                ot = _local_attention(rb[0:128], kc, kp, vc, vp, pos + b * BLK)
                po[g, b * 64:(b + 1) * 64, :] = pltpu.bitcast(ot.astype(bf16).T, u32)
                kp, vp = kc, vc
            khalo[g] = kp
            vhalo[g] = vp

        pbuf[...] = jnp.zeros(pbuf.shape, f32)

        def zero_scores(k, c):
            for sb in sbufs:
                sb[blk_rows(k, 32), :] = jnp.zeros((32, NQ), f32)
            return c
        lax.fori_loop(0, 2 * MK // 32, zero_scores, 0)
        for cp in x01_copies:
            cp.wait()
        for b in range(2):
            for r in range(BLK // 16):
                pxn[b * 64 + r * 8:b * 64 + (r + 1) * 8, :] = ln1(b, r)
        for cp in wa_copies(0):
            cp.wait()
        transpose_wa(0)

        def body(g, c):
            for cp in wa_copies(g + 1):
                cp.wait()
            prev = pbuf[...]
            pbuf[...] = project(g)
            transpose_wa(g + 1)
            attend(jnp.maximum(g - 1, 0), prev)
            return c
        lax.fori_loop(0, NG - 1, body, 0)

        x2_copy.wait()
        prev = pbuf[...]
        r = project(NG - 1)
        xn_next = jnp.concatenate([ln1(2, r16) for r16 in range(BLK // 16)], axis=0)
        xn1[0][...] = xn_next
        attend(NG - 2, _after(prev, _token(xn_next[56:64, 0:128])))
        stage(0, 0, qkv_group(0, _as_bf16(xn_next)))
        attend(NG - 1, r)

        for cp in iter_copies(0):
            cp.wait()
        for t in range(NG):
            wv = pltpu.bitcast(woa[:, t * 128:(t + 1) * 128], u32)
            for g in range(NG):
                store_permuted(woap.at[t], g * 64, wv[g * 64:(g + 1) * 64])
        for b in range(2):
            o = jnp.concatenate([po[g, b * 64:(b + 1) * 64, :] for g in range(NG)], axis=1)
            rows = blk_rows(b)
            x_ref[rows, :] = proj_residual(_as_bf16(o), woa_cols, xio[rows, :].astype(f32))
            wbt[b] = pltpu.bitcast(wb_nat[b].T, u32)
        repack(wkp, wk, 0, 128)
        for r16 in range(BLK // 16):
            ln2(0, r16)
        for g in range(NG):
            stg[g][1][1] = khalo[g]
            stg[g][2][1] = vhalo[g]
        for cp in iter_copies(1):
            cp.wait()

    def phase_a(rep):
        @pl.when(rep == 1)
        def _():
            for g in range(NG):
                for ref in stg[g][1:]:
                    ref[1] = jnp.zeros((64, BLK), u32)
            xn_first = jnp.concatenate([ln1(0, r) for r in range(BLK // 16)], axis=0)
            xn1[0][...] = xn_first
            stage(0, 0, qkv_group(0, _as_bf16(xn_first)))

        def body(it, c):
            @pl.when(it == 2 - rep * NB)
            def _():
                for cp in iter_copies(2):
                    cp.wait()

            @pl.when(it == 3 - rep * NB)
            def _():
                for k in range(3, NB // APB):
                    for cp in iter_copies(k):
                        cp.wait()

            for u in range(APB):
                a_block(it * APB + u, u % 2)
            return c
        with _scope("a_loop"):
            lax.fori_loop(1 - rep, NB // APB, body, 0)
        for r in range(BLK // 16):
            ln2(NB - 1, r)

    def phase_b_proj():
        def body(j, c):
            rows = blk_rows(j, TB // 2)
            xn = _as_bf16(xn2[rows, :])
            for n in range(2):
                y = _pack(_dot(xn, wk_cols(n)))
                for t in range(4):
                    kN[4 * n + t, rows, :] = y[:, t * 128:(t + 1) * 128]
            for r in range(4):
                w = _as_bf16(wbt[2 * r:2 * r + 2].reshape(128, D))
                y = _pack(_dot_nt(w, xn) * QSCALE)
                for b in range(TB // NQ):
                    qT[j * (TB // NQ) + b, r * 128:(r + 1) * 128, :] = y[:, b * NQ:(b + 1) * NQ]
            for r in range(4):
                w = _as_bf16(wbt[8 + 2 * r:8 + 2 * r + 2].reshape(128, D))
                y = _pack(_dot_nt(w, xn))
                for b in range(TB // MK):
                    vT[j * (TB // MK) + b, r * 128:(r + 1) * 128, :] = y[:, b * MK:(b + 1) * MK]
            return c
        lax.fori_loop(0, S // TB, body, 0)

    def flush_o(g, val):
        y = pltpu.bitcast(_as_bf16(val).T, u32)
        oN[g % NG, blk_rows(g // NG, NQ // 2), :] = y

    def phase_b_attn(rep):
        off = [0, 0]

        def qm_of(t, qi, j):
            q = _as_bf16(qT[qi, pl.ds(pl.multiple_of(t * 64 + j * 16, 16), 16), :])
            parts = []
            if j > 0:
                parts.append(jnp.zeros((32 * j, NQ), bf16))
            parts.append(q)
            if j < 3:
                parts.append(jnp.zeros((32 * (3 - j), NQ), bf16))
            return jnp.concatenate(parts, axis=0)

        def qk_chunk(t, qm, c, par, m):
            k = _as_bf16(kN[t, c * (MK // 2):(c + 1) * (MK // 2), :])
            s = _dot(k, qm)
            sbufs[c][pl.ds(pl.multiple_of(off[0] + par * MK, 8), MK), :] = s
            sm = _tree(s.reshape(MK // 8, 8, NQ), jnp.maximum)
            return sm if m is None else jnp.maximum(m, sm)

        def pv_chunk(h, c, par, mrow, l, o):
            s = sbufs[c][pl.ds(pl.multiple_of(off[1] + par * MK, 8), MK), :]
            p = jnp.exp2(s - mrow)
            ls = jnp.sum(p.reshape(MK // 8, 8, NQ), axis=0)
            l = ls if l is None else l + ls
            v = _as_bf16(vT[c, pl.ds(pl.multiple_of(h * 16, 16), 16), :])
            oc = _dot(v, p.astype(bf16))
            o = oc if o is None else o + oc
            return l, o

        n_groups = NQT * NG
        lag = NC + DL
        n_steps = 4 * NC

        def set_offsets(zero):
            off[0] = lax.shift_right_logical(zero, 16) * 8
            off[1] = lax.shift_right_logical(zero, 17) * 8

        def pv_step(g, n, ms, st, flush=True):
            j, c = divmod(n, NC)
            l, o, mrow = st
            if c == 0:
                mrow = jnp.max(ms[j], axis=0, keepdims=True)
                l = o = None
            l, o = pv_chunk((g % NG) * 4 + j, c, j % 2, mrow, l, o)
            if c == NC - 1:
                lrow = jnp.sum(l, axis=0, keepdims=True)
                otbuf[j * 16:(j + 1) * 16, :] = _pack(o * (1.0 / lrow))
                if j == 3 and flush:
                    flush_o(g, otbuf[...])
            return l, o, mrow

        def group(g, g_prev, carry, side_job=None):
            st, ms_prev = carry[:3], {3: carry[3]}
            ms = {}
            for n in range(n_steps):
                j, c = divmod(n, NC)
                if c == 0:
                    qm = qm_of(g % NG, g // NG, j)
                ms[j] = qk_chunk(g % NG, qm, c, j % 2, ms.get(j))
                if n < lag:
                    st = pv_step(g_prev, n + n_steps - lag, ms_prev, st)
                else:
                    st = pv_step(g, n - lag, ms, st)
                if side_job is not None and n == n_steps // 2:
                    side_job(_token(st[0][:, 0:128]))
            return st + (ms[3],)

        def body(it, carry):
            def side_job(tok):
                repack(wobp, wob, it, D * GPB // n_groups, tok)

            set_offsets(it)
            carry = carry[:4]
            for u in range(GPB):
                g = it * GPB + u
                carry = group(g, jnp.maximum(g - 1, 0), carry, side_job if u == 0 else None)
            return carry + (it,)

        otbuf[...] = jnp.zeros(otbuf.shape, u32)
        init = (jnp.zeros((8, NQ), f32), jnp.zeros((DH, NQ), f32),
                jnp.zeros((1, NQ), f32), jnp.zeros((8, NQ), f32), jnp.int32(0))
        carry = lax.fori_loop(0, n_groups // GPB, body, init)
        set_offsets(carry[4])
        st, ms = carry[:3], {3: carry[3]}
        o0 = o_rows(0, TF)
        done = 0
        for k, n in enumerate(range(n_steps - lag, n_steps)):
            while done < NG and done * lag <= k * NG:
                cols = slice(done * 128, (done + 1) * 128)
                y = x_ref[0:TF, cols] + _dot(o0, _as_bf16(wobp[done]))
                xio[0:TF, cols] = y.astype(bf16)
                done += 1
            st = pv_step(n_groups - 1, n, ms, st, False)

        @pl.when(rep == 1)
        def _():
            out_copy(0).start()
        off[0] = off[1] = 0

    def out_tile(j, rep):
        rows = blk_rows(j, TF)
        xv = proj_residual(o_rows(j, TF), wob_cols, x_ref[rows, :])
        xio[rows, :] = xv.astype(bf16)

        @pl.when(rep == 1)
        def _():
            out_copy(j).start()

    def phase_b_out(rep):
        def body(jj, c):
            for u in range(OPB):
                out_tile(OPRE + jj * OPB + u, rep)
            flush_o(NQT * NG - 1, otbuf[...])
            return c
        lax.fori_loop(0, (S // TF - OPRE) // OPB, body, 0)

    if ONLY == "A":
        phase_a(lax.fori_loop(0, 2, lambda i, c: c + i, 0))
        xio[0:8, :] = (_as_bf16(wbt[0, 0:4, :]) + _as_bf16(xn2[0:4, :])
                       + jnp.concatenate([_as_bf16(wkp[0, 0:4, :])] * 8, axis=1))
        return
    if ONLY == "S":
        for cp in x01_copies + [x2_copy] + iter_copies(0) + iter_copies(1):
            cp.start()
        for g in range(NG):
            for cp in wa_copies(g):
                cp.start()
        startup()
        xio[0:8, :] = (_as_bf16(wbt[0, 0:4, :]) + _as_bf16(xn2[0:4, :]) + _as_bf16(xn1[0][0:4, :])
                       + x_ref[0:8, :].astype(bf16)
                       + jnp.concatenate([_as_bf16(wkp[0, 0:4, :]) + _as_bf16(wat[1, 0, 0:4, :])
                                          + _as_bf16(stg[0][1][0, 0:4, :]) + _as_bf16(stg[3][2][1, 0:4, :])] * 8, axis=1))
        return
    if ONLY == "B":
        phase_b_attn(0)
        xio[0:8, :] = jnp.concatenate(
            [_as_bf16(oN[0, 0:4, :]) + _as_bf16(wobp[0, 0:4, :])] * 8, axis=1)
        return

    for cp in x01_copies:
        cp.start()
    for g in range(NG):
        if g == NG - 2:
            x2_copy.start()
        for cp in wa_copies(g):
            cp.start()
    for it in range(NB // APB):
        for cp in iter_copies(it):
            cp.start()
    wob_copy.start()

    with _scope("startup"):
        startup()

    def layer_pair(rep, c):
        with _scope("phase_a"):
            phase_a(rep)

        @pl.when(rep == 0)
        def _():
            wob_copy.wait()

        with _scope("b_proj"):
            phase_b_proj()
        with _scope("b_attn"):
            phase_b_attn(rep)
        with _scope("b_out"):
            phase_b_out(rep)
        return c
    lax.fori_loop(0, 2, layer_pair, 0)
    for j in range(S // TF):
        out_copy(j).wait()


@jax.jit
def pallas_interleave_layers__sliding_local_dilated__softmax_full_mha__prompt_kernel(
    A_x: jax.Array,
    A_wqkv: jax.Array,
    A_wo: jax.Array,
    B_x: jax.Array,
    B_wqkv: jax.Array,
    B_wo: jax.Array,
):
    del B_x
    x = A_x.reshape(S, D)
    vm = pltpu.VMEM
    scratch = [
        vm((S, D), f32),
        vm((S, D), bf16),
        vm((BLK // 2, D), u32),
        vm((BLK // 2, D), u32),
        vm((S // 2, D), u32),
        vm((3 * NG, D, 128), bf16),
        vm((NG, NG, 192, 128), u32),
        vm((D, D), bf16),
        vm((NG, D // 2, 128), u32),
        vm((2 * NG, D, 128), bf16),
        vm((2 * NG, 64, D), u32),
        vm((D, D), bf16),
        vm((NG, D // 2, 128), u32),
        vm((D, D), bf16),
        vm((NG, D // 2, 128), u32),
        vm((NG, 64, BLK), u32),
        vm((NG, 64, BLK), u32),
        vm((NG, 192, 128), u32),
        vm((BLK, D), u32),
        vm((384, 2 * BLK), f32),
        vm((NG, BLK, 128), u32),
        vm((NQT, D // 2, NQ), u32),
        vm((NG, S // 2, 128), u32),
        vm((NC, D // 2, MK), u32),
        vm((NG, S // 2, 128), u32),
        vm((64, NQ), u32),
        pltpu.SemaphoreType.DMA((N_SEM,)),
    ] + [vm((2 * MK, NQ), f32)] * NC + [
        vm((2, 128, BLK), f32), vm((2, 64, BLK), u32), vm((2, 64, BLK), u32)] * NG
    out = pl.pallas_call(
        _kernel,
        out_shape=jax.ShapeDtypeStruct((S, D), bf16),
        in_specs=[pl.BlockSpec(memory_space=pl.ANY)] * 5,
        out_specs=pl.BlockSpec(memory_space=pl.ANY),
        scratch_shapes=scratch,
        compiler_params=pltpu.CompilerParams(vmem_limit_bytes=110 * 1024 * 1024),
        name="interleave_attn",
    )(x, A_wqkv, A_wo, B_wqkv, B_wo)
    return out.reshape(1, S, D)
```

```python
import jax
import jax.numpy as jnp
from jax import lax
import jax.experimental.pallas as pl
import jax.experimental.pallas.tpu as pltpu

S, D, H, DH = 2048, 1024, 32, 32
W_LOC, DIL = 8, 2
EPS = 1e-5
LOG2E = 1.4426950408889634
QSCALE = (DH ** -0.5) * LOG2E
NEG = -1e9 * LOG2E

BLK = 128
NB = S // BLK
NG = D // 128
NQ = 256
NQT = S // NQ
MK = 128
NC = S // MK
DL = 6
APB = 2
GPB = 4
TB = 256
TF = 128
OPRE = 1
OPB = 3

SEM_X01, SEM_X2, SEM_WOB, SEM_OUT = 0, 1, 2, 3
SEM_WA = 4
SEM_IT = SEM_WA + NG
N_SEM = SEM_IT + 4

UCH = 2
L1S = (0, 0, 1, 1, 1, 2, 3, 4)
L2S = (4, 5, 6, 6, 7, 7, 8, 8)
WBSLOT = 6
WKSLOT = 2


bf16 = jnp.bfloat16
f32 = jnp.float32
u32 = jnp.uint32
NT = (((1,), (1,)), ((), ()))


def _pack(x):
    return pltpu.bitcast(x.astype(bf16), u32)


def _as_bf16(x):
    return pltpu.bitcast(x, bf16)


def _dot(a, b):
    return jnp.dot(a, b, preferred_element_type=f32)


def _dot_nt(a, b):
    return lax.dot_general(a, b, NT, preferred_element_type=f32)


def _token(v):
    t = pltpu.bitcast(v[0:8, :], u32)
    return lax.shift_right_logical(jnp.bitwise_and(t, jnp.uint32(0xFFFF)), jnp.uint32(16))


def _after(x, tok):
    n, m = x.shape
    z = jnp.concatenate([jnp.concatenate([tok] * (m // 128), axis=1)] * (n // 8), axis=0)
    return pltpu.bitcast(jnp.bitwise_or(pltpu.bitcast(x, u32), z), x.dtype)


def _ln16(x):
    mu = jnp.sum(x, axis=1, keepdims=True) * (1.0 / D)
    xc = x - mu
    var = jnp.sum(xc * xc, axis=1, keepdims=True) * (1.0 / D)
    return _pack(xc * lax.rsqrt(var + EPS))


def _tree(x, op):
    n = x.shape[0]
    while n > 1:
        n //= 2
        x = op(x[:n], x[n:])
    return x[0]


def _local_attention(q, kc, kp, vc, vp, pos):
    lane = lax.broadcasted_iota(jnp.int32, (UCH * 4, 128), 1)

    def shifted(cur, prev, u, w):
        rows = slice(u * UCH * 4, (u + 1) * UCH * 4)
        x = cur[rows]
        if w:
            x = jnp.where(lane >= 128 - DIL * w, prev[rows], x)
            x = pltpu.roll(x, DIL * w, axis=1)
        return _as_bf16(x).astype(f32).reshape(UCH, 8, 128)

    nu = 16 // UCH
    even = lax.broadcasted_iota(jnp.int32, (8, 128), 0) % 2 == 0
    acc = [None] * W_LOC
    for u in range(nu):
        qu = q[u * UCH * 8:(u + 1) * UCH * 8].reshape(UCH, 8, 128)
        for w in range(W_LOC):
            t = _tree(qu * shifted(kc, kp, u, w), jnp.add)
            acc[w] = t if acc[w] is None else acc[w] + t
    logits = []
    for w in range(W_LOC):
        t = acc[w]
        t = t + jnp.where(even, pltpu.roll(t, 7, axis=0), pltpu.roll(t, 1, axis=0))
        t = t * QSCALE
        if w:
            t = jnp.where(pos >= DIL * w, t, NEG)
        logits.append(t)
    m = logits[0]
    for t in logits[1:]:
        m = jnp.maximum(m, t)
    ps = [jnp.exp2(t - m) for t in logits]
    l = ps[0]
    for p in ps[1:]:
        l = l + p
    r = 1.0 / l
    ps = [(p * r)[None] for p in ps]
    outs = []
    for u in range(nu):
        o = None
        for w in range(W_LOC):
            t = shifted(vc, vp, u, w) * ps[w]
            o = t if o is None else o + t
        outs.append(o.reshape(UCH * 8, 128))
    return jnp.concatenate(outs, axis=0)


def _kernel(x_hbm, wa_hbm, woa_hbm, wb_hbm, wob_hbm, out_hbm,
            x_ref, xio, xn1a, xn1b, xn2, wa_nat, wat, woa, woap, wb_nat, wbt, wk, wkp, wob, wobp,
            khalo, vhalo, wstage, pxn, pbuf, po,
            qT, kN, vT, oN, otbuf,
            sem, *bufs):
    xn1 = (xn1a, xn1b)
    sbufs = bufs[:NC]
    stg = [bufs[NC + 3 * g:NC + 3 * g + 3] for g in range(NG)]

    def x_copy(i, sid):
        rows = pl.ds(i * BLK, BLK)
        return pltpu.make_async_copy(x_hbm.at[rows, :], xio.at[rows, :], sem.at[sid])

    def wa_copies(g):
        return [pltpu.make_async_copy(
            wa_hbm.at[:, pl.ds(pl.multiple_of(sec * D + g * 128, 128), 128)],
            wa_nat.at[g * 3 + sec], sem.at[SEM_WA + g]) for sec in range(3)]

    def wb_copy(c, sid):
        col = c * 128 + (c // 8) * D
        return pltpu.make_async_copy(
            wb_hbm.at[:, pl.ds(col, 128)], wb_nat.at[c], sem.at[sid])

    def wk_copy(c, sid):
        rows = pl.ds(c * 128, 128)
        return pltpu.make_async_copy(
            wb_hbm.at[rows, pl.ds(D, D)], wk.at[rows, :], sem.at[sid])

    def iter_copies(it):
        sid = SEM_IT + min(it, 3)
        if it == 0:
            cps = [pltpu.make_async_copy(woa_hbm, woa, sem.at[sid])]
        else:
            cps = [x_copy(i, sid) for i in (2 * it + 1, 2 * it + 2) if i < NB]
        return cps + [wb_copy(2 * it, sid), wb_copy(2 * it + 1, sid), wk_copy(it, sid)]

    x01_copies = [x_copy(0, SEM_X01), x_copy(1, SEM_X01)]
    x2_copy = x_copy(2, SEM_X2)
    wob_copy = pltpu.make_async_copy(wob_hbm, wob, sem.at[SEM_WOB])

    def out_copy(j):
        rows = pl.ds(pl.multiple_of(j * TF, TF), TF)
        return pltpu.make_async_copy(xio.at[rows, :], out_hbm.at[rows, :], sem.at[SEM_OUT])

    def blk_rows(i, n=BLK):
        return pl.ds(pl.multiple_of(i * n, n), n)

    def qkv_group(g, xn):
        w = jnp.concatenate([wat[g, kt] for kt in range(NG)], axis=1)
        q, k, v = [_dot_nt(_as_bf16(w[a:a + 64]), xn) for a in (0, 64, 128)]
        return q, _pack(k), _pack(v)

    def o_rows(i, n):
        rows = blk_rows(i, n // 2)
        return _as_bf16(jnp.concatenate([oN[t, rows, :] for t in range(NG)], axis=1))

    def proj_residual(o, w_cols, xv):
        cols = []
        for n in range(2):
            cols.append(xv[:, n * 512:(n + 1) * 512] + _dot(o, w_cols(n)))
        return jnp.concatenate(cols, axis=1)

    def packed_cols(w_ref):
        return lambda n: _as_bf16(
            jnp.concatenate([w_ref[4 * n + t] for t in range(4)], axis=1))

    woa_cols, wob_cols, wk_cols = packed_cols(woap), packed_cols(wobp), packed_cols(wkp)

    def repack(dst_ref, src_ref, c, n, tok=None):
        wv = pltpu.bitcast(src_ref[blk_rows(c, n), :], u32)
        if tok is not None:
            wv = _after(wv, tok)
        for t in range(NG):
            dst_ref[t, blk_rows(c, n // 2), :] = wv[:, t * 128:(t + 1) * 128]

    def store_permuted(dst_ref, row0, val):
        for h in range(4):
            dst_ref[pl.ds(row0 + h, 16, stride=4), :] = val[h * 16:(h + 1) * 16]

    def rows16(blk, r):
        return pl.ds(pl.multiple_of(blk * BLK + r * 16, 16), 16)

    def ln1(blk, r, tok=None):
        xv = xio[rows16(blk, r), :].astype(f32)
        return _ln16(xv if tok is None else _after(xv, tok))

    def ln2(blk, r, tok=None):
        xv = x_ref[rows16(blk, r), :]
        xn2[pl.ds(pl.multiple_of(blk * (BLK // 2) + r * 8, 8), 8), :] = _ln16(
            xv if tok is None else _after(xv, tok))

    def stage(g, slot, qkv):
        for ref, val in zip(stg[g], qkv):
            ref[slot] = val

    def a_block(i, par):
        ip = jnp.maximum(i - 1, 0)
        inx = jnp.minimum(i + 1, NB - 1)
        pos = i * BLK + lax.broadcasted_iota(jnp.int32, (8, 128), 1)

        def side_jobs(slot, src):
            if slot not in L1S + L2S + (WBSLOT, WKSLOT):
                return
            tok = _token(src)
            if slot == WBSLOT:
                wsrc = _as_bf16(_after(pltpu.bitcast(wb_nat[i], u32), tok))
                wbt[i] = pltpu.bitcast(wsrc.T, u32)
            if slot == WKSLOT:
                repack(wkp, wk, i, 64, tok)
            for r in range(8):
                if L1S[r] == slot:
                    xn1[1 - par][r * 8:(r + 1) * 8, :] = ln1(inx, r, tok)
            for r in range(8):
                if L2S[r] == slot:
                    ln2(ip, r, tok)

        o_cols = []
        for g in range(NG):
            if g:
                stage(g, par, qkv_group(g, _as_bf16(xn1[par][...])))
            qs, ks, vs = stg[g]
            ot = _local_attention(qs[par], ks[par], ks[1 - par], vs[par], vs[1 - par], pos)
            o_cols.append(ot.astype(bf16).T)
            side_jobs(g, ot[120:128])
        qkv = qkv_group(0, _as_bf16(xn1[1 - par][...]))
        stage(0, 1 - par, qkv)
        side_jobs(NG, qkv[1])
        rows = blk_rows(i)
        x_ref[rows, :] = proj_residual(
            jnp.concatenate(o_cols, axis=1), woa_cols, xio[rows, :].astype(f32))

    def startup():
        def transpose_wa(g):
            for sec in range(3):
                wv = pltpu.bitcast(wa_nat[g * 3 + sec].T, u32)
                for kt in range(NG):
                    store_permuted(wstage.at[kt], sec * 64, wv[:, kt * 128:(kt + 1) * 128])

        def project(g):
            w = wstage[...]
            wat[g] = w
            w = jnp.concatenate([w[kt] for kt in range(NG)], axis=1)
            return _dot_nt(_as_bf16(w), _as_bf16(pxn[...]))

        def attend(g, r):
            pos = lax.broadcasted_iota(jnp.int32, (8, 128), 1)
            kp = vp = jnp.zeros((64, BLK), u32)
            for b in range(2):
                rb = r[:, b * BLK:(b + 1) * BLK]
                kc = _pack(rb[128:256])
                vc = _pack(rb[256:384])
                ot = _local_attention(rb[0:128], kc, kp, vc, vp, pos + b * BLK)
                po[g, b * 64:(b + 1) * 64, :] = pltpu.bitcast(ot.astype(bf16).T, u32)
                kp, vp = kc, vc
            khalo[g] = kp
            vhalo[g] = vp

        pbuf[...] = jnp.zeros(pbuf.shape, f32)

        def zero_scores(k, c):
            for sb in sbufs:
                sb[blk_rows(k, 32), :] = jnp.zeros((32, NQ), f32)
            return c
        lax.fori_loop(0, 2 * MK // 32, zero_scores, 0)
        for cp in x01_copies:
            cp.wait()
        for b in range(2):
            for r in range(BLK // 16):
                pxn[b * 64 + r * 8:b * 64 + (r + 1) * 8, :] = ln1(b, r)
        for cp in wa_copies(0):
            cp.wait()
        transpose_wa(0)

        def body(g, c):
            for cp in wa_copies(g + 1):
                cp.wait()
            prev = pbuf[...]
            pbuf[...] = project(g)
            transpose_wa(g + 1)
            attend(jnp.maximum(g - 1, 0), prev)
            return c
        lax.fori_loop(0, NG - 1, body, 0)

        x2_copy.wait()
        prev = pbuf[...]
        r = project(NG - 1)
        xn_next = jnp.concatenate([ln1(2, r16) for r16 in range(BLK // 16)], axis=0)
        xn1[0][...] = xn_next
        attend(NG - 2, _after(prev, _token(xn_next[56:64, 0:128])))
        stage(0, 0, qkv_group(0, _as_bf16(xn_next)))
        attend(NG - 1, r)

        for cp in iter_copies(0):
            cp.wait()
        for t in range(NG):
            wv = pltpu.bitcast(woa[:, t * 128:(t + 1) * 128], u32)
            for g in range(NG):
                store_permuted(woap.at[t], g * 64, wv[g * 64:(g + 1) * 64])
        for b in range(2):
            o = jnp.concatenate([po[g, b * 64:(b + 1) * 64, :] for g in range(NG)], axis=1)
            rows = blk_rows(b)
            x_ref[rows, :] = proj_residual(_as_bf16(o), woa_cols, xio[rows, :].astype(f32))
            wbt[b] = pltpu.bitcast(wb_nat[b].T, u32)
        repack(wkp, wk, 0, 128)
        for r16 in range(BLK // 16):
            ln2(0, r16)
        for g in range(NG):
            stg[g][1][1] = khalo[g]
            stg[g][2][1] = vhalo[g]
        for cp in iter_copies(1):
            cp.wait()

    def phase_a(rep):
        @pl.when(rep == 1)
        def _():
            for g in range(NG):
                for ref in stg[g][1:]:
                    ref[1] = jnp.zeros((64, BLK), u32)
            xn_first = jnp.concatenate([ln1(0, r) for r in range(BLK // 16)], axis=0)
            xn1[0][...] = xn_first
            stage(0, 0, qkv_group(0, _as_bf16(xn_first)))

        def body(it, c):
            @pl.when(it == 2 - rep * NB)
            def _():
                for cp in iter_copies(2):
                    cp.wait()

            @pl.when(it == 3 - rep * NB)
            def _():
                for k in range(3, NB // APB):
                    for cp in iter_copies(k):
                        cp.wait()

            for u in range(APB):
                a_block(it * APB + u, u % 2)
            return c
        lax.fori_loop(1 - rep, NB // APB, body, 0)
        for r in range(BLK // 16):
            ln2(NB - 1, r)

    def phase_b_proj():
        def body(j, c):
            rows = blk_rows(j, TB // 2)
            xn = _as_bf16(xn2[rows, :])
            for n in range(2):
                y = _pack(_dot(xn, wk_cols(n)))
                for t in range(4):
                    kN[4 * n + t, rows, :] = y[:, t * 128:(t + 1) * 128]
            for r in range(4):
                w = _as_bf16(wbt[2 * r:2 * r + 2].reshape(128, D))
                y = _pack(_dot_nt(w, xn) * QSCALE)
                for b in range(TB // NQ):
                    qT[j * (TB // NQ) + b, r * 128:(r + 1) * 128, :] = y[:, b * NQ:(b + 1) * NQ]
            for r in range(4):
                w = _as_bf16(wbt[8 + 2 * r:8 + 2 * r + 2].reshape(128, D))
                y = _pack(_dot_nt(w, xn))
                for b in range(TB // MK):
                    vT[j * (TB // MK) + b, r * 128:(r + 1) * 128, :] = y[:, b * MK:(b + 1) * MK]
            return c
        lax.fori_loop(0, S // TB, body, 0)

    def flush_o(g, val):
        y = pltpu.bitcast(_as_bf16(val).T, u32)
        oN[g % NG, blk_rows(g // NG, NQ // 2), :] = y

    def phase_b_attn(rep):
        off = [0, 0]

        def qm_of(t, qi, j):
            q = _as_bf16(qT[qi, pl.ds(pl.multiple_of(t * 64 + j * 16, 16), 16), :])
            parts = []
            if j > 0:
                parts.append(jnp.zeros((32 * j, NQ), bf16))
            parts.append(q)
            if j < 3:
                parts.append(jnp.zeros((32 * (3 - j), NQ), bf16))
            return jnp.concatenate(parts, axis=0)

        def qk_chunk(t, qm, c, par, m):
            k = _as_bf16(kN[t, c * (MK // 2):(c + 1) * (MK // 2), :])
            s = _dot(k, qm)
            sbufs[c][pl.ds(pl.multiple_of(off[0] + par * MK, 8), MK), :] = s
            sm = _tree(s.reshape(MK // 8, 8, NQ), jnp.maximum)
            return sm if m is None else jnp.maximum(m, sm)

        def pv_chunk(h, c, par, mrow, l, o):
            s = sbufs[c][pl.ds(pl.multiple_of(off[1] + par * MK, 8), MK), :]
            p = jnp.exp2(s - mrow)
            ls = jnp.sum(p.reshape(MK // 8, 8, NQ), axis=0)
            l = ls if l is None else l + ls
            v = _as_bf16(vT[c, pl.ds(pl.multiple_of(h * 16, 16), 16), :])
            oc = _dot(v, p.astype(bf16))
            o = oc if o is None else o + oc
            return l, o

        n_groups = NQT * NG
        lag = NC + DL
        n_steps = 4 * NC

        def set_offsets(zero):
            off[0] = lax.shift_right_logical(zero, 16) * 8
            off[1] = lax.shift_right_logical(zero, 17) * 8

        def pv_step(g, n, ms, st, flush=True):
            j, c = divmod(n, NC)
            l, o, mrow = st
            if c == 0:
                mrow = jnp.max(ms[j], axis=0, keepdims=True)
                l = o = None
            l, o = pv_chunk((g % NG) * 4 + j, c, j % 2, mrow, l, o)
            if c == NC - 1:
                lrow = jnp.sum(l, axis=0, keepdims=True)
                otbuf[j * 16:(j + 1) * 16, :] = _pack(o * (1.0 / lrow))
                if j == 3 and flush:
                    flush_o(g, otbuf[...])
            return l, o, mrow

        def group(g, g_prev, carry, side_job=None):
            st, ms_prev = carry[:3], {3: carry[3]}
            ms = {}
            for n in range(n_steps):
                j, c = divmod(n, NC)
                if c == 0:
                    qm = qm_of(g % NG, g // NG, j)
                ms[j] = qk_chunk(g % NG, qm, c, j % 2, ms.get(j))
                if n < lag:
                    st = pv_step(g_prev, n + n_steps - lag, ms_prev, st)
                else:
                    st = pv_step(g, n - lag, ms, st)
                if side_job is not None and n == n_steps // 2:
                    side_job(_token(st[0][:, 0:128]))
            return st + (ms[3],)

        def body(it, carry):
            def side_job(tok):
                repack(wobp, wob, it, D * GPB // n_groups, tok)

            set_offsets(it)
            carry = carry[:4]
            for u in range(GPB):
                g = it * GPB + u
                carry = group(g, jnp.maximum(g - 1, 0), carry, side_job if u == 0 else None)
            return carry + (it,)

        otbuf[...] = jnp.zeros(otbuf.shape, u32)
        init = (jnp.zeros((8, NQ), f32), jnp.zeros((DH, NQ), f32),
                jnp.zeros((1, NQ), f32), jnp.zeros((8, NQ), f32), jnp.int32(0))
        carry = lax.fori_loop(0, n_groups // GPB, body, init)
        set_offsets(carry[4])
        st, ms = carry[:3], {3: carry[3]}
        o0 = o_rows(0, TF)
        done = 0
        for k, n in enumerate(range(n_steps - lag, n_steps)):
            while done < NG and done * lag <= k * NG:
                cols = slice(done * 128, (done + 1) * 128)
                y = x_ref[0:TF, cols] + _dot(o0, _as_bf16(wobp[done]))
                xio[0:TF, cols] = y.astype(bf16)
                done += 1
            st = pv_step(n_groups - 1, n, ms, st, False)

        @pl.when(rep == 1)
        def _():
            out_copy(0).start()
        off[0] = off[1] = 0

    def out_tile(j, rep):
        rows = blk_rows(j, TF)
        xv = proj_residual(o_rows(j, TF), wob_cols, x_ref[rows, :])
        xio[rows, :] = xv.astype(bf16)

        @pl.when(rep == 1)
        def _():
            out_copy(j).start()

    def phase_b_out(rep):
        def body(jj, c):
            for u in range(OPB):
                out_tile(OPRE + jj * OPB + u, rep)
            flush_o(NQT * NG - 1, otbuf[...])
            return c
        lax.fori_loop(0, (S // TF - OPRE) // OPB, body, 0)

    for cp in x01_copies:
        cp.start()
    for g in range(NG):
        if g == NG - 2:
            x2_copy.start()
        for cp in wa_copies(g):
            cp.start()
    for it in range(NB // APB):
        for cp in iter_copies(it):
            cp.start()
    wob_copy.start()

    startup()

    def layer_pair(rep, c):
        phase_a(rep)

        @pl.when(rep == 0)
        def _():
            wob_copy.wait()

        phase_b_proj()
        phase_b_attn(rep)
        phase_b_out(rep)
        return c
    lax.fori_loop(0, 2, layer_pair, 0)
    for j in range(S // TF):
        out_copy(j).wait()


@jax.jit
def pallas_interleave_layers__sliding_local_dilated__softmax_full_mha__prompt_kernel(
    A_x: jax.Array,
    A_wqkv: jax.Array,
    A_wo: jax.Array,
    B_x: jax.Array,
    B_wqkv: jax.Array,
    B_wo: jax.Array,
):
    del B_x
    x = A_x.reshape(S, D)
    vm = pltpu.VMEM
    scratch = [
        vm((S, D), f32),
        vm((S, D), bf16),
        vm((BLK // 2, D), u32),
        vm((BLK // 2, D), u32),
        vm((S // 2, D), u32),
        vm((3 * NG, D, 128), bf16),
        vm((NG, NG, 192, 128), u32),
        vm((D, D), bf16),
        vm((NG, D // 2, 128), u32),
        vm((2 * NG, D, 128), bf16),
        vm((2 * NG, 64, D), u32),
        vm((D, D), bf16),
        vm((NG, D // 2, 128), u32),
        vm((D, D), bf16),
        vm((NG, D // 2, 128), u32),
        vm((NG, 64, BLK), u32),
        vm((NG, 64, BLK), u32),
        vm((NG, 192, 128), u32),
        vm((BLK, D), u32),
        vm((384, 2 * BLK), f32),
        vm((NG, BLK, 128), u32),
        vm((NQT, D // 2, NQ), u32),
        vm((NG, S // 2, 128), u32),
        vm((NC, D // 2, MK), u32),
        vm((NG, S // 2, 128), u32),
        vm((64, NQ), u32),
        pltpu.SemaphoreType.DMA((N_SEM,)),
    ] + [vm((2 * MK, NQ), f32)] * NC + [
        vm((2, 128, BLK), f32), vm((2, 64, BLK), u32), vm((2, 64, BLK), u32)] * NG
    out = pl.pallas_call(
        _kernel,
        out_shape=jax.ShapeDtypeStruct((S, D), bf16),
        in_specs=[pl.BlockSpec(memory_space=pl.ANY)] * 5,
        out_specs=pl.BlockSpec(memory_space=pl.ANY),
        scratch_shapes=scratch,
        compiler_params=pltpu.CompilerParams(vmem_limit_bytes=110 * 1024 * 1024),
        name="interleave_attn",
    )(x, A_wqkv, A_wo, B_wqkv, B_wo)
    return out.reshape(1, S, D)
```

```python
import jax
import jax.numpy as jnp
from jax import lax
import jax.experimental.pallas as pl
import jax.experimental.pallas.tpu as pltpu

S, D, H, DH = 2048, 1024, 32, 32
W_LOC, DIL = 8, 2
EPS = 1e-5
LOG2E = 1.4426950408889634
QSCALE = (DH ** -0.5) * LOG2E
NEG = -1e9 * LOG2E

BLK = 128
NB = S // BLK
NG = D // 128
NQ = 256
NQT = S // NQ
MK = 128
NC = S // MK
DL = 6
APB = 2
GPB = 4
TB = 256
TF = 128
OPRE = 1
OPB = 3

SEM_X01, SEM_X2, SEM_WOB, SEM_OUT = 0, 1, 2, 3
SEM_WA = 4
SEM_IT = SEM_WA + NG
N_SEM = SEM_IT + 4

UCH = 2
L1S = (0, 0, 1, 2, 2, 3, 4, 4)
L2S = (7, 8)
WBSLOT = 3
WKSLOT = 7
L2BS = (10, 0, 4, 9, 8, 5, 2, 5, 4, 8, 3, 6, 2, 1, 9, 7)


bf16 = jnp.bfloat16
f32 = jnp.float32
u32 = jnp.uint32
NT = (((1,), (1,)), ((), ()))


def _pack(x):
    return pltpu.bitcast(x.astype(bf16), u32)


def _as_bf16(x):
    return pltpu.bitcast(x, bf16)


def _dot(a, b):
    return jnp.dot(a, b, preferred_element_type=f32)


def _dot_nt(a, b):
    return lax.dot_general(a, b, NT, preferred_element_type=f32)


def _token(v):
    t = pltpu.bitcast(v[0:8, :], u32)
    return lax.shift_right_logical(jnp.bitwise_and(t, jnp.uint32(0xFFFF)), jnp.uint32(16))


def _after(x, tok):
    n, m = x.shape
    z = jnp.concatenate([jnp.concatenate([tok] * (m // 128), axis=1)] * (n // 8), axis=0)
    return pltpu.bitcast(jnp.bitwise_or(pltpu.bitcast(x, u32), z), x.dtype)


def _ln16(x):
    mu = jnp.sum(x, axis=1, keepdims=True) * (1.0 / D)
    xc = x - mu
    var = jnp.sum(xc * xc, axis=1, keepdims=True) * (1.0 / D)
    return _pack(xc * lax.rsqrt(var + EPS))


def _tree(x, op):
    n = x.shape[0]
    while n > 1:
        n //= 2
        x = op(x[:n], x[n:])
    return x[0]


def _local_attention(q, kc, kp, vc, vp, pos):
    lane = lax.broadcasted_iota(jnp.int32, (UCH * 4, 128), 1)

    def shifted(cur, prev, u, w):
        rows = slice(u * UCH * 4, (u + 1) * UCH * 4)
        x = cur[rows]
        if w:
            x = jnp.where(lane >= 128 - DIL * w, prev[rows], x)
            x = pltpu.roll(x, DIL * w, axis=1)
        return _as_bf16(x).astype(f32).reshape(UCH, 8, 128)

    nu = 16 // UCH
    even = lax.broadcasted_iota(jnp.int32, (8, 128), 0) % 2 == 0
    acc = [None] * W_LOC
    for u in range(nu):
        qu = q[u * UCH * 8:(u + 1) * UCH * 8].reshape(UCH, 8, 128)
        for w in range(W_LOC):
            t = _tree(qu * shifted(kc, kp, u, w), jnp.add)
            acc[w] = t if acc[w] is None else acc[w] + t
    logits = []
    for w in range(W_LOC):
        t = acc[w]
        t = t + jnp.where(even, pltpu.roll(t, 7, axis=0), pltpu.roll(t, 1, axis=0))
        t = t * QSCALE
        if w:
            t = jnp.where(pos >= DIL * w, t, NEG)
        logits.append(t)
    m = logits[0]
    for t in logits[1:]:
        m = jnp.maximum(m, t)
    ps = [jnp.exp2(t - m) for t in logits]
    l = ps[0]
    for p in ps[1:]:
        l = l + p
    r = 1.0 / l
    ps = [(p * r)[None] for p in ps]
    outs = []
    for u in range(nu):
        o = None
        for w in range(W_LOC):
            t = shifted(vc, vp, u, w) * ps[w]
            o = t if o is None else o + t
        outs.append(o.reshape(UCH * 8, 128))
    return jnp.concatenate(outs, axis=0)


def _kernel(x_hbm, wa_hbm, woa_hbm, wb_hbm, wob_hbm, out_hbm,
            x_ref, xio, xn1a, xn1b, xn2, wa_nat, wat, woa, woap, wb_nat, wbt, wk, wkp, wob, wobp,
            khalo, vhalo, wstage, pbuf, po,
            qT, kN, vT, oN, otbuf,
            sem, *bufs):
    xn1 = (xn1a, xn1b)
    sbufs = bufs[:NC]
    stg = [bufs[NC + 3 * g:NC + 3 * g + 3] for g in range(NG)]

    def x_copy(i, sid):
        rows = pl.ds(i * BLK, BLK)
        return pltpu.make_async_copy(x_hbm.at[rows, :], xio.at[rows, :], sem.at[sid])

    def wa_copies(g):
        return [pltpu.make_async_copy(
            wa_hbm.at[:, pl.ds(pl.multiple_of(sec * D + g * 128, 128), 128)],
            wa_nat.at[g * 3 + sec], sem.at[SEM_WA + g]) for sec in range(3)]

    def wb_copy(c, sid):
        col = c * 128 + (c // 8) * D
        return pltpu.make_async_copy(
            wb_hbm.at[:, pl.ds(col, 128)], wb_nat.at[c], sem.at[sid])

    def wk_copy(c, sid):
        rows = pl.ds(c * 128, 128)
        return pltpu.make_async_copy(
            wb_hbm.at[rows, pl.ds(D, D)], wk.at[rows, :], sem.at[sid])

    def iter_copies(it):
        sid = SEM_IT + min(it, 3)
        if it == 0:
            cps = [pltpu.make_async_copy(woa_hbm, woa, sem.at[sid])]
        else:
            cps = [x_copy(i, sid) for i in (2 * it + 1, 2 * it + 2) if i < NB]
        return cps + [wb_copy(2 * it, sid), wb_copy(2 * it + 1, sid), wk_copy(it, sid)]

    x01_copies = [x_copy(0, SEM_X01), x_copy(1, SEM_X01)]
    x2_copy = x_copy(2, SEM_X2)
    wob_copy = pltpu.make_async_copy(wob_hbm, wob, sem.at[SEM_WOB])

    def out_copy(j):
        rows = pl.ds(pl.multiple_of(j * TF, TF), TF)
        return pltpu.make_async_copy(xio.at[rows, :], out_hbm.at[rows, :], sem.at[SEM_OUT])

    def blk_rows(i, n=BLK):
        return pl.ds(pl.multiple_of(i * n, n), n)

    def qkv_group(g, xn):
        w = jnp.concatenate([wat[g, kt] for kt in range(NG)], axis=1)
        q, k, v = [_dot_nt(_as_bf16(w[a:a + 64]), xn) for a in (0, 64, 128)]
        return q, _pack(k), _pack(v)

    def o_rows(i, n):
        rows = blk_rows(i, n // 2)
        return _as_bf16(jnp.concatenate([oN[t, rows, :] for t in range(NG)], axis=1))

    def proj_residual(o, w_cols, xv):
        cols = []
        for n in range(2):
            cols.append(xv[:, n * 512:(n + 1) * 512] + _dot(o, w_cols(n)))
        return jnp.concatenate(cols, axis=1)

    def packed_cols(w_ref):
        return lambda n: _as_bf16(
            jnp.concatenate([w_ref[4 * n + t] for t in range(4)], axis=1))

    woa_cols, wob_cols, wk_cols = packed_cols(woap), packed_cols(wobp), packed_cols(wkp)

    def repack(dst_ref, src_ref, c, n, tok=None):
        wv = pltpu.bitcast(src_ref[blk_rows(c, n), :], u32)
        if tok is not None:
            wv = _after(wv, tok)
        for t in range(NG):
            dst_ref[t, blk_rows(c, n // 2), :] = wv[:, t * 128:(t + 1) * 128]

    def store_permuted(dst_ref, row0, val):
        for h in range(4):
            dst_ref[pl.ds(row0 + h, 16, stride=4), :] = val[h * 16:(h + 1) * 16]

    def rows16(blk, r):
        return pl.ds(pl.multiple_of(blk * BLK + r * 16, 16), 16)

    def ln1(blk, r, tok=None):
        xv = xio[rows16(blk, r), :].astype(f32)
        return _ln16(xv if tok is None else _after(xv, tok))

    def ln2(tile, r, tok):
        xv = x_ref[pl.ds(pl.multiple_of(tile * TB + r * 16, 16), 16), :]
        xn2[pl.ds(pl.multiple_of(r * 8, 8), 8), :] = _ln16(_after(xv, tok))

    def stage(g, slot, qkv):
        for ref, val in zip(stg[g], qkv):
            ref[slot] = val

    def a_block(i, par):
        inx = jnp.minimum(i + 1, NB - 1)
        pos = i * BLK + lax.broadcasted_iota(jnp.int32, (8, 128), 1)

        def side_jobs(slot, src):
            if slot not in L1S + L2S + (WBSLOT, WKSLOT):
                return
            tok = _token(src)
            if slot == WBSLOT:
                wsrc = _as_bf16(_after(pltpu.bitcast(wb_nat[i], u32), tok))
                wbt[i] = pltpu.bitcast(wsrc.T, u32)
            if slot == WKSLOT:
                repack(wkp, wk, i, 64, tok)
            for r in range(8):
                if L1S[r] == slot:
                    xn1[1 - par][r * 8:(r + 1) * 8, :] = ln1(inx, r, tok)
            for e in range(2):
                if L2S[e] == slot:
                    ln2(0, 2 * jnp.clip(i - 2, 0, TB // 32 - 1) + e, tok)

        o_cols = []
        for g in range(NG):
            if g:
                stage(g, par, qkv_group(g, _as_bf16(xn1[par][...])))
            qs, ks, vs = stg[g]
            ot = _local_attention(qs[par], ks[par], ks[1 - par], vs[par], vs[1 - par], pos)
            o_cols.append(ot.astype(bf16).T)
            side_jobs(g, ot[120:128])
        qkv = qkv_group(0, _as_bf16(xn1[1 - par][...]))
        stage(0, 1 - par, qkv)
        side_jobs(NG, qkv[1])
        rows = blk_rows(i)
        x_ref[rows, :] = proj_residual(
            jnp.concatenate(o_cols, axis=1), woa_cols, xio[rows, :].astype(f32))

    def startup():
        def transpose_wa(g):
            for sec in range(3):
                wv = pltpu.bitcast(wa_nat[g * 3 + sec].T, u32)
                for kt in range(NG):
                    store_permuted(wstage.at[kt], sec * 64, wv[:, kt * 128:(kt + 1) * 128])

        def project(g):
            w = wstage[...]
            wat[g] = w
            w = jnp.concatenate([w[kt] for kt in range(NG)], axis=1)
            return _dot_nt(_as_bf16(w), _as_bf16(xn2[...]))

        def attend(g, r):
            pos = lax.broadcasted_iota(jnp.int32, (8, 128), 1)
            kp = vp = jnp.zeros((64, BLK), u32)
            for b in range(2):
                rb = r[:, b * BLK:(b + 1) * BLK]
                kc = _pack(rb[128:256])
                vc = _pack(rb[256:384])
                ot = _local_attention(rb[0:128], kc, kp, vc, vp, pos + b * BLK)
                po[g, b * 64:(b + 1) * 64, :] = pltpu.bitcast(ot.astype(bf16).T, u32)
                kp, vp = kc, vc
            khalo[g] = kp
            vhalo[g] = vp

        pbuf[...] = jnp.zeros(pbuf.shape, f32)

        def zero_scores(k, c):
            for sb in sbufs:
                sb[blk_rows(k, 32), :] = jnp.zeros((32, NQ), f32)
            return c
        lax.fori_loop(0, 2 * MK // 32, zero_scores, 0)
        for cp in x01_copies:
            cp.wait()
        for b in range(2):
            for r in range(BLK // 16):
                xn2[b * 64 + r * 8:b * 64 + (r + 1) * 8, :] = ln1(b, r)
        for cp in wa_copies(0):
            cp.wait()
        transpose_wa(0)

        def body(g, c):
            for cp in wa_copies(g + 1):
                cp.wait()
            prev = pbuf[...]
            pbuf[...] = project(g)
            transpose_wa(g + 1)
            attend(jnp.maximum(g - 1, 0), prev)
            return c
        lax.fori_loop(0, NG - 1, body, 0)

        x2_copy.wait()
        prev = pbuf[...]
        r = project(NG - 1)
        xn_next = jnp.concatenate([ln1(2, r16) for r16 in range(BLK // 16)], axis=0)
        xn1[0][...] = xn_next
        attend(NG - 2, _after(prev, _token(xn_next[56:64, 0:128])))
        stage(0, 0, qkv_group(0, _as_bf16(xn_next)))
        attend(NG - 1, r)

        for cp in iter_copies(0):
            cp.wait()
        for t in range(NG):
            wv = pltpu.bitcast(woa[:, t * 128:(t + 1) * 128], u32)
            for g in range(NG):
                store_permuted(woap.at[t], g * 64, wv[g * 64:(g + 1) * 64])
        for b in range(2):
            o = jnp.concatenate([po[g, b * 64:(b + 1) * 64, :] for g in range(NG)], axis=1)
            rows = blk_rows(b)
            x_ref[rows, :] = proj_residual(_as_bf16(o), woa_cols, xio[rows, :].astype(f32))
            wbt[b] = pltpu.bitcast(wb_nat[b].T, u32)
        repack(wkp, wk, 0, 128)
        for g in range(NG):
            stg[g][1][1] = khalo[g]
            stg[g][2][1] = vhalo[g]
        for cp in iter_copies(1):
            cp.wait()

    def phase_a(rep):
        @pl.when(rep == 1)
        def _():
            for g in range(NG):
                for ref in stg[g][1:]:
                    ref[1] = jnp.zeros((64, BLK), u32)
            xn_first = jnp.concatenate([ln1(0, r) for r in range(BLK // 16)], axis=0)
            xn1[0][...] = xn_first
            stage(0, 0, qkv_group(0, _as_bf16(xn_first)))

        def body(it, c):
            @pl.when(it == 2 - rep * NB)
            def _():
                for cp in iter_copies(2):
                    cp.wait()

            @pl.when(it == 3 - rep * NB)
            def _():
                for k in range(3, NB // APB):
                    for cp in iter_copies(k):
                        cp.wait()

            for u in range(APB):
                a_block(it * APB + u, u % 2)
            return c
        lax.fori_loop(1 - rep, NB // APB, body, 0)

    def phase_b_proj():
        def body(j, c):
            rows = blk_rows(j, TB // 2)
            xn = _as_bf16(xn2[...])
            toks = []
            for n in range(2):
                y = _pack(_dot(xn, wk_cols(n)))
                for t in range(4):
                    kN[4 * n + t, rows, :] = y[:, t * 128:(t + 1) * 128]
                toks += [y[:, 0:128], y[:, 256:384]]
            for r in range(4):
                w = _as_bf16(wbt[2 * r:2 * r + 2].reshape(128, D))
                y = _pack(_dot_nt(w, xn) * QSCALE)
                for b in range(TB // NQ):
                    qT[j * (TB // NQ) + b, r * 128:(r + 1) * 128, :] = y[:, b * NQ:(b + 1) * NQ]
                toks.append(y[:, 0:128])
            for r in range(4):
                w = _as_bf16(wbt[8 + 2 * r:8 + 2 * r + 2].reshape(128, D))
                y = _pack(_dot_nt(w, xn))
                for b in range(TB // MK):
                    vT[j * (TB // MK) + b, r * 128:(r + 1) * 128, :] = y[:, b * MK:(b + 1) * MK]
                toks.append(y[:, 0:128])
            jn = jnp.minimum(j + 1, S // TB - 1)
            for r in range(TB // 16):
                ln2(jn, r, _token(toks[L2BS[r]]))
            return c
        lax.fori_loop(0, S // TB, body, 0)

    def flush_o(g, val):
        y = pltpu.bitcast(_as_bf16(val).T, u32)
        oN[g % NG, blk_rows(g // NG, NQ // 2), :] = y

    def phase_b_attn(rep):
        off = [0, 0]

        def qm_of(t, qi, j):
            q = _as_bf16(qT[qi, pl.ds(pl.multiple_of(t * 64 + j * 16, 16), 16), :])
            parts = []
            if j > 0:
                parts.append(jnp.zeros((32 * j, NQ), bf16))
            parts.append(q)
            if j < 3:
                parts.append(jnp.zeros((32 * (3 - j), NQ), bf16))
            return jnp.concatenate(parts, axis=0)

        def qk_chunk(t, qm, c, par, m):
            k = _as_bf16(kN[t, c * (MK // 2):(c + 1) * (MK // 2), :])
            s = _dot(k, qm)
            sbufs[c][pl.ds(pl.multiple_of(off[0] + par * MK, 8), MK), :] = s
            sm = _tree(s.reshape(MK // 8, 8, NQ), jnp.maximum)
            return sm if m is None else jnp.maximum(m, sm)

        def pv_chunk(h, c, par, mrow, l, o):
            s = sbufs[c][pl.ds(pl.multiple_of(off[1] + par * MK, 8), MK), :]
            p = jnp.exp2(s - mrow)
            ls = jnp.sum(p.reshape(MK // 8, 8, NQ), axis=0)
            l = ls if l is None else l + ls
            v = _as_bf16(vT[c, pl.ds(pl.multiple_of(h * 16, 16), 16), :])
            oc = _dot(v, p.astype(bf16))
            o = oc if o is None else o + oc
            return l, o

        n_groups = NQT * NG
        lag = NC + DL
        n_steps = 4 * NC

        def set_offsets(zero):
            off[0] = lax.shift_right_logical(zero, 16) * 8
            off[1] = lax.shift_right_logical(zero, 17) * 8

        def pv_step(g, n, ms, st, flush=True):
            j, c = divmod(n, NC)
            l, o, mrow = st
            if c == 0:
                mrow = jnp.max(ms[j], axis=0, keepdims=True)
                l = o = None
            l, o = pv_chunk((g % NG) * 4 + j, c, j % 2, mrow, l, o)
            if c == NC - 1:
                lrow = jnp.sum(l, axis=0, keepdims=True)
                otbuf[j * 16:(j + 1) * 16, :] = _pack(o * (1.0 / lrow))
                if j == 3 and flush:
                    flush_o(g, otbuf[...])
            return l, o, mrow

        def group(g, g_prev, carry, side_job=None):
            st, ms_prev = carry[:3], {3: carry[3]}
            ms = {}
            for n in range(n_steps):
                j, c = divmod(n, NC)
                if c == 0:
                    qm = qm_of(g % NG, g // NG, j)
                ms[j] = qk_chunk(g % NG, qm, c, j % 2, ms.get(j))
                if n < lag:
                    st = pv_step(g_prev, n + n_steps - lag, ms_prev, st)
                else:
                    st = pv_step(g, n - lag, ms, st)
                if side_job is not None and n == n_steps // 2:
                    side_job(_token(st[0][:, 0:128]))
            return st + (ms[3],)

        def body(it, carry):
            def side_job(tok):
                repack(wobp, wob, it, D * GPB // n_groups, tok)

            set_offsets(it)
            carry = carry[:4]
            for u in range(GPB):
                g = it * GPB + u
                carry = group(g, jnp.maximum(g - 1, 0), carry, side_job if u == 0 else None)
            return carry + (it,)

        otbuf[...] = jnp.zeros(otbuf.shape, u32)
        init = (jnp.zeros((8, NQ), f32), jnp.zeros((DH, NQ), f32),
                jnp.zeros((1, NQ), f32), jnp.zeros((8, NQ), f32), jnp.int32(0))
        carry = lax.fori_loop(0, n_groups // GPB, body, init)
        set_offsets(carry[4])
        st, ms = carry[:3], {3: carry[3]}
        o0 = o_rows(0, TF)
        done = 0
        for k, n in enumerate(range(n_steps - lag, n_steps)):
            while done < NG and done * lag <= k * NG:
                cols = slice(done * 128, (done + 1) * 128)
                y = x_ref[0:TF, cols] + _dot(o0, _as_bf16(wobp[done]))
                xio[0:TF, cols] = y.astype(bf16)
                done += 1
            st = pv_step(n_groups - 1, n, ms, st, False)

        @pl.when(rep == 1)
        def _():
            out_copy(0).start()
        off[0] = off[1] = 0

    def out_tile(j, rep):
        rows = blk_rows(j, TF)
        xv = proj_residual(o_rows(j, TF), wob_cols, x_ref[rows, :])
        xio[rows, :] = xv.astype(bf16)

        @pl.when(rep == 1)
        def _():
            out_copy(j).start()

    def phase_b_out(rep):
        def body(jj, c):
            for u in range(OPB):
                out_tile(OPRE + jj * OPB + u, rep)
            flush_o(NQT * NG - 1, otbuf[...])
            return c
        lax.fori_loop(0, (S // TF - OPRE) // OPB, body, 0)

    for cp in x01_copies:
        cp.start()
    for g in range(NG):
        if g == NG - 2:
            x2_copy.start()
        for cp in wa_copies(g):
            cp.start()
    for it in range(NB // APB):
        for cp in iter_copies(it):
            cp.start()
    wob_copy.start()

    startup()

    def layer_pair(rep, c):
        phase_a(rep)

        @pl.when(rep == 0)
        def _():
            wob_copy.wait()

        phase_b_proj()
        phase_b_attn(rep)
        phase_b_out(rep)
        return c
    lax.fori_loop(0, 2, layer_pair, 0)
    for j in range(S // TF):
        out_copy(j).wait()


@jax.jit
def pallas_interleave_layers__sliding_local_dilated__softmax_full_mha__prompt_kernel(
    A_x: jax.Array,
    A_wqkv: jax.Array,
    A_wo: jax.Array,
    B_x: jax.Array,
    B_wqkv: jax.Array,
    B_wo: jax.Array,
):
    del B_x
    x = A_x.reshape(S, D)
    vm = pltpu.VMEM
    scratch = [
        vm((S, D), f32),
        vm((S, D), bf16),
        vm((BLK // 2, D), u32),
        vm((BLK // 2, D), u32),
        vm((TB // 2, D), u32),
        vm((3 * NG, D, 128), bf16),
        vm((NG, NG, 192, 128), u32),
        vm((D, D), bf16),
        vm((NG, D // 2, 128), u32),
        vm((2 * NG, D, 128), bf16),
        vm((2 * NG, 64, D), u32),
        vm((D, D), bf16),
        vm((NG, D // 2, 128), u32),
        vm((D, D), bf16),
        vm((NG, D // 2, 128), u32),
        vm((NG, 64, BLK), u32),
        vm((NG, 64, BLK), u32),
        vm((NG, 192, 128), u32),
        vm((384, 2 * BLK), f32),
        vm((NG, BLK, 128), u32),
        vm((NQT, D // 2, NQ), u32),
        vm((NG, S // 2, 128), u32),
        vm((NC, D // 2, MK), u32),
        vm((NG, S // 2, 128), u32),
        vm((64, NQ), u32),
        pltpu.SemaphoreType.DMA((N_SEM,)),
    ] + [vm((2 * MK, NQ), f32)] * NC + [
        vm((2, 128, BLK), f32), vm((2, 64, BLK), u32), vm((2, 64, BLK), u32)] * NG
    out = pl.pallas_call(
        _kernel,
        out_shape=jax.ShapeDtypeStruct((S, D), bf16),
        in_specs=[pl.BlockSpec(memory_space=pl.ANY)] * 5,
        out_specs=pl.BlockSpec(memory_space=pl.ANY),
        scratch_shapes=scratch,
        compiler_params=pltpu.CompilerParams(vmem_limit_bytes=110 * 1024 * 1024),
        name="interleave_attn",
    )(x, A_wqkv, A_wo, B_wqkv, B_wo)
    return out.reshape(1, S, D)
```

```python
import jax
import jax.numpy as jnp
from jax import lax
import jax.experimental.pallas as pl
import jax.experimental.pallas.tpu as pltpu

S, D, H, DH = 2048, 1024, 32, 32
W_LOC, DIL = 8, 2
EPS = 1e-5
LOG2E = 1.4426950408889634
QSCALE = (DH ** -0.5) * LOG2E
NEG = -1e9 * LOG2E

BLK = 128
NB = S // BLK
NG = D // 128
NQ = 256
NQT = S // NQ
MK = 128
NC = S // MK
DL = 6
APB = 2
GPB = 4
TB = 256
TF = 128
OPRE = 1
OPB = 3

SEM_X01, SEM_X2, SEM_WOB, SEM_OUT = 0, 1, 2, 3
SEM_WA = 4
SEM_IT = SEM_WA + NG
N_SEM = SEM_IT + 4

UCH = 2
L1S = (0, 0, 1, 2, 3, 4, 6, 7)
L2S = (3, 5)
WBSLOT = 6
WKSLOT = 0
L2BS = (10, 0, 4, 9, 8, 5, 2, 5, 4, 8, 3, 6, 2, 1, 9, 7)


bf16 = jnp.bfloat16
f32 = jnp.float32
u32 = jnp.uint32
NT = (((1,), (1,)), ((), ()))


def _pack(x):
    return pltpu.bitcast(x.astype(bf16), u32)


def _as_bf16(x):
    return pltpu.bitcast(x, bf16)


def _dot(a, b):
    return jnp.dot(a, b, preferred_element_type=f32)


def _dot_nt(a, b):
    return lax.dot_general(a, b, NT, preferred_element_type=f32)


def _token(v):
    t = pltpu.bitcast(v[0:8, :], u32)
    return lax.shift_right_logical(jnp.bitwise_and(t, jnp.uint32(0xFFFF)), jnp.uint32(16))


def _after(x, tok):
    n, m = x.shape
    z = jnp.concatenate([jnp.concatenate([tok] * (m // 128), axis=1)] * (n // 8), axis=0)
    return pltpu.bitcast(jnp.bitwise_or(pltpu.bitcast(x, u32), z), x.dtype)


def _ln16(x):
    mu = jnp.sum(x, axis=1, keepdims=True) * (1.0 / D)
    xc = x - mu
    var = jnp.sum(xc * xc, axis=1, keepdims=True) * (1.0 / D)
    return _pack(xc * lax.rsqrt(var + EPS))


def _tree(x, op):
    n = x.shape[0]
    while n > 1:
        n //= 2
        x = op(x[:n], x[n:])
    return x[0]


def _local_attention(q, kc, kp, vc, vp, pos):
    lane = lax.broadcasted_iota(jnp.int32, (UCH * 4, 128), 1)

    def shifted(cur, prev, u, w):
        rows = slice(u * UCH * 4, (u + 1) * UCH * 4)
        x = cur[rows]
        if w:
            x = jnp.where(lane >= 128 - DIL * w, prev[rows], x)
            x = pltpu.roll(x, DIL * w, axis=1)
        return _as_bf16(x).astype(f32).reshape(UCH, 8, 128)

    nu = 16 // UCH
    even = lax.broadcasted_iota(jnp.int32, (8, 128), 0) % 2 == 0
    acc = [None] * W_LOC
    for u in range(nu):
        qu = q[u * UCH * 8:(u + 1) * UCH * 8].reshape(UCH, 8, 128)
        for w in range(W_LOC):
            t = _tree(qu * shifted(kc, kp, u, w), jnp.add)
            acc[w] = t if acc[w] is None else acc[w] + t
    logits = []
    for w in range(W_LOC):
        t = acc[w]
        t = t + jnp.where(even, pltpu.roll(t, 7, axis=0), pltpu.roll(t, 1, axis=0))
        t = t * QSCALE
        if w:
            t = jnp.where(pos >= DIL * w, t, NEG)
        logits.append(t)
    m = logits[0]
    for t in logits[1:]:
        m = jnp.maximum(m, t)
    ps = [jnp.exp2(t - m) for t in logits]
    l = ps[0]
    for p in ps[1:]:
        l = l + p
    r = 1.0 / l
    ps = [(p * r)[None] for p in ps]
    outs = []
    for u in range(nu):
        o = None
        for w in range(W_LOC):
            t = shifted(vc, vp, u, w) * ps[w]
            o = t if o is None else o + t
        outs.append(o.reshape(UCH * 8, 128))
    return jnp.concatenate(outs, axis=0)


def _kernel(x_hbm, wa_hbm, woa_hbm, wb_hbm, wob_hbm, out_hbm,
            x_ref, xio, xn1a, xn1b, xn2, wa_nat, wat, woa, woap, wb_nat, wbt, wk, wkp, wob, wobp,
            khalo, vhalo, wstage, pbuf, po,
            qT, kN, vT, oN, otbuf,
            sem, *bufs):
    xn1 = (xn1a, xn1b)
    sbufs = bufs[:NC]
    stg = [bufs[NC + 3 * g:NC + 3 * g + 3] for g in range(NG)]

    def x_copy(i, sid):
        rows = pl.ds(i * BLK, BLK)
        return pltpu.make_async_copy(x_hbm.at[rows, :], xio.at[rows, :], sem.at[sid])

    def wa_copies(g):
        return [pltpu.make_async_copy(
            wa_hbm.at[:, pl.ds(pl.multiple_of(sec * D + g * 128, 128), 128)],
            wa_nat.at[g * 3 + sec], sem.at[SEM_WA + g]) for sec in range(3)]

    def wb_copy(c, sid):
        col = c * 128 + (c // 8) * D
        return pltpu.make_async_copy(
            wb_hbm.at[:, pl.ds(col, 128)], wb_nat.at[c], sem.at[sid])

    def wk_copy(c, sid):
        rows = pl.ds(c * 128, 128)
        return pltpu.make_async_copy(
            wb_hbm.at[rows, pl.ds(D, D)], wk.at[rows, :], sem.at[sid])

    def woa_copy(half, sid):
        rows = pl.ds(half * (D // 2), D // 2)
        return pltpu.make_async_copy(woa_hbm.at[rows, :], woa.at[rows, :], sem.at[sid])

    def iter_copies(it):
        sid = SEM_IT + min(it, 3)
        if it == 0:
            cps = [woa_copy(1, sid)]
        else:
            cps = [x_copy(i, sid) for i in (2 * it + 1, 2 * it + 2) if i < NB]
        return cps + [wb_copy(2 * it, sid), wb_copy(2 * it + 1, sid), wk_copy(it, sid)]

    x01_copies = [x_copy(0, SEM_X01), x_copy(1, SEM_X01)]
    x2_copies = [x_copy(2, SEM_X2), woa_copy(0, SEM_X2)]
    wob_copy = pltpu.make_async_copy(wob_hbm, wob, sem.at[SEM_WOB])

    def out_copy(j):
        rows = pl.ds(pl.multiple_of(j * TF, TF), TF)
        return pltpu.make_async_copy(xio.at[rows, :], out_hbm.at[rows, :], sem.at[SEM_OUT])

    def blk_rows(i, n=BLK):
        return pl.ds(pl.multiple_of(i * n, n), n)

    def qkv_group(g, xn):
        w = jnp.concatenate([wat[g, kt] for kt in range(NG)], axis=1)
        q, k, v = [_dot_nt(_as_bf16(w[a:a + 64]), xn) for a in (0, 64, 128)]
        return q, _pack(k), _pack(v)

    def o_rows(i, n):
        rows = blk_rows(i, n // 2)
        return _as_bf16(jnp.concatenate([oN[t, rows, :] for t in range(NG)], axis=1))

    def proj_residual(o, w_cols, xv):
        cols = []
        for n in range(2):
            cols.append(xv[:, n * 512:(n + 1) * 512] + _dot(o, w_cols(n)))
        return jnp.concatenate(cols, axis=1)

    def woa_half(half, o_cols, xv):
        o = jnp.concatenate(o_cols, axis=1)
        rows = slice(half * (D // 4), (half + 1) * (D // 4))
        cols = []
        for n in range(2):
            w = _as_bf16(jnp.concatenate([woap[4 * n + t, rows, :] for t in range(4)], axis=1))
            cols.append(xv[:, n * 512:(n + 1) * 512] + _dot(o, w))
        return jnp.concatenate(cols, axis=1)

    def packed_cols(w_ref):
        return lambda n: _as_bf16(
            jnp.concatenate([w_ref[4 * n + t] for t in range(4)], axis=1))

    wob_cols, wk_cols = packed_cols(wobp), packed_cols(wkp)

    def repack(dst_ref, src_ref, c, n, tok=None):
        wv = pltpu.bitcast(src_ref[blk_rows(c, n), :], u32)
        if tok is not None:
            wv = _after(wv, tok)
        for t in range(NG):
            dst_ref[t, blk_rows(c, n // 2), :] = wv[:, t * 128:(t + 1) * 128]

    def store_permuted(dst_ref, row0, val):
        for h in range(4):
            dst_ref[pl.ds(row0 + h, 16, stride=4), :] = val[h * 16:(h + 1) * 16]

    def rows16(blk, r):
        return pl.ds(pl.multiple_of(blk * BLK + r * 16, 16), 16)

    def ln1(blk, r, tok=None):
        xv = xio[rows16(blk, r), :].astype(f32)
        return _ln16(xv if tok is None else _after(xv, tok))

    def ln2(tile, r, tok):
        xv = x_ref[pl.ds(pl.multiple_of(tile * TB + r * 16, 16), 16), :]
        xn2[pl.ds(pl.multiple_of(r * 8, 8), 8), :] = _ln16(_after(xv, tok))

    def stage(g, slot, qkv):
        for ref, val in zip(stg[g], qkv):
            ref[slot] = val

    def a_block(i, par):
        inx = jnp.minimum(i + 1, NB - 1)
        pos = i * BLK + lax.broadcasted_iota(jnp.int32, (8, 128), 1)

        def side_jobs(slot, src):
            if slot not in L1S + L2S + (WBSLOT, WKSLOT):
                return
            tok = _token(src)
            if slot == WBSLOT:
                wsrc = _as_bf16(_after(pltpu.bitcast(wb_nat[i], u32), tok))
                wbt[i] = pltpu.bitcast(wsrc.T, u32)
            if slot == WKSLOT:
                repack(wkp, wk, i, 64, tok)
            for r in range(8):
                if L1S[r] == slot:
                    xn1[1 - par][r * 8:(r + 1) * 8, :] = ln1(inx, r, tok)
            for e in range(2):
                if L2S[e] == slot:
                    ln2(0, 2 * jnp.clip(i - 2, 0, TB // 32 - 1) + e, tok)

        o_cols = []
        for g in range(NG):
            stage(g, par, qkv_group(g, _as_bf16(xn1[par][...])))
            qs, ks, vs = stg[g]
            ot = _local_attention(qs[par], ks[par], ks[1 - par], vs[par], vs[1 - par], pos)
            o_cols.append(ot.astype(bf16).T)
            side_jobs(g, ot[120:128])
        rows = blk_rows(i)
        xv = woa_half(0, o_cols[:NG // 2], xio[rows, :].astype(f32))
        x_ref[rows, :] = woa_half(1, o_cols[NG // 2:], xv)

    def startup():
        def transpose_wa(g):
            for sec in range(3):
                wv = pltpu.bitcast(wa_nat[g * 3 + sec].T, u32)
                for kt in range(NG):
                    store_permuted(wstage.at[kt], sec * 64, wv[:, kt * 128:(kt + 1) * 128])

        def project(g):
            w = wstage[...]
            wat[g] = w
            w = jnp.concatenate([w[kt] for kt in range(NG)], axis=1)
            return _dot_nt(_as_bf16(w), _as_bf16(xn2[...]))

        def attend(g, r):
            pos = lax.broadcasted_iota(jnp.int32, (8, 128), 1)
            kp = vp = jnp.zeros((64, BLK), u32)
            for b in range(2):
                rb = r[:, b * BLK:(b + 1) * BLK]
                kc = _pack(rb[128:256])
                vc = _pack(rb[256:384])
                ot = _local_attention(rb[0:128], kc, kp, vc, vp, pos + b * BLK)
                po[g, b * 64:(b + 1) * 64, :] = pltpu.bitcast(ot.astype(bf16).T, u32)
                kp, vp = kc, vc
            khalo[g] = kp
            vhalo[g] = vp

        pbuf[...] = jnp.zeros(pbuf.shape, f32)

        def zero_scores(k, c):
            for sb in sbufs:
                sb[blk_rows(k, 32), :] = jnp.zeros((32, NQ), f32)
            return c
        lax.fori_loop(0, 2 * MK // 32, zero_scores, 0)
        for cp in x01_copies:
            cp.wait()
        for b in range(2):
            for r in range(BLK // 16):
                xn2[b * 64 + r * 8:b * 64 + (r + 1) * 8, :] = ln1(b, r)
        for cp in wa_copies(0):
            cp.wait()
        transpose_wa(0)

        def body(g, c):
            for cp in wa_copies(g + 1):
                cp.wait()
            prev = pbuf[...]
            pbuf[...] = project(g)
            transpose_wa(g + 1)
            attend(jnp.maximum(g - 1, 0), prev)
            return c
        lax.fori_loop(0, NG - 1, body, 0)

        def out_half(half):
            for t in range(NG):
                wv = pltpu.bitcast(
                    woa[half * (D // 2):(half + 1) * (D // 2), t * 128:(t + 1) * 128], u32)
                for g in range(NG // 2):
                    store_permuted(woap.at[t], half * (D // 4) + g * 64, wv[g * 64:(g + 1) * 64])
            for b in range(2):
                rows = blk_rows(b)
                o_cols = [_as_bf16(po[half * (NG // 2) + g, b * 64:(b + 1) * 64, :])
                          for g in range(NG // 2)]
                base = x_ref[rows, :] if half else xio[rows, :].astype(f32)
                x_ref[rows, :] = woa_half(half, o_cols, base)

        for cp in x2_copies:
            cp.wait()
        prev = pbuf[...]
        r = project(NG - 1)
        xn1[0][...] = jnp.concatenate([ln1(2, r16) for r16 in range(BLK // 16)], axis=0)
        attend(NG - 2, prev)
        out_half(0)
        attend(NG - 1, r)

        for cp in iter_copies(0):
            cp.wait()
        out_half(1)
        for b in range(2):
            wbt[b] = pltpu.bitcast(wb_nat[b].T, u32)
        repack(wkp, wk, 0, 128)
        for g in range(NG):
            stg[g][1][1] = khalo[g]
            stg[g][2][1] = vhalo[g]
        for cp in iter_copies(1):
            cp.wait()

    def phase_a(rep):
        @pl.when(rep == 1)
        def _():
            for g in range(NG):
                for ref in stg[g][1:]:
                    ref[1] = jnp.zeros((64, BLK), u32)
            xn1[0][...] = jnp.concatenate([ln1(0, r) for r in range(BLK // 16)], axis=0)


        def body(it, c):
            @pl.when(it == 2 - rep * NB)
            def _():
                for cp in iter_copies(2):
                    cp.wait()

            @pl.when(it == 3 - rep * NB)
            def _():
                for k in range(3, NB // APB):
                    for cp in iter_copies(k):
                        cp.wait()

            for u in range(APB):
                a_block(it * APB + u, u % 2)
            return c
        lax.fori_loop(1 - rep, NB // APB, body, 0)

    def phase_b_proj():
        def body(j, c):
            rows = blk_rows(j, TB // 2)
            xn = _as_bf16(xn2[...])
            toks = []
            for n in range(2):
                y = _pack(_dot(xn, wk_cols(n)))
                for t in range(4):
                    kN[4 * n + t, rows, :] = y[:, t * 128:(t + 1) * 128]
                toks += [y[:, 0:128], y[:, 256:384]]
            for r in range(4):
                w = _as_bf16(wbt[2 * r:2 * r + 2].reshape(128, D))
                y = _pack(_dot_nt(w, xn) * QSCALE)
                for b in range(TB // NQ):
                    qT[j * (TB // NQ) + b, r * 128:(r + 1) * 128, :] = y[:, b * NQ:(b + 1) * NQ]
                toks.append(y[:, 0:128])
            for r in range(4):
                w = _as_bf16(wbt[8 + 2 * r:8 + 2 * r + 2].reshape(128, D))
                y = _pack(_dot_nt(w, xn))
                for b in range(TB // MK):
                    vT[j * (TB // MK) + b, r * 128:(r + 1) * 128, :] = y[:, b * MK:(b + 1) * MK]
                toks.append(y[:, 0:128])
            jn = jnp.minimum(j + 1, S // TB - 1)
            for r in range(TB // 16):
                ln2(jn, r, _token(toks[L2BS[r]]))
            return c
        lax.fori_loop(0, S // TB, body, 0)

    def flush_o(g, val):
        y = pltpu.bitcast(_as_bf16(val).T, u32)
        oN[g % NG, blk_rows(g // NG, NQ // 2), :] = y

    def phase_b_attn(rep):
        off = [0, 0]

        def qm_of(t, qi, j):
            q = _as_bf16(qT[qi, pl.ds(pl.multiple_of(t * 64 + j * 16, 16), 16), :])
            parts = []
            if j > 0:
                parts.append(jnp.zeros((32 * j, NQ), bf16))
            parts.append(q)
            if j < 3:
                parts.append(jnp.zeros((32 * (3 - j), NQ), bf16))
            return jnp.concatenate(parts, axis=0)

        def qk_chunk(t, qm, c, par, m):
            k = _as_bf16(kN[t, c * (MK // 2):(c + 1) * (MK // 2), :])
            s = _dot(k, qm)
            sbufs[c][pl.ds(pl.multiple_of(off[0] + par * MK, 8), MK), :] = s
            sm = _tree(s.reshape(MK // 8, 8, NQ), jnp.maximum)
            return sm if m is None else jnp.maximum(m, sm)

        def pv_chunk(h, c, par, mrow, l, o):
            s = sbufs[c][pl.ds(pl.multiple_of(off[1] + par * MK, 8), MK), :]
            p = jnp.exp2(s - mrow)
            ls = jnp.sum(p.reshape(MK // 8, 8, NQ), axis=0)
            l = ls if l is None else l + ls
            v = _as_bf16(vT[c, pl.ds(pl.multiple_of(h * 16, 16), 16), :])
            oc = _dot(v, p.astype(bf16))
            o = oc if o is None else o + oc
            return l, o

        n_groups = NQT * NG
        lag = NC + DL
        n_steps = 4 * NC

        def set_offsets(zero):
            off[0] = lax.shift_right_logical(zero, 16) * 8
            off[1] = lax.shift_right_logical(zero, 17) * 8

        def pv_step(g, n, ms, st, flush=True):
            j, c = divmod(n, NC)
            l, o, mrow = st
            if c == 0:
                mrow = jnp.max(ms[j], axis=0, keepdims=True)
                l = o = None
            l, o = pv_chunk((g % NG) * 4 + j, c, j % 2, mrow, l, o)
            if c == NC - 1:
                lrow = jnp.sum(l, axis=0, keepdims=True)
                otbuf[j * 16:(j + 1) * 16, :] = _pack(o * (1.0 / lrow))
                if j == 3 and flush:
                    flush_o(g, otbuf[...])
            return l, o, mrow

        def group(g, g_prev, carry, side_job=None):
            st, ms_prev = carry[:3], {3: carry[3]}
            ms = {}
            for n in range(n_steps):
                j, c = divmod(n, NC)
                if c == 0:
                    qm = qm_of(g % NG, g // NG, j)
                ms[j] = qk_chunk(g % NG, qm, c, j % 2, ms.get(j))
                if n < lag:
                    st = pv_step(g_prev, n + n_steps - lag, ms_prev, st)
                else:
                    st = pv_step(g, n - lag, ms, st)
                if side_job is not None and n == n_steps // 2:
                    side_job(_token(st[0][:, 0:128]))
            return st + (ms[3],)

        def body(it, carry):
            def side_job(tok):
                repack(wobp, wob, it, D * GPB // n_groups, tok)

            set_offsets(it)
            carry = carry[:4]
            for u in range(GPB):
                g = it * GPB + u
                carry = group(g, jnp.maximum(g - 1, 0), carry, side_job if u == 0 else None)
            return carry + (it,)

        otbuf[...] = jnp.zeros(otbuf.shape, u32)
        init = (jnp.zeros((8, NQ), f32), jnp.zeros((DH, NQ), f32),
                jnp.zeros((1, NQ), f32), jnp.zeros((8, NQ), f32), jnp.int32(0))
        carry = lax.fori_loop(0, n_groups // GPB, body, init)
        set_offsets(carry[4])
        st, ms = carry[:3], {3: carry[3]}
        o0 = o_rows(0, TF)
        done = 0
        for k, n in enumerate(range(n_steps - lag, n_steps)):
            while done < NG and done * lag <= k * NG:
                cols = slice(done * 128, (done + 1) * 128)
                y = x_ref[0:TF, cols] + _dot(o0, _as_bf16(wobp[done]))
                xio[0:TF, cols] = y.astype(bf16)
                done += 1
            st = pv_step(n_groups - 1, n, ms, st, False)

        @pl.when(rep == 1)
        def _():
            out_copy(0).start()
        off[0] = off[1] = 0

    def out_tile(j, rep):
        rows = blk_rows(j, TF)
        xv = proj_residual(o_rows(j, TF), wob_cols, x_ref[rows, :])
        xio[rows, :] = xv.astype(bf16)

        @pl.when(rep == 1)
        def _():
            out_copy(j).start()

    def phase_b_out(rep):
        def body(jj, c):
            for u in range(OPB):
                out_tile(OPRE + jj * OPB + u, rep)
            flush_o(NQT * NG - 1, otbuf[...])
            return c
        lax.fori_loop(0, (S // TF - OPRE) // OPB, body, 0)

    for cp in x01_copies:
        cp.start()
    for g in range(NG):
        for cp in wa_copies(g):
            cp.start()
    for cp in x2_copies:
        cp.start()
    for it in range(NB // APB):
        for cp in iter_copies(it):
            cp.start()
    wob_copy.start()

    startup()

    def layer_pair(rep, c):
        phase_a(rep)

        @pl.when(rep == 0)
        def _():
            wob_copy.wait()

        phase_b_proj()
        phase_b_attn(rep)
        phase_b_out(rep)
        return c
    lax.fori_loop(0, 2, layer_pair, 0)
    for j in range(S // TF):
        out_copy(j).wait()


@jax.jit
def pallas_interleave_layers__sliding_local_dilated__softmax_full_mha__prompt_kernel(
    A_x: jax.Array,
    A_wqkv: jax.Array,
    A_wo: jax.Array,
    B_x: jax.Array,
    B_wqkv: jax.Array,
    B_wo: jax.Array,
):
    del B_x
    x = A_x.reshape(S, D)
    vm = pltpu.VMEM
    scratch = [
        vm((S, D), f32),
        vm((S, D), bf16),
        vm((BLK // 2, D), u32),
        vm((BLK // 2, D), u32),
        vm((TB // 2, D), u32),
        vm((3 * NG, D, 128), bf16),
        vm((NG, NG, 192, 128), u32),
        vm((D, D), bf16),
        vm((NG, D // 2, 128), u32),
        vm((2 * NG, D, 128), bf16),
        vm((2 * NG, 64, D), u32),
        vm((D, D), bf16),
        vm((NG, D // 2, 128), u32),
        vm((D, D), bf16),
        vm((NG, D // 2, 128), u32),
        vm((NG, 64, BLK), u32),
        vm((NG, 64, BLK), u32),
        vm((NG, 192, 128), u32),
        vm((384, 2 * BLK), f32),
        vm((NG, BLK, 128), u32),
        vm((NQT, D // 2, NQ), u32),
        vm((NG, S // 2, 128), u32),
        vm((NC, D // 2, MK), u32),
        vm((NG, S // 2, 128), u32),
        vm((64, NQ), u32),
        pltpu.SemaphoreType.DMA((N_SEM,)),
    ] + [vm((2 * MK, NQ), f32)] * NC + [
        vm((2, 128, BLK), f32), vm((2, 64, BLK), u32), vm((2, 64, BLK), u32)] * NG
    out = pl.pallas_call(
        _kernel,
        out_shape=jax.ShapeDtypeStruct((S, D), bf16),
        in_specs=[pl.BlockSpec(memory_space=pl.ANY)] * 5,
        out_specs=pl.BlockSpec(memory_space=pl.ANY),
        scratch_shapes=scratch,
        compiler_params=pltpu.CompilerParams(vmem_limit_bytes=110 * 1024 * 1024),
        name="interleave_attn",
    )(x, A_wqkv, A_wo, B_wqkv, B_wo)
    return out.reshape(1, S, D)
```

```python
import jax
import jax.numpy as jnp
from jax import lax
import jax.experimental.pallas as pl
import jax.experimental.pallas.tpu as pltpu

S, D, H, DH = 2048, 1024, 32, 32
W_LOC, DIL = 8, 2
EPS = 1e-5
LOG2E = 1.4426950408889634
QSCALE = (DH ** -0.5) * LOG2E
NEG = -1e9 * LOG2E

BLK = 128
NB = S // BLK
NG = D // 128
NQ = 256
NQT = S // NQ
MK = 128
NC = S // MK
DL = 6
APB = 2
GPB = 4
TB = 256
TF = 128
OPRE = 1
OPB = 3

SEM_X01, SEM_X2, SEM_WOB, SEM_OUT = 0, 1, 2, 3
SEM_WA = 4
SEM_IT = SEM_WA + NG
N_SEM = SEM_IT + 4

UCH = 2
L1S = (0, 0, 1, 2, 3, 4, 6, 7)
L2S = (3, 5)
WBSLOT = 6
WKSLOT = 0
L2BS = (10, 0, 4, 9, 8, 5, 2, 5, 4, 8, 3, 6, 2, 1, 9, 7)


bf16 = jnp.bfloat16
f32 = jnp.float32
u32 = jnp.uint32
NT = (((1,), (1,)), ((), ()))


def _pack(x):
    return pltpu.bitcast(x.astype(bf16), u32)


def _as_bf16(x):
    return pltpu.bitcast(x, bf16)


def _dot(a, b):
    return jnp.dot(a, b, preferred_element_type=f32)


def _dot_nt(a, b):
    return lax.dot_general(a, b, NT, preferred_element_type=f32)


def _token(v):
    t = pltpu.bitcast(v[0:8, :], u32)
    return lax.shift_right_logical(jnp.bitwise_and(t, jnp.uint32(0xFFFF)), jnp.uint32(16))


def _after(x, tok):
    n, m = x.shape
    z = jnp.concatenate([jnp.concatenate([tok] * (m // 128), axis=1)] * (n // 8), axis=0)
    return pltpu.bitcast(jnp.bitwise_or(pltpu.bitcast(x, u32), z), x.dtype)


def _ln16(x):
    mu = jnp.sum(x, axis=1, keepdims=True) * (1.0 / D)
    xc = x - mu
    var = jnp.sum(xc * xc, axis=1, keepdims=True) * (1.0 / D)
    return _pack(xc * lax.rsqrt(var + EPS))


def _tree(x, op):
    n = x.shape[0]
    while n > 1:
        n //= 2
        x = op(x[:n], x[n:])
    return x[0]


def _local_attention(q, kc, kp, vc, vp, pos):
    lane = lax.broadcasted_iota(jnp.int32, (UCH * 4, 128), 1)

    def shifted(cur, prev, u, w):
        rows = slice(u * UCH * 4, (u + 1) * UCH * 4)
        x = cur[rows]
        if w:
            x = jnp.where(lane >= 128 - DIL * w, prev[rows], x)
            x = pltpu.roll(x, DIL * w, axis=1)
        return _as_bf16(x).astype(f32).reshape(UCH, 8, 128)

    nu = 16 // UCH
    even = lax.broadcasted_iota(jnp.int32, (8, 128), 0) % 2 == 0
    acc = [None] * W_LOC
    for u in range(nu):
        qu = q[u * UCH * 8:(u + 1) * UCH * 8].reshape(UCH, 8, 128)
        for w in range(W_LOC):
            t = _tree(qu * shifted(kc, kp, u, w), jnp.add)
            acc[w] = t if acc[w] is None else acc[w] + t
    logits = []
    for w in range(W_LOC):
        t = acc[w]
        t = t + jnp.where(even, pltpu.roll(t, 7, axis=0), pltpu.roll(t, 1, axis=0))
        t = t * QSCALE
        if w:
            t = jnp.where(pos >= DIL * w, t, NEG)
        logits.append(t)
    m = logits[0]
    for t in logits[1:]:
        m = jnp.maximum(m, t)
    ps = [jnp.exp2(t - m) for t in logits]
    l = ps[0]
    for p in ps[1:]:
        l = l + p
    r = 1.0 / l
    ps = [(p * r)[None] for p in ps]
    outs = []
    for u in range(nu):
        o = None
        for w in range(W_LOC):
            t = shifted(vc, vp, u, w) * ps[w]
            o = t if o is None else o + t
        outs.append(o.reshape(UCH * 8, 128))
    return jnp.concatenate(outs, axis=0)


def _kernel(x_hbm, wa_hbm, woa_hbm, wb_hbm, wob_hbm, out_hbm,
            x_ref, xio, xn1a, xn1b, xn2, wa_nat, wat, woa, woap, wb_nat, wbt, wk, wkp, wob, wobp,
            khalo, vhalo, wstage, pbuf, po,
            qT, kN, vT, oN, otbuf,
            sem, *bufs):
    xn1 = (xn1a, xn1b)
    sbufs = bufs[:NC]
    stg = [bufs[NC + 3 * g:NC + 3 * g + 3] for g in range(NG)]

    def x_copy(i, sid):
        rows = pl.ds(i * BLK, BLK)
        return pltpu.make_async_copy(x_hbm.at[rows, :], xio.at[rows, :], sem.at[sid])

    def wa_copies(g):
        return [pltpu.make_async_copy(
            wa_hbm.at[:, pl.ds(pl.multiple_of(sec * D + g * 128, 128), 128)],
            wa_nat.at[g * 3 + sec], sem.at[SEM_WA + g]) for sec in range(3)]

    def wb_copy(c, sid):
        col = c * 128 + (c // 8) * D
        return pltpu.make_async_copy(
            wb_hbm.at[:, pl.ds(col, 128)], wb_nat.at[c], sem.at[sid])

    def wk_copy(c, sid):
        rows = pl.ds(c * 128, 128)
        return pltpu.make_async_copy(
            wb_hbm.at[rows, pl.ds(D, D)], wk.at[rows, :], sem.at[sid])

    def woa_copy(half, sid):
        rows = pl.ds(half * (D // 2), D // 2)
        return pltpu.make_async_copy(woa_hbm.at[rows, :], woa.at[rows, :], sem.at[sid])

    def iter_copies(it):
        sid = SEM_IT + min(it, 3)
        if it == 0:
            cps = [woa_copy(1, sid)]
        else:
            cps = [x_copy(i, sid) for i in (2 * it + 1, 2 * it + 2) if i < NB]
        return cps + [wb_copy(2 * it, sid), wb_copy(2 * it + 1, sid), wk_copy(it, sid)]

    x01_copies = [x_copy(0, SEM_X01), x_copy(1, SEM_X01)]
    x2_copies = [x_copy(2, SEM_X2), woa_copy(0, SEM_X2)]
    wob_copy = pltpu.make_async_copy(wob_hbm, wob, sem.at[SEM_WOB])

    def out_copy(j):
        rows = pl.ds(pl.multiple_of(j * TF, TF), TF)
        return pltpu.make_async_copy(xio.at[rows, :], out_hbm.at[rows, :], sem.at[SEM_OUT])

    def blk_rows(i, n=BLK):
        return pl.ds(pl.multiple_of(i * n, n), n)

    def qkv_group(g, xn):
        w = jnp.concatenate([wat[g, kt] for kt in range(NG)], axis=1)
        q, k, v = [_dot_nt(_as_bf16(w[a:a + 64]), xn) for a in (0, 64, 128)]
        return q, _pack(k), _pack(v)

    def o_rows(i, n):
        rows = blk_rows(i, n // 2)
        return _as_bf16(jnp.concatenate([oN[t, rows, :] for t in range(NG)], axis=1))

    def proj_residual(o, w_cols, xv):
        cols = []
        for n in range(2):
            cols.append(xv[:, n * 512:(n + 1) * 512] + _dot(o, w_cols(n)))
        return jnp.concatenate(cols, axis=1)

    def woa_half(half, o_cols, xv):
        o = jnp.concatenate(o_cols, axis=1)
        rows = slice(half * (D // 4), (half + 1) * (D // 4))
        cols = []
        for n in range(2):
            w = _as_bf16(jnp.concatenate([woap[4 * n + t, rows, :] for t in range(4)], axis=1))
            cols.append(xv[:, n * 512:(n + 1) * 512] + _dot(o, w))
        return jnp.concatenate(cols, axis=1)

    def packed_cols(w_ref):
        return lambda n: _as_bf16(
            jnp.concatenate([w_ref[4 * n + t] for t in range(4)], axis=1))

    wob_cols, wk_cols = packed_cols(wobp), packed_cols(wkp)

    def repack(dst_ref, src_ref, c, n, tok=None):
        wv = pltpu.bitcast(src_ref[blk_rows(c, n), :], u32)
        if tok is not None:
            wv = _after(wv, tok)
        for t in range(NG):
            dst_ref[t, blk_rows(c, n // 2), :] = wv[:, t * 128:(t + 1) * 128]

    def store_permuted(dst_ref, row0, val):
        for h in range(4):
            dst_ref[pl.ds(row0 + h, 16, stride=4), :] = val[h * 16:(h + 1) * 16]

    def rows16(blk, r):
        return pl.ds(pl.multiple_of(blk * BLK + r * 16, 16), 16)

    def ln1(blk, r, tok=None):
        xv = xio[rows16(blk, r), :].astype(f32)
        return _ln16(xv if tok is None else _after(xv, tok))

    def ln2(tile, r, tok):
        xv = x_ref[pl.ds(pl.multiple_of(tile * TB + r * 16, 16), 16), :]
        xn2[pl.ds(pl.multiple_of(r * 8, 8), 8), :] = _ln16(_after(xv, tok))

    def stage(g, slot, qkv):
        for ref, val in zip(stg[g], qkv):
            ref[slot] = val

    def a_block(i, par):
        inx = jnp.minimum(i + 1, NB - 1)
        pos = i * BLK + lax.broadcasted_iota(jnp.int32, (8, 128), 1)

        def side_jobs(slot, src):
            if slot not in L1S + L2S + (WBSLOT, WKSLOT):
                return
            tok = _token(src)
            if slot == WBSLOT:
                wsrc = _as_bf16(_after(pltpu.bitcast(wb_nat[i], u32), tok))
                wbt[i] = pltpu.bitcast(wsrc.T, u32)
            if slot == WKSLOT:
                repack(wkp, wk, i, 64, tok)
            for r in range(8):
                if L1S[r] == slot:
                    xn1[1 - par][r * 8:(r + 1) * 8, :] = ln1(inx, r, tok)
            for e in range(2):
                if L2S[e] == slot:
                    ln2(0, 2 * jnp.clip(i - 2, 0, TB // 32 - 1) + e, tok)

        o_cols = []
        for g in range(NG):
            stage(g, par, qkv_group(g, _as_bf16(xn1[par][...])))
            qs, ks, vs = stg[g]
            ot = _local_attention(qs[par], ks[par], ks[1 - par], vs[par], vs[1 - par], pos)
            o_cols.append(ot.astype(bf16).T)
            side_jobs(g, ot[120:128])
        rows = blk_rows(i)
        xv = woa_half(0, o_cols[:NG // 2], xio[rows, :].astype(f32))
        x_ref[rows, :] = woa_half(1, o_cols[NG // 2:], xv)

    def startup():
        def transpose_wa(g):
            for sec in range(3):
                wv = pltpu.bitcast(wa_nat[g * 3 + sec].T, u32)
                for kt in range(NG):
                    store_permuted(wstage.at[kt], sec * 64, wv[:, kt * 128:(kt + 1) * 128])

        def project(g):
            w = wstage[...]
            wat[g] = w
            w = jnp.concatenate([w[kt] for kt in range(NG)], axis=1)
            return _dot_nt(_as_bf16(w), _as_bf16(xn2[...]))

        def attend(g, r):
            pos = lax.broadcasted_iota(jnp.int32, (8, 128), 1)
            kp = vp = jnp.zeros((64, BLK), u32)
            for b in range(2):
                rb = r[:, b * BLK:(b + 1) * BLK]
                kc = _pack(rb[128:256])
                vc = _pack(rb[256:384])
                ot = _local_attention(rb[0:128], kc, kp, vc, vp, pos + b * BLK)
                po[g, b * 64:(b + 1) * 64, :] = pltpu.bitcast(ot.astype(bf16).T, u32)
                kp, vp = kc, vc
            khalo[g] = kp
            vhalo[g] = vp

        pbuf[...] = jnp.zeros(pbuf.shape, f32)

        def zero_scores(k, c):
            for sb in sbufs:
                sb[blk_rows(k, 32), :] = jnp.zeros((32, NQ), f32)
            return c
        lax.fori_loop(0, 2 * MK // 32, zero_scores, 0)
        for cp in x01_copies:
            cp.wait()
        for b in range(2):
            for r in range(BLK // 16):
                xn2[b * 64 + r * 8:b * 64 + (r + 1) * 8, :] = ln1(b, r)
        for cp in wa_copies(0):
            cp.wait()
        transpose_wa(0)

        def body(g, c):
            for cp in wa_copies(g + 1):
                cp.wait()
            prev = pbuf[...]
            pbuf[...] = project(g)
            transpose_wa(g + 1)
            attend(jnp.maximum(g - 1, 0), prev)
            return c
        lax.fori_loop(0, NG - 1, body, 0)

        def out_half(half):
            for t in range(NG):
                wv = pltpu.bitcast(
                    woa[half * (D // 2):(half + 1) * (D // 2), t * 128:(t + 1) * 128], u32)
                for g in range(NG // 2):
                    store_permuted(woap.at[t], half * (D // 4) + g * 64, wv[g * 64:(g + 1) * 64])
            for b in range(2):
                rows = blk_rows(b)
                o_cols = [_as_bf16(po[half * (NG // 2) + g, b * 64:(b + 1) * 64, :])
                          for g in range(NG // 2)]
                base = x_ref[rows, :] if half else xio[rows, :].astype(f32)
                x_ref[rows, :] = woa_half(half, o_cols, base)

        for cp in x2_copies:
            cp.wait()
        prev = pbuf[...]
        r = project(NG - 1)
        xn1[0][...] = jnp.concatenate([ln1(2, r16) for r16 in range(BLK // 16)], axis=0)
        attend(NG - 2, prev)
        out_half(0)
        attend(NG - 1, r)

        for cp in iter_copies(0):
            cp.wait()
        out_half(1)
        for b in range(2):
            wbt[b] = pltpu.bitcast(wb_nat[b].T, u32)
        repack(wkp, wk, 0, 128)
        for g in range(NG):
            stg[g][1][1] = khalo[g]
            stg[g][2][1] = vhalo[g]
        for cp in iter_copies(1):
            cp.wait()

    def phase_a(rep):
        @pl.when(rep == 1)
        def _():
            for g in range(NG):
                for ref in stg[g][1:]:
                    ref[1] = jnp.zeros((64, BLK), u32)
            xn1[0][...] = jnp.concatenate([ln1(0, r) for r in range(BLK // 16)], axis=0)


        def body(it, c):
            @pl.when(it == 2 - rep * NB)
            def _():
                for cp in iter_copies(2):
                    cp.wait()

            @pl.when(it == 3 - rep * NB)
            def _():
                for k in range(3, NB // APB):
                    for cp in iter_copies(k):
                        cp.wait()

            for u in range(APB):
                a_block(it * APB + u, u % 2)
            return c
        lax.fori_loop(1 - rep, NB // APB, body, 0)

    def phase_b_proj():
        def body(j, c):
            rows = blk_rows(j, TB // 2)
            xn = _as_bf16(xn2[...])
            toks = []
            for n in range(2):
                y = _pack(_dot(xn, wk_cols(n)))
                for t in range(4):
                    kN[4 * n + t, rows, :] = y[:, t * 128:(t + 1) * 128]
                toks += [y[:, 0:128], y[:, 256:384]]
            for r in range(4):
                w = _as_bf16(wbt[2 * r:2 * r + 2].reshape(128, D))
                y = _pack(_dot_nt(w, xn) * QSCALE)
                for b in range(TB // NQ):
                    qT[j * (TB // NQ) + b, r * 128:(r + 1) * 128, :] = y[:, b * NQ:(b + 1) * NQ]
                toks.append(y[:, 0:128])
            for r in range(4):
                w = _as_bf16(wbt[8 + 2 * r:8 + 2 * r + 2].reshape(128, D))
                y = _pack(_dot_nt(w, xn))
                for b in range(TB // MK):
                    vT[j * (TB // MK) + b, r * 128:(r + 1) * 128, :] = y[:, b * MK:(b + 1) * MK]
                toks.append(y[:, 0:128])
            jn = jnp.minimum(j + 1, S // TB - 1)
            for r in range(TB // 16):
                ln2(jn, r, _token(toks[L2BS[r]]))
            return c
        lax.fori_loop(0, S // TB, body, 0)

    def flush_o(g, val):
        y = pltpu.bitcast(_as_bf16(val).T, u32)
        oN[g[0], blk_rows(g[1], NQ // 2), :] = y

    def phase_b_attn(rep):
        off = [0, 0]

        def qm_of(t, qi, j):
            q = _as_bf16(qT[qi, pl.ds(pl.multiple_of(t * 64 + j * 16, 16), 16), :])
            parts = []
            if j > 0:
                parts.append(jnp.zeros((32 * j, NQ), bf16))
            parts.append(q)
            if j < 3:
                parts.append(jnp.zeros((32 * (3 - j), NQ), bf16))
            return jnp.concatenate(parts, axis=0)

        def qk_chunk(t, qm, c, par, m):
            k = _as_bf16(kN[t, c * (MK // 2):(c + 1) * (MK // 2), :])
            s = _dot(k, qm)
            sbufs[c][pl.ds(pl.multiple_of(off[0] + par * MK, 8), MK), :] = s
            sm = _tree(s.reshape(MK // 8, 8, NQ), jnp.maximum)
            return sm if m is None else jnp.maximum(m, sm)

        def pv_chunk(h, c, par, mrow, l, o):
            s = sbufs[c][pl.ds(pl.multiple_of(off[1] + par * MK, 8), MK), :]
            p = jnp.exp2(s - mrow)
            ls = jnp.sum(p.reshape(MK // 8, 8, NQ), axis=0)
            l = ls if l is None else l + ls
            v = _as_bf16(vT[c, pl.ds(pl.multiple_of(h * 16, 16), 16), :])
            oc = _dot(v, p.astype(bf16))
            o = oc if o is None else o + oc
            return l, o

        n_groups = NQT * NG
        lag = NC + DL
        n_steps = 4 * NC

        def set_offsets(zero):
            off[0] = lax.shift_right_logical(zero, 16) * 8
            off[1] = lax.shift_right_logical(zero, 17) * 8

        def pv_step(g, n, ms, st, flush=True):
            j, c = divmod(n, NC)
            l, o, mrow = st
            if c == 0:
                mrow = jnp.max(ms[j], axis=0, keepdims=True)
                l = o = None
            l, o = pv_chunk(g[0] * 4 + j, c, j % 2, mrow, l, o)
            if c == NC - 1:
                lrow = jnp.sum(l, axis=0, keepdims=True)
                otbuf[j * 16:(j + 1) * 16, :] = _pack(o * (1.0 / lrow))
                if j == 3 and flush:
                    flush_o(g, otbuf[...])
            return l, o, mrow

        def group(g, g_prev, carry, side_job=None):
            st, ms_prev = carry[:3], {3: carry[3]}
            ms = {}
            qms = {}
            order = [(kind, n) for n in range(n_steps) for kind in ("qk", "pv")]
            if side_job is not None:
                order[1], order[2] = order[2], order[1]
            for kind, n in order:
                if kind == "qk":
                    j, c = divmod(n, NC)
                    if c == 0:
                        qms[j] = qm_of(g[0], g[1], j)
                    ms[j] = qk_chunk(g[0], qms[j], c, j % 2, ms.get(j))
                    continue
                if n < lag:
                    st = pv_step(g_prev, n + n_steps - lag, ms_prev, st)
                else:
                    st = pv_step(g, n - lag, ms, st)
                if side_job is not None and n == n_steps // 2:
                    side_job(_token(st[0][:, 0:128]))
            return st + (ms[3],)

        def body(it, carry):
            def side_job(tok):
                repack(wobp, wob, it, D * GPB // n_groups, tok)

            set_offsets(it)
            carry = carry[:4]
            def split(g):
                return jnp.bitwise_and(g, NG - 1), lax.shift_right_logical(g, 3)

            g_prev = split(jnp.maximum(it * GPB - 1, 0))
            t0, qi = split(it * GPB)
            for u in range(GPB):
                g = (t0 + u, qi)
                carry = group(g, g_prev, carry, side_job if u == 0 else None)
                g_prev = g
            return carry + (it,)

        otbuf[...] = jnp.zeros(otbuf.shape, u32)
        init = (jnp.zeros((8, NQ), f32), jnp.zeros((DH, NQ), f32),
                jnp.zeros((1, NQ), f32), jnp.zeros((8, NQ), f32), jnp.int32(0))
        carry = lax.fori_loop(0, n_groups // GPB, body, init)
        set_offsets(carry[4])
        st, ms = carry[:3], {3: carry[3]}
        o0 = o_rows(0, TF)
        done = 0
        for k, n in enumerate(range(n_steps - lag, n_steps)):
            while done < NG and done * lag <= k * NG:
                cols = slice(done * 128, (done + 1) * 128)
                y = x_ref[0:TF, cols] + _dot(o0, _as_bf16(wobp[done]))
                xio[0:TF, cols] = y.astype(bf16)
                done += 1
            st = pv_step((NG - 1, NQT - 1), n, ms, st, False)

        @pl.when(rep == 1)
        def _():
            out_copy(0).start()
        off[0] = off[1] = 0

    def out_tile(j, rep):
        rows = blk_rows(j, TF)
        xv = proj_residual(o_rows(j, TF), wob_cols, x_ref[rows, :])
        xio[rows, :] = xv.astype(bf16)

        @pl.when(rep == 1)
        def _():
            out_copy(j).start()

    def phase_b_out(rep):
        def body(jj, c):
            for u in range(OPB):
                out_tile(OPRE + jj * OPB + u, rep)
            flush_o((NG - 1, NQT - 1), otbuf[...])
            return c
        lax.fori_loop(0, (S // TF - OPRE) // OPB, body, 0)

    for cp in x01_copies:
        cp.start()
    for g in range(NG):
        for cp in wa_copies(g):
            cp.start()
    for cp in x2_copies:
        cp.start()
    for it in range(NB // APB):
        for cp in iter_copies(it):
            cp.start()
    wob_copy.start()

    startup()

    def layer_pair(rep, c):
        phase_a(rep)

        @pl.when(rep == 0)
        def _():
            wob_copy.wait()

        phase_b_proj()
        phase_b_attn(rep)
        phase_b_out(rep)
        return c
    lax.fori_loop(0, 2, layer_pair, 0)
    for j in range(S // TF):
        out_copy(j).wait()


@jax.jit
def pallas_interleave_layers__sliding_local_dilated__softmax_full_mha__prompt_kernel(
    A_x: jax.Array,
    A_wqkv: jax.Array,
    A_wo: jax.Array,
    B_x: jax.Array,
    B_wqkv: jax.Array,
    B_wo: jax.Array,
):
    del B_x
    x = A_x.reshape(S, D)
    vm = pltpu.VMEM
    scratch = [
        vm((S, D), f32),
        vm((S, D), bf16),
        vm((BLK // 2, D), u32),
        vm((BLK // 2, D), u32),
        vm((TB // 2, D), u32),
        vm((3 * NG, D, 128), bf16),
        vm((NG, NG, 192, 128), u32),
        vm((D, D), bf16),
        vm((NG, D // 2, 128), u32),
        vm((2 * NG, D, 128), bf16),
        vm((2 * NG, 64, D), u32),
        vm((D, D), bf16),
        vm((NG, D // 2, 128), u32),
        vm((D, D), bf16),
        vm((NG, D // 2, 128), u32),
        vm((NG, 64, BLK), u32),
        vm((NG, 64, BLK), u32),
        vm((NG, 192, 128), u32),
        vm((384, 2 * BLK), f32),
        vm((NG, BLK, 128), u32),
        vm((NQT, D // 2, NQ), u32),
        vm((NG, S // 2, 128), u32),
        vm((NC, D // 2, MK), u32),
        vm((NG, S // 2, 128), u32),
        vm((64, NQ), u32),
        pltpu.SemaphoreType.DMA((N_SEM,)),
    ] + [vm((2 * MK, NQ), f32)] * NC + [
        vm((2, 128, BLK), f32), vm((2, 64, BLK), u32), vm((2, 64, BLK), u32)] * NG
    out = pl.pallas_call(
        _kernel,
        out_shape=jax.ShapeDtypeStruct((S, D), bf16),
        in_specs=[pl.BlockSpec(memory_space=pl.ANY)] * 5,
        out_specs=pl.BlockSpec(memory_space=pl.ANY),
        scratch_shapes=scratch,
        compiler_params=pltpu.CompilerParams(vmem_limit_bytes=110 * 1024 * 1024),
        name="interleave_attn",
    )(x, A_wqkv, A_wo, B_wqkv, B_wo)
    return out.reshape(1, S, D)
```

```python
import jax
import jax.numpy as jnp
from jax import lax
import jax.experimental.pallas as pl
import jax.experimental.pallas.tpu as pltpu

S, D, H, DH = 2048, 1024, 32, 32
W_LOC, DIL = 8, 2
EPS = 1e-5
LOG2E = 1.4426950408889634
QSCALE = (DH ** -0.5) * LOG2E
NEG = -1e9 * LOG2E

BLK = 128
NB = S // BLK
NG = D // 128
NQ = 256
NQT = S // NQ
MK = 128
NC = S // MK
DL = 6
APB = 2
GPB = 4
TB = 256
TF = 128
OPRE = 1
OPB = 3

SEM_X01, SEM_X2, SEM_WOB, SEM_OUT = 0, 1, 2, 3
SEM_WA = 4
SEM_IT = SEM_WA + NG
N_SEM = SEM_IT + 4

UCH = 2
L1S = (0, 0, 1, 2, 3, 4, 6, 7)
L2S = (3, 5)
WBSLOT = 6
WKSLOT = 0
L1O = (5, 6, 2, 0, 3, 7, 1, 8)
L2BS = (10, 0, 4, 9, 8, 5, 2, 5, 4, 8, 3, 6, 2, 1, 9, 7)


bf16 = jnp.bfloat16
f32 = jnp.float32
u32 = jnp.uint32
NT = (((1,), (1,)), ((), ()))


def _pack(x):
    return pltpu.bitcast(x.astype(bf16), u32)


def _as_bf16(x):
    return pltpu.bitcast(x, bf16)


def _dot(a, b):
    return jnp.dot(a, b, preferred_element_type=f32)


def _dot_nt(a, b):
    return lax.dot_general(a, b, NT, preferred_element_type=f32)


def _token(v):
    t = pltpu.bitcast(v[0:8, :], u32)
    return lax.shift_right_logical(jnp.bitwise_and(t, jnp.uint32(0xFFFF)), jnp.uint32(16))


def _after(x, tok):
    n, m = x.shape
    z = jnp.concatenate([jnp.concatenate([tok] * (m // 128), axis=1)] * (n // 8), axis=0)
    return pltpu.bitcast(jnp.bitwise_or(pltpu.bitcast(x, u32), z), x.dtype)


def _ln16(x):
    mu = jnp.sum(x, axis=1, keepdims=True) * (1.0 / D)
    xc = x - mu
    var = jnp.sum(xc * xc, axis=1, keepdims=True) * (1.0 / D)
    return _pack(xc * lax.rsqrt(var + EPS))


def _tree(x, op):
    n = x.shape[0]
    while n > 1:
        n //= 2
        x = op(x[:n], x[n:])
    return x[0]


def _local_attention(q, kc, kp, vc, vp, pos):
    lane = lax.broadcasted_iota(jnp.int32, (UCH * 4, 128), 1)

    def shifted(cur, prev, u, w):
        rows = slice(u * UCH * 4, (u + 1) * UCH * 4)
        x = cur[rows]
        if w:
            x = jnp.where(lane >= 128 - DIL * w, prev[rows], x)
            x = pltpu.roll(x, DIL * w, axis=1)
        return _as_bf16(x).astype(f32).reshape(UCH, 8, 128)

    nu = 16 // UCH
    even = lax.broadcasted_iota(jnp.int32, (8, 128), 0) % 2 == 0
    acc = [None] * W_LOC
    for u in range(nu):
        qu = q[u * UCH * 8:(u + 1) * UCH * 8].reshape(UCH, 8, 128)
        for w in range(W_LOC):
            t = _tree(qu * shifted(kc, kp, u, w), jnp.add)
            acc[w] = t if acc[w] is None else acc[w] + t
    logits = []
    for w in range(W_LOC):
        t = acc[w]
        t = t + jnp.where(even, pltpu.roll(t, 7, axis=0), pltpu.roll(t, 1, axis=0))
        t = t * QSCALE
        if w:
            t = jnp.where(pos >= DIL * w, t, NEG)
        logits.append(t)
    m = logits[0]
    for t in logits[1:]:
        m = jnp.maximum(m, t)
    ps = [jnp.exp2(t - m) for t in logits]
    l = ps[0]
    for p in ps[1:]:
        l = l + p
    r = 1.0 / l
    ps = [(p * r)[None] for p in ps]
    outs = []
    for u in range(nu):
        o = None
        for w in range(W_LOC):
            t = shifted(vc, vp, u, w) * ps[w]
            o = t if o is None else o + t
        outs.append(o.reshape(UCH * 8, 128))
    return jnp.concatenate(outs, axis=0)


def _kernel(x_hbm, wa_hbm, woa_hbm, wb_hbm, wob_hbm, out_hbm,
            x_ref, xio, xn1a, xn1b, xn2, wa_nat, wat, woa, woap, wb_nat, wbt, wk, wkp, wob, wobp,
            khalo, vhalo, wstage, pbuf, po, x0buf,
            qT, kN, vT, oN, otbuf,
            sem, *bufs):
    xn1 = (xn1a, xn1b)
    sbufs = bufs[:NC]
    stg = [bufs[NC + 3 * g:NC + 3 * g + 3] for g in range(NG)]

    def x_copy(i, sid):
        rows = pl.ds(i * BLK, BLK)
        return pltpu.make_async_copy(x_hbm.at[rows, :], xio.at[rows, :], sem.at[sid])

    def wa_copies(g):
        return [pltpu.make_async_copy(
            wa_hbm.at[:, pl.ds(pl.multiple_of(sec * D + g * 128, 128), 128)],
            wa_nat.at[g * 3 + sec], sem.at[SEM_WA + g]) for sec in range(3)]

    def wb_copy(c, sid):
        col = c * 128 + (c // 8) * D
        return pltpu.make_async_copy(
            wb_hbm.at[:, pl.ds(col, 128)], wb_nat.at[c], sem.at[sid])

    def wk_copy(c, sid):
        rows = pl.ds(c * 128, 128)
        return pltpu.make_async_copy(
            wb_hbm.at[rows, pl.ds(D, D)], wk.at[rows, :], sem.at[sid])

    def woa_copy(half, sid):
        rows = pl.ds(half * (D // 2), D // 2)
        return pltpu.make_async_copy(woa_hbm.at[rows, :], woa.at[rows, :], sem.at[sid])

    def iter_copies(it):
        sid = SEM_IT + min(it, 3)
        if it == 0:
            cps = [woa_copy(1, sid)]
        else:
            cps = [x_copy(i, sid) for i in (2 * it + 1, 2 * it + 2) if i < NB]
        return cps + [wb_copy(2 * it, sid), wb_copy(2 * it + 1, sid), wk_copy(it, sid)]

    x01_copies = [x_copy(0, SEM_X01), x_copy(1, SEM_X01)]
    x2_copies = [x_copy(2, SEM_X2), woa_copy(0, SEM_X2)]
    wob_copy = pltpu.make_async_copy(wob_hbm, wob, sem.at[SEM_WOB])

    def out_copy(j):
        rows = pl.ds(pl.multiple_of(j * TF, TF), TF)
        return pltpu.make_async_copy(xio.at[rows, :], out_hbm.at[rows, :], sem.at[SEM_OUT])

    def blk_rows(i, n=BLK):
        return pl.ds(pl.multiple_of(i * n, n), n)

    def qkv_group(g, xn):
        w = jnp.concatenate([wat[g, kt] for kt in range(NG)], axis=1)
        q, k, v = [_dot_nt(_as_bf16(w[a:a + 64]), xn) for a in (0, 64, 128)]
        return q, _pack(k), _pack(v)

    def o_rows(i, n):
        rows = blk_rows(i, n // 2)
        return _as_bf16(jnp.concatenate([oN[t, rows, :] for t in range(NG)], axis=1))

    def proj_residual(o, w_cols, xv):
        cols = []
        for n in range(2):
            cols.append(xv[:, n * 512:(n + 1) * 512] + _dot(o, w_cols(n)))
        return jnp.concatenate(cols, axis=1)

    def woa_half(half, o_cols, xv):
        o = jnp.concatenate(o_cols, axis=1)
        rows = slice(half * (D // 4), (half + 1) * (D // 4))
        cols = []
        for n in range(2):
            w = _as_bf16(jnp.concatenate([woap[4 * n + t, rows, :] for t in range(4)], axis=1))
            cols.append(xv[:, n * 512:(n + 1) * 512] + _dot(o, w))
        return jnp.concatenate(cols, axis=1)

    def packed_cols(w_ref):
        return lambda n: _as_bf16(
            jnp.concatenate([w_ref[4 * n + t] for t in range(4)], axis=1))

    wob_cols, wk_cols = packed_cols(wobp), packed_cols(wkp)

    def repack(dst_ref, src_ref, c, n, tok=None):
        wv = pltpu.bitcast(src_ref[blk_rows(c, n), :], u32)
        if tok is not None:
            wv = _after(wv, tok)
        for t in range(NG):
            dst_ref[t, blk_rows(c, n // 2), :] = wv[:, t * 128:(t + 1) * 128]

    def store_permuted(dst_ref, row0, val):
        for h in range(4):
            dst_ref[pl.ds(row0 + h, 16, stride=4), :] = val[h * 16:(h + 1) * 16]

    def rows16(blk, r):
        return pl.ds(pl.multiple_of(blk * BLK + r * 16, 16), 16)

    def ln1(blk, r, tok=None):
        xv = xio[rows16(blk, r), :].astype(f32)
        return _ln16(xv if tok is None else _after(xv, tok))

    def ln2(tile, r, tok):
        xv = x_ref[pl.ds(pl.multiple_of(tile * TB + r * 16, 16), 16), :]
        xn2[pl.ds(pl.multiple_of(r * 8, 8), 8), :] = _ln16(_after(xv, tok))

    def stage(g, slot, qkv):
        for ref, val in zip(stg[g], qkv):
            ref[slot] = val

    def a_block(i, par):
        inx = jnp.minimum(i + 1, NB - 1)
        pos = i * BLK + lax.broadcasted_iota(jnp.int32, (8, 128), 1)

        def side_jobs(slot, src):
            if slot not in L1S + L2S + (WBSLOT, WKSLOT):
                return
            tok = _token(src)
            if slot == WBSLOT:
                wsrc = _as_bf16(_after(pltpu.bitcast(wb_nat[i], u32), tok))
                wbt[i] = pltpu.bitcast(wsrc.T, u32)
            if slot == WKSLOT:
                repack(wkp, wk, i, 64, tok)
            for r in range(8):
                if L1S[r] == slot:
                    xn1[1 - par][r * 8:(r + 1) * 8, :] = ln1(inx, r, tok)
            for e in range(2):
                if L2S[e] == slot:
                    ln2(0, 2 * jnp.clip(i - 2, 0, TB // 32 - 1) + e, tok)

        o_cols = []
        for g in range(NG):
            stage(g, par, qkv_group(g, _as_bf16(xn1[par][...])))
            qs, ks, vs = stg[g]
            ot = _local_attention(qs[par], ks[par], ks[1 - par], vs[par], vs[1 - par], pos)
            o_cols.append(ot.astype(bf16).T)
            side_jobs(g, ot[120:128])
        rows = blk_rows(i)
        xv = woa_half(0, o_cols[:NG // 2], xio[rows, :].astype(f32))
        x_ref[rows, :] = woa_half(1, o_cols[NG // 2:], xv)

    def startup():
        def transpose_wa(g):
            for sec in range(3):
                wv = pltpu.bitcast(wa_nat[g * 3 + sec].T, u32)
                for kt in range(NG):
                    store_permuted(wstage.at[kt], sec * 64, wv[:, kt * 128:(kt + 1) * 128])

        def project(g):
            w = wstage[...]
            wat[g] = w
            w = jnp.concatenate([w[kt] for kt in range(NG)], axis=1)
            return _dot_nt(_as_bf16(w), _as_bf16(xn2[...]))

        def attend(g, r):
            pos = lax.broadcasted_iota(jnp.int32, (8, 128), 1)
            kp = vp = jnp.zeros((64, BLK), u32)
            for b in range(2):
                rb = r[:, b * BLK:(b + 1) * BLK]
                kc = _pack(rb[128:256])
                vc = _pack(rb[256:384])
                ot = _local_attention(rb[0:128], kc, kp, vc, vp, pos + b * BLK)
                po[g, b * 64:(b + 1) * 64, :] = pltpu.bitcast(ot.astype(bf16).T, u32)
                kp, vp = kc, vc
            khalo[g] = kp
            vhalo[g] = vp

        pbuf[...] = jnp.zeros(pbuf.shape, f32)

        def zero_scores(k, c):
            for sb in sbufs:
                sb[blk_rows(k, 32), :] = jnp.zeros((32, NQ), f32)
            return c
        lax.fori_loop(0, 2 * MK // 32, zero_scores, 0)
        for cp in x01_copies:
            cp.wait()
        for b in range(2):
            for r in range(BLK // 16):
                xn2[b * 64 + r * 8:b * 64 + (r + 1) * 8, :] = ln1(b, r)
        for cp in wa_copies(0):
            cp.wait()
        transpose_wa(0)

        def body(g, c):
            for cp in wa_copies(g + 1):
                cp.wait()
            prev = pbuf[...]
            pbuf[...] = project(g)
            transpose_wa(g + 1)
            attend(jnp.maximum(g - 1, 0), prev)
            return c
        lax.fori_loop(0, NG - 1, body, 0)

        def out_half(half):
            for t in range(NG):
                wv = pltpu.bitcast(
                    woa[half * (D // 2):(half + 1) * (D // 2), t * 128:(t + 1) * 128], u32)
                for g in range(NG // 2):
                    store_permuted(woap.at[t], half * (D // 4) + g * 64, wv[g * 64:(g + 1) * 64])
            for b in range(2):
                rows = blk_rows(b)
                o_cols = [_as_bf16(po[half * (NG // 2) + g, b * 64:(b + 1) * 64, :])
                          for g in range(NG // 2)]
                base = x_ref[rows, :] if half else xio[rows, :].astype(f32)
                x_ref[rows, :] = woa_half(half, o_cols, base)

        for cp in x2_copies:
            cp.wait()
        prev = pbuf[...]
        r = project(NG - 1)
        xn1[0][...] = jnp.concatenate([ln1(2, r16) for r16 in range(BLK // 16)], axis=0)
        attend(NG - 2, prev)
        out_half(0)
        attend(NG - 1, r)

        for cp in iter_copies(0):
            cp.wait()
        out_half(1)
        for b in range(2):
            wbt[b] = pltpu.bitcast(wb_nat[b].T, u32)
        repack(wkp, wk, 0, 128)
        for g in range(NG):
            stg[g][1][1] = khalo[g]
            stg[g][2][1] = vhalo[g]
        for cp in iter_copies(1):
            cp.wait()

    def phase_a(rep):
        def body(it, c):
            @pl.when(it == 2 - rep * NB)
            def _():
                for cp in iter_copies(2):
                    cp.wait()

            @pl.when(it == 3 - rep * NB)
            def _():
                for k in range(3, NB // APB):
                    for cp in iter_copies(k):
                        cp.wait()

            for u in range(APB):
                a_block(it * APB + u, u % 2)
            return c
        lax.fori_loop(1 - rep, NB // APB, body, 0)

    def phase_b_proj():
        def body(j, c):
            rows = blk_rows(j, TB // 2)
            xn = _as_bf16(xn2[...])
            toks = []
            for n in range(2):
                y = _pack(_dot(xn, wk_cols(n)))
                for t in range(4):
                    kN[4 * n + t, rows, :] = y[:, t * 128:(t + 1) * 128]
                toks += [y[:, 0:128], y[:, 256:384]]
            for r in range(4):
                w = _as_bf16(wbt[2 * r:2 * r + 2].reshape(128, D))
                y = _pack(_dot_nt(w, xn) * QSCALE)
                for b in range(TB // NQ):
                    qT[j * (TB // NQ) + b, r * 128:(r + 1) * 128, :] = y[:, b * NQ:(b + 1) * NQ]
                toks.append(y[:, 0:128])
            for r in range(4):
                w = _as_bf16(wbt[8 + 2 * r:8 + 2 * r + 2].reshape(128, D))
                y = _pack(_dot_nt(w, xn))
                for b in range(TB // MK):
                    vT[j * (TB // MK) + b, r * 128:(r + 1) * 128, :] = y[:, b * MK:(b + 1) * MK]
                toks.append(y[:, 0:128])
            jn = jnp.minimum(j + 1, S // TB - 1)
            for r in range(TB // 16):
                ln2(jn, r, _token(toks[L2BS[r]]))
            return c
        lax.fori_loop(0, S // TB, body, 0)

    def flush_o(g, val):
        y = pltpu.bitcast(_as_bf16(val).T, u32)
        oN[g[0], blk_rows(g[1], NQ // 2), :] = y

    def phase_b_attn(rep):
        off = [0, 0]

        def qm_of(t, qi, j):
            q = _as_bf16(qT[qi, pl.ds(pl.multiple_of(t * 64 + j * 16, 16), 16), :])
            parts = []
            if j > 0:
                parts.append(jnp.zeros((32 * j, NQ), bf16))
            parts.append(q)
            if j < 3:
                parts.append(jnp.zeros((32 * (3 - j), NQ), bf16))
            return jnp.concatenate(parts, axis=0)

        def qk_chunk(t, qm, c, par, m):
            k = _as_bf16(kN[t, c * (MK // 2):(c + 1) * (MK // 2), :])
            s = _dot(k, qm)
            sbufs[c][pl.ds(pl.multiple_of(off[0] + par * MK, 8), MK), :] = s
            sm = _tree(s.reshape(MK // 8, 8, NQ), jnp.maximum)
            return sm if m is None else jnp.maximum(m, sm)

        def pv_chunk(h, c, par, mrow, l, o):
            s = sbufs[c][pl.ds(pl.multiple_of(off[1] + par * MK, 8), MK), :]
            p = jnp.exp2(s - mrow)
            ls = jnp.sum(p.reshape(MK // 8, 8, NQ), axis=0)
            l = ls if l is None else l + ls
            v = _as_bf16(vT[c, pl.ds(pl.multiple_of(h * 16, 16), 16), :])
            oc = _dot(v, p.astype(bf16))
            o = oc if o is None else o + oc
            return l, o

        n_groups = NQT * NG
        lag = NC + DL
        n_steps = 4 * NC

        def set_offsets(zero):
            off[0] = lax.shift_right_logical(zero, 16) * 8
            off[1] = lax.shift_right_logical(zero, 17) * 8

        def pv_step(g, n, ms, st, flush=True):
            j, c = divmod(n, NC)
            l, o, mrow = st
            if c == 0:
                mrow = jnp.max(ms[j], axis=0, keepdims=True)
                l = o = None
            l, o = pv_chunk(g[0] * 4 + j, c, j % 2, mrow, l, o)
            if c == NC - 1:
                lrow = jnp.sum(l, axis=0, keepdims=True)
                otbuf[j * 16:(j + 1) * 16, :] = _pack(o * (1.0 / lrow))
                if j == 3 and flush:
                    flush_o(g, otbuf[...])
            return l, o, mrow

        def group(g, g_prev, carry, side_job=None):
            st, ms_prev = carry[:3], {3: carry[3]}
            ms = {}
            qms = {}
            order = [(kind, n) for n in range(n_steps) for kind in ("qk", "pv")]
            if side_job is not None:
                order[1], order[2] = order[2], order[1]
            for kind, n in order:
                if kind == "qk":
                    j, c = divmod(n, NC)
                    if c == 0:
                        qms[j] = qm_of(g[0], g[1], j)
                    ms[j] = qk_chunk(g[0], qms[j], c, j % 2, ms.get(j))
                    continue
                if n < lag:
                    st = pv_step(g_prev, n + n_steps - lag, ms_prev, st)
                else:
                    st = pv_step(g, n - lag, ms, st)
                if side_job is not None and n == n_steps // 2:
                    side_job(_token(st[0][:, 0:128]))
            return st + (ms[3],)

        def body(it, carry):
            def side_job(tok):
                repack(wobp, wob, it, D * GPB // n_groups, tok)

            set_offsets(it)
            carry = carry[:4]
            def split(g):
                return jnp.bitwise_and(g, NG - 1), lax.shift_right_logical(g, 3)

            g_prev = split(jnp.maximum(it * GPB - 1, 0))
            t0, qi = split(it * GPB)
            for u in range(GPB):
                g = (t0 + u, qi)
                carry = group(g, g_prev, carry, side_job if u == 0 else None)
                g_prev = g
            return carry + (it,)

        otbuf[...] = jnp.zeros(otbuf.shape, u32)
        init = (jnp.zeros((8, NQ), f32), jnp.zeros((DH, NQ), f32),
                jnp.zeros((1, NQ), f32), jnp.zeros((8, NQ), f32), jnp.int32(0))
        carry = lax.fori_loop(0, n_groups // GPB, body, init)
        set_offsets(carry[4])
        st, ms = carry[:3], {3: carry[3]}
        o0 = o_rows(0, TF)
        done = 0
        for k, n in enumerate(range(n_steps - lag, n_steps)):
            while done < NG and done * lag <= k * NG:
                cols = slice(done * 128, (done + 1) * 128)
                y = (x_ref[0:TF, cols] + _dot(o0, _as_bf16(wobp[done]))).astype(bf16)
                xio[0:TF, cols] = y
                y = pltpu.bitcast(y, u32)
                x0buf[:, cols] = y
                for ref in stg[done][1:]:
                    ref[1] = jnp.concatenate([_token(y)] * 8, axis=0)
                done += 1
            st = pv_step((NG - 1, NQT - 1), n, ms, st, False)

        @pl.when(rep == 1)
        def _():
            out_copy(0).start()
        off[0] = off[1] = 0

    def out_tile(j, rep, side_jobs):
        rows = blk_rows(j, TF)
        xv = proj_residual(o_rows(j, TF), wob_cols, x_ref[rows, :])
        xio[rows, :] = xv.astype(bf16)
        side_jobs(xv)

        @pl.when(rep == 1)
        def _():
            out_copy(j).start()

    def phase_b_out(rep):
        def body(jj, c):
            for u in range(OPB):
                def side_jobs(xv, u=u):
                    for r in range(8):
                        if L1O[r] // 4 == u:
                            k = L1O[r] % 4
                            xr = _as_bf16(x0buf[r * 8:(r + 1) * 8, :]).astype(f32)
                            tok = _token(xv[0:8, k * 256:k * 256 + 128])
                            xn1[0][r * 8:(r + 1) * 8, :] = _ln16(_after(xr, tok))
                out_tile(OPRE + jj * OPB + u, rep, side_jobs)
            flush_o((NG - 1, NQT - 1), otbuf[...])
            return c
        lax.fori_loop(0, (S // TF - OPRE) // OPB, body, 0)

    for cp in x01_copies:
        cp.start()
    for g in range(NG):
        for cp in wa_copies(g):
            cp.start()
    for cp in x2_copies:
        cp.start()
    for it in range(NB // APB):
        for cp in iter_copies(it):
            cp.start()
    wob_copy.start()

    startup()

    def layer_pair(rep, c):
        phase_a(rep)

        @pl.when(rep == 0)
        def _():
            wob_copy.wait()

        phase_b_proj()
        phase_b_attn(rep)
        phase_b_out(rep)
        return c
    lax.fori_loop(0, 2, layer_pair, 0)
    for j in range(S // TF):
        out_copy(j).wait()


@jax.jit
def pallas_interleave_layers__sliding_local_dilated__softmax_full_mha__prompt_kernel(
    A_x: jax.Array,
    A_wqkv: jax.Array,
    A_wo: jax.Array,
    B_x: jax.Array,
    B_wqkv: jax.Array,
    B_wo: jax.Array,
):
    del B_x
    x = A_x.reshape(S, D)
    vm = pltpu.VMEM
    scratch = [
        vm((S, D), f32),
        vm((S, D), bf16),
        vm((BLK // 2, D), u32),
        vm((BLK // 2, D), u32),
        vm((TB // 2, D), u32),
        vm((3 * NG, D, 128), bf16),
        vm((NG, NG, 192, 128), u32),
        vm((D, D), bf16),
        vm((NG, D // 2, 128), u32),
        vm((2 * NG, D, 128), bf16),
        vm((2 * NG, 64, D), u32),
        vm((D, D), bf16),
        vm((NG, D // 2, 128), u32),
        vm((D, D), bf16),
        vm((NG, D // 2, 128), u32),
        vm((NG, 64, BLK), u32),
        vm((NG, 64, BLK), u32),
        vm((NG, 192, 128), u32),
        vm((384, 2 * BLK), f32),
        vm((NG, BLK, 128), u32),
        vm((BLK // 2, D), u32),
        vm((NQT, D // 2, NQ), u32),
        vm((NG, S // 2, 128), u32),
        vm((NC, D // 2, MK), u32),
        vm((NG, S // 2, 128), u32),
        vm((64, NQ), u32),
        pltpu.SemaphoreType.DMA((N_SEM,)),
    ] + [vm((2 * MK, NQ), f32)] * NC + [
        vm((2, 128, BLK), f32), vm((2, 64, BLK), u32), vm((2, 64, BLK), u32)] * NG
    out = pl.pallas_call(
        _kernel,
        out_shape=jax.ShapeDtypeStruct((S, D), bf16),
        in_specs=[pl.BlockSpec(memory_space=pl.ANY)] * 5,
        out_specs=pl.BlockSpec(memory_space=pl.ANY),
        scratch_shapes=scratch,
        compiler_params=pltpu.CompilerParams(vmem_limit_bytes=110 * 1024 * 1024),
        name="interleave_attn",
    )(x, A_wqkv, A_wo, B_wqkv, B_wo)
    return out.reshape(1, S, D)
```

```python
import jax
import jax.numpy as jnp
from jax import lax
import jax.experimental.pallas as pl
import jax.experimental.pallas.tpu as pltpu

S, D, H, DH = 2048, 1024, 32, 32
W_LOC, DIL = 8, 2
EPS = 1e-5
LOG2E = 1.4426950408889634
QSCALE = (DH ** -0.5) * LOG2E
NEG = -1e9 * LOG2E

BLK = 128
NB = S // BLK
NG = D // 128
NQ = 256
NQT = S // NQ
MK = 128
NC = S // MK
DL = 6
APB = 2
GPB = 4
TB = 256
TF = 128
OPRE = 1
OPB = 3

SEM_X01, SEM_X2, SEM_WOB, SEM_OUT = 0, 1, 2, 3
SEM_WA = 4
SEM_IT = SEM_WA + NG
N_SEM = SEM_IT + 4

UCH = 2
L1S = (0, 0, 1, 2, 3, 4, 6, 7)
L2S = (3, 5)
WBSLOT = 6
WKSLOT = 0
SL1 = (0, 48, 96, 144, 192, 240, 288, 336)
L1O = (5, 6, 2, 0, 3, 7, 1, 8)
L2BS = (10, 0, 4, 9, 8, 5, 2, 5, 4, 8, 3, 6, 2, 1, 9, 7)


bf16 = jnp.bfloat16
f32 = jnp.float32
u32 = jnp.uint32
NT = (((1,), (1,)), ((), ()))


def _pack(x):
    return pltpu.bitcast(x.astype(bf16), u32)


def _as_bf16(x):
    return pltpu.bitcast(x, bf16)


def _dot(a, b):
    return jnp.dot(a, b, preferred_element_type=f32)


def _dot_nt(a, b):
    return lax.dot_general(a, b, NT, preferred_element_type=f32)


def _token(v):
    t = pltpu.bitcast(v[0:8, :], u32)
    return lax.shift_right_logical(jnp.bitwise_and(t, jnp.uint32(0xFFFF)), jnp.uint32(16))


def _after(x, tok):
    n, m = x.shape
    z = jnp.concatenate([jnp.concatenate([tok] * (m // 128), axis=1)] * (n // 8), axis=0)
    return pltpu.bitcast(jnp.bitwise_or(pltpu.bitcast(x, u32), z), x.dtype)


def _ln16(x):
    mu = jnp.sum(x, axis=1, keepdims=True) * (1.0 / D)
    xc = x - mu
    var = jnp.sum(xc * xc, axis=1, keepdims=True) * (1.0 / D)
    return _pack(xc * lax.rsqrt(var + EPS))


def _tree(x, op):
    n = x.shape[0]
    while n > 1:
        n //= 2
        x = op(x[:n], x[n:])
    return x[0]


def _local_attention(q, kc, kp, vc, vp, pos):
    lane = lax.broadcasted_iota(jnp.int32, (UCH * 4, 128), 1)

    def shifted(cur, prev, u, w):
        rows = slice(u * UCH * 4, (u + 1) * UCH * 4)
        x = cur[rows]
        if w:
            x = jnp.where(lane >= 128 - DIL * w, prev[rows], x)
            x = pltpu.roll(x, DIL * w, axis=1)
        return _as_bf16(x).astype(f32).reshape(UCH, 8, 128)

    nu = 16 // UCH
    even = lax.broadcasted_iota(jnp.int32, (8, 128), 0) % 2 == 0
    acc = [None] * W_LOC
    for u in range(nu):
        qu = q[u * UCH * 8:(u + 1) * UCH * 8].reshape(UCH, 8, 128)
        for w in range(W_LOC):
            t = _tree(qu * shifted(kc, kp, u, w), jnp.add)
            acc[w] = t if acc[w] is None else acc[w] + t
    logits = []
    for w in range(W_LOC):
        t = acc[w]
        t = t + jnp.where(even, pltpu.roll(t, 7, axis=0), pltpu.roll(t, 1, axis=0))
        t = t * QSCALE
        if w:
            t = jnp.where(pos >= DIL * w, t, NEG)
        logits.append(t)
    m = logits[0]
    for t in logits[1:]:
        m = jnp.maximum(m, t)
    ps = [jnp.exp2(t - m) for t in logits]
    l = ps[0]
    for p in ps[1:]:
        l = l + p
    r = 1.0 / l
    ps = [(p * r)[None] for p in ps]
    outs = []
    for u in range(nu):
        o = None
        for w in range(W_LOC):
            t = shifted(vc, vp, u, w) * ps[w]
            o = t if o is None else o + t
        outs.append(o.reshape(UCH * 8, 128))
    return jnp.concatenate(outs, axis=0)


def _kernel(x_hbm, wa_hbm, woa_hbm, wb_hbm, wob_hbm, out_hbm,
            x_ref, xio, xn1a, xn1b, xn2, wa_nat, wat, woa, woap, wb_nat, wbt, wk, wkp, wob, wobp,
            khalo, vhalo, wstage, pbuf, po, x0buf,
            qT, kN, vT, oN, otbuf,
            sem, *bufs):
    xn1 = (xn1a, xn1b)
    sbufs = bufs[:NC]
    stg = [bufs[NC + 3 * g:NC + 3 * g + 3] for g in range(NG)]

    def x_copy(i, sid):
        rows = pl.ds(i * BLK, BLK)
        return pltpu.make_async_copy(x_hbm.at[rows, :], xio.at[rows, :], sem.at[sid])

    def wa_copies(g):
        return [pltpu.make_async_copy(
            wa_hbm.at[:, pl.ds(pl.multiple_of(sec * D + g * 128, 128), 128)],
            wa_nat.at[g * 3 + sec], sem.at[SEM_WA + g]) for sec in range(3)]

    def wb_copy(c, sid):
        col = c * 128 + (c // 8) * D
        return pltpu.make_async_copy(
            wb_hbm.at[:, pl.ds(col, 128)], wb_nat.at[c], sem.at[sid])

    def wk_copy(c, sid):
        rows = pl.ds(c * 128, 128)
        return pltpu.make_async_copy(
            wb_hbm.at[rows, pl.ds(D, D)], wk.at[rows, :], sem.at[sid])

    def woa_copy(half, sid):
        rows = pl.ds(half * (D // 2), D // 2)
        return pltpu.make_async_copy(woa_hbm.at[rows, :], woa.at[rows, :], sem.at[sid])

    def iter_copies(it):
        sid = SEM_IT + min(it, 3)
        if it == 0:
            cps = [woa_copy(1, sid)]
        else:
            cps = [x_copy(i, sid) for i in (2 * it + 1, 2 * it + 2) if i < NB]
        return cps + [wb_copy(2 * it, sid), wb_copy(2 * it + 1, sid), wk_copy(it, sid)]

    x01_copies = [x_copy(0, SEM_X01), x_copy(1, SEM_X01)]
    x2_copies = [x_copy(2, SEM_X2), woa_copy(0, SEM_X2)]
    wob_copy = pltpu.make_async_copy(wob_hbm, wob, sem.at[SEM_WOB])

    def out_copy(j):
        rows = pl.ds(pl.multiple_of(j * TF, TF), TF)
        return pltpu.make_async_copy(xio.at[rows, :], out_hbm.at[rows, :], sem.at[SEM_OUT])

    def blk_rows(i, n=BLK):
        return pl.ds(pl.multiple_of(i * n, n), n)

    def qkv_group(g, xn):
        w = jnp.concatenate([wat[g, kt] for kt in range(NG)], axis=1)
        q, k, v = [_dot_nt(_as_bf16(w[a:a + 64]), xn) for a in (0, 64, 128)]
        return q, _pack(k), _pack(v)

    def o_rows(i, n):
        rows = blk_rows(i, n // 2)
        return _as_bf16(jnp.concatenate([oN[t, rows, :] for t in range(NG)], axis=1))

    def proj_residual(o, w_cols, xv):
        cols = []
        for n in range(2):
            cols.append(xv[:, n * 512:(n + 1) * 512] + _dot(o, w_cols(n)))
        return jnp.concatenate(cols, axis=1)

    def woa_half(half, o_cols, xv):
        o = jnp.concatenate(o_cols, axis=1)
        rows = slice(half * (D // 4), (half + 1) * (D // 4))
        cols = []
        for n in range(2):
            w = _as_bf16(jnp.concatenate([woap[4 * n + t, rows, :] for t in range(4)], axis=1))
            cols.append(xv[:, n * 512:(n + 1) * 512] + _dot(o, w))
        return jnp.concatenate(cols, axis=1)

    def packed_cols(w_ref):
        return lambda n: _as_bf16(
            jnp.concatenate([w_ref[4 * n + t] for t in range(4)], axis=1))

    wob_cols, wk_cols = packed_cols(wobp), packed_cols(wkp)

    def repack(dst_ref, src_ref, c, n, tok=None):
        wv = pltpu.bitcast(src_ref[blk_rows(c, n), :], u32)
        if tok is not None:
            wv = _after(wv, tok)
        for t in range(NG):
            dst_ref[t, blk_rows(c, n // 2), :] = wv[:, t * 128:(t + 1) * 128]

    def store_permuted(dst_ref, row0, val):
        for h in range(4):
            dst_ref[pl.ds(row0 + h, 16, stride=4), :] = val[h * 16:(h + 1) * 16]

    def rows16(blk, r):
        return pl.ds(pl.multiple_of(blk * BLK + r * 16, 16), 16)

    def ln1(blk, r, tok=None):
        xv = xio[rows16(blk, r), :].astype(f32)
        return _ln16(xv if tok is None else _after(xv, tok))

    def ln2(tile, r, tok):
        xv = x_ref[pl.ds(pl.multiple_of(tile * TB + r * 16, 16), 16), :]
        xn2[pl.ds(pl.multiple_of(r * 8, 8), 8), :] = _ln16(_after(xv, tok))

    def stage(g, slot, qkv):
        for ref, val in zip(stg[g], qkv):
            ref[slot] = val

    def a_block(i, par):
        inx = jnp.minimum(i + 1, NB - 1)
        pos = i * BLK + lax.broadcasted_iota(jnp.int32, (8, 128), 1)

        def side_jobs(slot, src):
            if slot not in L1S + L2S + (WBSLOT, WKSLOT):
                return
            tok = _token(src)
            if slot == WBSLOT:
                wsrc = _as_bf16(_after(pltpu.bitcast(wb_nat[i], u32), tok))
                wbt[i] = pltpu.bitcast(wsrc.T, u32)
            if slot == WKSLOT:
                repack(wkp, wk, i, 64, tok)
            for r in range(8):
                if L1S[r] == slot:
                    xn1[1 - par][r * 8:(r + 1) * 8, :] = ln1(inx, r, tok)
            for e in range(2):
                if L2S[e] == slot:
                    ln2(0, 2 * jnp.clip(i - 2, 0, TB // 32 - 1) + e, tok)

        o_cols = []
        for g in range(NG):
            stage(g, par, qkv_group(g, _as_bf16(xn1[par][...])))
            qs, ks, vs = stg[g]
            ot = _local_attention(qs[par], ks[par], ks[1 - par], vs[par], vs[1 - par], pos)
            o_cols.append(ot.astype(bf16).T)
            side_jobs(g, ot[120:128])
        rows = blk_rows(i)
        xv = woa_half(0, o_cols[:NG // 2], xio[rows, :].astype(f32))
        x_ref[rows, :] = woa_half(1, o_cols[NG // 2:], xv)

    def startup():
        def transpose_wa(g):
            for sec in range(3):
                wv = pltpu.bitcast(wa_nat[g * 3 + sec].T, u32)
                for kt in range(NG):
                    store_permuted(wstage.at[kt], sec * 64, wv[:, kt * 128:(kt + 1) * 128])

        def project(g):
            w = wstage[...]
            wat[g] = w
            w = jnp.concatenate([w[kt] for kt in range(NG)], axis=1)
            return _dot_nt(_as_bf16(w), _as_bf16(xn2[...]))

        def attend(g, r):
            pos = lax.broadcasted_iota(jnp.int32, (8, 128), 1)
            kp = vp = jnp.zeros((64, BLK), u32)
            for b in range(2):
                rb = r[:, b * BLK:(b + 1) * BLK]
                kc = _pack(rb[128:256])
                vc = _pack(rb[256:384])
                ot = _local_attention(rb[0:128], kc, kp, vc, vp, pos + b * BLK)
                po[g, b * 64:(b + 1) * 64, :] = pltpu.bitcast(ot.astype(bf16).T, u32)
                kp, vp = kc, vc
            khalo[g] = kp
            vhalo[g] = vp

        pbuf[...] = jnp.zeros(pbuf.shape, f32)

        def zero_scores(k, c):
            for sb in sbufs:
                sb[blk_rows(k, 32), :] = jnp.zeros((32, NQ), f32)
            return c
        lax.fori_loop(0, 2 * MK // 32, zero_scores, 0)
        for cp in x01_copies:
            cp.wait()
        for b in range(2):
            for r in range(BLK // 16):
                xn2[b * 64 + r * 8:b * 64 + (r + 1) * 8, :] = ln1(b, r)
        for cp in wa_copies(0):
            cp.wait()
        transpose_wa(0)

        def body(g, c):
            for cp in wa_copies(g + 1):
                cp.wait()
            prev = pbuf[...]
            pbuf[...] = project(g)
            transpose_wa(g + 1)
            attend(jnp.maximum(g - 1, 0), prev)
            return c
        lax.fori_loop(0, NG - 1, body, 0)

        def out_half(half):
            toks = []
            for t in range(NG):
                wv = pltpu.bitcast(
                    woa[half * (D // 2):(half + 1) * (D // 2), t * 128:(t + 1) * 128], u32)
                for g in range(NG // 2):
                    store_permuted(woap.at[t], half * (D // 4) + g * 64, wv[g * 64:(g + 1) * 64])
            for b in range(2):
                rows = blk_rows(b)
                o_cols = [_as_bf16(po[half * (NG // 2) + g, b * 64:(b + 1) * 64, :])
                          for g in range(NG // 2)]
                base = x_ref[rows, :] if half else xio[rows, :].astype(f32)
                xv = woa_half(half, o_cols, base)
                x_ref[rows, :] = xv
                toks.append(_token(xv[0:8, 0:128]))
            return toks

        for cp in x2_copies:
            cp.wait()
        prev = pbuf[...]
        r = project(NG - 1)
        for r16 in range(BLK // 16):
            tok = _token(r[SL1[r16]:SL1[r16] + 8, 0:128])
            xn1[0][r16 * 8:(r16 + 1) * 8, :] = ln1(2, r16, tok)
        attend(NG - 2, prev)
        out_half(0)
        attend(NG - 1, r)

        for cp in iter_copies(0):
            cp.wait()
        toks = out_half(1)
        for b in range(2):
            wbt[b] = pltpu.bitcast(wb_nat[b].T, u32)
        repack(wkp, wk, 0, 128, toks[0])
        for g in range(NG):
            stg[g][1][1] = khalo[g]
            stg[g][2][1] = vhalo[g]
        for cp in iter_copies(1):
            cp.wait()

    def phase_a(rep):
        def body(it, c):
            @pl.when(it == 2 - rep * NB)
            def _():
                for cp in iter_copies(2):
                    cp.wait()

            @pl.when(it == 3 - rep * NB)
            def _():
                for k in range(3, NB // APB):
                    for cp in iter_copies(k):
                        cp.wait()

            for u in range(APB):
                a_block(it * APB + u, u % 2)
            return c
        lax.fori_loop(1 - rep, NB // APB, body, 0)

    def phase_b_proj():
        def body(j, c):
            rows = blk_rows(j, TB // 2)
            xn = _as_bf16(xn2[...])
            toks = []
            for n in range(2):
                y = _pack(_dot(xn, wk_cols(n)))
                for t in range(4):
                    kN[4 * n + t, rows, :] = y[:, t * 128:(t + 1) * 128]
                toks += [y[:, 0:128], y[:, 256:384]]
            for r in range(4):
                w = _as_bf16(wbt[2 * r:2 * r + 2].reshape(128, D))
                y = _pack(_dot_nt(w, xn) * QSCALE)
                for b in range(TB // NQ):
                    qT[j * (TB // NQ) + b, r * 128:(r + 1) * 128, :] = y[:, b * NQ:(b + 1) * NQ]
                toks.append(y[:, 0:128])
            for r in range(4):
                w = _as_bf16(wbt[8 + 2 * r:8 + 2 * r + 2].reshape(128, D))
                y = _pack(_dot_nt(w, xn))
                for b in range(TB // MK):
                    vT[j * (TB // MK) + b, r * 128:(r + 1) * 128, :] = y[:, b * MK:(b + 1) * MK]
                toks.append(y[:, 0:128])
            jn = jnp.minimum(j + 1, S // TB - 1)
            for r in range(TB // 16):
                ln2(jn, r, _token(toks[L2BS[r]]))
            return c
        lax.fori_loop(0, S // TB, body, 0)

    def flush_o(g, val):
        y = pltpu.bitcast(_as_bf16(val).T, u32)
        oN[g[0], blk_rows(g[1], NQ // 2), :] = y

    def phase_b_attn(rep):
        off = [0, 0]

        def qm_of(t, qi, j):
            q = _as_bf16(qT[qi, pl.ds(pl.multiple_of(t * 64 + j * 16, 16), 16), :])
            parts = []
            if j > 0:
                parts.append(jnp.zeros((32 * j, NQ), bf16))
            parts.append(q)
            if j < 3:
                parts.append(jnp.zeros((32 * (3 - j), NQ), bf16))
            return jnp.concatenate(parts, axis=0)

        def qk_chunk(t, qm, c, par, m):
            k = _as_bf16(kN[t, c * (MK // 2):(c + 1) * (MK // 2), :])
            s = _dot(k, qm)
            sbufs[c][pl.ds(pl.multiple_of(off[0] + par * MK, 8), MK), :] = s
            sm = _tree(s.reshape(MK // 8, 8, NQ), jnp.maximum)
            return sm if m is None else jnp.maximum(m, sm)

        def pv_chunk(h, c, par, mrow, l, o):
            s = sbufs[c][pl.ds(pl.multiple_of(off[1] + par * MK, 8), MK), :]
            p = jnp.exp2(s - mrow)
            ls = jnp.sum(p.reshape(MK // 8, 8, NQ), axis=0)
            l = ls if l is None else l + ls
            v = _as_bf16(vT[c, pl.ds(pl.multiple_of(h * 16, 16), 16), :])
            oc = _dot(v, p.astype(bf16))
            o = oc if o is None else o + oc
            return l, o

        n_groups = NQT * NG
        lag = NC + DL
        n_steps = 4 * NC

        def set_offsets(zero):
            off[0] = lax.shift_right_logical(zero, 16) * 8
            off[1] = lax.shift_right_logical(zero, 17) * 8

        def pv_step(g, n, ms, st, flush=True):
            j, c = divmod(n, NC)
            l, o, mrow = st
            if c == 0:
                mrow = jnp.max(ms[j], axis=0, keepdims=True)
                l = o = None
            l, o = pv_chunk(g[0] * 4 + j, c, j % 2, mrow, l, o)
            if c == NC - 1:
                lrow = jnp.sum(l, axis=0, keepdims=True)
                otbuf[j * 16:(j + 1) * 16, :] = _pack(o * (1.0 / lrow))
                if j == 3 and flush:
                    flush_o(g, otbuf[...])
            return l, o, mrow

        def group(g, g_prev, carry, side_job=None):
            st, ms_prev = carry[:3], {3: carry[3]}
            ms = {}
            qms = {}
            order = [(kind, n) for n in range(n_steps) for kind in ("qk", "pv")]
            if side_job is not None:
                order[1], order[2] = order[2], order[1]
            for kind, n in order:
                if kind == "qk":
                    j, c = divmod(n, NC)
                    if c == 0:
                        qms[j] = qm_of(g[0], g[1], j)
                    ms[j] = qk_chunk(g[0], qms[j], c, j % 2, ms.get(j))
                    continue
                if n < lag:
                    st = pv_step(g_prev, n + n_steps - lag, ms_prev, st)
                else:
                    st = pv_step(g, n - lag, ms, st)
                if side_job is not None and n == n_steps // 2:
                    side_job(_token(st[0][:, 0:128]))
            return st + (ms[3],)

        def body(it, carry):
            def side_job(tok):
                repack(wobp, wob, it, D * GPB // n_groups, tok)

            set_offsets(it)
            carry = carry[:4]
            def split(g):
                return jnp.bitwise_and(g, NG - 1), lax.shift_right_logical(g, 3)

            g_prev = split(jnp.maximum(it * GPB - 1, 0))
            t0, qi = split(it * GPB)
            for u in range(GPB):
                g = (t0 + u, qi)
                carry = group(g, g_prev, carry, side_job if u == 0 else None)
                g_prev = g
            return carry + (it,)

        otbuf[...] = jnp.zeros(otbuf.shape, u32)
        init = (jnp.zeros((8, NQ), f32), jnp.zeros((DH, NQ), f32),
                jnp.zeros((1, NQ), f32), jnp.zeros((8, NQ), f32), jnp.int32(0))
        carry = lax.fori_loop(0, n_groups // GPB, body, init)
        set_offsets(carry[4])
        st, ms = carry[:3], {3: carry[3]}
        o0 = o_rows(0, TF)
        done = 0
        for k, n in enumerate(range(n_steps - lag, n_steps)):
            while done < NG and done * lag <= k * NG:
                cols = slice(done * 128, (done + 1) * 128)
                y = (x_ref[0:TF, cols] + _dot(o0, _as_bf16(wobp[done]))).astype(bf16)
                xio[0:TF, cols] = y
                y = pltpu.bitcast(y, u32)
                x0buf[:, cols] = y
                for ref in stg[done][1:]:
                    ref[1] = jnp.concatenate([_token(y)] * 8, axis=0)
                done += 1
            st = pv_step((NG - 1, NQT - 1), n, ms, st, False)

        @pl.when(rep == 1)
        def _():
            out_copy(0).start()
        off[0] = off[1] = 0

    def out_tile(j, rep, side_jobs):
        rows = blk_rows(j, TF)
        xv = proj_residual(o_rows(j, TF), wob_cols, x_ref[rows, :])
        xio[rows, :] = xv.astype(bf16)
        side_jobs(xv)

        @pl.when(rep == 1)
        def _():
            out_copy(j).start()

    def phase_b_out(rep):
        def body(jj, c):
            for u in range(OPB):
                def side_jobs(xv, u=u):
                    for r in range(8):
                        if L1O[r] // 4 == u:
                            k = L1O[r] % 4
                            xr = _as_bf16(x0buf[r * 8:(r + 1) * 8, :]).astype(f32)
                            tok = _token(xv[0:8, k * 256:k * 256 + 128])
                            xn1[0][r * 8:(r + 1) * 8, :] = _ln16(_after(xr, tok))
                out_tile(OPRE + jj * OPB + u, rep, side_jobs)
            flush_o((NG - 1, NQT - 1), otbuf[...])
            return c
        lax.fori_loop(0, (S // TF - OPRE) // OPB, body, 0)

    for cp in x01_copies:
        cp.start()
    for g in range(NG):
        for cp in wa_copies(g):
            cp.start()
    for cp in x2_copies:
        cp.start()
    for it in range(NB // APB):
        for cp in iter_copies(it):
            cp.start()
    wob_copy.start()

    startup()

    def layer_pair(rep, c):
        phase_a(rep)

        @pl.when(rep == 0)
        def _():
            wob_copy.wait()

        phase_b_proj()
        phase_b_attn(rep)
        phase_b_out(rep)
        return c
    lax.fori_loop(0, 2, layer_pair, 0)
    for j in range(S // TF):
        out_copy(j).wait()


@jax.jit
def pallas_interleave_layers__sliding_local_dilated__softmax_full_mha__prompt_kernel(
    A_x: jax.Array,
    A_wqkv: jax.Array,
    A_wo: jax.Array,
    B_x: jax.Array,
    B_wqkv: jax.Array,
    B_wo: jax.Array,
):
    del B_x
    x = A_x.reshape(S, D)
    vm = pltpu.VMEM
    scratch = [
        vm((S, D), f32),
        vm((S, D), bf16),
        vm((BLK // 2, D), u32),
        vm((BLK // 2, D), u32),
        vm((TB // 2, D), u32),
        vm((3 * NG, D, 128), bf16),
        vm((NG, NG, 192, 128), u32),
        vm((D, D), bf16),
        vm((NG, D // 2, 128), u32),
        vm((2 * NG, D, 128), bf16),
        vm((2 * NG, 64, D), u32),
        vm((D, D), bf16),
        vm((NG, D // 2, 128), u32),
        vm((D, D), bf16),
        vm((NG, D // 2, 128), u32),
        vm((NG, 64, BLK), u32),
        vm((NG, 64, BLK), u32),
        vm((NG, 192, 128), u32),
        vm((384, 2 * BLK), f32),
        vm((NG, BLK, 128), u32),
        vm((BLK // 2, D), u32),
        vm((NQT, D // 2, NQ), u32),
        vm((NG, S // 2, 128), u32),
        vm((NC, D // 2, MK), u32),
        vm((NG, S // 2, 128), u32),
        vm((64, NQ), u32),
        pltpu.SemaphoreType.DMA((N_SEM,)),
    ] + [vm((2 * MK, NQ), f32)] * NC + [
        vm((2, 128, BLK), f32), vm((2, 64, BLK), u32), vm((2, 64, BLK), u32)] * NG
    out = pl.pallas_call(
        _kernel,
        out_shape=jax.ShapeDtypeStruct((S, D), bf16),
        in_specs=[pl.BlockSpec(memory_space=pl.ANY)] * 5,
        out_specs=pl.BlockSpec(memory_space=pl.ANY),
        scratch_shapes=scratch,
        compiler_params=pltpu.CompilerParams(vmem_limit_bytes=110 * 1024 * 1024),
        name="interleave_attn",
    )(x, A_wqkv, A_wo, B_wqkv, B_wo)
    return out.reshape(1, S, D)
```
